```python
import jax
import jax.numpy as jnp

def _softmax(x, axis=-1):
    return jax.nn.softmax(x, axis=axis)

def _gelu(x):
    return jax.nn.gelu(x, approximate=True)

def _silu(x):
    return jax.nn.silu(x)

def _sigmoid(x):
    return jax.nn.sigmoid(x)

def _layernorm(x, axis=-1, eps=1e-05):
    m = jnp.mean(x, axis=axis, keepdims=True)
    v = jnp.var(x, axis=axis, keepdims=True)
    return (x - m) / jnp.sqrt(v + eps)

def _scatter_add(tgt, idx, src, axis=0):
    return tgt.at[idx].add(src)

def _segment_sum(src, seg, n):
    return jax.ops.segment_sum(src, seg, n)

class _Rng:

    def __init__(self, key):
        self._k = key

    def _next(self):
        self._k, sub = jax.random.split(self._k)
        return sub

    def normal(self, shape):
        return jax.random.normal(self._next(), shape, dtype=jnp.bfloat16)

    def randint(self, lo, hi, shape):
        return jax.random.randint(self._next(), shape, lo, hi, dtype=jnp.int32)

    def uniform(self, shape, lo=0.0, hi=1.0):
        return jax.random.uniform(self._next(), shape, jnp.bfloat16, lo, hi)

    def permutation(self, n):
        return jax.random.permutation(self._next(), n)
kernel_name = 'interleave_layers__memory_aug_recurrent_mem_tr__sliding_local_dilated__prompt'

def setup_inputs():
    _rng = _Rng(jax.random.key(int.from_bytes(__import__("os").urandom(4), "little")))
    _w = lambda a: (lambda t: t.astype(jnp.bfloat16) if jnp.issubdtype(t.dtype, jnp.floating) else t)(jnp.asarray(a))

    def _A_setup():
        B, S, Dm = (1, 2048, 640)
        H, Dh = (32, 192)
        M, seg = (8, 32)
        seg = min(seg, S)
        S = S // seg * seg
        return {'x': _w((lambda *s: _rng.normal(s) * 0.05)(B, S, Dm)), 'mem0': _w((lambda *s: _rng.normal(s) * 0.05)(B, M, Dm)), 'Wq': _w((lambda *s: _rng.normal(s) * 0.05)(Dm, H, Dh) * Dm ** (-0.5)), 'Wk': _w((lambda *s: _rng.normal(s) * 0.05)(Dm, H, Dh) * Dm ** (-0.5)), 'Wv': _w((lambda *s: _rng.normal(s) * 0.05)(Dm, H, Dh) * Dm ** (-0.5)), 'Wo': _w((lambda *s: _rng.normal(s) * 0.05)(H, Dh, Dm) * (H * Dh) ** (-0.5)), 'seg_len': seg}
    _A_in = _A_setup()

    def _B_setup():
        B, S, D = (1, 2048, 640)
        return {'x': _w((lambda *s: _rng.normal(s) * 0.05)(B, S, D)), 'wqkv': _w((lambda *s: _rng.normal(s) * 0.05)(D, 3 * D)), 'wo': _w((lambda *s: _rng.normal(s) * 0.05)(D, D))}
    _B_in = _B_setup()
    return {'A_x': _A_in['x'], 'A_mem0': _A_in['mem0'], 'A_Wq': _A_in['Wq'], 'A_Wk': _A_in['Wk'], 'A_Wv': _A_in['Wv'], 'A_Wo': _A_in['Wo'], 'A_seg_len': _A_in['seg_len'], 'B_x': _B_in['x'], 'B_wqkv': _B_in['wqkv'], 'B_wo': _B_in['wo']}

def reference(A_x, A_mem0, A_Wq, A_Wk, A_Wv, A_Wo, A_seg_len, B_x, B_wqkv, B_wo):

    def _A_ref(x, mem0, Wq, Wk, Wv, Wo, seg_len):
        B, S, Dm = x.shape
        H, Dh = (Wq.shape[1], Wq.shape[2])
        M = mem0.shape[1]
        scale = Dh ** (-0.5)
        n_seg = S // seg_len
        L = M + seg_len
        idx = jnp.arange(L)
        mask = (idx[:, None] < M) | (idx[:, None] >= idx[None, :])
        mem = mem0
        outs = []
        for s in range(n_seg):
            xs = x[:, s * seg_len:(s + 1) * seg_len, :].copy()
            h = jnp.concatenate([mem, xs], axis=1)
            q = jnp.einsum('btd,dhe->bhte', h, Wq)
            k = jnp.einsum('btd,dhe->bhte', h, Wk)
            v = jnp.einsum('btd,dhe->bhte', h, Wv)
            scores = jnp.einsum('bhqe,bhke->bhqk', q, k) * scale
            scores = jnp.where(mask[None, None], scores, -1000000000.0)
            p = _softmax(scores, axis=-1)
            o = jnp.einsum('bhqk,bhke->bhqe', p, v)
            o = jnp.einsum('bhte,hed->btd', o, Wo)
            mem = o[:, :M, :].copy()
            outs.append(o[:, M:, :])
        return jnp.concatenate(outs, axis=1)

    def _B_ref(x, wqkv, wo):
        B, S, D = x.shape
        H = 32
        Dh = D // H
        W, dil = (8, 2)
        qkv = (lambda x, *d: x.transpose(*d))((x @ wqkv).reshape(B, S, 3, H, Dh), 2, 0, 3, 1, 4)
        q, k, v = (qkv[0], qkv[1], qkv[2])
        scale = Dh ** (-0.5)
        pos = jnp.arange(S)
        off = jnp.arange(W) * dil
        idx = pos[:, None] - off[None, :]
        mask = idx >= 0
        idx_c = jnp.where(mask, idx, 0).reshape(-1)
        kg = k[:, :, idx_c, :].reshape(B, H, S, W, Dh)
        vg = v[:, :, idx_c, :].reshape(B, H, S, W, Dh)
        logits = jnp.einsum('bhsd,bhswd->bhsw', q, kg) * scale
        logits = jnp.where(mask[None, None, :, :], logits, -1000000000.0)
        attn = _softmax(logits, axis=-1)
        o = jnp.einsum('bhsw,bhswd->bhsd', attn, vg)
        return (lambda x, *d: x.transpose(*d))(o, 0, 2, 1, 3).reshape(B, S, D) @ wo
    x = A_x
    x = x + _A_ref(_layernorm(x, axis=-1), A_mem0, A_Wq, A_Wk, A_Wv, A_Wo, A_seg_len)
    x = x + _B_ref(_layernorm(x, axis=-1), B_wqkv, B_wo)
    x = x + _A_ref(_layernorm(x, axis=-1), A_mem0, A_Wq, A_Wk, A_Wv, A_Wo, A_seg_len)
    x = x + _B_ref(_layernorm(x, axis=-1), B_wqkv, B_wo)
    return x
```

```python
import functools

import jax
import jax.numpy as jnp
from jax import lax
import jax.experimental.pallas as pl
import jax.experimental.pallas.tpu as pltpu

F32 = jnp.float32
BF16 = jnp.bfloat16

EPS = 1e-5
NEG = -1000000000.0
PADNEG = -3.0e38
B_HEADS = 32
B_WIN = 8
B_DIL = 2
HIST = 16


def _ln(x):
    m = jnp.mean(x, axis=-1, keepdims=True)
    xc = x - m
    v = jnp.mean(xc * xc, axis=-1, keepdims=True)
    return xc * lax.rsqrt(v + EPS)


def _dot_nt(a, b):
    return lax.dot_general(a, b, (((1,), (1,)), ((), ())), preferred_element_type=F32)


def _dot(a, b):
    return jnp.dot(a, b, preferred_element_type=F32)


def _kernel(x_ref, mem0_ref, wq_ref, wk_ref, wv_ref, wo_ref, bqkv_ref, bwo_ref,
            out_ref,
            bqkv_p, bwo_p, mem_ref, xa_ref, x2_ref, kv_ref,
            *, S, D, H, DH, M, SEG):
    NSEG = S // SEG
    PW = 2 * DH
    NP = H // 2
    RL = SEG + 2 * M
    RT = 2 * SEG + 2 * M
    a_scale = DH ** (-0.5)
    b_dh = D // B_HEADS
    b_scale = b_dh ** (-0.5)
    NT = D // 128

    r_i = lax.broadcasted_iota(jnp.int32, (D, D), 0)
    c_i = lax.broadcasted_iota(jnp.int32, (D, D), 1)
    perm = jnp.where(r_i == (c_i & (B_HEADS - 1)) * b_dh + (c_i >> 5), 1.0, 0.0).astype(BF16)
    perm_t = jnp.where(c_i == (r_i & (B_HEADS - 1)) * b_dh + (r_i >> 5), 1.0, 0.0).astype(BF16)
    for j in range(3):
        bqkv_p[:, j * D:(j + 1) * D] = _dot(bqkv_ref[:, j * D:(j + 1) * D], perm).astype(BF16)
    bwo_p[...] = _dot(perm_t, bwo_ref[...]).astype(BF16)

    mem0 = mem0_ref[...].astype(F32)
    mem_ref[0:M, :] = mem0
    mem_ref[M:2 * M, :] = mem0
    xa_ref[...] = jnp.zeros(xa_ref.shape, F32)
    x2_ref[...] = jnp.zeros(x2_ref.shape, F32)
    kv_ref[...] = jnp.zeros(kv_ref.shape, F32)

    def layer_b(t):
        xb = xa_ref[...]
        qkv = _dot(_ln(xb).astype(BF16), bqkv_p[...])
        outs = []
        for l in range(2):
            q = qkv[l * SEG:(l + 1) * SEG, 0:D]
            kv_ref[l, HIST:HIST + SEG, :] = qkv[l * SEG:(l + 1) * SEG, D:3 * D]
            seg = t - 1 - 2 * l
            pos = seg * SEG + lax.broadcasted_iota(jnp.int32, (SEG, 128), 0)
            logits = []
            for w in range(B_WIN):
                o = HIST - B_DIL * w
                prod = q * kv_ref[l, o:o + SEG, 0:D]
                s = prod[:, 0:128]
                for j in range(1, NT):
                    s = s + prod[:, j * 128:(j + 1) * 128]
                s = s + pltpu.roll(s, 64, 1)
                s = s + pltpu.roll(s, 32, 1)
                logits.append(jnp.where(pos >= B_DIL * w, s * b_scale, NEG))
            m = logits[0]
            for w in range(1, B_WIN):
                m = jnp.maximum(m, logits[w])
            es = [jnp.exp(lg - m) for lg in logits]
            den = es[0]
            for w in range(1, B_WIN):
                den = den + es[w]
            inv = 1.0 / den
            acc = None
            for w in range(B_WIN):
                o = HIST - B_DIL * w
                p = es[w] * inv
                term = jnp.concatenate([p] * NT, axis=1) * kv_ref[l, o:o + SEG, D:2 * D]
                acc = term if acc is None else acc + term
            outs.append(acc)
            kv_ref[l, 0:HIST, :] = kv_ref[l, SEG:SEG + HIST, :]
        ob = _dot(jnp.concatenate(outs, axis=0).astype(BF16), bwo_p[...])
        y = xb + ob
        row = pl.multiple_of(jnp.maximum(t - 3, 0) * SEG, SEG)
        out_ref[pl.ds(row, SEG), :] = y[SEG:2 * SEG].astype(out_ref.dtype)
        return y[0:SEG]

    RV = SEG + M
    rr = lax.broadcasted_iota(jnp.int32, (RV, 2 * RL), 0)
    cc = lax.broadcasted_iota(jnp.int32, (RV, 2 * RL), 1)
    first = cc < RL
    kc = jnp.where(first, cc, cc - RL)
    valid1 = (kc < RV) & ((kc >= SEG) | (kc <= rr))
    fill1 = jnp.where(kc < RV, NEG, PADNEG)
    valid2 = (kc >= M) & ((rr < M) | (kc - M <= rr))
    fill2 = jnp.where(kc >= M, NEG, PADNEG)
    lane128 = lax.broadcasted_iota(jnp.int32, (RT, 128), 1)
    lo = lane128 < (DH - 128)

    def softmax2(s, valid, fill):
        s = jnp.where(valid, s * a_scale, fill)
        m1 = jnp.max(jnp.where(first, s, PADNEG), axis=-1, keepdims=True)
        m2 = jnp.max(jnp.where(first, PADNEG, s), axis=-1, keepdims=True)
        e = jnp.exp(s - jnp.where(first, m1, m2))
        l1 = jnp.sum(jnp.where(first, e, 0.0), axis=-1, keepdims=True)
        l2 = jnp.sum(jnp.where(first, 0.0, e), axis=-1, keepdims=True)
        return e * (1.0 / jnp.where(first, l1, l2))

    def blockdiag(a):
        t0 = a[:, 0:128].astype(BF16)
        mid = a[:, 128:256]
        t1a = jnp.where(lo, mid, 0.0).astype(BF16)
        t1b = jnp.where(lo, 0.0, mid).astype(BF16)
        t2 = a[:, 256:384].astype(BF16)
        z = jnp.zeros((RL, 128), BF16)
        res = []
        for s0 in (0, SEG):
            top = jnp.concatenate([t0[s0:s0 + RL], t1a[s0:s0 + RL], z], axis=1)
            bot = jnp.concatenate([z, t1b[s0:s0 + RL], t2[s0:s0 + RL]], axis=1)
            res.append(jnp.concatenate([top, bot], axis=0))
        return res

    def step(t, carry):
        row = pl.multiple_of(jnp.minimum(t, NSEG - 1) * SEG, SEG)
        x0 = x_ref[pl.ds(row, SEG), :].astype(F32)
        x2 = x2_ref[...]
        h = jnp.concatenate([_ln(x0), mem_ref[...], _ln(x2)], axis=0).astype(BF16)
        acc = None
        zrow = jnp.zeros((M, 2 * RL), F32)
        for p in range(NP):
            sl = slice(p * PW, (p + 1) * PW)
            q = _dot_nt(h, wq_ref[sl, :]).astype(BF16)
            k1, k2 = blockdiag(_dot_nt(h, wk_ref[sl, :]))
            v1, v2 = blockdiag(_dot_nt(h, wv_ref[sl, :]))
            s1 = _dot_nt(q[0:RL], k1)
            s2 = _dot_nt(q[SEG:SEG + RL], k2)
            p1 = softmax2(s1[0:RV], valid1, fill1)
            p2 = softmax2(s2[M:RL], valid2, fill2)
            p1 = jnp.concatenate([p1, zrow], axis=0).astype(BF16)
            p2 = jnp.concatenate([zrow, p2], axis=0).astype(BF16)
            o1 = _dot(p1, v1)
            o2 = _dot(p2, v2)
            o = jnp.concatenate([o1[0:RV], o2[M:RL]], axis=0).astype(BF16)
            part = _dot(o, wo_ref[sl, :])
            acc = part if acc is None else acc + part
        x2_new = layer_b(t)
        xa_ref[0:SEG, :] = x0 + acc[0:SEG]
        xa_ref[SEG:2 * SEG, :] = x2 + acc[SEG + 2 * M:RT]
        mem_ref[0:M, :] = acc[SEG:SEG + M]
        mem_ref[M:2 * M, :] = jnp.where(t >= 2, acc[SEG + M:SEG + 2 * M], mem0)
        x2_ref[...] = x2_new
        return carry

    lax.fori_loop(0, NSEG + 2, step, 0)
    layer_b(NSEG + 2)


@functools.partial(jax.jit, static_argnames=("A_seg_len",))
def pallas_interleave_layers__memory_aug_recurrent_mem_tr__sliding_local_dilated__prompt_kernel(
    A_x: jax.Array,
    A_mem0: jax.Array,
    A_Wq: jax.Array,
    A_Wk: jax.Array,
    A_Wv: jax.Array,
    A_Wo: jax.Array,
    A_seg_len,
    B_x: jax.Array,
    B_wqkv: jax.Array,
    B_wo: jax.Array,
):
    B, S, D = A_x.shape
    H, DH = A_Wq.shape[1], A_Wq.shape[2]
    M = A_mem0.shape[1]
    SEG = int(A_seg_len)
    assert B == 1 and M == 8 and SEG == 32 and DH == 192 and D % 128 == 0 and S % SEG == 0

    x = A_x.reshape(S, D)
    mem0 = A_mem0.reshape(M, D)
    wq = jnp.transpose(A_Wq, (1, 2, 0)).reshape(H * DH, D)
    wk = jnp.transpose(A_Wk, (1, 2, 0)).reshape(H * DH, D)
    wv = jnp.transpose(A_Wv, (1, 2, 0)).reshape(H * DH, D)
    wo = A_Wo.reshape(H * DH, D)

    out = pl.pallas_call(
        functools.partial(_kernel, S=S, D=D, H=H, DH=DH, M=M, SEG=SEG),
        out_shape=jax.ShapeDtypeStruct((S, D), A_x.dtype),
        scratch_shapes=[
            pltpu.VMEM((D, 3 * D), BF16),
            pltpu.VMEM((D, D), BF16),
            pltpu.VMEM((2 * M, D), F32),
            pltpu.VMEM((2 * SEG, D), F32),
            pltpu.VMEM((SEG, D), F32),
            pltpu.VMEM((2, HIST + SEG, 2 * D), F32),
        ],
        compiler_params=pltpu.CompilerParams(vmem_limit_bytes=100 * 1024 * 1024),
    )(x, mem0, wq, wk, wv, wo, B_wqkv, B_wo)
    return out.reshape(B, S, D)
```

```python
import functools

import jax
import jax.numpy as jnp
from jax import lax
import jax.experimental.pallas as pl
import jax.experimental.pallas.tpu as pltpu

F32 = jnp.float32
BF16 = jnp.bfloat16

EPS = 1e-5
NEG = -1000000000.0
PADNEG = -3.0e38
B_HEADS = 32
B_WIN = 8
B_DIL = 2
HIST = 16


def _ln(x):
    m = jnp.mean(x, axis=-1, keepdims=True)
    xc = x - m
    v = jnp.mean(xc * xc, axis=-1, keepdims=True)
    return xc * lax.rsqrt(v + EPS)


def _dot_nt(a, b):
    return lax.dot_general(a, b, (((1,), (1,)), ((), ())), preferred_element_type=F32)


def _dot(a, b):
    return jnp.dot(a, b, preferred_element_type=F32)


def _kernel(x_ref, mem0_ref, wq_ref, wk_ref, wv_ref, wo_ref, bqkv_ref, bwo_ref,
            out_ref,
            bqkv_p, bwo_p, mem_ref, xa_ref, x2_ref, kv_ref,
            *, S, D, H, DH, M, SEG):
    NSEG = S // SEG
    PW = 2 * DH
    NP = H // 2
    RL = SEG + 2 * M
    RT = 2 * SEG + 2 * M
    a_scale = DH ** (-0.5)
    b_dh = D // B_HEADS
    b_scale = b_dh ** (-0.5)
    NT = D // 128

    r_i = lax.broadcasted_iota(jnp.int32, (D, D), 0)
    c_i = lax.broadcasted_iota(jnp.int32, (D, D), 1)
    perm = jnp.where(r_i == (c_i & (B_HEADS - 1)) * b_dh + (c_i >> 5), 1.0, 0.0).astype(BF16)
    perm_t = jnp.where(c_i == (r_i & (B_HEADS - 1)) * b_dh + (r_i >> 5), 1.0, 0.0).astype(BF16)
    for j in range(3):
        bqkv_p[:, j * D:(j + 1) * D] = _dot(bqkv_ref[:, j * D:(j + 1) * D], perm).astype(BF16)
    bwo_p[...] = _dot(perm_t, bwo_ref[...]).astype(BF16)

    mem0 = mem0_ref[...].astype(F32)
    mem_ref[0:M, :] = mem0
    mem_ref[M:2 * M, :] = mem0
    xa_ref[...] = jnp.zeros(xa_ref.shape, F32)
    x2_ref[...] = jnp.zeros(x2_ref.shape, F32)
    kv_ref[...] = jnp.zeros(kv_ref.shape, F32)

    def b_qkv():
        xb = xa_ref[...]
        return xb, _dot(_ln(xb).astype(BF16), bqkv_p[...])

    def b_attn(t, qkv):
        outs = []
        for l in range(2):
            q = qkv[l * SEG:(l + 1) * SEG, 0:D]
            kv_ref[l, HIST:HIST + SEG, :] = qkv[l * SEG:(l + 1) * SEG, D:3 * D]
            seg = t - 1 - 2 * l
            pos = seg * SEG + lax.broadcasted_iota(jnp.int32, (SEG, 128), 0)
            logits = []
            for w in range(B_WIN):
                o = HIST - B_DIL * w
                prod = q * kv_ref[l, o:o + SEG, 0:D]
                s = prod[:, 0:128]
                for j in range(1, NT):
                    s = s + prod[:, j * 128:(j + 1) * 128]
                s = s + pltpu.roll(s, 64, 1)
                s = s + pltpu.roll(s, 32, 1)
                logits.append(jnp.where(pos >= B_DIL * w, s * b_scale, NEG))
            m = logits[0]
            for w in range(1, B_WIN):
                m = jnp.maximum(m, logits[w])
            es = [jnp.exp(lg - m) for lg in logits]
            den = es[0]
            for w in range(1, B_WIN):
                den = den + es[w]
            inv = 1.0 / den
            acc = None
            for w in range(B_WIN):
                o = HIST - B_DIL * w
                p = es[w] * inv
                term = jnp.concatenate([p] * NT, axis=1) * kv_ref[l, o:o + SEG, D:2 * D]
                acc = term if acc is None else acc + term
            outs.append(acc)
            kv_ref[l, 0:HIST, :] = kv_ref[l, SEG:SEG + HIST, :]
        return jnp.concatenate(outs, axis=0).astype(BF16)

    def b_out(t, xb, ob):
        y = xb + _dot(ob, bwo_p[...])
        row = pl.multiple_of(jnp.maximum(t - 3, 0) * SEG, SEG)
        out_ref[pl.ds(row, SEG), :] = y[SEG:2 * SEG].astype(out_ref.dtype)
        return y[0:SEG]

    RV = SEG + M
    rr = lax.broadcasted_iota(jnp.int32, (RV, 2 * RL), 0)
    cc = lax.broadcasted_iota(jnp.int32, (RV, 2 * RL), 1)
    first = cc < RL
    kc = jnp.where(first, cc, cc - RL)
    valid1 = (kc < RV) & ((kc >= SEG) | (kc <= rr))
    fill1 = jnp.where(kc < RV, NEG, PADNEG)
    valid2 = (kc >= M) & ((rr < M) | (kc - M <= rr))
    fill2 = jnp.where(kc >= M, NEG, PADNEG)
    lane128 = lax.broadcasted_iota(jnp.int32, (RT, 128), 1)
    lo = lane128 < (DH - 128)

    def softmax2(s, valid, fill):
        s = jnp.where(valid, s * a_scale, fill)
        m1 = jnp.max(jnp.where(first, s, PADNEG), axis=-1, keepdims=True)
        m2 = jnp.max(jnp.where(first, PADNEG, s), axis=-1, keepdims=True)
        e = jnp.exp(s - jnp.where(first, m1, m2))
        l1 = jnp.sum(jnp.where(first, e, 0.0), axis=-1, keepdims=True)
        l2 = jnp.sum(jnp.where(first, 0.0, e), axis=-1, keepdims=True)
        return e * (1.0 / jnp.where(first, l1, l2))

    def blockdiag(a):
        t0 = a[:, 0:128].astype(BF16)
        mid = a[:, 128:256]
        t1a = jnp.where(lo, mid, 0.0).astype(BF16)
        t1b = jnp.where(lo, 0.0, mid).astype(BF16)
        t2 = a[:, 256:384].astype(BF16)
        z = jnp.zeros((RL, 128), BF16)
        res = []
        for s0 in (0, SEG):
            top = jnp.concatenate([t0[s0:s0 + RL], t1a[s0:s0 + RL], z], axis=1)
            bot = jnp.concatenate([z, t1b[s0:s0 + RL], t2[s0:s0 + RL]], axis=1)
            res.append(jnp.concatenate([top, bot], axis=0))
        return res

    def step(t, carry):
        row = pl.multiple_of(jnp.minimum(t, NSEG - 1) * SEG, SEG)
        x0 = x_ref[pl.ds(row, SEG), :].astype(F32)
        x2 = x2_ref[...]
        h = jnp.concatenate([_ln(x0), mem_ref[...], _ln(x2)], axis=0).astype(BF16)
        zrow = jnp.zeros((M, 2 * RL), F32)

        def sl(p):
            return slice(p * PW, (p + 1) * PW)

        def proj_q(p):
            return _dot_nt(h, wq_ref[sl(p), :]).astype(BF16)

        def proj_k(p):
            return blockdiag(_dot_nt(h, wk_ref[sl(p), :]))

        def proj_v(p):
            return blockdiag(_dot_nt(h, wv_ref[sl(p), :]))

        def qk(q, k):
            s1 = _dot_nt(q[0:RL], k[0])
            s2 = _dot_nt(q[SEG:SEG + RL], k[1])
            p1 = softmax2(s1[0:RV], valid1, fill1)
            p2 = softmax2(s2[M:RL], valid2, fill2)
            p1 = jnp.concatenate([p1, zrow], axis=0).astype(BF16)
            p2 = jnp.concatenate([zrow, p2], axis=0).astype(BF16)
            return p1, p2

        def pv(pr, v):
            o1 = _dot(pr[0], v[0])
            o2 = _dot(pr[1], v[1])
            return jnp.concatenate([o1[0:RV], o2[M:RL]], axis=0).astype(BF16)

        acc = [None]

        def oproj(p, o):
            part = _dot(o, wo_ref[sl(p), :])
            acc[0] = part if acc[0] is None else acc[0] + part

        q = proj_q(0)
        k = proj_k(0)
        v = proj_v(0)
        os_ = {}
        for p in range(NP):
            pr = qk(q, k)
            if p + 1 < NP:
                q = proj_q(p + 1)
                k = proj_k(p + 1)
            else:
                x2_new = b_out(t, xb, ob)
                oproj(p - 2, os_.pop(p - 2))
            os_[p] = pv(pr, v)
            if p + 1 < NP:
                v = proj_v(p + 1)
            if p == 0:
                xb, qkv = b_qkv()
                ob = b_attn(t, qkv)
            if p >= 2 and p + 1 < NP:
                oproj(p - 2, os_.pop(p - 2))
        oproj(NP - 2, os_.pop(NP - 2))
        oproj(NP - 1, os_.pop(NP - 1))
        a = acc[0]
        xa_ref[0:SEG, :] = x0 + a[0:SEG]
        xa_ref[SEG:2 * SEG, :] = x2 + a[SEG + 2 * M:RT]
        mem_ref[0:M, :] = a[SEG:SEG + M]
        mem_ref[M:2 * M, :] = jnp.where(t >= 2, a[SEG + M:SEG + 2 * M], mem0)
        x2_ref[...] = x2_new
        return carry

    lax.fori_loop(0, NSEG + 2, step, 0)
    xb, qkv = b_qkv()
    b_out(NSEG + 2, xb, b_attn(NSEG + 2, qkv))


@functools.partial(jax.jit, static_argnames=("A_seg_len",))
def pallas_interleave_layers__memory_aug_recurrent_mem_tr__sliding_local_dilated__prompt_kernel(
    A_x: jax.Array,
    A_mem0: jax.Array,
    A_Wq: jax.Array,
    A_Wk: jax.Array,
    A_Wv: jax.Array,
    A_Wo: jax.Array,
    A_seg_len,
    B_x: jax.Array,
    B_wqkv: jax.Array,
    B_wo: jax.Array,
):
    B, S, D = A_x.shape
    H, DH = A_Wq.shape[1], A_Wq.shape[2]
    M = A_mem0.shape[1]
    SEG = int(A_seg_len)
    assert B == 1 and M == 8 and SEG == 32 and DH == 192 and D % 128 == 0 and S % SEG == 0

    x = A_x.reshape(S, D)
    mem0 = A_mem0.reshape(M, D)
    wq = jnp.transpose(A_Wq, (1, 2, 0)).reshape(H * DH, D)
    wk = jnp.transpose(A_Wk, (1, 2, 0)).reshape(H * DH, D)
    wv = jnp.transpose(A_Wv, (1, 2, 0)).reshape(H * DH, D)
    wo = A_Wo.reshape(H * DH, D)

    out = pl.pallas_call(
        functools.partial(_kernel, S=S, D=D, H=H, DH=DH, M=M, SEG=SEG),
        out_shape=jax.ShapeDtypeStruct((S, D), A_x.dtype),
        scratch_shapes=[
            pltpu.VMEM((D, 3 * D), BF16),
            pltpu.VMEM((D, D), BF16),
            pltpu.VMEM((2 * M, D), F32),
            pltpu.VMEM((2 * SEG, D), F32),
            pltpu.VMEM((SEG, D), F32),
            pltpu.VMEM((2, HIST + SEG, 2 * D), F32),
        ],
        compiler_params=pltpu.CompilerParams(vmem_limit_bytes=100 * 1024 * 1024),
    )(x, mem0, wq, wk, wv, wo, B_wqkv, B_wo)
    return out.reshape(B, S, D)
```

```python
import functools

import jax
import jax.numpy as jnp
from jax import lax
import jax.experimental.pallas as pl
import jax.experimental.pallas.tpu as pltpu

F32 = jnp.float32
BF16 = jnp.bfloat16

EPS = 1e-5
NEG = -1000000000.0
PADNEG = -3.0e38
B_HEADS = 32
B_WIN = 8
B_DIL = 2
HIST = 16


def _ln(x):
    m = jnp.mean(x, axis=-1, keepdims=True)
    xc = x - m
    v = jnp.mean(xc * xc, axis=-1, keepdims=True)
    return xc * lax.rsqrt(v + EPS)


def _dot_nt(a, b):
    return lax.dot_general(a, b, (((1,), (1,)), ((), ())), preferred_element_type=F32)


def _dot(a, b):
    return jnp.dot(a, b, preferred_element_type=F32)


def _kernel(x_ref, mem0_ref, wq_ref, wk_ref, wv_ref, wo_ref, bqkv_ref, bwo_ref,
            out_ref,
            bqkv_p, bwo_p, h_ref, xa_ref, x2_ref, kv_ref,
            *, S, D, H, DH, M, SEG):
    NSEG = S // SEG
    PW = 2 * DH
    NP = H // 2
    RL = SEG + 2 * M
    RT = 2 * SEG + 2 * M
    a_scale = DH ** (-0.5)
    b_dh = D // B_HEADS
    b_scale = b_dh ** (-0.5)
    NT = D // 128

    r_i = lax.broadcasted_iota(jnp.int32, (D, D), 0)
    c_i = lax.broadcasted_iota(jnp.int32, (D, D), 1)
    perm = jnp.where(r_i == (c_i & (B_HEADS - 1)) * b_dh + (c_i >> 5), 1.0, 0.0).astype(BF16)
    perm_t = jnp.where(c_i == (r_i & (B_HEADS - 1)) * b_dh + (r_i >> 5), 1.0, 0.0).astype(BF16)
    for j in range(3):
        bqkv_p[:, j * D:(j + 1) * D] = _dot(bqkv_ref[:, j * D:(j + 1) * D], perm).astype(BF16)
    bwo_p[...] = _dot(perm_t, bwo_ref[...]).astype(BF16)

    mem0 = mem0_ref[...].astype(F32)
    h_ref[0:SEG, :] = _ln(x_ref[0:SEG, :].astype(F32)).astype(BF16)
    h_ref[SEG:SEG + 2 * M, :] = jnp.concatenate([mem0, mem0], axis=0).astype(BF16)
    h_ref[SEG + 2 * M:RT, :] = jnp.zeros((SEG, D), BF16)
    xa_ref[...] = jnp.zeros(xa_ref.shape, F32)
    x2_ref[...] = jnp.zeros(x2_ref.shape, F32)
    kv_ref[...] = jnp.zeros(kv_ref.shape, F32)

    def b_qkv():
        xb = xa_ref[...]
        return xb, _dot(_ln(xb).astype(BF16), bqkv_p[...])

    def b_attn(t, qkv):
        outs = []
        for l in range(2):
            rows = slice(l * SEG, (l + 1) * SEG)
            q = [qkv[rows, j * 128:(j + 1) * 128] for j in range(NT)]
            for j in range(2 * NT):
                kv_ref[l, j, HIST:HIST + SEG, :] = qkv[rows, D + j * 128:D + (j + 1) * 128]
            seg = t - 1 - 2 * l
            pos = seg * SEG + lax.broadcasted_iota(jnp.int32, (SEG, 128), 0)
            logits = []
            for w in range(B_WIN):
                o = HIST - B_DIL * w
                s = q[0] * kv_ref[l, 0, o:o + SEG, :]
                for j in range(1, NT):
                    s = s + q[j] * kv_ref[l, j, o:o + SEG, :]
                s = s + pltpu.roll(s, 64, 1)
                s = s + pltpu.roll(s, 32, 1)
                logits.append(jnp.where(pos >= B_DIL * w, s * b_scale, NEG))
            m = logits[0]
            for w in range(1, B_WIN):
                m = jnp.maximum(m, logits[w])
            es = [jnp.exp(lg - m) for lg in logits]
            den = es[0]
            for w in range(1, B_WIN):
                den = den + es[w]
            inv = 1.0 / den
            tiles = []
            for j in range(NT):
                acc = None
                for w in range(B_WIN):
                    o = HIST - B_DIL * w
                    term = es[w] * kv_ref[l, NT + j, o:o + SEG, :]
                    acc = term if acc is None else acc + term
                tiles.append(acc * inv)
            outs.append(jnp.concatenate(tiles, axis=1))
            for j in range(2 * NT):
                kv_ref[l, j, 0:HIST, :] = qkv[l * SEG + SEG - HIST:(l + 1) * SEG, D + j * 128:D + (j + 1) * 128]
        return jnp.concatenate(outs, axis=0).astype(BF16)

    def b_out(t, xb, ob):
        y = xb + _dot(ob, bwo_p[...])
        row = pl.multiple_of(jnp.maximum(t - 3, 0) * SEG, SEG)
        out_ref[pl.ds(row, SEG), :] = y[SEG:2 * SEG].astype(out_ref.dtype)
        return y[0:SEG]

    RV = SEG + M
    rr = lax.broadcasted_iota(jnp.int32, (RV, 2 * RL), 0)
    cc = lax.broadcasted_iota(jnp.int32, (RV, 2 * RL), 1)
    first = cc < RL
    kc = jnp.where(first, cc, cc - RL)
    valid1 = (kc < RV) & ((kc >= SEG) | (kc <= rr))
    fill1 = jnp.where(kc < RV, NEG, PADNEG)
    valid2 = (kc >= M) & ((rr < M) | (kc - M <= rr))
    fill2 = jnp.where(kc >= M, NEG, PADNEG)
    lane128 = lax.broadcasted_iota(jnp.int32, (RT, 128), 1)
    lo = lane128 < (DH - 128)

    def softmax2(s, valid, fill):
        s = jnp.where(valid, s * a_scale, fill)
        m1 = jnp.max(jnp.where(first, s, PADNEG), axis=-1, keepdims=True)
        m2 = jnp.max(jnp.where(first, PADNEG, s), axis=-1, keepdims=True)
        e = jnp.exp(s - jnp.where(first, m1, m2))
        l1 = jnp.sum(jnp.where(first, e, 0.0), axis=-1, keepdims=True)
        l2 = jnp.sum(jnp.where(first, 0.0, e), axis=-1, keepdims=True)
        return e * (1.0 / jnp.where(first, l1, l2))

    def blockdiag(a):
        t0 = a[:, 0:128].astype(BF16)
        mid = a[:, 128:256]
        t1a = jnp.where(lo, mid, 0.0).astype(BF16)
        t1b = jnp.where(lo, 0.0, mid).astype(BF16)
        t2 = a[:, 256:384].astype(BF16)
        z = jnp.zeros((RL, 128), BF16)
        res = []
        for s0 in (0, SEG):
            top = jnp.concatenate([t0[s0:s0 + RL], t1a[s0:s0 + RL], z], axis=1)
            bot = jnp.concatenate([z, t1b[s0:s0 + RL], t2[s0:s0 + RL]], axis=1)
            res.append(jnp.concatenate([top, bot], axis=0))
        return res

    def step(t, carry):
        h = h_ref[...]
        zrow = jnp.zeros((M, 2 * RL), F32)

        def sl(p):
            return slice(p * PW, (p + 1) * PW)

        def proj_q(p):
            return _dot_nt(h, wq_ref[sl(p), :]).astype(BF16)

        def proj_k(p):
            return blockdiag(_dot_nt(h, wk_ref[sl(p), :]))

        def proj_v(p):
            return blockdiag(_dot_nt(h, wv_ref[sl(p), :]))

        def qk(q, k):
            s1 = _dot_nt(q[0:RL], k[0])
            s2 = _dot_nt(q[SEG:SEG + RL], k[1])
            p1 = softmax2(s1[0:RV], valid1, fill1)
            p2 = softmax2(s2[M:RL], valid2, fill2)
            p1 = jnp.concatenate([p1, zrow], axis=0).astype(BF16)
            p2 = jnp.concatenate([zrow, p2], axis=0).astype(BF16)
            return p1, p2

        def pv(pr, v):
            o1 = _dot(pr[0], v[0])
            o2 = _dot(pr[1], v[1])
            return jnp.concatenate([o1[0:RV], o2[M:RL]], axis=0).astype(BF16)

        acc = [None]

        def oproj(p, o):
            part = _dot(o, wo_ref[sl(p), :])
            acc[0] = part if acc[0] is None else acc[0] + part

        q = proj_q(0)
        k = proj_k(0)
        v = proj_v(0)
        os_ = {}
        for p in range(NP):
            pr = qk(q, k)
            if p + 1 < NP:
                q = proj_q(p + 1)
                k = proj_k(p + 1)
            else:
                x2 = x2_ref[...]
                x2_new = b_out(t, xb, ob)
                x2_ref[...] = x2_new
                h_ref[SEG + 2 * M:RT, :] = _ln(x2_new).astype(BF16)
                rown = pl.multiple_of(jnp.minimum(t + 1, NSEG - 1) * SEG, SEG)
                h_ref[0:SEG, :] = _ln(x_ref[pl.ds(rown, SEG), :].astype(F32)).astype(BF16)
                oproj(p - 2, os_.pop(p - 2))
            os_[p] = pv(pr, v)
            if p + 1 < NP:
                v = proj_v(p + 1)
            if p == 0:
                xb, qkv = b_qkv()
                ob = b_attn(t, qkv)
            if p >= 2 and p + 1 < NP:
                oproj(p - 2, os_.pop(p - 2))
        oproj(NP - 2, os_.pop(NP - 2))
        oproj(NP - 1, os_.pop(NP - 1))
        a = acc[0]
        row = pl.multiple_of(jnp.minimum(t, NSEG - 1) * SEG, SEG)
        x0 = x_ref[pl.ds(row, SEG), :].astype(F32)
        xa_ref[0:SEG, :] = x0 + a[0:SEG]
        xa_ref[SEG:2 * SEG, :] = x2 + a[SEG + 2 * M:RT]
        mem2 = jnp.where(t >= 2, a[SEG + M:SEG + 2 * M], mem0)
        h_ref[SEG:SEG + 2 * M, :] = jnp.concatenate([a[SEG:SEG + M], mem2], axis=0).astype(BF16)
        return carry

    lax.fori_loop(0, NSEG + 2, step, 0)
    xb, qkv = b_qkv()
    b_out(NSEG + 2, xb, b_attn(NSEG + 2, qkv))


@functools.partial(jax.jit, static_argnames=("A_seg_len",))
def pallas_interleave_layers__memory_aug_recurrent_mem_tr__sliding_local_dilated__prompt_kernel(
    A_x: jax.Array,
    A_mem0: jax.Array,
    A_Wq: jax.Array,
    A_Wk: jax.Array,
    A_Wv: jax.Array,
    A_Wo: jax.Array,
    A_seg_len,
    B_x: jax.Array,
    B_wqkv: jax.Array,
    B_wo: jax.Array,
):
    B, S, D = A_x.shape
    H, DH = A_Wq.shape[1], A_Wq.shape[2]
    M = A_mem0.shape[1]
    SEG = int(A_seg_len)
    assert B == 1 and M == 8 and SEG == 32 and DH == 192 and D % 128 == 0 and S % SEG == 0

    x = A_x.reshape(S, D)
    mem0 = A_mem0.reshape(M, D)
    wq = jnp.transpose(A_Wq, (1, 2, 0)).reshape(H * DH, D)
    wk = jnp.transpose(A_Wk, (1, 2, 0)).reshape(H * DH, D)
    wv = jnp.transpose(A_Wv, (1, 2, 0)).reshape(H * DH, D)
    wo = A_Wo.reshape(H * DH, D)

    out = pl.pallas_call(
        functools.partial(_kernel, S=S, D=D, H=H, DH=DH, M=M, SEG=SEG),
        out_shape=jax.ShapeDtypeStruct((S, D), A_x.dtype),
        scratch_shapes=[
            pltpu.VMEM((D, 3 * D), BF16),
            pltpu.VMEM((D, D), BF16),
            pltpu.VMEM((2 * SEG + 2 * M, D), BF16),
            pltpu.VMEM((2 * SEG, D), F32),
            pltpu.VMEM((SEG, D), F32),
            pltpu.VMEM((2, 2 * D // 128, HIST + SEG, 128), F32),
        ],
        compiler_params=pltpu.CompilerParams(vmem_limit_bytes=100 * 1024 * 1024),
    )(x, mem0, wq, wk, wv, wo, B_wqkv, B_wo)
    return out.reshape(B, S, D)
```

```python
import functools

import jax
import jax.numpy as jnp
from jax import lax
import jax.experimental.pallas as pl
import jax.experimental.pallas.tpu as pltpu

F32 = jnp.float32
BF16 = jnp.bfloat16

EPS = 1e-5
NEG = -1000000000.0
PADNEG = -3.0e38
B_HEADS = 32
B_WIN = 8
B_DIL = 2
HIST = 16


def _ln(x):
    m = jnp.mean(x, axis=-1, keepdims=True)
    xc = x - m
    v = jnp.mean(xc * xc, axis=-1, keepdims=True)
    return xc * lax.rsqrt(v + EPS)


def _dot_nt(a, b):
    return lax.dot_general(a, b, (((1,), (1,)), ((), ())), preferred_element_type=F32)


def _dot(a, b):
    return jnp.dot(a, b, preferred_element_type=F32)


def _kernel(x_ref, mem0_ref, wq_ref, wk_ref, wv_ref, wo_ref, bqkv_ref, bwo_ref,
            out_ref,
            bqkv_p, bwo_p, h_ref, xa_ref, x2_ref, kv_ref,
            *, S, D, H, DH, M, SEG):
    NSEG = S // SEG
    PW = 2 * DH
    NP = H // 2
    RL = SEG + 2 * M
    RT = 2 * SEG + 2 * M
    a_scale = DH ** (-0.5)
    b_dh = D // B_HEADS
    b_scale = b_dh ** (-0.5)
    NT = D // 128

    r_i = lax.broadcasted_iota(jnp.int32, (D, D), 0)
    c_i = lax.broadcasted_iota(jnp.int32, (D, D), 1)
    perm = jnp.where(r_i == (c_i & (B_HEADS - 1)) * b_dh + (c_i >> 5), 1.0, 0.0).astype(BF16)
    perm_t = jnp.where(c_i == (r_i & (B_HEADS - 1)) * b_dh + (r_i >> 5), 1.0, 0.0).astype(BF16)
    for j in range(3):
        bqkv_p[:, j * D:(j + 1) * D] = _dot(bqkv_ref[:, j * D:(j + 1) * D], perm).astype(BF16)
    bwo_p[...] = _dot(perm_t, bwo_ref[...]).astype(BF16)

    mem0 = mem0_ref[...].astype(F32)
    h_ref[0:SEG, :] = _ln(x_ref[0:SEG, :].astype(F32)).astype(BF16)
    h_ref[SEG:SEG + 2 * M, :] = jnp.concatenate([mem0, mem0], axis=0).astype(BF16)
    h_ref[SEG + 2 * M:RT, :] = jnp.zeros((SEG, D), BF16)
    xa_ref[...] = jnp.zeros(xa_ref.shape, F32)
    x2_ref[...] = jnp.zeros(x2_ref.shape, F32)
    kv_ref[...] = jnp.zeros(kv_ref.shape, F32)

    def b_qkv():
        xb = xa_ref[...]
        return xb, _dot(_ln(xb).astype(BF16), bqkv_p[...])

    def b_attn(t, qkv):
        outs = []
        for l in range(2):
            rows = slice(l * SEG, (l + 1) * SEG)
            q = [qkv[rows, j * 128:(j + 1) * 128] for j in range(NT)]
            for j in range(2 * NT):
                kv_ref[l, j, HIST:HIST + SEG, :] = qkv[rows, D + j * 128:D + (j + 1) * 128]
            seg = t - 1 - 2 * l
            pos = seg * SEG + lax.broadcasted_iota(jnp.int32, (SEG, 128), 0)
            logits = []
            for w in range(B_WIN):
                o = HIST - B_DIL * w
                s = q[0] * kv_ref[l, 0, o:o + SEG, :]
                for j in range(1, NT):
                    s = s + q[j] * kv_ref[l, j, o:o + SEG, :]
                s = s + pltpu.roll(s, 64, 1)
                s = s + pltpu.roll(s, 32, 1)
                logits.append(jnp.where(pos >= B_DIL * w, s * b_scale, NEG))
            m = logits[0]
            for w in range(1, B_WIN):
                m = jnp.maximum(m, logits[w])
            es = [jnp.exp(lg - m) for lg in logits]
            den = es[0]
            for w in range(1, B_WIN):
                den = den + es[w]
            inv = 1.0 / den
            tiles = []
            for j in range(NT):
                acc = None
                for w in range(B_WIN):
                    o = HIST - B_DIL * w
                    term = es[w] * kv_ref[l, NT + j, o:o + SEG, :]
                    acc = term if acc is None else acc + term
                tiles.append(acc * inv)
            outs.append(jnp.concatenate(tiles, axis=1))
            for j in range(2 * NT):
                kv_ref[l, j, 0:HIST, :] = qkv[l * SEG + SEG - HIST:(l + 1) * SEG, D + j * 128:D + (j + 1) * 128]
        return jnp.concatenate(outs, axis=0).astype(BF16)

    def b_out(t, xb, ob):
        y = xb + _dot(ob, bwo_p[...])
        row = pl.multiple_of(jnp.maximum(t - 3, 0) * SEG, SEG)
        out_ref[pl.ds(row, SEG), :] = y[SEG:2 * SEG].astype(out_ref.dtype)
        return y[0:SEG]

    RV = SEG + M
    rr = lax.broadcasted_iota(jnp.int32, (RT, 128), 0)
    cc = lax.broadcasted_iota(jnp.int32, (RT, 128), 1)
    lay1 = rr < RV
    first = cc < jnp.where(lay1, RL, RT)
    key = jnp.where(first, cc, cc - RL)
    exists = jnp.where(lay1, RV - 1 - key, key - RV) >= 0
    allowed = (key <= rr) | (lay1 & (key >= SEG)) | ((rr >= RV) & (rr < RL))
    valid = exists & allowed
    fill = jnp.where(exists, NEG, PADNEG)
    lo = cc < (DH - 128)

    def split_pair(a):
        t0 = a[:, 0:128].astype(BF16)
        mid = a[:, 128:256]
        tlo = jnp.where(lo, mid, 0.0).astype(BF16)
        thi = jnp.where(lo, 0.0, mid).astype(BF16)
        t2 = a[:, 256:384].astype(BF16)
        z48 = jnp.zeros((128 - RT, 128), BF16)
        z32 = jnp.zeros((128 - 2 * RL, 128), BF16)
        return (jnp.concatenate([t0, z48], axis=0),
                jnp.concatenate([tlo[0:RL], thi[0:RL], z32], axis=0),
                jnp.concatenate([z32, tlo[SEG:RT], thi[SEG:RT]], axis=0),
                jnp.concatenate([z48, t2], axis=0))

    def qk(q, k):
        t0 = _dot_nt(q[:, 0:128], k[0])
        t2 = _dot_nt(q[:, 256:384], k[3])
        t1a = _dot_nt(q[0:RL, 128:256], k[1])
        t1b = _dot_nt(q[SEG:RT, 128:256], k[2])
        s = jnp.where(first, t0, t2) + jnp.concatenate([t1a[0:RV], t1b[M:RL]], axis=0)
        s = jnp.where(valid, s * a_scale, fill)
        m1 = jnp.max(jnp.where(first, s, PADNEG), axis=-1, keepdims=True)
        m2 = jnp.max(jnp.where(first, PADNEG, s), axis=-1, keepdims=True)
        e = jnp.exp(s - jnp.where(first, m1, m2))
        e1 = jnp.where(first, e, 0.0)
        e2 = jnp.where(first, 0.0, e)
        l1 = jnp.sum(e1, axis=-1, keepdims=True)
        l2 = jnp.sum(e2, axis=-1, keepdims=True)
        inv = 1.0 / jnp.where(first, l1, l2)
        return (e1 * inv).astype(BF16), (e * inv).astype(BF16), (e2 * inv).astype(BF16)

    def pv(pr, v):
        o0 = _dot(pr[0], v[0])
        o2 = _dot(pr[2], v[3])
        o1a = _dot(pr[1][0:RL], v[1])
        o1b = _dot(pr[1][SEG:RT], v[2])
        o1 = jnp.concatenate([o1a[0:RV], o1b[M:RL]], axis=0)
        return jnp.concatenate([o0, o1, o2], axis=1).astype(BF16)

    def step(t, carry):
        h = h_ref[...]

        def sl(p):
            return slice(p * PW, (p + 1) * PW)

        def proj_q(p):
            return _dot_nt(h, wq_ref[sl(p), :]).astype(BF16)

        def proj_k(p):
            return split_pair(_dot_nt(h, wk_ref[sl(p), :]))

        def proj_v(p):
            return split_pair(_dot_nt(h, wv_ref[sl(p), :]))

        acc = [None]

        def oproj(p, o):
            part = _dot(o, wo_ref[sl(p), :])
            acc[0] = part if acc[0] is None else acc[0] + part

        q = proj_q(0)
        k = proj_k(0)
        v = proj_v(0)
        os_ = {}
        for p in range(NP):
            pr = qk(q, k)
            if p + 1 < NP:
                q = proj_q(p + 1)
                k = proj_k(p + 1)
            else:
                x2 = x2_ref[...]
                x2_new = b_out(t, xb, ob)
                x2_ref[...] = x2_new
                h_ref[SEG + 2 * M:RT, :] = _ln(x2_new).astype(BF16)
                rown = pl.multiple_of(jnp.minimum(t + 1, NSEG - 1) * SEG, SEG)
                h_ref[0:SEG, :] = _ln(x_ref[pl.ds(rown, SEG), :].astype(F32)).astype(BF16)
                oproj(p - 2, os_.pop(p - 2))
            os_[p] = pv(pr, v)
            if p + 1 < NP:
                v = proj_v(p + 1)
            if p == 0:
                xb, qkv = b_qkv()
                ob = b_attn(t, qkv)
            if p >= 2 and p + 1 < NP:
                oproj(p - 2, os_.pop(p - 2))
        oproj(NP - 2, os_.pop(NP - 2))
        oproj(NP - 1, os_.pop(NP - 1))
        a = acc[0]
        row = pl.multiple_of(jnp.minimum(t, NSEG - 1) * SEG, SEG)
        x0 = x_ref[pl.ds(row, SEG), :].astype(F32)
        xa_ref[0:SEG, :] = x0 + a[0:SEG]
        xa_ref[SEG:2 * SEG, :] = x2 + a[SEG + 2 * M:RT]
        mem2 = jnp.where(t >= 2, a[SEG + M:SEG + 2 * M], mem0)
        h_ref[SEG:SEG + 2 * M, :] = jnp.concatenate([a[SEG:SEG + M], mem2], axis=0).astype(BF16)
        return carry

    lax.fori_loop(0, NSEG + 2, step, 0)
    xb, qkv = b_qkv()
    b_out(NSEG + 2, xb, b_attn(NSEG + 2, qkv))


@functools.partial(jax.jit, static_argnames=("A_seg_len",))
def pallas_interleave_layers__memory_aug_recurrent_mem_tr__sliding_local_dilated__prompt_kernel(
    A_x: jax.Array,
    A_mem0: jax.Array,
    A_Wq: jax.Array,
    A_Wk: jax.Array,
    A_Wv: jax.Array,
    A_Wo: jax.Array,
    A_seg_len,
    B_x: jax.Array,
    B_wqkv: jax.Array,
    B_wo: jax.Array,
):
    B, S, D = A_x.shape
    H, DH = A_Wq.shape[1], A_Wq.shape[2]
    M = A_mem0.shape[1]
    SEG = int(A_seg_len)
    assert B == 1 and M == 8 and SEG == 32 and DH == 192 and D % 128 == 0 and S % SEG == 0

    x = A_x.reshape(S, D)
    mem0 = A_mem0.reshape(M, D)
    wq = jnp.transpose(A_Wq, (1, 2, 0)).reshape(H * DH, D)
    wk = jnp.transpose(A_Wk, (1, 2, 0)).reshape(H * DH, D)
    wv = jnp.transpose(A_Wv, (1, 2, 0)).reshape(H * DH, D)
    wo = A_Wo.reshape(H * DH, D)

    out = pl.pallas_call(
        functools.partial(_kernel, S=S, D=D, H=H, DH=DH, M=M, SEG=SEG),
        out_shape=jax.ShapeDtypeStruct((S, D), A_x.dtype),
        scratch_shapes=[
            pltpu.VMEM((D, 3 * D), BF16),
            pltpu.VMEM((D, D), BF16),
            pltpu.VMEM((2 * SEG + 2 * M, D), BF16),
            pltpu.VMEM((2 * SEG, D), F32),
            pltpu.VMEM((SEG, D), F32),
            pltpu.VMEM((2, 2 * D // 128, HIST + SEG, 128), F32),
        ],
        compiler_params=pltpu.CompilerParams(vmem_limit_bytes=100 * 1024 * 1024),
    )(x, mem0, wq, wk, wv, wo, B_wqkv, B_wo)
    return out.reshape(B, S, D)
```

```python
import functools

import jax
import jax.numpy as jnp
from jax import lax
import jax.experimental.pallas as pl
import jax.experimental.pallas.tpu as pltpu

F32 = jnp.float32
BF16 = jnp.bfloat16

EPS = 1e-5
NEG = -1000000000.0
PADNEG = -3.0e38
B_HEADS = 32
B_WIN = 8
B_DIL = 2
HIST = 16


def _ln(x):
    m = jnp.mean(x, axis=-1, keepdims=True)
    xc = x - m
    v = jnp.mean(xc * xc, axis=-1, keepdims=True)
    return xc * lax.rsqrt(v + EPS)


def _dot_nt(a, b):
    return lax.dot_general(a, b, (((1,), (1,)), ((), ())), preferred_element_type=F32)


def _dot(a, b):
    return jnp.dot(a, b, preferred_element_type=F32)


def _cat0(xs):
    return jnp.concatenate(xs, axis=0)


def _cat1(xs):
    return jnp.concatenate(xs, axis=1)


def _kernel(mem0_ref, x_hbm, wq_hbm, wk_hbm, wv_hbm, wo_hbm, bqkv_hbm, bwo_hbm,
            out_hbm,
            x_ref, out_ref, wq_ref, wk_ref, wv_ref, wo_ref, bqkv_ref, bwo_ref,
            bqkv_p, bwo_p, h_ref, xa_ref, x2_ref, kv_ref, wsem, sem,
            *, S, D, H, DH, M, SEG):
    NSEG = S // SEG
    PW = 2 * DH
    NP = H // 2
    RV = SEG + M
    RL = SEG + 2 * M
    RT = 2 * SEG + 2 * M
    a_scale = DH ** (-0.5)
    b_dh = D // B_HEADS
    b_scale = b_dh ** (-0.5)
    NT = D // 128
    X0 = 2 * SEG

    def sl(p):
        return slice(p * PW, (p + 1) * PW)

    cp_x0 = pltpu.make_async_copy(x_hbm.at[0:X0], x_ref.at[0:X0], sem.at[0])
    cp_x1 = pltpu.make_async_copy(x_hbm.at[X0:S], x_ref.at[X0:S], sem.at[1])
    cp_bqkv = pltpu.make_async_copy(bqkv_hbm, bqkv_ref, sem.at[2])
    cp_bwo = pltpu.make_async_copy(bwo_hbm, bwo_ref, sem.at[3])
    w_pairs = ((wq_hbm, wq_ref), (wk_hbm, wk_ref), (wv_hbm, wv_ref), (wo_hbm, wo_ref))

    def cp_w(i, p):
        src, dst = w_pairs[i]
        return pltpu.make_async_copy(src.at[sl(p)], dst.at[sl(p)], wsem.at[i * NP + p])

    def start_group(p):
        for i in range(4):
            cp_w(i, p).start()

    def wait_group(p):
        for i in range(4):
            cp_w(i, p).wait()

    cp_x0.start()
    start_group(0)
    start_group(1)

    mem0 = mem0_ref[...].astype(F32)
    xa_ref[...] = jnp.zeros(xa_ref.shape, F32)
    kv_ref[...] = jnp.zeros(kv_ref.shape, F32)
    h_ref[SEG:RL, :] = _cat0([mem0, mem0]).astype(BF16)
    cp_x0.wait()
    h_ref[0:SEG, :] = _ln(x_ref[0:SEG, :].astype(F32)).astype(BF16)

    def perm_piece(i):
        j, c = divmod(i, NT)
        if j < 3:
            r_i = lax.broadcasted_iota(jnp.int32, (D, 128), 0)
            c_i = lax.broadcasted_iota(jnp.int32, (D, 128), 1) + c * 128
            perm = jnp.where(r_i == (c_i & (B_HEADS - 1)) * b_dh + (c_i >> 5), 1.0, 0.0).astype(BF16)
            bqkv_p[:, j * D + c * 128:j * D + (c + 1) * 128] = _dot(
                bqkv_ref[:, j * D:(j + 1) * D], perm).astype(BF16)
        else:
            r_i = lax.broadcasted_iota(jnp.int32, (128, D), 0) + c * 128
            c_i = lax.broadcasted_iota(jnp.int32, (128, D), 1)
            perm_t = jnp.where(c_i == (r_i & (B_HEADS - 1)) * b_dh + (r_i >> 5), 1.0, 0.0).astype(BF16)
            bwo_p[c * 128:(c + 1) * 128, :] = _dot(perm_t, bwo_ref[...]).astype(BF16)

    def first_step_hook(p):
        wait_group(p)
        if p == 0:
            cp_bqkv.start()
            cp_bwo.start()
        if p + 2 < NP:
            start_group(p + 2)
        if p + 2 == NP:
            cp_x1.start()
        if p == 3:
            cp_bqkv.wait()
            cp_bwo.wait()
        if p >= 3:
            for i in range(2 * (p - 3), min(2 * (p - 2), 4 * NT)):
                perm_piece(i)

    def b_qkv(layers):
        xb = xa_ref[layers[0] * SEG:(layers[-1] + 1) * SEG, :]
        return xb, _dot(_ln(xb).astype(BF16), bqkv_p[...])

    def b_attn(t, qkv, layers):
        outs = []
        for i, l in enumerate(layers):
            rows = slice(i * SEG, (i + 1) * SEG)
            q = [qkv[rows, j * 128:(j + 1) * 128] for j in range(NT)]
            for j in range(2 * NT):
                kv_ref[l, j, HIST:HIST + SEG, :] = qkv[rows, D + j * 128:D + (j + 1) * 128]
            seg = t - 1 - 2 * l
            pos = seg * SEG + lax.broadcasted_iota(jnp.int32, (SEG, 128), 0)
            logits = []
            for w in range(B_WIN):
                o = HIST - B_DIL * w
                s = q[0] * kv_ref[l, 0, o:o + SEG, :]
                for j in range(1, NT):
                    s = s + q[j] * kv_ref[l, j, o:o + SEG, :]
                s = s + pltpu.roll(s, 64, 1)
                s = s + pltpu.roll(s, 32, 1)
                logits.append(jnp.where(pos >= B_DIL * w, s * b_scale, NEG))
            m = logits[0]
            for w in range(1, B_WIN):
                m = jnp.maximum(m, logits[w])
            es = [jnp.exp(lg - m) for lg in logits]
            den = es[0]
            for w in range(1, B_WIN):
                den = den + es[w]
            inv = 1.0 / den
            tiles = []
            for j in range(NT):
                acc = None
                for w in range(B_WIN):
                    o = HIST - B_DIL * w
                    term = es[w] * kv_ref[l, NT + j, o:o + SEG, :]
                    acc = term if acc is None else acc + term
                tiles.append(acc * inv)
            outs.append(_cat1(tiles))
            for j in range(2 * NT):
                kv_ref[l, j, 0:HIST, :] = qkv[(i + 1) * SEG - HIST:(i + 1) * SEG,
                                              D + j * 128:D + (j + 1) * 128]
        return _cat0(outs).astype(BF16)

    def b_out(t, xb, ob, layers):
        y = xb + _dot(ob, bwo_p[...])
        for i, l in enumerate(layers):
            yl = y[i * SEG:(i + 1) * SEG]
            if l == 0:
                x2_ref[...] = yl
                h_ref[RL:RT, :] = _ln(yl).astype(BF16)
            else:
                if isinstance(t, int):
                    row = (t - 3) * SEG
                else:
                    row = pl.multiple_of(jnp.maximum(t - 3, 0) * SEG, SEG)
                out_ref[pl.ds(row, SEG), :] = yl.astype(out_ref.dtype)

    def softmax2(s, first, valid, fill):
        s = jnp.where(valid, s * a_scale, fill)
        m1 = jnp.max(jnp.where(first, s, PADNEG), axis=-1, keepdims=True)
        m2 = jnp.max(jnp.where(first, PADNEG, s), axis=-1, keepdims=True)
        e = jnp.exp(s - jnp.where(first, m1, m2))
        e1 = jnp.where(first, e, 0.0)
        e2 = jnp.where(first, 0.0, e)
        l1 = jnp.sum(e1, axis=-1, keepdims=True)
        l2 = jnp.sum(e2, axis=-1, keepdims=True)
        inv = 1.0 / jnp.where(first, l1, l2)
        return e, e1, e2, inv

    def make_joint():
        rr = lax.broadcasted_iota(jnp.int32, (RT, 128), 0)
        cc = lax.broadcasted_iota(jnp.int32, (RT, 128), 1)
        lay1 = rr < RV
        first = cc < jnp.where(lay1, RL, RT)
        key = jnp.where(first, cc, cc - RL)
        exists = jnp.where(lay1, RV - 1 - key, key - RV) >= 0
        allowed = (key <= rr) | (lay1 & (key >= SEG)) | ((rr >= RV) & (rr < RL))
        valid = exists & allowed
        fill = jnp.where(exists, NEG, PADNEG)
        lo = cc < (DH - 128)
        z48 = jnp.zeros((128 - RT, 128), F32)
        z32 = jnp.zeros((128 - 2 * RL, 128), F32)

        def prep_q(a):
            return (a[:, 0:128].astype(BF16), a[0:RL, 128:256].astype(BF16),
                    a[SEG:RT, 128:256].astype(BF16), a[:, 256:384].astype(BF16))

        def prep_kv(a):
            mid = a[:, 128:256]
            tlo = jnp.where(lo, mid, 0.0)
            thi = jnp.where(lo, 0.0, mid)
            return (_cat0([a[:, 0:128], z48]).astype(BF16),
                    _cat0([tlo[0:RL], thi[0:RL], z32]).astype(BF16),
                    _cat0([z32, tlo[SEG:RT], thi[SEG:RT]]).astype(BF16),
                    _cat0([z48, a[:, 256:384]]).astype(BF16))

        def qk(q, k):
            t0 = _dot_nt(q[0], k[0])
            t2 = _dot_nt(q[3], k[3])
            t1a = _dot_nt(q[1], k[1])
            t1b = _dot_nt(q[2], k[2])
            s = jnp.where(first, t0, t2) + _cat0([t1a[0:RV], t1b[M:RL]])
            e, e1, e2, inv = softmax2(s, first, valid, fill)
            pa = e * inv
            return ((e1 * inv).astype(BF16), pa[0:RL].astype(BF16),
                    pa[SEG:RT].astype(BF16), (e2 * inv).astype(BF16))

        def pv(pr, v):
            o0 = _dot(pr[0], v[0])
            o2 = _dot(pr[3], v[3])
            o1a = _dot(pr[1], v[1])
            o1b = _dot(pr[2], v[2])
            return _cat1([o0, _cat0([o1a[0:RV], o1b[M:RL]]), o2]).astype(BF16)

        return prep_q, prep_kv, qk, pv

    def make_single(layer):
        rr = lax.broadcasted_iota(jnp.int32, (RV, 2 * RL), 0)
        cc = lax.broadcasted_iota(jnp.int32, (RV, 2 * RL), 1)
        first = cc < RL
        kc = jnp.where(first, cc, cc - RL)
        if layer == 0:
            exists = kc < RV
            valid = exists & ((kc >= SEG) | (kc <= rr))
            r0 = 0
        else:
            exists = kc >= M
            valid = exists & ((rr < M) | (kc - M <= rr))
            r0 = M
        fill = jnp.where(exists, NEG, PADNEG)
        lo = lax.broadcasted_iota(jnp.int32, (RL, PW), 1) < DH
        zrow = jnp.zeros((M, 2 * RL), F32)

        def prep_q(a):
            return a.astype(BF16)

        def prep_kv(a):
            return _cat0([jnp.where(lo, a, 0.0), jnp.where(lo, 0.0, a)]).astype(BF16)

        def qk(q, k):
            s = _dot_nt(q, k)[r0:r0 + RV]
            e, _, _, inv = softmax2(s, first, valid, fill)
            pa = e * inv
            return _cat0([pa, zrow] if layer == 0 else [zrow, pa]).astype(BF16)

        def pv(pr, v):
            return _dot(pr, v).astype(BF16)

        return prep_q, prep_kv, qk, pv

    def step(t, a_layers, b_layers, wait_w=False, wait_x=False):
        r0 = 0 if 0 in a_layers else SEG
        r1 = RT if 1 in a_layers else RL
        h = h_ref[r0:r1, :]
        if len(a_layers) == 2:
            prep_q, prep_kv, qk, pv = make_joint()
        else:
            prep_q, prep_kv, qk, pv = make_single(a_layers[0])

        def proj(i, p):
            if wait_w and i == 0:
                first_step_hook(p)
            return _dot_nt(h, w_pairs[i][1][sl(p), :])

        acc = [None]

        def oproj(p, o):
            part = _dot(o, wo_ref[sl(p), :])
            acc[0] = part if acc[0] is None else acc[0] + part

        def xrows(seg):
            if isinstance(seg, int):
                return x_ref[seg * SEG:(seg + 1) * SEG, :].astype(F32)
            return x_ref[pl.ds(pl.multiple_of(seg * SEG, SEG), SEG), :].astype(F32)

        q = prep_q(proj(0, 0))
        k = prep_kv(proj(1, 0))
        v = prep_kv(proj(2, 0))
        os_ = {}
        x2 = None
        for p in range(NP):
            pr = qk(q, k)
            if p + 1 < NP:
                q = prep_q(proj(0, p + 1))
                k = prep_kv(proj(1, p + 1))
            else:
                if 1 in a_layers:
                    x2 = x2_ref[...]
                if b_layers:
                    b_out(t, xb, ob, b_layers)
                if 0 in a_layers:
                    if wait_x:
                        cp_x1.wait()
                    nxt = t + 1 if isinstance(t, int) else jnp.minimum(t + 1, NSEG - 1)
                    h_ref[0:SEG, :] = _ln(xrows(nxt)).astype(BF16)
                oproj(p - 2, os_.pop(p - 2))
            os_[p] = pv(pr, v)
            if p + 1 < NP:
                v = prep_kv(proj(2, p + 1))
            if p == 0 and b_layers:
                xb, qkv = b_qkv(b_layers)
                ob = b_attn(t, qkv, b_layers)
            if p >= 2 and p + 1 < NP:
                oproj(p - 2, os_.pop(p - 2))
        oproj(NP - 2, os_.pop(NP - 2))
        oproj(NP - 1, os_.pop(NP - 1))
        a = acc[0]
        if 0 in a_layers:
            xa_ref[0:SEG, :] = xrows(t) + a[0:SEG]
        if 1 in a_layers:
            xa_ref[SEG:2 * SEG, :] = x2 + a[RL - r0:RT - r0]
        mem1 = a[SEG - r0:RV - r0]
        mem2 = a[RV - r0:RL - r0] if 1 in a_layers else mem0
        h_ref[SEG:RL, :] = _cat0([mem1, mem2]).astype(BF16)

    step(0, (0,), (), wait_w=True)
    step(1, (0,), (0,), wait_x=True)

    def body(t, carry):
        step(t, (0, 1), (0, 1))
        return carry

    lax.fori_loop(2, NSEG, body, 0)
    done = (NSEG - 3) * SEG
    cp_o0 = pltpu.make_async_copy(out_ref.at[0:done], out_hbm.at[0:done], sem.at[4])
    cp_o0.start()
    step(NSEG, (1,), (0, 1))
    step(NSEG + 1, (1,), (1,))
    xb, qkv = b_qkv((1,))
    b_out(NSEG + 2, xb, b_attn(NSEG + 2, qkv, (1,)), (1,))
    cp_o1 = pltpu.make_async_copy(out_ref.at[done:S], out_hbm.at[done:S], sem.at[5])
    cp_o1.start()
    cp_o0.wait()
    cp_o1.wait()


@functools.partial(jax.jit, static_argnames=("A_seg_len",))
def pallas_interleave_layers__memory_aug_recurrent_mem_tr__sliding_local_dilated__prompt_kernel(
    A_x: jax.Array,
    A_mem0: jax.Array,
    A_Wq: jax.Array,
    A_Wk: jax.Array,
    A_Wv: jax.Array,
    A_Wo: jax.Array,
    A_seg_len,
    B_x: jax.Array,
    B_wqkv: jax.Array,
    B_wo: jax.Array,
):
    B, S, D = A_x.shape
    H, DH = A_Wq.shape[1], A_Wq.shape[2]
    M = A_mem0.shape[1]
    SEG = int(A_seg_len)
    assert B == 1 and M == 8 and SEG == 32 and DH == 192 and D % 128 == 0 and S % SEG == 0

    x = A_x.reshape(S, D)
    mem0 = A_mem0.reshape(M, D)
    wq = jnp.transpose(A_Wq, (1, 2, 0)).reshape(H * DH, D)
    wk = jnp.transpose(A_Wk, (1, 2, 0)).reshape(H * DH, D)
    wv = jnp.transpose(A_Wv, (1, 2, 0)).reshape(H * DH, D)
    wo = A_Wo.reshape(H * DH, D)

    hbm = pl.BlockSpec(memory_space=pl.ANY)
    out = pl.pallas_call(
        functools.partial(_kernel, S=S, D=D, H=H, DH=DH, M=M, SEG=SEG),
        out_shape=jax.ShapeDtypeStruct((S, D), A_x.dtype),
        in_specs=[pl.BlockSpec(memory_space=pltpu.VMEM)] + [hbm] * 7,
        out_specs=hbm,
        scratch_shapes=[
            pltpu.VMEM((S, D), BF16),
            pltpu.VMEM((S, D), BF16),
            pltpu.VMEM((H * DH, D), BF16),
            pltpu.VMEM((H * DH, D), BF16),
            pltpu.VMEM((H * DH, D), BF16),
            pltpu.VMEM((H * DH, D), BF16),
            pltpu.VMEM((D, 3 * D), BF16),
            pltpu.VMEM((D, D), BF16),
            pltpu.VMEM((D, 3 * D), BF16),
            pltpu.VMEM((D, D), BF16),
            pltpu.VMEM((2 * SEG + 2 * M, D), BF16),
            pltpu.VMEM((2 * SEG, D), F32),
            pltpu.VMEM((SEG, D), F32),
            pltpu.VMEM((2, 2 * D // 128, HIST + SEG, 128), F32),
            pltpu.SemaphoreType.DMA((4 * (H // 2),)),
            pltpu.SemaphoreType.DMA((6,)),
        ],
        compiler_params=pltpu.CompilerParams(vmem_limit_bytes=100 * 1024 * 1024),
    )(mem0, x, wq, wk, wv, wo, B_wqkv, B_wo)
    return out.reshape(B, S, D)
```

```python
import functools

import jax
import jax.numpy as jnp
from jax import lax
import jax.experimental.pallas as pl
import jax.experimental.pallas.tpu as pltpu

F32 = jnp.float32
BF16 = jnp.bfloat16
U32 = jnp.uint32

EPS = 1e-5
NEG = -1000000000.0
PADNEG = -3.0e38
B_HEADS = 32
B_WIN = 8
B_DIL = 2
HIST = 16


def _ln(x):
    m = jnp.mean(x, axis=-1, keepdims=True)
    xc = x - m
    v = jnp.mean(xc * xc, axis=-1, keepdims=True)
    return xc * lax.rsqrt(v + EPS)


def _dot_nt(a, b):
    return lax.dot_general(a, b, (((1,), (1,)), ((), ())), preferred_element_type=F32)


def _dot(a, b):
    return jnp.dot(a, b, preferred_element_type=F32)


def _pack(a):
    return pltpu.bitcast(a, U32)


def _unpack(a):
    return pltpu.bitcast(a, BF16)


def _cat0(xs):
    return jnp.concatenate(xs, axis=0)


def _cat1(xs):
    return jnp.concatenate(xs, axis=1)


def _kernel(mem0_ref, x_hbm, wq_hbm, wk_hbm, wv_hbm, wo_hbm, bqkv_hbm, bwo_hbm,
            out_hbm,
            x_ref, out_ref, wq_ref, wk_ref, wv_ref, wo_ref, bqkv_ref, bwo_ref,
            wqkv_p, wo_p, bqkv_p, bwo_p, h_ref, xa_ref, x2_ref, kv_ref, wsem, sem,
            *, S, D, H, DH, M, SEG):
    NSEG = S // SEG
    PW = 2 * DH
    NP = H // 2
    RV = SEG + M
    RL = SEG + 2 * M
    RT = 2 * SEG + 2 * M
    a_scale = DH ** (-0.5)
    b_dh = D // B_HEADS
    b_scale = b_dh ** (-0.5)
    NT = D // 128
    X0 = 2 * SEG

    def sl(p):
        return slice(p * PW, (p + 1) * PW)

    cp_x0 = pltpu.make_async_copy(x_hbm.at[0:X0], x_ref.at[0:X0], sem.at[0])
    cp_x1 = pltpu.make_async_copy(x_hbm.at[X0:S], x_ref.at[X0:S], sem.at[1])
    cp_bqkv = pltpu.make_async_copy(bqkv_hbm, bqkv_ref, sem.at[2])
    cp_bwo = pltpu.make_async_copy(bwo_hbm, bwo_ref, sem.at[3])
    w_pairs = ((wq_hbm, wq_ref), (wk_hbm, wk_ref), (wv_hbm, wv_ref), (wo_hbm, wo_ref))

    def cp_w(i, p):
        src, dst = w_pairs[i]
        return pltpu.make_async_copy(src.at[sl(p)], dst.at[sl(p)], wsem.at[i * NP + p])

    def start_group(p):
        for i in range(4):
            cp_w(i, p).start()

    def wait_group(p):
        for i in range(4):
            cp_w(i, p).wait()

    cp_x0.start()
    start_group(0)
    start_group(1)

    mem0 = mem0_ref[...].astype(F32)
    xa_ref[...] = jnp.zeros(xa_ref.shape, F32)
    kv_ref[...] = jnp.zeros(kv_ref.shape, F32)
    h_ref[SEG:RL, :] = _cat0([mem0, mem0]).astype(BF16)
    cp_x0.wait()
    h_ref[0:SEG, :] = _ln(x_ref[0:SEG, :].astype(F32)).astype(BF16)

    def perm_piece(i):
        j, c = divmod(i, NT)
        if j < 3:
            r_i = lax.broadcasted_iota(jnp.int32, (D, 128), 0)
            c_i = lax.broadcasted_iota(jnp.int32, (D, 128), 1) + c * 128
            perm = jnp.where(r_i == (c_i & (B_HEADS - 1)) * b_dh + (c_i >> 5), 1.0, 0.0).astype(BF16)
            bqkv_p[:, j * D + c * 128:j * D + (c + 1) * 128] = _pack(_dot(
                bqkv_ref[:, j * D:(j + 1) * D], perm).astype(BF16))
        else:
            r_i = lax.broadcasted_iota(jnp.int32, (128, D), 0) + c * 128
            c_i = lax.broadcasted_iota(jnp.int32, (128, D), 1)
            perm_t = jnp.where(c_i == (r_i & (B_HEADS - 1)) * b_dh + (r_i >> 5), 1.0, 0.0).astype(BF16)
            bwo_p[c * 64:(c + 1) * 64, :] = _pack(_dot(perm_t, bwo_ref[...]).astype(BF16))

    def first_step_hook(p):
        wait_group(p)
        if p == 0:
            cp_bqkv.start()
            cp_bwo.start()
        if p + 2 < NP:
            start_group(p + 2)
        if p + 2 == NP:
            cp_x1.start()
        for i in range(3):
            wqkv_p[i, p] = _pack(w_pairs[i][1][sl(p), :].T)
        wo_p[p] = _pack(wo_ref[sl(p), :])
        if p == 3:
            cp_bqkv.wait()
            cp_bwo.wait()
        if p >= 3:
            for i in range(2 * (p - 3), min(2 * (p - 2), 4 * NT)):
                perm_piece(i)

    def b_qkv(layers):
        xb = xa_ref[layers[0] * SEG:(layers[-1] + 1) * SEG, :]
        return xb, _dot(_ln(xb).astype(BF16), _unpack(bqkv_p[...]))

    def b_attn(t, qkv, layers):
        outs = []
        for i, l in enumerate(layers):
            rows = slice(i * SEG, (i + 1) * SEG)
            q = [qkv[rows, j * 128:(j + 1) * 128] for j in range(NT)]
            for j in range(2 * NT):
                kv_ref[l, j, HIST:HIST + SEG, :] = qkv[rows, D + j * 128:D + (j + 1) * 128]
            seg = t - 1 - 2 * l
            pos = seg * SEG + lax.broadcasted_iota(jnp.int32, (SEG, 128), 0)
            logits = []
            for w in range(B_WIN):
                o = HIST - B_DIL * w
                s = q[0] * kv_ref[l, 0, o:o + SEG, :]
                for j in range(1, NT):
                    s = s + q[j] * kv_ref[l, j, o:o + SEG, :]
                s = s + pltpu.roll(s, 64, 1)
                s = s + pltpu.roll(s, 32, 1)
                logits.append(jnp.where(pos >= B_DIL * w, s * b_scale, NEG))
            m = logits[0]
            for w in range(1, B_WIN):
                m = jnp.maximum(m, logits[w])
            es = [jnp.exp(lg - m) for lg in logits]
            den = es[0]
            for w in range(1, B_WIN):
                den = den + es[w]
            inv = 1.0 / den
            tiles = []
            for j in range(NT):
                acc = None
                for w in range(B_WIN):
                    o = HIST - B_DIL * w
                    term = es[w] * kv_ref[l, NT + j, o:o + SEG, :]
                    acc = term if acc is None else acc + term
                tiles.append(acc * inv)
            outs.append(_cat1(tiles))
            for j in range(2 * NT):
                kv_ref[l, j, 0:HIST, :] = qkv[(i + 1) * SEG - HIST:(i + 1) * SEG,
                                              D + j * 128:D + (j + 1) * 128]
        return _cat0(outs).astype(BF16)

    def b_out(t, xb, ob, layers):
        y = xb + _dot(ob, _unpack(bwo_p[...]))
        for i, l in enumerate(layers):
            yl = y[i * SEG:(i + 1) * SEG]
            if l == 0:
                x2_ref[...] = yl
                h_ref[RL:RT, :] = _ln(yl).astype(BF16)
            else:
                if isinstance(t, int):
                    row = (t - 3) * SEG
                else:
                    row = pl.multiple_of(jnp.maximum(t - 3, 0) * SEG, SEG)
                out_ref[pl.ds(row, SEG), :] = yl.astype(out_ref.dtype)

    def softmax2(s, first, valid, fill):
        s = jnp.where(valid, s * a_scale, fill)
        m1 = jnp.max(jnp.where(first, s, PADNEG), axis=-1, keepdims=True)
        m2 = jnp.max(jnp.where(first, PADNEG, s), axis=-1, keepdims=True)
        e = jnp.exp(s - jnp.where(first, m1, m2))
        e1 = jnp.where(first, e, 0.0)
        e2 = jnp.where(first, 0.0, e)
        l1 = jnp.sum(e1, axis=-1, keepdims=True)
        l2 = jnp.sum(e2, axis=-1, keepdims=True)
        inv = 1.0 / jnp.where(first, l1, l2)
        return e, e1, e2, inv

    def make_joint():
        rr = lax.broadcasted_iota(jnp.int32, (RT, 128), 0)
        cc = lax.broadcasted_iota(jnp.int32, (RT, 128), 1)
        lay1 = rr < RV
        first = cc < jnp.where(lay1, RL, RT)
        key = jnp.where(first, cc, cc - RL)
        exists = jnp.where(lay1, RV - 1 - key, key - RV) >= 0
        allowed = (key <= rr) | (lay1 & (key >= SEG)) | ((rr >= RV) & (rr < RL))
        valid = exists & allowed
        fill = jnp.where(exists, NEG, PADNEG)
        lo = cc < (DH - 128)
        z48 = jnp.zeros((128 - RT, 128), F32)
        z32 = jnp.zeros((128 - 2 * RL, 128), F32)

        def prep_q(a):
            return (a[:, 0:128].astype(BF16), a[0:RL, 128:256].astype(BF16),
                    a[SEG:RT, 128:256].astype(BF16), a[:, 256:384].astype(BF16))

        def prep_kv(a):
            mid = a[:, 128:256]
            tlo = jnp.where(lo, mid, 0.0)
            thi = jnp.where(lo, 0.0, mid)
            return (_cat0([a[:, 0:128], z48]).astype(BF16),
                    _cat0([tlo[0:RL], thi[0:RL], z32]).astype(BF16),
                    _cat0([z32, tlo[SEG:RT], thi[SEG:RT]]).astype(BF16),
                    _cat0([z48, a[:, 256:384]]).astype(BF16))

        def qk(q, k):
            t0 = _dot_nt(q[0], k[0])
            t2 = _dot_nt(q[3], k[3])
            t1a = _dot_nt(q[1], k[1])
            t1b = _dot_nt(q[2], k[2])
            s = jnp.where(first, t0, t2) + _cat0([t1a[0:RV], t1b[M:RL]])
            e, e1, e2, inv = softmax2(s, first, valid, fill)
            pa = e * inv
            return ((e1 * inv).astype(BF16), pa[0:RL].astype(BF16),
                    pa[SEG:RT].astype(BF16), (e2 * inv).astype(BF16))

        def pv(pr, v):
            o0 = _dot(pr[0], v[0])
            o2 = _dot(pr[3], v[3])
            o1a = _dot(pr[1], v[1])
            o1b = _dot(pr[2], v[2])
            return _cat1([o0, _cat0([o1a[0:RV], o1b[M:RL]]), o2]).astype(BF16)

        return prep_q, prep_kv, qk, pv

    def make_single(layer):
        rr = lax.broadcasted_iota(jnp.int32, (RV, 2 * RL), 0)
        cc = lax.broadcasted_iota(jnp.int32, (RV, 2 * RL), 1)
        first = cc < RL
        kc = jnp.where(first, cc, cc - RL)
        if layer == 0:
            exists = kc < RV
            valid = exists & ((kc >= SEG) | (kc <= rr))
            r0 = 0
        else:
            exists = kc >= M
            valid = exists & ((rr < M) | (kc - M <= rr))
            r0 = M
        fill = jnp.where(exists, NEG, PADNEG)
        lo = lax.broadcasted_iota(jnp.int32, (RL, PW), 1) < DH
        zrow = jnp.zeros((M, 2 * RL), F32)

        def prep_q(a):
            return a.astype(BF16)

        def prep_kv(a):
            return _cat0([jnp.where(lo, a, 0.0), jnp.where(lo, 0.0, a)]).astype(BF16)

        def qk(q, k):
            s = _dot_nt(q, k)[r0:r0 + RV]
            e, _, _, inv = softmax2(s, first, valid, fill)
            pa = e * inv
            return _cat0([pa, zrow] if layer == 0 else [zrow, pa]).astype(BF16)

        def pv(pr, v):
            return _dot(pr, v).astype(BF16)

        return prep_q, prep_kv, qk, pv

    def step(t, a_layers, b_layers, wait_w=False, wait_x=False):
        r0 = 0 if 0 in a_layers else SEG
        r1 = RT if 1 in a_layers else RL
        h = h_ref[r0:r1, :]
        if len(a_layers) == 2:
            prep_q, prep_kv, qk, pv = make_joint()
        else:
            prep_q, prep_kv, qk, pv = make_single(a_layers[0])

        def proj(i, p):
            if wait_w and i == 0:
                first_step_hook(p)
            return _dot(h, _unpack(wqkv_p[i, p]))

        acc = [None]

        def oproj(p, o):
            part = _dot(o, _unpack(wo_p[p]))
            acc[0] = part if acc[0] is None else acc[0] + part

        def xrows(seg):
            if isinstance(seg, int):
                return x_ref[seg * SEG:(seg + 1) * SEG, :].astype(F32)
            return x_ref[pl.ds(pl.multiple_of(seg * SEG, SEG), SEG), :].astype(F32)

        q = prep_q(proj(0, 0))
        k = prep_kv(proj(1, 0))
        v = prep_kv(proj(2, 0))
        os_ = {}
        x2 = None
        for p in range(NP):
            pr = qk(q, k)
            if p + 1 < NP:
                q = prep_q(proj(0, p + 1))
                k = prep_kv(proj(1, p + 1))
            else:
                if 1 in a_layers:
                    x2 = x2_ref[...]
                if b_layers:
                    b_out(t, xb, ob, b_layers)
                if 0 in a_layers:
                    if wait_x:
                        cp_x1.wait()
                    nxt = t + 1 if isinstance(t, int) else jnp.minimum(t + 1, NSEG - 1)
                    h_ref[0:SEG, :] = _ln(xrows(nxt)).astype(BF16)
                oproj(p - 2, os_.pop(p - 2))
            os_[p] = pv(pr, v)
            if p + 1 < NP:
                v = prep_kv(proj(2, p + 1))
            if p == 0 and b_layers:
                xb, qkv = b_qkv(b_layers)
                ob = b_attn(t, qkv, b_layers)
            if p >= 2 and p + 1 < NP:
                oproj(p - 2, os_.pop(p - 2))
        oproj(NP - 2, os_.pop(NP - 2))
        oproj(NP - 1, os_.pop(NP - 1))
        a = acc[0]
        if 0 in a_layers:
            xa_ref[0:SEG, :] = xrows(t) + a[0:SEG]
        if 1 in a_layers:
            xa_ref[SEG:2 * SEG, :] = x2 + a[RL - r0:RT - r0]
        mem1 = a[SEG - r0:RV - r0]
        mem2 = a[RV - r0:RL - r0] if 1 in a_layers else mem0
        h_ref[SEG:RL, :] = _cat0([mem1, mem2]).astype(BF16)

    step(0, (0,), (), wait_w=True)
    step(1, (0,), (0,), wait_x=True)

    def body(t, carry):
        step(t, (0, 1), (0, 1))
        return carry

    lax.fori_loop(2, NSEG, body, 0)
    done = (NSEG - 3) * SEG
    cp_o0 = pltpu.make_async_copy(out_ref.at[0:done], out_hbm.at[0:done], sem.at[4])
    cp_o0.start()
    step(NSEG, (1,), (0, 1))
    step(NSEG + 1, (1,), (1,))
    xb, qkv = b_qkv((1,))
    b_out(NSEG + 2, xb, b_attn(NSEG + 2, qkv, (1,)), (1,))
    cp_o1 = pltpu.make_async_copy(out_ref.at[done:S], out_hbm.at[done:S], sem.at[5])
    cp_o1.start()
    cp_o0.wait()
    cp_o1.wait()


@functools.partial(jax.jit, static_argnames=("A_seg_len",))
def pallas_interleave_layers__memory_aug_recurrent_mem_tr__sliding_local_dilated__prompt_kernel(
    A_x: jax.Array,
    A_mem0: jax.Array,
    A_Wq: jax.Array,
    A_Wk: jax.Array,
    A_Wv: jax.Array,
    A_Wo: jax.Array,
    A_seg_len,
    B_x: jax.Array,
    B_wqkv: jax.Array,
    B_wo: jax.Array,
):
    B, S, D = A_x.shape
    H, DH = A_Wq.shape[1], A_Wq.shape[2]
    M = A_mem0.shape[1]
    SEG = int(A_seg_len)
    assert B == 1 and M == 8 and SEG == 32 and DH == 192 and D % 128 == 0 and S % SEG == 0

    x = A_x.reshape(S, D)
    mem0 = A_mem0.reshape(M, D)
    wq = jnp.transpose(A_Wq, (1, 2, 0)).reshape(H * DH, D)
    wk = jnp.transpose(A_Wk, (1, 2, 0)).reshape(H * DH, D)
    wv = jnp.transpose(A_Wv, (1, 2, 0)).reshape(H * DH, D)
    wo = A_Wo.reshape(H * DH, D)

    hbm = pl.BlockSpec(memory_space=pl.ANY)
    out = pl.pallas_call(
        functools.partial(_kernel, S=S, D=D, H=H, DH=DH, M=M, SEG=SEG),
        out_shape=jax.ShapeDtypeStruct((S, D), A_x.dtype),
        in_specs=[pl.BlockSpec(memory_space=pltpu.VMEM)] + [hbm] * 7,
        out_specs=hbm,
        scratch_shapes=[
            pltpu.VMEM((S, D), BF16),
            pltpu.VMEM((S, D), BF16),
            pltpu.VMEM((H * DH, D), BF16),
            pltpu.VMEM((H * DH, D), BF16),
            pltpu.VMEM((H * DH, D), BF16),
            pltpu.VMEM((H * DH, D), BF16),
            pltpu.VMEM((D, 3 * D), BF16),
            pltpu.VMEM((D, D), BF16),
            pltpu.VMEM((3, H // 2, D // 2, 2 * DH), U32),
            pltpu.VMEM((H // 2, DH, D), U32),
            pltpu.VMEM((D // 2, 3 * D), U32),
            pltpu.VMEM((D // 2, D), U32),
            pltpu.VMEM((2 * SEG + 2 * M, D), BF16),
            pltpu.VMEM((2 * SEG, D), F32),
            pltpu.VMEM((SEG, D), F32),
            pltpu.VMEM((2, 2 * D // 128, HIST + SEG, 128), F32),
            pltpu.SemaphoreType.DMA((4 * (H // 2),)),
            pltpu.SemaphoreType.DMA((6,)),
        ],
        compiler_params=pltpu.CompilerParams(vmem_limit_bytes=100 * 1024 * 1024),
    )(mem0, x, wq, wk, wv, wo, B_wqkv, B_wo)
    return out.reshape(B, S, D)
```

```python
import functools

import jax
import jax.numpy as jnp
from jax import lax
import jax.experimental.pallas as pl
import jax.experimental.pallas.tpu as pltpu

F32 = jnp.float32
BF16 = jnp.bfloat16
U32 = jnp.uint32

EPS = 1e-5
NEG = -1000000000.0
PADNEG = -3.0e38
B_HEADS = 32
B_WIN = 8
B_DIL = 2
HIST = 16


def _ln(x):
    m = jnp.mean(x, axis=-1, keepdims=True)
    xc = x - m
    v = jnp.mean(xc * xc, axis=-1, keepdims=True)
    return xc * lax.rsqrt(v + EPS)


def _dot_nt(a, b):
    return lax.dot_general(a, b, (((1,), (1,)), ((), ())), preferred_element_type=F32)


def _dot(a, b):
    return jnp.dot(a, b, preferred_element_type=F32)


def _pack(a):
    return pltpu.bitcast(a, U32)


def _unpack(a):
    return pltpu.bitcast(a, BF16)


def _cat0(xs):
    return jnp.concatenate(xs, axis=0)


def _cat1(xs):
    return jnp.concatenate(xs, axis=1)


def _kernel(mem0_ref, x_hbm, wq_hbm, wk_hbm, wv_hbm, wo_hbm, bqkv_hbm, bwo_hbm,
            out_hbm,
            x_ref, out_ref, wq_ref, wk_ref, wv_ref, wo_ref, bqkv_ref, bwo_ref,
            wqkv_p, wo_p, bqkv_p, bwo_p, h_ref, xa_ref, x2_ref, kv_ref, acc_ref, wsem, sem,
            *, S, D, H, DH, M, SEG):
    NSEG = S // SEG
    PW = 2 * DH
    NP = H // 2
    RV = SEG + M
    RL = SEG + 2 * M
    RT = 2 * SEG + 2 * M
    a_scale = DH ** (-0.5)
    b_dh = D // B_HEADS
    b_scale = b_dh ** (-0.5)
    NT = D // 128
    X0 = 2 * SEG
    WIN = 3
    PERM0 = 3

    def sl(p):
        return slice(p * PW, (p + 1) * PW)

    cp_x0 = pltpu.make_async_copy(x_hbm.at[0:X0], x_ref.at[0:X0], sem.at[0])
    cp_x1 = pltpu.make_async_copy(x_hbm.at[X0:S], x_ref.at[X0:S], sem.at[1])
    cp_b = [pltpu.make_async_copy(bqkv_hbm.at[:, j * D:(j + 1) * D], bqkv_ref.at[j], sem.at[2 + j])
            for j in range(3)]
    cp_b.append(pltpu.make_async_copy(bwo_hbm, bwo_ref, sem.at[5]))
    w_pairs = ((wq_hbm, wq_ref), (wk_hbm, wk_ref), (wv_hbm, wv_ref), (wo_hbm, wo_ref))

    def rows_of(p):
        if isinstance(p, int):
            return pl.ds(p * PW, PW)
        return pl.ds(pl.multiple_of(p * PW, 128), PW)

    def cp_w(i, p):
        src, dst = w_pairs[i]
        return pltpu.make_async_copy(src.at[rows_of(p)], dst.at[rows_of(p)], wsem.at[i * NP + p])

    def start_group(p):
        for i in range(4):
            cp_w(i, p).start()

    def wait_group(p):
        for i in range(4):
            cp_w(i, p).wait()

    cp_x0.start()
    for p in range(WIN):
        start_group(p)
    for cp in cp_b:
        cp.start()

    mem0 = mem0_ref[...].astype(F32)
    xa_ref[...] = jnp.zeros(xa_ref.shape, F32)
    kv_ref[...] = jnp.zeros(kv_ref.shape, F32)
    acc_ref[...] = jnp.zeros(acc_ref.shape, F32)
    h_ref[SEG:RL, :] = _cat0([mem0, mem0]).astype(BF16)
    cp_x0.wait()
    h_ref[0:SEG, :] = _ln(x_ref[0:SEG, :].astype(F32)).astype(BF16)

    def perm_qkv_piece(j, c):
        r_i = lax.broadcasted_iota(jnp.int32, (D, 128), 0)
        c_i = lax.broadcasted_iota(jnp.int32, (D, 128), 1) + c * 128
        perm = jnp.where(r_i == (c_i & (B_HEADS - 1)) * b_dh + (c_i >> 5), 1.0, 0.0).astype(BF16)
        bqkv_p[j * NT + c] = _pack(_dot(bqkv_ref[j], perm).astype(BF16))

    def perm_wo_piece(c):
        r_i = lax.broadcasted_iota(jnp.int32, (128, D), 0) + c * 128
        c_i = lax.broadcasted_iota(jnp.int32, (128, D), 1)
        perm_t = jnp.where(c_i == (r_i & (B_HEADS - 1)) * b_dh + (r_i >> 5), 1.0, 0.0).astype(BF16)
        bwo_p[pl.ds(pl.multiple_of(c * 64, 64), 64), :] = _pack(_dot(perm_t, bwo_ref[...]).astype(BF16))

    def b_qkv(layers):
        xb = xa_ref[layers[0] * SEG:(layers[-1] + 1) * SEG, :]
        hb = _ln(xb).astype(BF16)
        return xb, [_dot(hb, _unpack(bqkv_p[n])) for n in range(3 * NT)]

    def b_attn(t, qkv, layers):
        outs = []
        for i, l in enumerate(layers):
            rows = slice(i * SEG, (i + 1) * SEG)
            q = [qkv[j][rows] for j in range(NT)]
            for j in range(2 * NT):
                kv_ref[l, j, HIST:HIST + SEG, :] = qkv[NT + j][rows]
            seg = t - 1 - 2 * l
            pos = seg * SEG + lax.broadcasted_iota(jnp.int32, (SEG, 128), 0)
            logits = []
            for w in range(B_WIN):
                o = HIST - B_DIL * w
                s = q[0] * kv_ref[l, 0, o:o + SEG, :]
                for j in range(1, NT):
                    s = s + q[j] * kv_ref[l, j, o:o + SEG, :]
                s = s + pltpu.roll(s, 64, 1)
                s = s + pltpu.roll(s, 32, 1)
                logits.append(jnp.where(pos >= B_DIL * w, s * b_scale, NEG))
            m = logits[0]
            for w in range(1, B_WIN):
                m = jnp.maximum(m, logits[w])
            es = [jnp.exp(lg - m) for lg in logits]
            den = es[0]
            for w in range(1, B_WIN):
                den = den + es[w]
            inv = 1.0 / den
            tiles = []
            for j in range(NT):
                acc = None
                for w in range(B_WIN):
                    o = HIST - B_DIL * w
                    term = es[w] * kv_ref[l, NT + j, o:o + SEG, :]
                    acc = term if acc is None else acc + term
                tiles.append(acc * inv)
            outs.append(_cat1(tiles))
            for j in range(2 * NT):
                kv_ref[l, j, 0:HIST, :] = qkv[NT + j][(i + 1) * SEG - HIST:(i + 1) * SEG]
        return _cat0(outs).astype(BF16)

    def b_out(t, xb, ob, layers):
        y = xb + _dot(ob, _unpack(bwo_p[...]))
        for i, l in enumerate(layers):
            yl = y[i * SEG:(i + 1) * SEG]
            if l == 0:
                x2_ref[...] = yl
                h_ref[RL:RT, :] = _ln(yl).astype(BF16)
            else:
                if isinstance(t, int):
                    row = (t - 3) * SEG
                else:
                    row = pl.multiple_of(jnp.maximum(t - 3, 0) * SEG, SEG)
                out_ref[pl.ds(row, SEG), :] = yl.astype(out_ref.dtype)

    def softmax2(s, first, valid, fill):
        s = jnp.where(valid, s * a_scale, fill)
        m1 = jnp.max(jnp.where(first, s, PADNEG), axis=-1, keepdims=True)
        m2 = jnp.max(jnp.where(first, PADNEG, s), axis=-1, keepdims=True)
        e = jnp.exp(s - jnp.where(first, m1, m2))
        e1 = jnp.where(first, e, 0.0)
        e2 = jnp.where(first, 0.0, e)
        l1 = jnp.sum(e1, axis=-1, keepdims=True)
        l2 = jnp.sum(e2, axis=-1, keepdims=True)
        inv = 1.0 / jnp.where(first, l1, l2)
        return e, e1, e2, inv

    def make_joint():
        rr = lax.broadcasted_iota(jnp.int32, (RT, 128), 0)
        cc = lax.broadcasted_iota(jnp.int32, (RT, 128), 1)
        lay1 = rr < RV
        first = cc < jnp.where(lay1, RL, RT)
        key = jnp.where(first, cc, cc - RL)
        exists = jnp.where(lay1, RV - 1 - key, key - RV) >= 0
        allowed = (key <= rr) | (lay1 & (key >= SEG)) | ((rr >= RV) & (rr < RL))
        valid = exists & allowed
        fill = jnp.where(exists, NEG, PADNEG)
        lo = cc < (DH - 128)
        z48 = jnp.zeros((128 - RT, 128), F32)
        z32 = jnp.zeros((128 - 2 * RL, 128), F32)

        def prep_q(a):
            return (a[:, 0:128].astype(BF16), a[0:RL, 128:256].astype(BF16),
                    a[SEG:RT, 128:256].astype(BF16), a[:, 256:384].astype(BF16))

        def prep_kv(a):
            mid = a[:, 128:256]
            tlo = jnp.where(lo, mid, 0.0)
            thi = jnp.where(lo, 0.0, mid)
            return (_cat0([a[:, 0:128], z48]).astype(BF16),
                    _cat0([tlo[0:RL], thi[0:RL], z32]).astype(BF16),
                    _cat0([z32, tlo[SEG:RT], thi[SEG:RT]]).astype(BF16),
                    _cat0([z48, a[:, 256:384]]).astype(BF16))

        def qk(q, k):
            t0 = _dot_nt(q[0], k[0])
            t2 = _dot_nt(q[3], k[3])
            t1a = _dot_nt(q[1], k[1])
            t1b = _dot_nt(q[2], k[2])
            s = jnp.where(first, t0, t2) + _cat0([t1a[0:RV], t1b[M:RL]])
            e, e1, e2, inv = softmax2(s, first, valid, fill)
            pa = e * inv
            return ((e1 * inv).astype(BF16), pa[0:RL].astype(BF16),
                    pa[SEG:RT].astype(BF16), (e2 * inv).astype(BF16))

        def pv(pr, v):
            o0 = _dot(pr[0], v[0])
            o2 = _dot(pr[3], v[3])
            o1a = _dot(pr[1], v[1])
            o1b = _dot(pr[2], v[2])
            return _cat1([o0, _cat0([o1a[0:RV], o1b[M:RL]]), o2]).astype(BF16)

        return prep_q, prep_kv, qk, pv

    def make_single(layer):
        rr = lax.broadcasted_iota(jnp.int32, (RV, 2 * RL), 0)
        cc = lax.broadcasted_iota(jnp.int32, (RV, 2 * RL), 1)
        first = cc < RL
        kc = jnp.where(first, cc, cc - RL)
        if layer == 0:
            exists = kc < RV
            valid = exists & ((kc >= SEG) | (kc <= rr))
            r0 = 0
        else:
            exists = kc >= M
            valid = exists & ((rr < M) | (kc - M <= rr))
            r0 = M
        fill = jnp.where(exists, NEG, PADNEG)
        lo = lax.broadcasted_iota(jnp.int32, (RL, PW), 1) < DH
        zrow = jnp.zeros((M, 2 * RL), F32)

        def prep_q(a):
            return a.astype(BF16)

        def prep_kv(a):
            return _cat0([jnp.where(lo, a, 0.0), jnp.where(lo, 0.0, a)]).astype(BF16)

        def qk(q, k):
            s = _dot_nt(q, k)[r0:r0 + RV]
            e, _, _, inv = softmax2(s, first, valid, fill)
            pa = e * inv
            return _cat0([pa, zrow] if layer == 0 else [zrow, pa]).astype(BF16)

        def pv(pr, v):
            return _dot(pr, v).astype(BF16)

        return prep_q, prep_kv, qk, pv

    def step(t, a_layers, b_layers, wait_x=False):
        r0 = 0 if 0 in a_layers else SEG
        r1 = RT if 1 in a_layers else RL
        h = h_ref[r0:r1, :]
        if len(a_layers) == 2:
            prep_q, prep_kv, qk, pv = make_joint()
        else:
            prep_q, prep_kv, qk, pv = make_single(a_layers[0])

        def proj(i, p):
            return _dot(h, _unpack(wqkv_p[i, p]))

        acc = [None]

        def oproj(p, o):
            part = _dot(o, _unpack(wo_p[p]))
            acc[0] = part if acc[0] is None else acc[0] + part

        def xrows(seg):
            if isinstance(seg, int):
                return x_ref[seg * SEG:(seg + 1) * SEG, :].astype(F32)
            return x_ref[pl.ds(pl.multiple_of(seg * SEG, SEG), SEG), :].astype(F32)

        q = prep_q(proj(0, 0))
        k = prep_kv(proj(1, 0))
        v = prep_kv(proj(2, 0))
        os_ = {}
        x2 = None
        for p in range(NP):
            pr = qk(q, k)
            if p + 1 < NP:
                q = prep_q(proj(0, p + 1))
                k = prep_kv(proj(1, p + 1))
            else:
                if 1 in a_layers:
                    x2 = x2_ref[...]
                if b_layers:
                    b_out(t, xb, ob, b_layers)
                if 0 in a_layers:
                    if wait_x:
                        cp_x1.wait()
                    nxt = t + 1 if isinstance(t, int) else jnp.minimum(t + 1, NSEG - 1)
                    h_ref[0:SEG, :] = _ln(xrows(nxt)).astype(BF16)
                oproj(p - 2, os_.pop(p - 2))
            os_[p] = pv(pr, v)
            if p + 1 < NP:
                v = prep_kv(proj(2, p + 1))
            if p == 0 and b_layers:
                xb, qkv = b_qkv(b_layers)
                ob = b_attn(t, qkv, b_layers)
            if p >= 2 and p + 1 < NP:
                oproj(p - 2, os_.pop(p - 2))
        oproj(NP - 2, os_.pop(NP - 2))
        oproj(NP - 1, os_.pop(NP - 1))
        a = acc[0]
        if 0 in a_layers:
            xa_ref[0:SEG, :] = xrows(t) + a[0:SEG]
        if 1 in a_layers:
            xa_ref[SEG:2 * SEG, :] = x2 + a[RL - r0:RT - r0]
        mem1 = a[SEG - r0:RV - r0]
        mem2 = a[RV - r0:RL - r0] if 1 in a_layers else mem0
        h_ref[SEG:RL, :] = _cat0([mem1, mem2]).astype(BF16)

    def first_step():
        prep_q, prep_kv, qk, pv = make_single(0)

        def body0(p, carry):
            wait_group(p)

            @pl.when(p + WIN < NP)
            def _():
                start_group(p + WIN)

            @pl.when(p == NP - 1)
            def _():
                cp_x1.start()

            h = h_ref[0:RL, :]
            w = [w_pairs[i][1][rows_of(p), :] for i in range(4)]
            q = prep_q(_dot_nt(h, w[0]))
            k = prep_kv(_dot_nt(h, w[1]))
            v = prep_kv(_dot_nt(h, w[2]))
            o = pv(qk(q, k), v)
            acc_ref[...] += _dot(o, w[3])
            for i in range(3):
                wqkv_p[i, p] = _pack(w[i].T)
            wo_p[p] = _pack(w[3])

            @pl.when(p == PERM0)
            def _():
                for cp in cp_b:
                    cp.wait()

            @pl.when((p >= PERM0) & (p < PERM0 + NT))
            def _():
                c = p - PERM0
                perm_qkv_piece(0, c)
                perm_qkv_piece(1, c)

            @pl.when((p >= PERM0 + NT) & (p < PERM0 + 2 * NT))
            def _():
                c = p - PERM0 - NT
                perm_qkv_piece(2, c)
                perm_wo_piece(c)

            return carry

        lax.fori_loop(0, NP, body0, 0)
        a = acc_ref[...]
        xa_ref[0:SEG, :] = x_ref[0:SEG, :].astype(F32) + a[0:SEG]
        h_ref[0:SEG, :] = _ln(x_ref[SEG:2 * SEG, :].astype(F32)).astype(BF16)
        h_ref[SEG:RL, :] = _cat0([a[SEG:RV], mem0]).astype(BF16)

    first_step()
    step(1, (0,), (0,), wait_x=True)

    def body(t, carry):
        step(t, (0, 1), (0, 1))
        return carry

    lax.fori_loop(2, NSEG, body, 0)
    done = (NSEG - 3) * SEG
    cp_o0 = pltpu.make_async_copy(out_ref.at[0:done], out_hbm.at[0:done], sem.at[6])
    cp_o0.start()
    step(NSEG, (1,), (0, 1))
    step(NSEG + 1, (1,), (1,))
    xb, qkv = b_qkv((1,))
    b_out(NSEG + 2, xb, b_attn(NSEG + 2, qkv, (1,)), (1,))
    cp_o1 = pltpu.make_async_copy(out_ref.at[done:S], out_hbm.at[done:S], sem.at[7])
    cp_o1.start()
    cp_o0.wait()
    cp_o1.wait()


@functools.partial(jax.jit, static_argnames=("A_seg_len",))
def pallas_interleave_layers__memory_aug_recurrent_mem_tr__sliding_local_dilated__prompt_kernel(
    A_x: jax.Array,
    A_mem0: jax.Array,
    A_Wq: jax.Array,
    A_Wk: jax.Array,
    A_Wv: jax.Array,
    A_Wo: jax.Array,
    A_seg_len,
    B_x: jax.Array,
    B_wqkv: jax.Array,
    B_wo: jax.Array,
):
    B, S, D = A_x.shape
    H, DH = A_Wq.shape[1], A_Wq.shape[2]
    M = A_mem0.shape[1]
    SEG = int(A_seg_len)
    assert B == 1 and M == 8 and SEG == 32 and DH == 192 and D % 128 == 0 and S % SEG == 0

    x = A_x.reshape(S, D)
    mem0 = A_mem0.reshape(M, D)
    wq = jnp.transpose(A_Wq, (1, 2, 0)).reshape(H * DH, D)
    wk = jnp.transpose(A_Wk, (1, 2, 0)).reshape(H * DH, D)
    wv = jnp.transpose(A_Wv, (1, 2, 0)).reshape(H * DH, D)
    wo = A_Wo.reshape(H * DH, D)

    hbm = pl.BlockSpec(memory_space=pl.ANY)
    out = pl.pallas_call(
        functools.partial(_kernel, S=S, D=D, H=H, DH=DH, M=M, SEG=SEG),
        out_shape=jax.ShapeDtypeStruct((S, D), A_x.dtype),
        in_specs=[pl.BlockSpec(memory_space=pltpu.VMEM)] + [hbm] * 7,
        out_specs=hbm,
        scratch_shapes=[
            pltpu.VMEM((S, D), BF16),
            pltpu.VMEM((S, D), BF16),
            pltpu.VMEM((H * DH, D), BF16),
            pltpu.VMEM((H * DH, D), BF16),
            pltpu.VMEM((H * DH, D), BF16),
            pltpu.VMEM((H * DH, D), BF16),
            pltpu.VMEM((3, D, D), BF16),
            pltpu.VMEM((D, D), BF16),
            pltpu.VMEM((3, H // 2, D // 2, 2 * DH), U32),
            pltpu.VMEM((H // 2, DH, D), U32),
            pltpu.VMEM((3 * D // 128, D // 2, 128), U32),
            pltpu.VMEM((D // 2, D), U32),
            pltpu.VMEM((2 * SEG + 2 * M, D), BF16),
            pltpu.VMEM((2 * SEG, D), F32),
            pltpu.VMEM((SEG, D), F32),
            pltpu.VMEM((2, 2 * D // 128, HIST + SEG, 128), F32),
            pltpu.VMEM((SEG + 2 * M, D), F32),
            pltpu.SemaphoreType.DMA((4 * (H // 2),)),
            pltpu.SemaphoreType.DMA((8,)),
        ],
        compiler_params=pltpu.CompilerParams(vmem_limit_bytes=100 * 1024 * 1024),
    )(mem0, x, wq, wk, wv, wo, B_wqkv, B_wo)
    return out.reshape(B, S, D)
```

```python
import functools

import jax
import jax.numpy as jnp
from jax import lax
import jax.experimental.pallas as pl
import jax.experimental.pallas.tpu as pltpu

F32 = jnp.float32
BF16 = jnp.bfloat16
U32 = jnp.uint32

EPS = 1e-5
NEG = -1000000000.0
PADNEG = -3.0e38
B_HEADS = 32
B_WIN = 8
B_DIL = 2
NPRE = 4
HIST = 16


def _ln(x):
    m = jnp.mean(x, axis=-1, keepdims=True)
    xc = x - m
    v = jnp.mean(xc * xc, axis=-1, keepdims=True)
    return xc * lax.rsqrt(v + EPS)


def _dot_nt(a, b):
    return lax.dot_general(a, b, (((1,), (1,)), ((), ())), preferred_element_type=F32)


def _dot(a, b):
    return jnp.dot(a, b, preferred_element_type=F32)


def _pack(a):
    return pltpu.bitcast(a, U32)


def _unpack(a):
    return pltpu.bitcast(a, BF16)


def _cat0(xs):
    return jnp.concatenate(xs, axis=0)


def _cat1(xs):
    return jnp.concatenate(xs, axis=1)


def _kernel(mem0_ref, x_hbm, wq_hbm, wk_hbm, wv_hbm, wo_hbm, bqkv_hbm, bwo_hbm,
            out_hbm,
            x_ref, out_ref, wq_ref, wk_ref, wv_ref, wo_ref, bqkv_ref, bwo_ref,
            wqkv_p, wo_p, bqkv_p, bwo_p, h_ref, xa_ref, x2_ref, kv_ref, acc_ref, hpre_ref, pre_ref, o_ref, wsem, sem,
            *, S, D, H, DH, M, SEG):
    NSEG = S // SEG
    PW = 2 * DH
    NP = H // 2
    RV = SEG + M
    RL = SEG + 2 * M
    RT = 2 * SEG + 2 * M
    a_scale = DH ** (-0.5)
    b_dh = D // B_HEADS
    b_scale = b_dh ** (-0.5)
    NT = D // 128
    X0 = (NPRE + 3) * SEG
    WIN = 3
    PERM0 = 3

    def sl(p):
        return slice(p * PW, (p + 1) * PW)

    cp_x0 = pltpu.make_async_copy(x_hbm.at[0:X0], x_ref.at[0:X0], sem.at[0])
    cp_x1 = pltpu.make_async_copy(x_hbm.at[X0:S], x_ref.at[X0:S], sem.at[1])
    cp_b = [pltpu.make_async_copy(bqkv_hbm.at[:, j * D:(j + 1) * D], bqkv_ref.at[j], sem.at[2 + j])
            for j in range(3)]
    cp_b.append(pltpu.make_async_copy(bwo_hbm, bwo_ref, sem.at[5]))
    w_pairs = ((wq_hbm, wq_ref), (wk_hbm, wk_ref), (wv_hbm, wv_ref), (wo_hbm, wo_ref))

    def rows_of(p):
        if isinstance(p, int):
            return pl.ds(p * PW, PW)
        return pl.ds(pl.multiple_of(p * PW, 128), PW)

    def cp_w(i, p):
        src, dst = w_pairs[i]
        return pltpu.make_async_copy(src.at[rows_of(p)], dst.at[rows_of(p)], wsem.at[i * NP + p])

    def start_group(p):
        for i in range(4):
            cp_w(i, p).start()

    def wait_group(p):
        for i in range(4):
            cp_w(i, p).wait()

    cp_x0.start()
    for p in range(WIN):
        start_group(p)
    for cp in cp_b:
        cp.start()

    mem0 = mem0_ref[...].astype(F32)
    xa_ref[...] = jnp.zeros(xa_ref.shape, F32)
    kv_ref[...] = jnp.zeros(kv_ref.shape, F32)
    acc_ref[...] = jnp.zeros(acc_ref.shape, F32)
    cp_x0.wait()
    h0 = _ln(x_ref[0:SEG, :].astype(F32))
    hpre_ref[0:RL // 2, :] = _pack(_cat0([h0, mem0, mem0]).astype(BF16))
    for i in range(NPRE):
        hi = _ln(x_ref[(2 + i) * SEG:(3 + i) * SEG, :].astype(F32)).astype(BF16)
        hpre_ref[(RL + i * SEG) // 2:(RL + (i + 1) * SEG) // 2, :] = _pack(hi)
    o_ref[...] = jnp.zeros(o_ref.shape, U32)

    def perm_qkv_piece(j, c):
        r_i = lax.broadcasted_iota(jnp.int32, (D, 128), 0)
        c_i = lax.broadcasted_iota(jnp.int32, (D, 128), 1) + c * 128
        perm = jnp.where(r_i == (c_i & (B_HEADS - 1)) * b_dh + (c_i >> 5), 1.0, 0.0).astype(BF16)
        bqkv_p[j * NT + c] = _pack(_dot(bqkv_ref[j], perm).astype(BF16))

    def perm_wo_piece(c):
        r_i = lax.broadcasted_iota(jnp.int32, (128, D), 0) + c * 128
        c_i = lax.broadcasted_iota(jnp.int32, (128, D), 1)
        perm_t = jnp.where(c_i == (r_i & (B_HEADS - 1)) * b_dh + (r_i >> 5), 1.0, 0.0).astype(BF16)
        bwo_p[pl.ds(pl.multiple_of(c * 64, 64), 64), :] = _pack(_dot(perm_t, bwo_ref[...]).astype(BF16))

    def b_qkv(layers):
        xb = xa_ref[layers[0] * SEG:(layers[-1] + 1) * SEG, :]
        hb = _ln(xb).astype(BF16)
        return xb, [_dot(hb, _unpack(bqkv_p[n])) for n in range(3 * NT)]

    def b_attn(t, qkv, layers):
        outs = []
        for i, l in enumerate(layers):
            rows = slice(i * SEG, (i + 1) * SEG)
            q = [qkv[j][rows] for j in range(NT)]
            for j in range(2 * NT):
                kv_ref[l, j, HIST:HIST + SEG, :] = qkv[NT + j][rows]
            seg = t - 1 - 2 * l
            pos = seg * SEG + lax.broadcasted_iota(jnp.int32, (SEG, 128), 0)
            logits = []
            for w in range(B_WIN):
                o = HIST - B_DIL * w
                s = q[0] * kv_ref[l, 0, o:o + SEG, :]
                for j in range(1, NT):
                    s = s + q[j] * kv_ref[l, j, o:o + SEG, :]
                s = s + pltpu.roll(s, 64, 1)
                s = s + pltpu.roll(s, 32, 1)
                logits.append(jnp.where(pos >= B_DIL * w, s * b_scale, NEG))
            m = logits[0]
            for w in range(1, B_WIN):
                m = jnp.maximum(m, logits[w])
            es = [jnp.exp(lg - m) for lg in logits]
            den = es[0]
            for w in range(1, B_WIN):
                den = den + es[w]
            inv = 1.0 / den
            tiles = []
            for j in range(NT):
                acc = None
                for w in range(B_WIN):
                    o = HIST - B_DIL * w
                    term = es[w] * kv_ref[l, NT + j, o:o + SEG, :]
                    acc = term if acc is None else acc + term
                tiles.append(acc * inv)
            outs.append(_cat1(tiles))
            for j in range(2 * NT):
                kv_ref[l, j, 0:HIST, :] = qkv[NT + j][(i + 1) * SEG - HIST:(i + 1) * SEG]
        return _cat0(outs).astype(BF16)

    def b_out(t, xb, ob, layers):
        y = xb + _dot(ob, _unpack(bwo_p[...]))
        for i, l in enumerate(layers):
            yl = y[i * SEG:(i + 1) * SEG]
            if l == 0:
                x2_ref[...] = yl
                h_ref[RL:RT, :] = _ln(yl).astype(BF16)
            else:
                if isinstance(t, int):
                    row = (t - 3) * SEG
                else:
                    row = pl.multiple_of(jnp.maximum(t - 3, 0) * SEG, SEG)
                out_ref[pl.ds(row, SEG), :] = yl.astype(out_ref.dtype)

    def softmax2(s, first, valid, fill):
        s = jnp.where(valid, s * a_scale, fill)
        m1 = jnp.max(jnp.where(first, s, PADNEG), axis=-1, keepdims=True)
        m2 = jnp.max(jnp.where(first, PADNEG, s), axis=-1, keepdims=True)
        e = jnp.exp(s - jnp.where(first, m1, m2))
        e1 = jnp.where(first, e, 0.0)
        e2 = jnp.where(first, 0.0, e)
        l1 = jnp.sum(e1, axis=-1, keepdims=True)
        l2 = jnp.sum(e2, axis=-1, keepdims=True)
        inv = 1.0 / jnp.where(first, l1, l2)
        return e, e1, e2, inv

    def make_joint():
        rr = lax.broadcasted_iota(jnp.int32, (RT, 128), 0)
        cc = lax.broadcasted_iota(jnp.int32, (RT, 128), 1)
        lay1 = rr < RV
        first = cc < jnp.where(lay1, RL, RT)
        key = jnp.where(first, cc, cc - RL)
        exists = jnp.where(lay1, RV - 1 - key, key - RV) >= 0
        allowed = (key <= rr) | (lay1 & (key >= SEG)) | ((rr >= RV) & (rr < RL))
        valid = exists & allowed
        fill = jnp.where(exists, NEG, PADNEG)
        lo = cc < (DH - 128)
        z48 = jnp.zeros((128 - RT, 128), F32)
        z32 = jnp.zeros((128 - 2 * RL, 128), F32)

        def prep_q(a):
            return (a[:, 0:128].astype(BF16), a[0:RL, 128:256].astype(BF16),
                    a[SEG:RT, 128:256].astype(BF16), a[:, 256:384].astype(BF16))

        def prep_kv(a):
            mid = a[:, 128:256]
            tlo = jnp.where(lo, mid, 0.0)
            thi = jnp.where(lo, 0.0, mid)
            return (_cat0([a[:, 0:128], z48]).astype(BF16),
                    _cat0([tlo[0:RL], thi[0:RL], z32]).astype(BF16),
                    _cat0([z32, tlo[SEG:RT], thi[SEG:RT]]).astype(BF16),
                    _cat0([z48, a[:, 256:384]]).astype(BF16))

        def qk(q, k):
            t0 = _dot_nt(q[0], k[0])
            t2 = _dot_nt(q[3], k[3])
            t1a = _dot_nt(q[1], k[1])
            t1b = _dot_nt(q[2], k[2])
            s = jnp.where(first, t0, t2) + _cat0([t1a[0:RV], t1b[M:RL]])
            e, e1, e2, inv = softmax2(s, first, valid, fill)
            pa = e * inv
            return ((e1 * inv).astype(BF16), pa[0:RL].astype(BF16),
                    pa[SEG:RT].astype(BF16), (e2 * inv).astype(BF16))

        def pv(pr, v):
            o0 = _dot(pr[0], v[0])
            o2 = _dot(pr[3], v[3])
            o1a = _dot(pr[1], v[1])
            o1b = _dot(pr[2], v[2])
            return _cat1([o0, _cat0([o1a[0:RV], o1b[M:RL]]), o2]).astype(BF16)

        return prep_q, prep_kv, qk, pv

    def make_single(layer):
        rr = lax.broadcasted_iota(jnp.int32, (RV, 2 * RL), 0)
        cc = lax.broadcasted_iota(jnp.int32, (RV, 2 * RL), 1)
        first = cc < RL
        kc = jnp.where(first, cc, cc - RL)
        if layer == 0:
            exists = kc < RV
            valid = exists & ((kc >= SEG) | (kc <= rr))
            r0 = 0
        else:
            exists = kc >= M
            valid = exists & ((rr < M) | (kc - M <= rr))
            r0 = M
        fill = jnp.where(exists, NEG, PADNEG)
        lo = lax.broadcasted_iota(jnp.int32, (RL, PW), 1) < DH
        zrow = jnp.zeros((M, 2 * RL), F32)

        def prep_q(a):
            return a.astype(BF16)

        def prep_kv(a):
            return _cat0([jnp.where(lo, a, 0.0), jnp.where(lo, 0.0, a)]).astype(BF16)

        def qk(q, k):
            s = _dot_nt(q, k)[r0:r0 + RV]
            e, _, _, inv = softmax2(s, first, valid, fill)
            pa = e * inv
            return _cat0([pa, zrow] if layer == 0 else [zrow, pa]).astype(BF16)

        def pv(pr, v):
            return _dot(pr, v).astype(BF16)

        return prep_q, prep_kv, qk, pv

    def step(t, a_layers, b_layers, light=False):
        r0 = 0 if 0 in a_layers else SEG
        r1 = RT if 1 in a_layers else RL
        h = h_ref[SEG if light else r0:r1, :]
        if len(a_layers) == 2:
            prep_q, prep_kv, qk, pv = make_joint()
        else:
            prep_q, prep_kv, qk, pv = make_single(a_layers[0])

        def proj(i, p):
            r = _dot(h, _unpack(wqkv_p[i, p]))
            if light:
                r = _cat0([pre_ref[i, p, pl.ds(pl.multiple_of((t - 2) * SEG, SEG), SEG), :], r])
            return r

        acc = [None]

        def oproj(p, o):
            part = _dot(o, _unpack(wo_p[p]))
            acc[0] = part if acc[0] is None else acc[0] + part

        def xrows(seg):
            if isinstance(seg, int):
                return x_ref[seg * SEG:(seg + 1) * SEG, :].astype(F32)
            return x_ref[pl.ds(pl.multiple_of(seg * SEG, SEG), SEG), :].astype(F32)

        q = prep_q(proj(0, 0))
        k = prep_kv(proj(1, 0))
        v = prep_kv(proj(2, 0))
        os_ = {}
        x2 = None
        for p in range(NP):
            pr = qk(q, k)
            if p + 1 < NP:
                q = prep_q(proj(0, p + 1))
                k = prep_kv(proj(1, p + 1))
            else:
                if 1 in a_layers:
                    x2 = x2_ref[...]
                if b_layers:
                    b_out(t, xb, ob, b_layers)
                if 0 in a_layers:
                    nxt = t + 1 if isinstance(t, int) else jnp.minimum(t + 1, NSEG - 1)
                    h_ref[0:SEG, :] = _ln(xrows(nxt)).astype(BF16)
                oproj(p - 2, os_.pop(p - 2))
            os_[p] = pv(pr, v)
            if p + 1 < NP:
                v = prep_kv(proj(2, p + 1))
            if p == 0 and b_layers:
                xb, qkv = b_qkv(b_layers)
                ob = b_attn(t, qkv, b_layers)
            if p >= 2 and p + 1 < NP:
                oproj(p - 2, os_.pop(p - 2))
        oproj(NP - 2, os_.pop(NP - 2))
        oproj(NP - 1, os_.pop(NP - 1))
        a = acc[0]
        if 0 in a_layers:
            xa_ref[0:SEG, :] = xrows(t) + a[0:SEG]
        if 1 in a_layers:
            xa_ref[SEG:2 * SEG, :] = x2 + a[RL - r0:RT - r0]
        mem1 = a[SEG - r0:RV - r0]
        mem2 = a[RV - r0:RL - r0] if 1 in a_layers else mem0
        h_ref[SEG:RL, :] = _cat0([mem1, mem2]).astype(BF16)

    def first_step():
        prep_q, prep_kv, qk, pv = make_single(0)

        def body0(p, carry):
            wait_group(p)

            @pl.when(p + WIN < NP)
            def _():
                start_group(p + WIN)

            @pl.when(p == NP - 1)
            def _():
                cp_x1.start()

            h = _unpack(hpre_ref[...])
            w = [w_pairs[i][1][rows_of(p), :] for i in range(4)]

            def proj(i):
                r = _dot_nt(h, w[i])
                pre_ref[i, p] = r[RL:]
                return r[0:RL]

            q = prep_q(proj(0))
            k = prep_kv(proj(1))
            pr = qk(q, k)
            acc_ref[...] += _dot(_unpack(o_ref[...]), wo_ref[rows_of(jnp.maximum(p - 1, 0)), :])
            v = prep_kv(proj(2))
            o_ref[...] = _pack(pv(pr, v))
            for i in range(3):
                wqkv_p[i, p] = _pack(w[i].T)
            wo_p[p] = _pack(w[3])

            @pl.when(p == PERM0)
            def _():
                for cp in cp_b:
                    cp.wait()

            @pl.when((p >= PERM0) & (p < PERM0 + NT))
            def _():
                c = p - PERM0
                perm_qkv_piece(0, c)
                perm_qkv_piece(1, c)

            @pl.when((p >= PERM0 + NT) & (p < PERM0 + 2 * NT))
            def _():
                c = p - PERM0 - NT
                perm_qkv_piece(2, c)
                perm_wo_piece(c)

            return carry

        lax.fori_loop(0, NP, body0, 0)
        a = acc_ref[...] + _dot(_unpack(o_ref[...]), wo_ref[rows_of(NP - 1), :])
        xa_ref[0:SEG, :] = x_ref[0:SEG, :].astype(F32) + a[0:SEG]
        h_ref[0:SEG, :] = _ln(x_ref[SEG:2 * SEG, :].astype(F32)).astype(BF16)
        h_ref[SEG:RL, :] = _cat0([a[SEG:RV], mem0]).astype(BF16)

    first_step()
    step(1, (0,), (0,))

    def body_light(t, carry):
        step(t, (0, 1), (0, 1), light=True)
        return carry

    lax.fori_loop(2, 2 + NPRE, body_light, 0)
    cp_x1.wait()

    def body(t, carry):
        step(t, (0, 1), (0, 1))
        return carry

    lax.fori_loop(2 + NPRE, NSEG, body, 0)
    done = (NSEG - 3) * SEG
    cp_o0 = pltpu.make_async_copy(out_ref.at[0:done], out_hbm.at[0:done], sem.at[6])
    cp_o0.start()
    step(NSEG, (1,), (0, 1))
    step(NSEG + 1, (1,), (1,))
    xb, qkv = b_qkv((1,))
    b_out(NSEG + 2, xb, b_attn(NSEG + 2, qkv, (1,)), (1,))
    cp_o1 = pltpu.make_async_copy(out_ref.at[done:S], out_hbm.at[done:S], sem.at[7])
    cp_o1.start()
    cp_o0.wait()
    cp_o1.wait()


@functools.partial(jax.jit, static_argnames=("A_seg_len",))
def pallas_interleave_layers__memory_aug_recurrent_mem_tr__sliding_local_dilated__prompt_kernel(
    A_x: jax.Array,
    A_mem0: jax.Array,
    A_Wq: jax.Array,
    A_Wk: jax.Array,
    A_Wv: jax.Array,
    A_Wo: jax.Array,
    A_seg_len,
    B_x: jax.Array,
    B_wqkv: jax.Array,
    B_wo: jax.Array,
):
    B, S, D = A_x.shape
    H, DH = A_Wq.shape[1], A_Wq.shape[2]
    M = A_mem0.shape[1]
    SEG = int(A_seg_len)
    assert B == 1 and M == 8 and SEG == 32 and DH == 192 and D % 128 == 0 and S % SEG == 0

    x = A_x.reshape(S, D)
    mem0 = A_mem0.reshape(M, D)
    wq = jnp.transpose(A_Wq, (1, 2, 0)).reshape(H * DH, D)
    wk = jnp.transpose(A_Wk, (1, 2, 0)).reshape(H * DH, D)
    wv = jnp.transpose(A_Wv, (1, 2, 0)).reshape(H * DH, D)
    wo = A_Wo.reshape(H * DH, D)

    hbm = pl.BlockSpec(memory_space=pl.ANY)
    out = pl.pallas_call(
        functools.partial(_kernel, S=S, D=D, H=H, DH=DH, M=M, SEG=SEG),
        out_shape=jax.ShapeDtypeStruct((S, D), A_x.dtype),
        in_specs=[pl.BlockSpec(memory_space=pltpu.VMEM)] + [hbm] * 7,
        out_specs=hbm,
        scratch_shapes=[
            pltpu.VMEM((S, D), BF16),
            pltpu.VMEM((S, D), BF16),
            pltpu.VMEM((H * DH, D), BF16),
            pltpu.VMEM((H * DH, D), BF16),
            pltpu.VMEM((H * DH, D), BF16),
            pltpu.VMEM((H * DH, D), BF16),
            pltpu.VMEM((3, D, D), BF16),
            pltpu.VMEM((D, D), BF16),
            pltpu.VMEM((3, H // 2, D // 2, 2 * DH), U32),
            pltpu.VMEM((H // 2, DH, D), U32),
            pltpu.VMEM((3 * D // 128, D // 2, 128), U32),
            pltpu.VMEM((D // 2, D), U32),
            pltpu.VMEM((2 * SEG + 2 * M, D), BF16),
            pltpu.VMEM((2 * SEG, D), F32),
            pltpu.VMEM((SEG, D), F32),
            pltpu.VMEM((2, 2 * D // 128, HIST + SEG, 128), F32),
            pltpu.VMEM((SEG + 2 * M, D), F32),
            pltpu.VMEM(((SEG + 2 * M + NPRE * SEG) // 2, D), U32),
            pltpu.VMEM((3, H // 2, NPRE * SEG, 2 * DH), F32),
            pltpu.VMEM(((SEG + 2 * M) // 2, 2 * DH), U32),
            pltpu.SemaphoreType.DMA((4 * (H // 2),)),
            pltpu.SemaphoreType.DMA((8,)),
        ],
        compiler_params=pltpu.CompilerParams(vmem_limit_bytes=110 * 1024 * 1024),
    )(mem0, x, wq, wk, wv, wo, B_wqkv, B_wo)
    return out.reshape(B, S, D)
```

```python
import functools

import jax
import jax.numpy as jnp
from jax import lax
import jax.experimental.pallas as pl
import jax.experimental.pallas.tpu as pltpu

F32 = jnp.float32
BF16 = jnp.bfloat16
U32 = jnp.uint32

EPS = 1e-5
NEG = -1000000000.0
PADNEG = -3.0e38
B_HEADS = 32
B_WIN = 8
B_DIL = 2
NPRE = 4
HIST = 16


def _ln(x):
    m = jnp.mean(x, axis=-1, keepdims=True)
    xc = x - m
    v = jnp.mean(xc * xc, axis=-1, keepdims=True)
    return xc * lax.rsqrt(v + EPS)


def _dot_nt(a, b):
    return lax.dot_general(a, b, (((1,), (1,)), ((), ())), preferred_element_type=F32)


def _dot(a, b):
    return jnp.dot(a, b, preferred_element_type=F32)


def _pack(a):
    return pltpu.bitcast(a, U32)


def _unpack(a):
    return pltpu.bitcast(a, BF16)


def _cat0(xs):
    return jnp.concatenate(xs, axis=0)


def _cat1(xs):
    return jnp.concatenate(xs, axis=1)


def _kernel(mem0_ref, x_hbm, wq_hbm, wk_hbm, wv_hbm, wo_hbm, bqkv_hbm, bwo_hbm,
            out_hbm,
            x_ref, out_ref, wq_ref, wk_ref, wv_ref, wo_ref, bqkv_ref, bwo_ref,
            wqkv_p, wo_p, bqkv_p, bwo_p, h_ref, xa_ref, x2_ref, kv_ref, acc_ref, hpre_ref, pre_ref, o_ref, wsem, sem,
            *, S, D, H, DH, M, SEG):
    NSEG = S // SEG
    PW = 2 * DH
    NP = H // 2
    RV = SEG + M
    RL = SEG + 2 * M
    RT = 2 * SEG + 2 * M
    a_scale = DH ** (-0.5)
    b_dh = D // B_HEADS
    b_scale = b_dh ** (-0.5)
    NT = D // 128
    X0 = (NPRE + 3) * SEG
    WIN = 3
    PERM0 = 3

    def sl(p):
        return slice(p * PW, (p + 1) * PW)

    cp_x0 = pltpu.make_async_copy(x_hbm.at[0:X0], x_ref.at[0:X0], sem.at[0])
    cp_x1 = pltpu.make_async_copy(x_hbm.at[X0:S], x_ref.at[X0:S], sem.at[1])
    cp_b = [pltpu.make_async_copy(bqkv_hbm.at[:, j * D:(j + 1) * D], bqkv_ref.at[j], sem.at[2 + j])
            for j in range(3)]
    cp_b.append(pltpu.make_async_copy(bwo_hbm, bwo_ref, sem.at[5]))
    w_pairs = ((wq_hbm, wq_ref), (wk_hbm, wk_ref), (wv_hbm, wv_ref), (wo_hbm, wo_ref))

    def rows_of(p):
        if isinstance(p, int):
            return pl.ds(p * PW, PW)
        return pl.ds(pl.multiple_of(p * PW, 128), PW)

    def cp_w(i, p):
        src, dst = w_pairs[i]
        return pltpu.make_async_copy(src.at[rows_of(p)], dst.at[rows_of(p)], wsem.at[i * NP + p])

    def start_group(p):
        for i in range(4):
            cp_w(i, p).start()

    def wait_group(p):
        for i in range(4):
            cp_w(i, p).wait()

    cp_x0.start()
    for p in range(WIN):
        start_group(p)
    for cp in cp_b:
        cp.start()

    mem0 = mem0_ref[...].astype(F32)
    xa_ref[...] = jnp.zeros(xa_ref.shape, F32)
    kv_ref[...] = jnp.zeros(kv_ref.shape, F32)
    acc_ref[...] = jnp.zeros(acc_ref.shape, F32)
    cp_x0.wait()
    h0 = _ln(x_ref[0:SEG, :].astype(F32))
    hpre_ref[0:RL // 2, :] = _pack(_cat0([h0, mem0, mem0]).astype(BF16))
    for i in range(NPRE):
        hi = _ln(x_ref[(2 + i) * SEG:(3 + i) * SEG, :].astype(F32)).astype(BF16)
        hpre_ref[(RL + i * SEG) // 2:(RL + (i + 1) * SEG) // 2, :] = _pack(hi)
    o_ref[...] = jnp.zeros(o_ref.shape, U32)

    def perm_qkv_piece(j, c):
        r_i = lax.broadcasted_iota(jnp.int32, (D, 128), 0)
        c_i = lax.broadcasted_iota(jnp.int32, (D, 128), 1) + c * 128
        perm = jnp.where(r_i == (c_i & (B_HEADS - 1)) * b_dh + (c_i >> 5), 1.0, 0.0).astype(BF16)
        bqkv_p[j * NT + c] = _pack(_dot(bqkv_ref[j], perm).astype(BF16))

    def perm_wo_piece(c):
        r_i = lax.broadcasted_iota(jnp.int32, (128, D), 0) + c * 128
        c_i = lax.broadcasted_iota(jnp.int32, (128, D), 1)
        perm_t = jnp.where(c_i == (r_i & (B_HEADS - 1)) * b_dh + (r_i >> 5), 1.0, 0.0).astype(BF16)
        bwo_p[pl.ds(pl.multiple_of(c * 64, 64), 64), :] = _pack(_dot(perm_t, bwo_ref[...]).astype(BF16))

    def b_qkv(layers):
        xb = xa_ref[layers[0] * SEG:(layers[-1] + 1) * SEG, :]
        hb = _ln(xb).astype(BF16)
        return xb, [_dot(hb, _unpack(bqkv_p[n])) for n in range(3 * NT)]

    def b_attn(t, qkv, layers):
        outs = []
        for i, l in enumerate(layers):
            rows = slice(i * SEG, (i + 1) * SEG)
            q = [qkv[j][rows] for j in range(NT)]
            for j in range(2 * NT):
                kv_ref[l, j, HIST:HIST + SEG, :] = qkv[NT + j][rows]
            seg = t - 1 - 2 * l
            pos = seg * SEG + lax.broadcasted_iota(jnp.int32, (SEG, 128), 0)
            logits = []
            for w in range(B_WIN):
                o = HIST - B_DIL * w
                s = q[0] * kv_ref[l, 0, o:o + SEG, :]
                for j in range(1, NT):
                    s = s + q[j] * kv_ref[l, j, o:o + SEG, :]
                s = s + pltpu.roll(s, 64, 1)
                s = s + pltpu.roll(s, 32, 1)
                logits.append(jnp.where(pos >= B_DIL * w, s * b_scale, NEG))
            m = logits[0]
            for w in range(1, B_WIN):
                m = jnp.maximum(m, logits[w])
            es = [jnp.exp(lg - m) for lg in logits]
            den = es[0]
            for w in range(1, B_WIN):
                den = den + es[w]
            inv = 1.0 / den
            tiles = []
            for j in range(NT):
                acc = None
                for w in range(B_WIN):
                    o = HIST - B_DIL * w
                    term = es[w] * kv_ref[l, NT + j, o:o + SEG, :]
                    acc = term if acc is None else acc + term
                tiles.append(acc * inv)
            outs.append(_cat1(tiles))
            for j in range(2 * NT):
                kv_ref[l, j, 0:HIST, :] = qkv[NT + j][(i + 1) * SEG - HIST:(i + 1) * SEG]
        return _cat0(outs).astype(BF16)

    def b_out(t, xb, ob, layers):
        y = xb + _dot(ob, _unpack(bwo_p[...]))
        for i, l in enumerate(layers):
            yl = y[i * SEG:(i + 1) * SEG]
            if l == 0:
                x2_ref[...] = yl
                h_ref[RL:RT, :] = _ln(yl).astype(BF16)
            else:
                if isinstance(t, int):
                    row = (t - 3) * SEG
                else:
                    row = pl.multiple_of(jnp.maximum(t - 3, 0) * SEG, SEG)
                out_ref[pl.ds(row, SEG), :] = yl.astype(out_ref.dtype)

    def softmax2(s, first, valid, fill):
        s = jnp.where(valid, s * a_scale, fill)
        m1 = jnp.max(jnp.where(first, s, PADNEG), axis=-1, keepdims=True)
        m2 = jnp.max(jnp.where(first, PADNEG, s), axis=-1, keepdims=True)
        e = jnp.exp(s - jnp.where(first, m1, m2))
        e1 = jnp.where(first, e, 0.0)
        e2 = jnp.where(first, 0.0, e)
        l1 = jnp.sum(e1, axis=-1, keepdims=True)
        l2 = jnp.sum(e2, axis=-1, keepdims=True)
        inv = 1.0 / jnp.where(first, l1, l2)
        return e, e1, e2, inv

    def make_joint():
        rr = lax.broadcasted_iota(jnp.int32, (RT, 128), 0)
        cc = lax.broadcasted_iota(jnp.int32, (RT, 128), 1)
        lay1 = rr < RV
        first = cc < jnp.where(lay1, RL, RT)
        key = jnp.where(first, cc, cc - RL)
        exists = jnp.where(lay1, RV - 1 - key, key - RV) >= 0
        allowed = (key <= rr) | (lay1 & (key >= SEG)) | ((rr >= RV) & (rr < RL))
        valid = exists & allowed
        fill = jnp.where(exists, NEG, PADNEG)
        lo = cc < (DH - 128)
        z48 = jnp.zeros((128 - RT, 128), F32)
        z32 = jnp.zeros((128 - 2 * RL, 128), F32)

        def prep_q(a):
            return (a[:, 0:128].astype(BF16), a[0:RL, 128:256].astype(BF16),
                    a[SEG:RT, 128:256].astype(BF16), a[:, 256:384].astype(BF16))

        def prep_kv(a):
            mid = a[:, 128:256]
            tlo = jnp.where(lo, mid, 0.0)
            thi = jnp.where(lo, 0.0, mid)
            return (_cat0([a[:, 0:128], z48]).astype(BF16),
                    _cat0([tlo[0:RL], thi[0:RL], z32]).astype(BF16),
                    _cat0([z32, tlo[SEG:RT], thi[SEG:RT]]).astype(BF16),
                    _cat0([z48, a[:, 256:384]]).astype(BF16))

        def qk(q, k):
            t0 = _dot_nt(q[0], k[0])
            t2 = _dot_nt(q[3], k[3])
            t1a = _dot_nt(q[1], k[1])
            t1b = _dot_nt(q[2], k[2])
            s = jnp.where(first, t0, t2) + _cat0([t1a[0:RV], t1b[M:RL]])
            e, e1, e2, inv = softmax2(s, first, valid, fill)
            pa = e * inv
            return ((e1 * inv).astype(BF16), pa[0:RL].astype(BF16),
                    pa[SEG:RT].astype(BF16), (e2 * inv).astype(BF16))

        def pv(pr, v):
            o0 = _dot(pr[0], v[0])
            o2 = _dot(pr[3], v[3])
            o1a = _dot(pr[1], v[1])
            o1b = _dot(pr[2], v[2])
            return _cat1([o0, _cat0([o1a[0:RV], o1b[M:RL]]), o2]).astype(BF16)

        return prep_q, prep_kv, qk, pv

    def make_single(layer):
        rr = lax.broadcasted_iota(jnp.int32, (RV, 2 * RL), 0)
        cc = lax.broadcasted_iota(jnp.int32, (RV, 2 * RL), 1)
        first = cc < RL
        kc = jnp.where(first, cc, cc - RL)
        if layer == 0:
            exists = kc < RV
            valid = exists & ((kc >= SEG) | (kc <= rr))
            r0 = 0
        else:
            exists = kc >= M
            valid = exists & ((rr < M) | (kc - M <= rr))
            r0 = M
        fill = jnp.where(exists, NEG, PADNEG)
        lo = lax.broadcasted_iota(jnp.int32, (RL, PW), 1) < DH
        zrow = jnp.zeros((M, 2 * RL), F32)

        def prep_q(a):
            return a.astype(BF16)

        def prep_kv(a):
            return _cat0([jnp.where(lo, a, 0.0), jnp.where(lo, 0.0, a)]).astype(BF16)

        def qk(q, k):
            s = _dot_nt(q, k)[r0:r0 + RV]
            e, _, _, inv = softmax2(s, first, valid, fill)
            pa = e * inv
            return _cat0([pa, zrow] if layer == 0 else [zrow, pa]).astype(BF16)

        def pv(pr, v):
            return _dot(pr, v).astype(BF16)

        return prep_q, prep_kv, qk, pv

    def step(t, a_layers, b_layers, light=False):
        r0 = 0 if 0 in a_layers else SEG
        r1 = RT if 1 in a_layers else RL
        h = h_ref[SEG if light else r0:r1, :]
        if len(a_layers) == 2:
            prep_q, prep_kv, qk, pv = make_joint()
        else:
            prep_q, prep_kv, qk, pv = make_single(a_layers[0])

        def proj(i, p):
            r = _dot(h, _unpack(wqkv_p[i, p]))
            if light:
                r = _cat0([pre_ref[i, p, pl.ds(pl.multiple_of((t - 2) * SEG, SEG), SEG), :], r])
            return r

        acc = [None]

        def oproj(p, o):
            part = _dot(o, _unpack(wo_p[p]))
            acc[0] = part if acc[0] is None else acc[0] + part

        def xrows(seg):
            if isinstance(seg, int):
                return x_ref[seg * SEG:(seg + 1) * SEG, :].astype(F32)
            return x_ref[pl.ds(pl.multiple_of(seg * SEG, SEG), SEG), :].astype(F32)

        q = prep_q(proj(0, 0))
        k = prep_kv(proj(1, 0))
        v = prep_kv(proj(2, 0))
        early_v = light or len(a_layers) == 1
        os_ = {}
        x2 = None
        for p in range(NP):
            pr = qk(q, k)
            if p + 1 < NP:
                q = prep_q(proj(0, p + 1))
                k = prep_kv(proj(1, p + 1))
                if early_v:
                    vn = prep_kv(proj(2, p + 1))
            else:
                if 1 in a_layers:
                    x2 = x2_ref[...]
                if b_layers:
                    b_out(t, xb, ob, b_layers)
                if 0 in a_layers:
                    nxt = t + 1 if isinstance(t, int) else jnp.minimum(t + 1, NSEG - 1)
                    h_ref[0:SEG, :] = _ln(xrows(nxt)).astype(BF16)
                oproj(p - 2, os_.pop(p - 2))
            os_[p] = pv(pr, v)
            if p + 1 < NP:
                v = vn if early_v else prep_kv(proj(2, p + 1))
            if p == 0 and b_layers:
                xb, qkv = b_qkv(b_layers)
                ob = b_attn(t, qkv, b_layers)
            if p >= 2 and p + 1 < NP:
                oproj(p - 2, os_.pop(p - 2))
        oproj(NP - 2, os_.pop(NP - 2))
        oproj(NP - 1, os_.pop(NP - 1))
        a = acc[0]
        if 0 in a_layers:
            xa_ref[0:SEG, :] = xrows(t) + a[0:SEG]
        if 1 in a_layers:
            xa_ref[SEG:2 * SEG, :] = x2 + a[RL - r0:RT - r0]
        mem1 = a[SEG - r0:RV - r0]
        mem2 = a[RV - r0:RL - r0] if 1 in a_layers else mem0
        h_ref[SEG:RL, :] = _cat0([mem1, mem2]).astype(BF16)

    def first_step():
        prep_q, prep_kv, qk, pv = make_single(0)

        def body0(p, carry):
            wait_group(p)

            @pl.when(p + WIN < NP)
            def _():
                start_group(p + WIN)

            @pl.when(p == NP - 1)
            def _():
                cp_x1.start()

            h = _unpack(hpre_ref[...])
            w = [w_pairs[i][1][rows_of(p), :] for i in range(4)]

            def proj(i):
                r = _dot_nt(h, w[i])
                pre_ref[i, p] = r[RL:]
                return r[0:RL]

            q = prep_q(proj(0))
            k = prep_kv(proj(1))
            pr = qk(q, k)
            acc_ref[...] += _dot(_unpack(o_ref[...]), wo_ref[rows_of(jnp.maximum(p - 1, 0)), :])
            v = prep_kv(proj(2))
            o_ref[...] = _pack(pv(pr, v))
            for i in range(3):
                wqkv_p[i, p] = _pack(w[i].T)
            wo_p[p] = _pack(w[3])

            @pl.when(p == PERM0)
            def _():
                for cp in cp_b:
                    cp.wait()

            @pl.when((p >= PERM0) & (p < PERM0 + NT))
            def _():
                c = p - PERM0
                perm_qkv_piece(0, c)
                perm_qkv_piece(1, c)

            @pl.when((p >= PERM0 + NT) & (p < PERM0 + 2 * NT))
            def _():
                c = p - PERM0 - NT
                perm_qkv_piece(2, c)
                perm_wo_piece(c)

            return carry

        lax.fori_loop(0, NP, body0, 0)
        a = acc_ref[...] + _dot(_unpack(o_ref[...]), wo_ref[rows_of(NP - 1), :])
        xa_ref[0:SEG, :] = x_ref[0:SEG, :].astype(F32) + a[0:SEG]
        h_ref[0:SEG, :] = _ln(x_ref[SEG:2 * SEG, :].astype(F32)).astype(BF16)
        h_ref[SEG:RL, :] = _cat0([a[SEG:RV], mem0]).astype(BF16)

    first_step()
    step(1, (0,), (0,))

    def body_light(t, carry):
        step(t, (0, 1), (0, 1), light=True)
        return carry

    lax.fori_loop(2, 2 + NPRE, body_light, 0)
    cp_x1.wait()

    def body(t, carry):
        step(t, (0, 1), (0, 1))
        return carry

    lax.fori_loop(2 + NPRE, NSEG, body, 0)
    done = (NSEG - 3) * SEG
    cp_o0 = pltpu.make_async_copy(out_ref.at[0:done], out_hbm.at[0:done], sem.at[6])
    cp_o0.start()
    step(NSEG, (1,), (0, 1))
    step(NSEG + 1, (1,), (1,))
    xb, qkv = b_qkv((1,))
    b_out(NSEG + 2, xb, b_attn(NSEG + 2, qkv, (1,)), (1,))
    cp_o1 = pltpu.make_async_copy(out_ref.at[done:S], out_hbm.at[done:S], sem.at[7])
    cp_o1.start()
    cp_o0.wait()
    cp_o1.wait()


@functools.partial(jax.jit, static_argnames=("A_seg_len",))
def pallas_interleave_layers__memory_aug_recurrent_mem_tr__sliding_local_dilated__prompt_kernel(
    A_x: jax.Array,
    A_mem0: jax.Array,
    A_Wq: jax.Array,
    A_Wk: jax.Array,
    A_Wv: jax.Array,
    A_Wo: jax.Array,
    A_seg_len,
    B_x: jax.Array,
    B_wqkv: jax.Array,
    B_wo: jax.Array,
):
    B, S, D = A_x.shape
    H, DH = A_Wq.shape[1], A_Wq.shape[2]
    M = A_mem0.shape[1]
    SEG = int(A_seg_len)
    assert B == 1 and M == 8 and SEG == 32 and DH == 192 and D % 128 == 0 and S % SEG == 0

    x = A_x.reshape(S, D)
    mem0 = A_mem0.reshape(M, D)
    wq = jnp.transpose(A_Wq, (1, 2, 0)).reshape(H * DH, D)
    wk = jnp.transpose(A_Wk, (1, 2, 0)).reshape(H * DH, D)
    wv = jnp.transpose(A_Wv, (1, 2, 0)).reshape(H * DH, D)
    wo = A_Wo.reshape(H * DH, D)

    hbm = pl.BlockSpec(memory_space=pl.ANY)
    out = pl.pallas_call(
        functools.partial(_kernel, S=S, D=D, H=H, DH=DH, M=M, SEG=SEG),
        out_shape=jax.ShapeDtypeStruct((S, D), A_x.dtype),
        in_specs=[pl.BlockSpec(memory_space=pltpu.VMEM)] + [hbm] * 7,
        out_specs=hbm,
        scratch_shapes=[
            pltpu.VMEM((S, D), BF16),
            pltpu.VMEM((S, D), BF16),
            pltpu.VMEM((H * DH, D), BF16),
            pltpu.VMEM((H * DH, D), BF16),
            pltpu.VMEM((H * DH, D), BF16),
            pltpu.VMEM((H * DH, D), BF16),
            pltpu.VMEM((3, D, D), BF16),
            pltpu.VMEM((D, D), BF16),
            pltpu.VMEM((3, H // 2, D // 2, 2 * DH), U32),
            pltpu.VMEM((H // 2, DH, D), U32),
            pltpu.VMEM((3 * D // 128, D // 2, 128), U32),
            pltpu.VMEM((D // 2, D), U32),
            pltpu.VMEM((2 * SEG + 2 * M, D), BF16),
            pltpu.VMEM((2 * SEG, D), F32),
            pltpu.VMEM((SEG, D), F32),
            pltpu.VMEM((2, 2 * D // 128, HIST + SEG, 128), F32),
            pltpu.VMEM((SEG + 2 * M, D), F32),
            pltpu.VMEM(((SEG + 2 * M + NPRE * SEG) // 2, D), U32),
            pltpu.VMEM((3, H // 2, NPRE * SEG, 2 * DH), F32),
            pltpu.VMEM(((SEG + 2 * M) // 2, 2 * DH), U32),
            pltpu.SemaphoreType.DMA((4 * (H // 2),)),
            pltpu.SemaphoreType.DMA((8,)),
        ],
        compiler_params=pltpu.CompilerParams(vmem_limit_bytes=110 * 1024 * 1024),
    )(mem0, x, wq, wk, wv, wo, B_wqkv, B_wo)
    return out.reshape(B, S, D)
```

```python
import functools

import jax
import jax.numpy as jnp
from jax import lax
import jax.experimental.pallas as pl
import jax.experimental.pallas.tpu as pltpu

F32 = jnp.float32
BF16 = jnp.bfloat16
U32 = jnp.uint32

EPS = 1e-5
NEG = -1000000000.0
PADNEG = -3.0e38
B_HEADS = 32
B_WIN = 8
B_DIL = 2
NPRE = 6
HIST = 16


def _ln(x):
    m = jnp.mean(x, axis=-1, keepdims=True)
    xc = x - m
    v = jnp.mean(xc * xc, axis=-1, keepdims=True)
    return xc * lax.rsqrt(v + EPS)


def _dot_nt(a, b):
    return lax.dot_general(a, b, (((1,), (1,)), ((), ())), preferred_element_type=F32)


def _dot(a, b):
    return jnp.dot(a, b, preferred_element_type=F32)


def _pack(a):
    return pltpu.bitcast(a, U32)


def _unpack(a):
    return pltpu.bitcast(a, BF16)


def _cat0(xs):
    return jnp.concatenate(xs, axis=0)


def _cat1(xs):
    return jnp.concatenate(xs, axis=1)


def _kernel(mem0_ref, x_hbm, wq_hbm, wk_hbm, wv_hbm, wo_hbm, bqkv_hbm, bwo_hbm,
            out_hbm,
            x_ref, out_ref, wq_ref, wk_ref, wv_ref, wo_ref, bqkv_ref, bwo_ref,
            wqkv_p, wo_p, bqkv_p, bwo_p, h_ref, xa_ref, x2_ref, kv_ref, acc_ref, hpre_ref, pre_ref, o_ref, tmp_ref, wsem, sem,
            *, S, D, H, DH, M, SEG):
    NSEG = S // SEG
    PW = 2 * DH
    NP = H // 2
    RV = SEG + M
    RL = SEG + 2 * M
    RT = 2 * SEG + 2 * M
    a_scale = DH ** (-0.5)
    b_dh = D // B_HEADS
    b_scale = b_dh ** (-0.5)
    NT = D // 128
    X0 = (NPRE + 3) * SEG
    WIN = 2
    PERM0 = 5

    def sl(p):
        return slice(p * PW, (p + 1) * PW)

    cp_x0 = pltpu.make_async_copy(x_hbm.at[0:X0], x_ref.at[0:X0], sem.at[0])
    cp_x1 = pltpu.make_async_copy(x_hbm.at[X0:S], x_ref.at[X0:S], sem.at[1])
    cp_b = [pltpu.make_async_copy(bqkv_hbm.at[:, j * D:(j + 1) * D], bqkv_ref.at[j], sem.at[2 + j])
            for j in range(3)]
    cp_b.append(pltpu.make_async_copy(bwo_hbm, bwo_ref, sem.at[5]))
    w_pairs = ((wq_hbm, wq_ref), (wk_hbm, wk_ref), (wv_hbm, wv_ref), (wo_hbm, wo_ref))

    def rows_of(p):
        if isinstance(p, int):
            return pl.ds(p * PW, PW)
        return pl.ds(pl.multiple_of(p * PW, 128), PW)

    def cp_w(i, p):
        src, dst = w_pairs[i]
        return pltpu.make_async_copy(src.at[rows_of(p)], dst.at[rows_of(p)], wsem.at[i * NP + p])

    def start_group(p):
        for i in range(4):
            cp_w(i, p).start()

    def wait_group(p):
        for i in range(4):
            cp_w(i, p).wait()

    cp_x0.start()
    for p in range(WIN):
        start_group(p)

    mem0 = mem0_ref[...].astype(F32)
    xa_ref[...] = jnp.zeros(xa_ref.shape, F32)
    kv_ref[...] = jnp.zeros(kv_ref.shape, F32)
    acc_ref[...] = jnp.zeros(acc_ref.shape, F32)
    cp_x0.wait()
    h0 = _ln(x_ref[0:SEG, :].astype(F32))
    hpre_ref[0:RL // 2, :] = _pack(_cat0([h0, mem0, mem0]).astype(BF16))
    for i in range(NPRE):
        hi = _ln(x_ref[(2 + i) * SEG:(3 + i) * SEG, :].astype(F32)).astype(BF16)
        hpre_ref[(RL + i * SEG) // 2:(RL + (i + 1) * SEG) // 2, :] = _pack(hi)
    o_ref[...] = jnp.zeros(o_ref.shape, U32)

    def perm_rows(a):
        a = a.astype(F32)
        for m in range(NT):
            tmp_ref[m] = a[:, m * 128:(m + 1) * 128]
        return _cat1([_cat0([tmp_ref[m, pl.ds(d, B_HEADS, stride=b_dh), :] for d in range(b_dh)])
                      for m in range(NT)]).astype(BF16)

    def perm_qkv(j):
        wp = perm_rows(bqkv_ref[j].T).T
        for c in range(NT):
            bqkv_p[j * NT + c] = _pack(wp[:, c * 128:(c + 1) * 128])

    def perm_wo():
        bwo_p[...] = _pack(perm_rows(bwo_ref[...]))

    def b_qkv(layers):
        xb = xa_ref[layers[0] * SEG:(layers[-1] + 1) * SEG, :]
        hb = _ln(xb).astype(BF16)
        return xb, [_dot(hb, _unpack(bqkv_p[n])) for n in range(3 * NT)]

    def b_attn(t, qkv, layers):
        outs = []
        for i, l in enumerate(layers):
            rows = slice(i * SEG, (i + 1) * SEG)
            q = [qkv[j][rows] for j in range(NT)]
            for j in range(2 * NT):
                kv_ref[l, j, HIST:HIST + SEG, :] = qkv[NT + j][rows]
            seg = t - 1 - 2 * l
            pos = seg * SEG + lax.broadcasted_iota(jnp.int32, (SEG, 128), 0)
            logits = []
            for w in range(B_WIN):
                o = HIST - B_DIL * w
                s = q[0] * kv_ref[l, 0, o:o + SEG, :]
                for j in range(1, NT):
                    s = s + q[j] * kv_ref[l, j, o:o + SEG, :]
                s = s + pltpu.roll(s, 64, 1)
                s = s + pltpu.roll(s, 32, 1)
                logits.append(jnp.where(pos >= B_DIL * w, s * b_scale, NEG))
            m = logits[0]
            for w in range(1, B_WIN):
                m = jnp.maximum(m, logits[w])
            es = [jnp.exp(lg - m) for lg in logits]
            den = es[0]
            for w in range(1, B_WIN):
                den = den + es[w]
            inv = 1.0 / den
            tiles = []
            for j in range(NT):
                acc = None
                for w in range(B_WIN):
                    o = HIST - B_DIL * w
                    term = es[w] * kv_ref[l, NT + j, o:o + SEG, :]
                    acc = term if acc is None else acc + term
                tiles.append(acc * inv)
            outs.append(_cat1(tiles))
            for j in range(2 * NT):
                kv_ref[l, j, 0:HIST, :] = qkv[NT + j][(i + 1) * SEG - HIST:(i + 1) * SEG]
        return _cat0(outs).astype(BF16)

    def b_out(t, xb, ob, layers):
        y = xb + _dot(ob, _unpack(bwo_p[...]))
        for i, l in enumerate(layers):
            yl = y[i * SEG:(i + 1) * SEG]
            if l == 0:
                x2_ref[...] = yl
                h_ref[RL:RT, :] = _ln(yl).astype(BF16)
            else:
                if isinstance(t, int):
                    row = (t - 3) * SEG
                else:
                    row = pl.multiple_of(jnp.maximum(t - 3, 0) * SEG, SEG)
                out_ref[pl.ds(row, SEG), :] = yl.astype(out_ref.dtype)

    def softmax2(s, first, valid, fill):
        s = jnp.where(valid, s * a_scale, fill)
        m1 = jnp.max(jnp.where(first, s, PADNEG), axis=-1, keepdims=True)
        m2 = jnp.max(jnp.where(first, PADNEG, s), axis=-1, keepdims=True)
        e = jnp.exp(s - jnp.where(first, m1, m2))
        e1 = jnp.where(first, e, 0.0)
        e2 = jnp.where(first, 0.0, e)
        l1 = jnp.sum(e1, axis=-1, keepdims=True)
        l2 = jnp.sum(e2, axis=-1, keepdims=True)
        inv = 1.0 / jnp.where(first, l1, l2)
        return e, e1, e2, inv

    def make_joint():
        rr = lax.broadcasted_iota(jnp.int32, (RT, 128), 0)
        cc = lax.broadcasted_iota(jnp.int32, (RT, 128), 1)
        lay1 = rr < RV
        first = cc < jnp.where(lay1, RL, RT)
        key = jnp.where(first, cc, cc - RL)
        exists = jnp.where(lay1, RV - 1 - key, key - RV) >= 0
        allowed = (key <= rr) | (lay1 & (key >= SEG)) | ((rr >= RV) & (rr < RL))
        valid = exists & allowed
        fill = jnp.where(exists, NEG, PADNEG)
        lo = cc < (DH - 128)
        z48 = jnp.zeros((128 - RT, 128), F32)
        z32 = jnp.zeros((128 - 2 * RL, 128), F32)

        def prep_q(a):
            return (a[:, 0:128].astype(BF16), a[0:RL, 128:256].astype(BF16),
                    a[SEG:RT, 128:256].astype(BF16), a[:, 256:384].astype(BF16))

        def prep_kv(a):
            mid = a[:, 128:256]
            tlo = jnp.where(lo, mid, 0.0)
            thi = jnp.where(lo, 0.0, mid)
            return (_cat0([a[:, 0:128], z48]).astype(BF16),
                    _cat0([tlo[0:RL], thi[0:RL], z32]).astype(BF16),
                    _cat0([z32, tlo[SEG:RT], thi[SEG:RT]]).astype(BF16),
                    _cat0([z48, a[:, 256:384]]).astype(BF16))

        def qk(q, k):
            t0 = _dot_nt(q[0], k[0])
            t2 = _dot_nt(q[3], k[3])
            t1a = _dot_nt(q[1], k[1])
            t1b = _dot_nt(q[2], k[2])
            s = jnp.where(first, t0, t2) + _cat0([t1a[0:RV], t1b[M:RL]])
            e, e1, e2, inv = softmax2(s, first, valid, fill)
            pa = e * inv
            return ((e1 * inv).astype(BF16), pa[0:RL].astype(BF16),
                    pa[SEG:RT].astype(BF16), (e2 * inv).astype(BF16))

        def pv(pr, v):
            o0 = _dot(pr[0], v[0])
            o2 = _dot(pr[3], v[3])
            o1a = _dot(pr[1], v[1])
            o1b = _dot(pr[2], v[2])
            return _cat1([o0, _cat0([o1a[0:RV], o1b[M:RL]]), o2]).astype(BF16)

        return prep_q, prep_kv, qk, pv

    def make_single(layer):
        rr = lax.broadcasted_iota(jnp.int32, (RV, 2 * RL), 0)
        cc = lax.broadcasted_iota(jnp.int32, (RV, 2 * RL), 1)
        first = cc < RL
        kc = jnp.where(first, cc, cc - RL)
        if layer == 0:
            exists = kc < RV
            valid = exists & ((kc >= SEG) | (kc <= rr))
            r0 = 0
        else:
            exists = kc >= M
            valid = exists & ((rr < M) | (kc - M <= rr))
            r0 = M
        fill = jnp.where(exists, NEG, PADNEG)
        lo = lax.broadcasted_iota(jnp.int32, (RL, PW), 1) < DH
        zrow = jnp.zeros((M, 2 * RL), F32)

        def prep_q(a):
            return a.astype(BF16)

        def prep_kv(a):
            return _cat0([jnp.where(lo, a, 0.0), jnp.where(lo, 0.0, a)]).astype(BF16)

        def qk(q, k):
            s = _dot_nt(q, k)[r0:r0 + RV]
            e, _, _, inv = softmax2(s, first, valid, fill)
            pa = e * inv
            return _cat0([pa, zrow] if layer == 0 else [zrow, pa]).astype(BF16)

        def pv(pr, v):
            return _dot(pr, v).astype(BF16)

        return prep_q, prep_kv, qk, pv

    def step(t, a_layers, b_layers, light=False):
        r0 = 0 if 0 in a_layers else SEG
        r1 = RT if 1 in a_layers else RL
        h = h_ref[SEG if light else r0:r1, :]
        if len(a_layers) == 2:
            prep_q, prep_kv, qk, pv = make_joint()
        else:
            prep_q, prep_kv, qk, pv = make_single(a_layers[0])

        def proj(i, p):
            r = _dot(h, _unpack(wqkv_p[i, p]))
            if light:
                r = _cat0([pre_ref[i, p, pl.ds(pl.multiple_of((t - 2) * SEG, SEG), SEG), :], r])
            return r

        acc = [None]

        def oproj(p, o):
            part = _dot(o, _unpack(wo_p[p]))
            acc[0] = part if acc[0] is None else acc[0] + part

        def xrows(seg):
            if isinstance(seg, int):
                return x_ref[seg * SEG:(seg + 1) * SEG, :].astype(F32)
            return x_ref[pl.ds(pl.multiple_of(seg * SEG, SEG), SEG), :].astype(F32)

        q = prep_q(proj(0, 0))
        k = prep_kv(proj(1, 0))
        v = prep_kv(proj(2, 0))
        early_v = light or len(a_layers) == 1
        os_ = {}
        x2 = None
        for p in range(NP):
            pr = qk(q, k)
            if p + 1 < NP:
                q = prep_q(proj(0, p + 1))
                k = prep_kv(proj(1, p + 1))
                if early_v:
                    vn = prep_kv(proj(2, p + 1))
            else:
                if 1 in a_layers:
                    x2 = x2_ref[...]
                if b_layers:
                    b_out(t, xb, ob, b_layers)
                if 0 in a_layers:
                    nxt = t + 1 if isinstance(t, int) else jnp.minimum(t + 1, NSEG - 1)
                    h_ref[0:SEG, :] = _ln(xrows(nxt)).astype(BF16)
                oproj(p - 2, os_.pop(p - 2))
            os_[p] = pv(pr, v)
            if p + 1 < NP:
                v = vn if early_v else prep_kv(proj(2, p + 1))
            if p == 0 and b_layers:
                xb, qkv = b_qkv(b_layers)
                ob = b_attn(t, qkv, b_layers)
            if p >= 2 and p + 1 < NP:
                oproj(p - 2, os_.pop(p - 2))
        oproj(NP - 2, os_.pop(NP - 2))
        oproj(NP - 1, os_.pop(NP - 1))
        a = acc[0]
        if 0 in a_layers:
            xa_ref[0:SEG, :] = xrows(t) + a[0:SEG]
        if 1 in a_layers:
            xa_ref[SEG:2 * SEG, :] = x2 + a[RL - r0:RT - r0]
        mem1 = a[SEG - r0:RV - r0]
        mem2 = a[RV - r0:RL - r0] if 1 in a_layers else mem0
        h_ref[SEG:RL, :] = _cat0([mem1, mem2]).astype(BF16)

    def first_step():
        prep_q, prep_kv, qk, pv = make_single(0)

        def body0(p, carry):
            wait_group(p)

            @pl.when(p + WIN < NP)
            def _():
                start_group(p + WIN)

            @pl.when(p == 1)
            def _():
                for cp in cp_b:
                    cp.start()

            @pl.when(p == NP - 1)
            def _():
                cp_x1.start()

            h = _unpack(hpre_ref[...])
            w = [w_pairs[i][1][rows_of(p), :] for i in range(4)]

            def proj(i):
                r = _dot_nt(h, w[i])
                pre_ref[i, p] = r[RL:]
                return r[0:RL]

            q = prep_q(proj(0))
            k = prep_kv(proj(1))
            pr = qk(q, k)
            acc_ref[...] += _dot(_unpack(o_ref[...]), wo_ref[rows_of(jnp.maximum(p - 1, 0)), :])
            v = prep_kv(proj(2))
            o_ref[...] = _pack(pv(pr, v))
            for i in range(3):
                wqkv_p[i, p] = _pack(w[i].T)
            wo_p[p] = _pack(w[3])

            @pl.when(p == PERM0)
            def _():
                for cp in cp_b:
                    cp.wait()
                perm_wo()

            @pl.when((p > PERM0) & (p <= PERM0 + 3))
            def _():
                perm_qkv(p - PERM0 - 1)

            return carry

        lax.fori_loop(0, NP, body0, 0)
        a = acc_ref[...] + _dot(_unpack(o_ref[...]), wo_ref[rows_of(NP - 1), :])
        xa_ref[0:SEG, :] = x_ref[0:SEG, :].astype(F32) + a[0:SEG]
        h_ref[0:SEG, :] = _ln(x_ref[SEG:2 * SEG, :].astype(F32)).astype(BF16)
        h_ref[SEG:RL, :] = _cat0([a[SEG:RV], mem0]).astype(BF16)

    first_step()
    step(1, (0,), (0,))

    def body_light(t, carry):
        step(t, (0, 1), (0, 1), light=True)
        return carry

    lax.fori_loop(2, 2 + NPRE, body_light, 0)
    cp_x1.wait()

    def body(t, carry):
        step(t, (0, 1), (0, 1))
        return carry

    lax.fori_loop(2 + NPRE, NSEG, body, 0)
    done = (NSEG - 3) * SEG
    cp_o0 = pltpu.make_async_copy(out_ref.at[0:done], out_hbm.at[0:done], sem.at[6])
    cp_o0.start()
    step(NSEG, (1,), (0, 1))
    step(NSEG + 1, (1,), (1,))
    xb, qkv = b_qkv((1,))
    b_out(NSEG + 2, xb, b_attn(NSEG + 2, qkv, (1,)), (1,))
    cp_o1 = pltpu.make_async_copy(out_ref.at[done:S], out_hbm.at[done:S], sem.at[7])
    cp_o1.start()
    cp_o0.wait()
    cp_o1.wait()


@functools.partial(jax.jit, static_argnames=("A_seg_len",))
def pallas_interleave_layers__memory_aug_recurrent_mem_tr__sliding_local_dilated__prompt_kernel(
    A_x: jax.Array,
    A_mem0: jax.Array,
    A_Wq: jax.Array,
    A_Wk: jax.Array,
    A_Wv: jax.Array,
    A_Wo: jax.Array,
    A_seg_len,
    B_x: jax.Array,
    B_wqkv: jax.Array,
    B_wo: jax.Array,
):
    B, S, D = A_x.shape
    H, DH = A_Wq.shape[1], A_Wq.shape[2]
    M = A_mem0.shape[1]
    SEG = int(A_seg_len)
    assert B == 1 and M == 8 and SEG == 32 and DH == 192 and D % 128 == 0 and S % SEG == 0

    x = A_x.reshape(S, D)
    mem0 = A_mem0.reshape(M, D)
    wq = jnp.transpose(A_Wq, (1, 2, 0)).reshape(H * DH, D)
    wk = jnp.transpose(A_Wk, (1, 2, 0)).reshape(H * DH, D)
    wv = jnp.transpose(A_Wv, (1, 2, 0)).reshape(H * DH, D)
    wo = A_Wo.reshape(H * DH, D)

    hbm = pl.BlockSpec(memory_space=pl.ANY)
    out = pl.pallas_call(
        functools.partial(_kernel, S=S, D=D, H=H, DH=DH, M=M, SEG=SEG),
        out_shape=jax.ShapeDtypeStruct((S, D), A_x.dtype),
        in_specs=[pl.BlockSpec(memory_space=pltpu.VMEM)] + [hbm] * 7,
        out_specs=hbm,
        scratch_shapes=[
            pltpu.VMEM((S, D), BF16),
            pltpu.VMEM((S, D), BF16),
            pltpu.VMEM((H * DH, D), BF16),
            pltpu.VMEM((H * DH, D), BF16),
            pltpu.VMEM((H * DH, D), BF16),
            pltpu.VMEM((H * DH, D), BF16),
            pltpu.VMEM((3, D, D), BF16),
            pltpu.VMEM((D, D), BF16),
            pltpu.VMEM((3, H // 2, D // 2, 2 * DH), U32),
            pltpu.VMEM((H // 2, DH, D), U32),
            pltpu.VMEM((3 * D // 128, D // 2, 128), U32),
            pltpu.VMEM((D // 2, D), U32),
            pltpu.VMEM((2 * SEG + 2 * M, D), BF16),
            pltpu.VMEM((2 * SEG, D), F32),
            pltpu.VMEM((SEG, D), F32),
            pltpu.VMEM((2, 2 * D // 128, HIST + SEG, 128), F32),
            pltpu.VMEM((SEG + 2 * M, D), F32),
            pltpu.VMEM(((SEG + 2 * M + NPRE * SEG) // 2, D), U32),
            pltpu.VMEM((3, H // 2, NPRE * SEG, 2 * DH), F32),
            pltpu.VMEM(((SEG + 2 * M) // 2, 2 * DH), U32),
            pltpu.VMEM((D // 128, D, 128), F32),
            pltpu.SemaphoreType.DMA((4 * (H // 2),)),
            pltpu.SemaphoreType.DMA((8,)),
        ],
        compiler_params=pltpu.CompilerParams(vmem_limit_bytes=110 * 1024 * 1024),
    )(mem0, x, wq, wk, wv, wo, B_wqkv, B_wo)
    return out.reshape(B, S, D)
```

```python
import functools

import jax
import jax.numpy as jnp
from jax import lax
import jax.experimental.pallas as pl
import jax.experimental.pallas.tpu as pltpu

F32 = jnp.float32
BF16 = jnp.bfloat16
U32 = jnp.uint32

EPS = 1e-5
NEG = -1000000000.0
PADNEG = -3.0e38
B_HEADS = 32
B_WIN = 8
B_DIL = 2
NPRE = 8
HIST = 16


def _ln(x):
    m = jnp.mean(x, axis=-1, keepdims=True)
    xc = x - m
    v = jnp.mean(xc * xc, axis=-1, keepdims=True)
    return xc * lax.rsqrt(v + EPS)


def _dot_nt(a, b):
    return lax.dot_general(a, b, (((1,), (1,)), ((), ())), preferred_element_type=F32)


def _dot(a, b):
    return jnp.dot(a, b, preferred_element_type=F32)


def _pack(a):
    return pltpu.bitcast(a, U32)


def _unpack(a):
    return pltpu.bitcast(a, BF16)


def _cat0(xs):
    return jnp.concatenate(xs, axis=0)


def _cat1(xs):
    return jnp.concatenate(xs, axis=1)


def _kernel(mem0_hbm, x_hbm, wq_hbm, wk_hbm, wv_hbm, wo_hbm, bqkv_hbm, bwo_hbm,
            out_hbm,
            mem0_ref, x_ref, out_ref, wq_ref, wk_ref, wv_ref, wo_ref, bqkv_ref, bwo_ref,
            wqkv_p, wo_p, bqkv_p, bwo_p, h_ref, xa_ref, x2_ref, kv_ref, acc_ref, hpre_ref, pre_ref, o_ref, tmp_ref, wsem, sem,
            *, S, D, H, DH, M, SEG):
    NSEG = S // SEG
    PW = 2 * DH
    NP = H // 2
    RV = SEG + M
    RL = SEG + 2 * M
    RT = 2 * SEG + 2 * M
    a_scale = DH ** (-0.5)
    b_dh = D // B_HEADS
    b_scale = b_dh ** (-0.5)
    NT = D // 128
    X0 = (NPRE + 3) * SEG

    def sl(p):
        return slice(p * PW, (p + 1) * PW)

    cp_m = pltpu.make_async_copy(mem0_hbm, mem0_ref, sem.at[8])
    cp_x0 = pltpu.make_async_copy(x_hbm.at[0:X0], x_ref.at[0:X0], sem.at[0])
    cp_x1 = pltpu.make_async_copy(x_hbm.at[X0:S], x_ref.at[X0:S], sem.at[1])
    cp_b = [pltpu.make_async_copy(bqkv_hbm.at[:, j * D:(j + 1) * D], bqkv_ref.at[j], sem.at[2 + j])
            for j in range(3)]
    cp_b.append(pltpu.make_async_copy(bwo_hbm, bwo_ref, sem.at[5]))
    w_pairs = ((wq_hbm, wq_ref), (wk_hbm, wk_ref), (wv_hbm, wv_ref), (wo_hbm, wo_ref))

    def rows_of(p):
        if isinstance(p, int):
            return pl.ds(p * PW, PW)
        return pl.ds(pl.multiple_of(p * PW, 128), PW)

    def cp_w(i, p):
        src, dst = w_pairs[i]
        return pltpu.make_async_copy(src.at[rows_of(p)], dst.at[rows_of(p)], wsem.at[i * NP + p])

    def start_group(p):
        for i in range(4):
            cp_w(i, p).start()

    def wait_group(p):
        for i in range(4):
            cp_w(i, p).wait()

    def start_groups(lo, hi):
        def f(p, carry):
            start_group(p)
            return carry
        lax.fori_loop(lo, hi, f, 0)

    cp_m.start()
    cp_x0.start()
    start_groups(0, NP)
    for cp in cp_b:
        cp.start()

    xa_ref[...] = jnp.zeros(xa_ref.shape, F32)
    kv_ref[...] = jnp.zeros(kv_ref.shape, F32)
    acc_ref[...] = jnp.zeros(acc_ref.shape, F32)
    cp_m.wait()
    cp_x0.wait()
    mem0 = mem0_ref[...].astype(F32)
    h0 = _ln(x_ref[0:SEG, :].astype(F32))
    hpre_ref[0:RL // 2, :] = _pack(_cat0([h0, mem0, mem0]).astype(BF16))
    for i in range(NPRE):
        hi = _ln(x_ref[(2 + i) * SEG:(3 + i) * SEG, :].astype(F32)).astype(BF16)
        hpre_ref[(RL + i * SEG) // 2:(RL + (i + 1) * SEG) // 2, :] = _pack(hi)
    o_ref[...] = jnp.zeros(o_ref.shape, U32)

    def perm_rows(a, slot):
        a = a.astype(F32)
        for m in range(NT):
            tmp_ref[slot, m] = a[:, m * 128:(m + 1) * 128]
        return _cat1([_cat0([tmp_ref[slot, m, pl.ds(d, B_HEADS, stride=b_dh), :] for d in range(b_dh)])
                      for m in range(NT)]).astype(BF16)

    def perm_qkv(j):
        wp = perm_rows(bqkv_ref[j].T, j).T
        for c in range(NT):
            bqkv_p[j * NT + c] = _pack(wp[:, c * 128:(c + 1) * 128])

    def perm_wo():
        bwo_p[...] = _pack(perm_rows(bwo_ref[...], 3))

    def b_qkv(layers):
        xb = xa_ref[layers[0] * SEG:(layers[-1] + 1) * SEG, :]
        hb = _ln(xb).astype(BF16)
        return xb, [_dot(hb, _unpack(bqkv_p[n])) for n in range(3 * NT)]

    def b_attn(t, qkv, layers):
        outs = []
        for i, l in enumerate(layers):
            rows = slice(i * SEG, (i + 1) * SEG)
            q = [qkv[j][rows] for j in range(NT)]
            for j in range(2 * NT):
                kv_ref[l, j, HIST:HIST + SEG, :] = qkv[NT + j][rows]
            seg = t - 1 - 2 * l
            pos = seg * SEG + lax.broadcasted_iota(jnp.int32, (SEG, 128), 0)
            logits = []
            for w in range(B_WIN):
                o = HIST - B_DIL * w
                s = q[0] * kv_ref[l, 0, o:o + SEG, :]
                for j in range(1, NT):
                    s = s + q[j] * kv_ref[l, j, o:o + SEG, :]
                s = s + pltpu.roll(s, 64, 1)
                s = s + pltpu.roll(s, 32, 1)
                logits.append(jnp.where(pos >= B_DIL * w, s * b_scale, NEG))
            m = logits[0]
            for w in range(1, B_WIN):
                m = jnp.maximum(m, logits[w])
            es = [jnp.exp(lg - m) for lg in logits]
            den = es[0]
            for w in range(1, B_WIN):
                den = den + es[w]
            inv = 1.0 / den
            tiles = []
            for j in range(NT):
                acc = None
                for w in range(B_WIN):
                    o = HIST - B_DIL * w
                    term = es[w] * kv_ref[l, NT + j, o:o + SEG, :]
                    acc = term if acc is None else acc + term
                tiles.append(acc * inv)
            outs.append(_cat1(tiles))
            for j in range(2 * NT):
                kv_ref[l, j, 0:HIST, :] = qkv[NT + j][(i + 1) * SEG - HIST:(i + 1) * SEG]
        return _cat0(outs).astype(BF16)

    def b_out(t, xb, ob, layers):
        y = xb + _dot(ob, _unpack(bwo_p[...]))
        for i, l in enumerate(layers):
            yl = y[i * SEG:(i + 1) * SEG]
            if l == 0:
                x2_ref[...] = yl
                h_ref[RL:RT, :] = _ln(yl).astype(BF16)
            else:
                if isinstance(t, int):
                    row = (t - 3) * SEG
                else:
                    row = pl.multiple_of(jnp.maximum(t - 3, 0) * SEG, SEG)
                out_ref[pl.ds(row, SEG), :] = yl.astype(out_ref.dtype)

    def softmax2(s, first, valid, fill):
        s = jnp.where(valid, s * a_scale, fill)
        m1 = jnp.max(jnp.where(first, s, PADNEG), axis=-1, keepdims=True)
        m2 = jnp.max(jnp.where(first, PADNEG, s), axis=-1, keepdims=True)
        e = jnp.exp(s - jnp.where(first, m1, m2))
        e1 = jnp.where(first, e, 0.0)
        e2 = jnp.where(first, 0.0, e)
        l1 = jnp.sum(e1, axis=-1, keepdims=True)
        l2 = jnp.sum(e2, axis=-1, keepdims=True)
        inv = 1.0 / jnp.where(first, l1, l2)
        return e, e1, e2, inv

    def make_joint():
        rr = lax.broadcasted_iota(jnp.int32, (RT, 128), 0)
        cc = lax.broadcasted_iota(jnp.int32, (RT, 128), 1)
        lay1 = rr < RV
        first = cc < jnp.where(lay1, RL, RT)
        key = jnp.where(first, cc, cc - RL)
        exists = jnp.where(lay1, RV - 1 - key, key - RV) >= 0
        allowed = (key <= rr) | (lay1 & (key >= SEG)) | ((rr >= RV) & (rr < RL))
        valid = exists & allowed
        fill = jnp.where(exists, NEG, PADNEG)
        lo = cc < (DH - 128)
        z48 = jnp.zeros((128 - RT, 128), F32)
        z32 = jnp.zeros((128 - 2 * RL, 128), F32)

        def prep_q(a):
            return (a[:, 0:128].astype(BF16), a[0:RL, 128:256].astype(BF16),
                    a[SEG:RT, 128:256].astype(BF16), a[:, 256:384].astype(BF16))

        def prep_kv(a):
            mid = a[:, 128:256]
            tlo = jnp.where(lo, mid, 0.0)
            thi = jnp.where(lo, 0.0, mid)
            return (_cat0([a[:, 0:128], z48]).astype(BF16),
                    _cat0([tlo[0:RL], thi[0:RL], z32]).astype(BF16),
                    _cat0([z32, tlo[SEG:RT], thi[SEG:RT]]).astype(BF16),
                    _cat0([z48, a[:, 256:384]]).astype(BF16))

        def qk(q, k):
            t0 = _dot_nt(q[0], k[0])
            t2 = _dot_nt(q[3], k[3])
            t1a = _dot_nt(q[1], k[1])
            t1b = _dot_nt(q[2], k[2])
            s = jnp.where(first, t0, t2) + _cat0([t1a[0:RV], t1b[M:RL]])
            e, e1, e2, inv = softmax2(s, first, valid, fill)
            pa = e * inv
            return ((e1 * inv).astype(BF16), pa[0:RL].astype(BF16),
                    pa[SEG:RT].astype(BF16), (e2 * inv).astype(BF16))

        def pv(pr, v):
            o0 = _dot(pr[0], v[0])
            o2 = _dot(pr[3], v[3])
            o1a = _dot(pr[1], v[1])
            o1b = _dot(pr[2], v[2])
            return _cat1([o0, _cat0([o1a[0:RV], o1b[M:RL]]), o2]).astype(BF16)

        return prep_q, prep_kv, qk, pv

    def make_single(layer):
        rr = lax.broadcasted_iota(jnp.int32, (RV, 2 * RL), 0)
        cc = lax.broadcasted_iota(jnp.int32, (RV, 2 * RL), 1)
        first = cc < RL
        kc = jnp.where(first, cc, cc - RL)
        if layer == 0:
            exists = kc < RV
            valid = exists & ((kc >= SEG) | (kc <= rr))
            r0 = 0
        else:
            exists = kc >= M
            valid = exists & ((rr < M) | (kc - M <= rr))
            r0 = M
        fill = jnp.where(exists, NEG, PADNEG)
        lo = lax.broadcasted_iota(jnp.int32, (RL, PW), 1) < DH
        zrow = jnp.zeros((M, 2 * RL), F32)

        def prep_q(a):
            return a.astype(BF16)

        def prep_kv(a):
            return _cat0([jnp.where(lo, a, 0.0), jnp.where(lo, 0.0, a)]).astype(BF16)

        def qk(q, k):
            s = _dot_nt(q, k)[r0:r0 + RV]
            e, _, _, inv = softmax2(s, first, valid, fill)
            pa = e * inv
            return _cat0([pa, zrow] if layer == 0 else [zrow, pa]).astype(BF16)

        def pv(pr, v):
            return _dot(pr, v).astype(BF16)

        return prep_q, prep_kv, qk, pv

    def step(t, a_layers, b_layers, light=False, b_at=0):
        r0 = 0 if 0 in a_layers else SEG
        r1 = RT if 1 in a_layers else RL
        h = h_ref[SEG if light else r0:r1, :]
        if len(a_layers) == 2:
            prep_q, prep_kv, qk, pv = make_joint()
        else:
            prep_q, prep_kv, qk, pv = make_single(a_layers[0])

        def proj(i, p):
            r = _dot(h, _unpack(wqkv_p[i, p]))
            if light:
                r = _cat0([pre_ref[i, p, pl.ds(pl.multiple_of((t - 2) * SEG, SEG), SEG), :], r])
            return r

        acc = [None]

        def oproj(p, o):
            part = _dot(o, _unpack(wo_p[p]))
            acc[0] = part if acc[0] is None else acc[0] + part

        def xrows(seg):
            if isinstance(seg, int):
                return x_ref[seg * SEG:(seg + 1) * SEG, :].astype(F32)
            return x_ref[pl.ds(pl.multiple_of(seg * SEG, SEG), SEG), :].astype(F32)

        q = prep_q(proj(0, 0))
        k = prep_kv(proj(1, 0))
        v = prep_kv(proj(2, 0))
        early_v = light or len(a_layers) == 1
        os_ = {}
        x2 = None
        for p in range(NP):
            pr = qk(q, k)
            if p + 1 < NP:
                q = prep_q(proj(0, p + 1))
                k = prep_kv(proj(1, p + 1))
                if early_v:
                    vn = prep_kv(proj(2, p + 1))
            else:
                if 1 in a_layers:
                    x2 = x2_ref[...]
                if b_layers:
                    b_out(t, xb, ob, b_layers)
                if 0 in a_layers:
                    nxt = t + 1 if isinstance(t, int) else jnp.minimum(t + 1, NSEG - 1)
                    h_ref[0:SEG, :] = _ln(xrows(nxt)).astype(BF16)
                oproj(p - 2, os_.pop(p - 2))
            os_[p] = pv(pr, v)
            if p + 1 < NP:
                v = vn if early_v else prep_kv(proj(2, p + 1))
            if p == b_at and b_layers:
                xb, qkv = b_qkv(b_layers)
                ob = b_attn(t, qkv, b_layers)
            if p >= 2 and p + 1 < NP:
                oproj(p - 2, os_.pop(p - 2))
        oproj(NP - 2, os_.pop(NP - 2))
        oproj(NP - 1, os_.pop(NP - 1))
        a = acc[0]
        if 0 in a_layers:
            xa_ref[0:SEG, :] = xrows(t) + a[0:SEG]
        if 1 in a_layers:
            xa_ref[SEG:2 * SEG, :] = x2 + a[RL - r0:RT - r0]
        mem1 = a[SEG - r0:RV - r0]
        mem2 = a[RV - r0:RL - r0] if 1 in a_layers else mem0
        h_ref[SEG:RL, :] = _cat0([mem1, mem2]).astype(BF16)

    def first_step():
        prep_q, prep_kv, qk, pv = make_single(0)

        def body0(p, carry):
            wait_group(p)

            h = _unpack(hpre_ref[...])
            w = [w_pairs[i][1][rows_of(p), :] for i in range(4)]

            def proj(i):
                r = _dot_nt(h, w[i])
                pre_ref[i, p] = r[RL:]
                return r[0:RL]

            q = prep_q(proj(0))
            k = prep_kv(proj(1))
            pr = qk(q, k)
            acc_ref[...] += _dot(_unpack(o_ref[...]), wo_ref[rows_of(jnp.maximum(p - 1, 0)), :])
            v = prep_kv(proj(2))
            o_ref[...] = _pack(pv(pr, v))
            for i in range(3):
                wqkv_p[i, p] = _pack(w[i].T)
            wo_p[p] = _pack(w[3])

            return carry

        lax.fori_loop(0, NP, body0, 0)
        a = acc_ref[...] + _dot(_unpack(o_ref[...]), wo_ref[rows_of(NP - 1), :])
        xa_ref[0:SEG, :] = x_ref[0:SEG, :].astype(F32) + a[0:SEG]
        h_ref[0:SEG, :] = _ln(x_ref[SEG:2 * SEG, :].astype(F32)).astype(BF16)
        h_ref[SEG:RL, :] = _cat0([a[SEG:RV], mem0]).astype(BF16)

    first_step()
    cp_x1.start()
    for cp in cp_b:
        cp.wait()
    for j in range(3):
        perm_qkv(j)
    perm_wo()
    step(1, (0,), (0,), b_at=9)

    def body_light(t, carry):
        step(t, (0, 1), (0, 1), light=True)
        return carry

    lax.fori_loop(2, 2 + NPRE, body_light, 0)
    cp_x1.wait()

    def body(t, carry):
        step(t, (0, 1), (0, 1))
        return carry

    lax.fori_loop(2 + NPRE, NSEG, body, 0)
    done = (NSEG - 3) * SEG
    cp_o0 = pltpu.make_async_copy(out_ref.at[0:done], out_hbm.at[0:done], sem.at[6])
    cp_o0.start()
    step(NSEG, (1,), (0, 1))
    step(NSEG + 1, (1,), (1,))
    xb, qkv = b_qkv((1,))
    b_out(NSEG + 2, xb, b_attn(NSEG + 2, qkv, (1,)), (1,))
    cp_o1 = pltpu.make_async_copy(out_ref.at[done:S], out_hbm.at[done:S], sem.at[7])
    cp_o1.start()
    cp_o0.wait()
    cp_o1.wait()


@functools.partial(jax.jit, static_argnames=("A_seg_len",))
def pallas_interleave_layers__memory_aug_recurrent_mem_tr__sliding_local_dilated__prompt_kernel(
    A_x: jax.Array,
    A_mem0: jax.Array,
    A_Wq: jax.Array,
    A_Wk: jax.Array,
    A_Wv: jax.Array,
    A_Wo: jax.Array,
    A_seg_len,
    B_x: jax.Array,
    B_wqkv: jax.Array,
    B_wo: jax.Array,
):
    B, S, D = A_x.shape
    H, DH = A_Wq.shape[1], A_Wq.shape[2]
    M = A_mem0.shape[1]
    SEG = int(A_seg_len)
    assert B == 1 and M == 8 and SEG == 32 and DH == 192 and D % 128 == 0 and S % SEG == 0

    x = A_x.reshape(S, D)
    mem0 = A_mem0.reshape(M, D)
    wq = jnp.transpose(A_Wq, (1, 2, 0)).reshape(H * DH, D)
    wk = jnp.transpose(A_Wk, (1, 2, 0)).reshape(H * DH, D)
    wv = jnp.transpose(A_Wv, (1, 2, 0)).reshape(H * DH, D)
    wo = A_Wo.reshape(H * DH, D)

    hbm = pl.BlockSpec(memory_space=pl.ANY)
    out = pl.pallas_call(
        functools.partial(_kernel, S=S, D=D, H=H, DH=DH, M=M, SEG=SEG),
        out_shape=jax.ShapeDtypeStruct((S, D), A_x.dtype),
        in_specs=[hbm] * 8,
        out_specs=hbm,
        scratch_shapes=[
            pltpu.VMEM((M, D), BF16),
            pltpu.VMEM((S, D), BF16),
            pltpu.VMEM((S, D), BF16),
            pltpu.VMEM((H * DH, D), BF16),
            pltpu.VMEM((H * DH, D), BF16),
            pltpu.VMEM((H * DH, D), BF16),
            pltpu.VMEM((H * DH, D), BF16),
            pltpu.VMEM((3, D, D), BF16),
            pltpu.VMEM((D, D), BF16),
            pltpu.VMEM((3, H // 2, D // 2, 2 * DH), U32),
            pltpu.VMEM((H // 2, DH, D), U32),
            pltpu.VMEM((3 * D // 128, D // 2, 128), U32),
            pltpu.VMEM((D // 2, D), U32),
            pltpu.VMEM((2 * SEG + 2 * M, D), BF16),
            pltpu.VMEM((2 * SEG, D), F32),
            pltpu.VMEM((SEG, D), F32),
            pltpu.VMEM((2, 2 * D // 128, HIST + SEG, 128), F32),
            pltpu.VMEM((SEG + 2 * M, D), F32),
            pltpu.VMEM(((SEG + 2 * M + NPRE * SEG) // 2, D), U32),
            pltpu.VMEM((3, H // 2, NPRE * SEG, 2 * DH), F32),
            pltpu.VMEM(((SEG + 2 * M) // 2, 2 * DH), U32),
            pltpu.VMEM((4, D // 128, D, 128), F32),
            pltpu.SemaphoreType.DMA((4 * (H // 2),)),
            pltpu.SemaphoreType.DMA((9,)),
        ],
        compiler_params=pltpu.CompilerParams(vmem_limit_bytes=120 * 1024 * 1024),
    )(mem0, x, wq, wk, wv, wo, B_wqkv, B_wo)
    return out.reshape(B, S, D)
```

```python
import functools

import jax
import jax.numpy as jnp
from jax import lax
import jax.experimental.pallas as pl
import jax.experimental.pallas.tpu as pltpu

F32 = jnp.float32
BF16 = jnp.bfloat16
U32 = jnp.uint32

EPS = 1e-5
NEG = -1000000000.0
PADNEG = -3.0e38
B_HEADS = 32
B_WIN = 8
B_DIL = 2
NPRE = 9
HIST = 16


def _ln(x):
    m = jnp.mean(x, axis=-1, keepdims=True)
    xc = x - m
    v = jnp.mean(xc * xc, axis=-1, keepdims=True)
    return xc * lax.rsqrt(v + EPS)


def _dot_nt(a, b):
    return lax.dot_general(a, b, (((1,), (1,)), ((), ())), preferred_element_type=F32)


def _dot(a, b):
    return jnp.dot(a, b, preferred_element_type=F32)


def _pack(a):
    return pltpu.bitcast(a, U32)


def _unpack(a):
    return pltpu.bitcast(a, BF16)


def _cat0(xs):
    return jnp.concatenate(xs, axis=0)


def _cat1(xs):
    return jnp.concatenate(xs, axis=1)


def _kernel(mem0_hbm, x_hbm, wq_hbm, wk_hbm, wv_hbm, wo_hbm, bqkv_hbm, bwo_hbm,
            out_hbm,
            mem0_ref, x_ref, out_ref, wq_ref, wk_ref, wv_ref, wo_ref, bqkv_ref, bwo_ref,
            wqkv_p, wo_p, bqkv_p, bwo_p, h_ref, xa_ref, x2_ref, kv_ref, hpre_ref, pre_ref, o_ref, tmp_ref, wsem, sem,
            *, S, D, H, DH, M, SEG):
    NSEG = S // SEG
    PW = 2 * DH
    NP = H // 2
    RV = SEG + M
    RL = SEG + 2 * M
    RT = 2 * SEG + 2 * M
    a_scale = DH ** (-0.5)
    b_dh = D // B_HEADS
    b_scale = b_dh ** (-0.5)
    NT = D // 128
    X0 = (NPRE + 3) * SEG

    def sl(p):
        return slice(p * PW, (p + 1) * PW)

    cp_m = pltpu.make_async_copy(mem0_hbm, mem0_ref, sem.at[8])
    cp_x0 = pltpu.make_async_copy(x_hbm.at[0:X0], x_ref.at[0:X0], sem.at[0])
    cp_x1 = pltpu.make_async_copy(x_hbm.at[X0:S], x_ref.at[X0:S], sem.at[1])
    cp_b = [pltpu.make_async_copy(bqkv_hbm.at[:, j * D:(j + 1) * D], bqkv_ref.at[j], sem.at[2 + j])
            for j in range(3)]
    cp_b.append(pltpu.make_async_copy(bwo_hbm, bwo_ref, sem.at[5]))
    cp_wo = pltpu.make_async_copy(wo_hbm, wo_ref, sem.at[9])
    w_pairs = ((wq_hbm, wq_ref), (wk_hbm, wk_ref), (wv_hbm, wv_ref))

    def rows_of(p):
        return pl.ds(pl.multiple_of(p * PW, 128), PW)

    def cp_group(p):
        return [pltpu.make_async_copy(src.at[rows_of(p)], dst.at[rows_of(p)], wsem.at[p])
                for src, dst in w_pairs]

    def start_group(p, carry):
        for cp in cp_group(p):
            cp.start()

        @pl.when(p == NP - 1)
        def _():
            cp_wo.start()

        return carry

    cp_m.start()
    cp_x0.start()
    lax.fori_loop(0, NP, start_group, 0)
    for cp in cp_b:
        cp.start()

    xa_ref[...] = jnp.zeros(xa_ref.shape, F32)
    kv_ref[...] = jnp.zeros(kv_ref.shape, F32)
    cp_m.wait()
    cp_x0.wait()
    mem0 = mem0_ref[...].astype(F32)
    h0 = _ln(x_ref[0:SEG, :].astype(F32))
    hpre_ref[0:RL // 2, :] = _pack(_cat0([h0, mem0, mem0]).astype(BF16))
    for i in range(NPRE):
        hi = _ln(x_ref[(2 + i) * SEG:(3 + i) * SEG, :].astype(F32)).astype(BF16)
        hpre_ref[(RL + i * SEG) // 2:(RL + (i + 1) * SEG) // 2, :] = _pack(hi)

    def perm_rows(a, slot):
        a = a.astype(F32)
        for m in range(NT):
            tmp_ref[slot, m] = a[:, m * 128:(m + 1) * 128]
        return _cat1([_cat0([tmp_ref[slot, m, pl.ds(d, B_HEADS, stride=b_dh), :] for d in range(b_dh)])
                      for m in range(NT)]).astype(BF16)

    def perm_qkv(j):
        wp = perm_rows(bqkv_ref[j].T, j).T
        for c in range(NT):
            bqkv_p[j * NT + c] = _pack(wp[:, c * 128:(c + 1) * 128])

    def perm_wo():
        bwo_p[...] = _pack(perm_rows(bwo_ref[...], 3))

    def b_qkv(layers):
        xb = xa_ref[layers[0] * SEG:(layers[-1] + 1) * SEG, :]
        hb = _ln(xb).astype(BF16)
        return xb, [_dot(hb, _unpack(bqkv_p[n])) for n in range(3 * NT)]

    def b_attn(t, qkv, layers):
        outs = []
        for i, l in enumerate(layers):
            rows = slice(i * SEG, (i + 1) * SEG)
            q = [qkv[j][rows] for j in range(NT)]
            for j in range(2 * NT):
                kv_ref[l, j, HIST:HIST + SEG, :] = qkv[NT + j][rows]
            seg = t - 1 - 2 * l
            pos = seg * SEG + lax.broadcasted_iota(jnp.int32, (SEG, 128), 0)
            logits = []
            for w in range(B_WIN):
                o = HIST - B_DIL * w
                s = q[0] * kv_ref[l, 0, o:o + SEG, :]
                for j in range(1, NT):
                    s = s + q[j] * kv_ref[l, j, o:o + SEG, :]
                s = s + pltpu.roll(s, 64, 1)
                s = s + pltpu.roll(s, 32, 1)
                logits.append(jnp.where(pos >= B_DIL * w, s * b_scale, NEG))
            m = logits[0]
            for w in range(1, B_WIN):
                m = jnp.maximum(m, logits[w])
            es = [jnp.exp(lg - m) for lg in logits]
            den = es[0]
            for w in range(1, B_WIN):
                den = den + es[w]
            inv = 1.0 / den
            tiles = []
            for j in range(NT):
                acc = None
                for w in range(B_WIN):
                    o = HIST - B_DIL * w
                    term = es[w] * kv_ref[l, NT + j, o:o + SEG, :]
                    acc = term if acc is None else acc + term
                tiles.append(acc * inv)
            outs.append(_cat1(tiles))
            for j in range(2 * NT):
                kv_ref[l, j, 0:HIST, :] = qkv[NT + j][(i + 1) * SEG - HIST:(i + 1) * SEG]
        return _cat0(outs).astype(BF16)

    def b_out(t, xb, ob, layers):
        y = xb + _dot(ob, _unpack(bwo_p[...]))
        for i, l in enumerate(layers):
            yl = y[i * SEG:(i + 1) * SEG]
            if l == 0:
                x2_ref[...] = yl
                h_ref[RL:RT, :] = _ln(yl).astype(BF16)
            else:
                if isinstance(t, int):
                    row = (t - 3) * SEG
                else:
                    row = pl.multiple_of(jnp.maximum(t - 3, 0) * SEG, SEG)
                out_ref[pl.ds(row, SEG), :] = yl.astype(out_ref.dtype)

    def softmax2(s, first, valid, fill):
        s = jnp.where(valid, s * a_scale, fill)
        m1 = jnp.max(jnp.where(first, s, PADNEG), axis=-1, keepdims=True)
        m2 = jnp.max(jnp.where(first, PADNEG, s), axis=-1, keepdims=True)
        e = jnp.exp(s - jnp.where(first, m1, m2))
        e1 = jnp.where(first, e, 0.0)
        e2 = jnp.where(first, 0.0, e)
        l1 = jnp.sum(e1, axis=-1, keepdims=True)
        l2 = jnp.sum(e2, axis=-1, keepdims=True)
        inv = 1.0 / jnp.where(first, l1, l2)
        return e, e1, e2, inv

    def make_joint():
        rr = lax.broadcasted_iota(jnp.int32, (RT, 128), 0)
        cc = lax.broadcasted_iota(jnp.int32, (RT, 128), 1)
        lay1 = rr < RV
        first = cc < jnp.where(lay1, RL, RT)
        key = jnp.where(first, cc, cc - RL)
        exists = jnp.where(lay1, RV - 1 - key, key - RV) >= 0
        allowed = (key <= rr) | (lay1 & (key >= SEG)) | ((rr >= RV) & (rr < RL))
        valid = exists & allowed
        fill = jnp.where(exists, NEG, PADNEG)
        lo = cc < (DH - 128)
        z48 = jnp.zeros((128 - RT, 128), F32)
        z32 = jnp.zeros((128 - 2 * RL, 128), F32)

        def prep_q(a):
            return (a[:, 0:128].astype(BF16), a[0:RL, 128:256].astype(BF16),
                    a[SEG:RT, 128:256].astype(BF16), a[:, 256:384].astype(BF16))

        def prep_kv(a):
            mid = a[:, 128:256]
            tlo = jnp.where(lo, mid, 0.0)
            thi = jnp.where(lo, 0.0, mid)
            return (_cat0([a[:, 0:128], z48]).astype(BF16),
                    _cat0([tlo[0:RL], thi[0:RL], z32]).astype(BF16),
                    _cat0([z32, tlo[SEG:RT], thi[SEG:RT]]).astype(BF16),
                    _cat0([z48, a[:, 256:384]]).astype(BF16))

        def qk(q, k):
            t0 = _dot_nt(q[0], k[0])
            t2 = _dot_nt(q[3], k[3])
            t1a = _dot_nt(q[1], k[1])
            t1b = _dot_nt(q[2], k[2])
            s = jnp.where(first, t0, t2) + _cat0([t1a[0:RV], t1b[M:RL]])
            e, e1, e2, inv = softmax2(s, first, valid, fill)
            pa = e * inv
            return ((e1 * inv).astype(BF16), pa[0:RL].astype(BF16),
                    pa[SEG:RT].astype(BF16), (e2 * inv).astype(BF16))

        def pv(pr, v):
            o0 = _dot(pr[0], v[0])
            o2 = _dot(pr[3], v[3])
            o1a = _dot(pr[1], v[1])
            o1b = _dot(pr[2], v[2])
            return _cat1([o0, _cat0([o1a[0:RV], o1b[M:RL]]), o2]).astype(BF16)

        return prep_q, prep_kv, qk, pv

    def make_single(layer):
        rr = lax.broadcasted_iota(jnp.int32, (RV, 2 * RL), 0)
        cc = lax.broadcasted_iota(jnp.int32, (RV, 2 * RL), 1)
        first = cc < RL
        kc = jnp.where(first, cc, cc - RL)
        if layer == 0:
            exists = kc < RV
            valid = exists & ((kc >= SEG) | (kc <= rr))
            r0 = 0
        else:
            exists = kc >= M
            valid = exists & ((rr < M) | (kc - M <= rr))
            r0 = M
        fill = jnp.where(exists, NEG, PADNEG)
        lo = lax.broadcasted_iota(jnp.int32, (RL, PW), 1) < DH
        zrow = jnp.zeros((M, 2 * RL), F32)

        def prep_q(a):
            return a.astype(BF16)

        def prep_kv(a):
            return _cat0([jnp.where(lo, a, 0.0), jnp.where(lo, 0.0, a)]).astype(BF16)

        def qk(q, k):
            s = _dot_nt(q, k)[r0:r0 + RV]
            e, _, _, inv = softmax2(s, first, valid, fill)
            pa = e * inv
            return _cat0([pa, zrow] if layer == 0 else [zrow, pa]).astype(BF16)

        def pv(pr, v):
            return _dot(pr, v).astype(BF16)

        return prep_q, prep_kv, qk, pv

    def step(t, a_layers, b_layers, light=False, b_at=0):
        r0 = 0 if 0 in a_layers else SEG
        r1 = RT if 1 in a_layers else RL
        h = h_ref[SEG if light else r0:r1, :]
        if len(a_layers) == 2:
            prep_q, prep_kv, qk, pv = make_joint()
        else:
            prep_q, prep_kv, qk, pv = make_single(a_layers[0])

        def proj(i, p):
            r = _dot(h, _unpack(wqkv_p[i, p]))
            if light:
                r = _cat0([pre_ref[i, p, pl.ds(pl.multiple_of((t - 2) * SEG, SEG), SEG), :], r])
            return r

        acc = [None]

        def oproj(p, o):
            part = _dot(o, _unpack(wo_p[p]))
            acc[0] = part if acc[0] is None else acc[0] + part

        def xrows(seg):
            if isinstance(seg, int):
                return x_ref[seg * SEG:(seg + 1) * SEG, :].astype(F32)
            return x_ref[pl.ds(pl.multiple_of(seg * SEG, SEG), SEG), :].astype(F32)

        q = prep_q(proj(0, 0))
        k = prep_kv(proj(1, 0))
        v = prep_kv(proj(2, 0))
        early_v = light or len(a_layers) == 1
        os_ = {}
        x2 = None
        for p in range(NP):
            pr = qk(q, k)
            if p + 1 < NP:
                q = prep_q(proj(0, p + 1))
                k = prep_kv(proj(1, p + 1))
                if early_v:
                    vn = prep_kv(proj(2, p + 1))
            else:
                if 1 in a_layers:
                    x2 = x2_ref[...]
                if b_layers:
                    b_out(t, xb, ob, b_layers)
                if 0 in a_layers:
                    nxt = t + 1 if isinstance(t, int) else jnp.minimum(t + 1, NSEG - 1)
                    h_ref[0:SEG, :] = _ln(xrows(nxt)).astype(BF16)
                oproj(p - 2, os_.pop(p - 2))
            os_[p] = pv(pr, v)
            if p + 1 < NP:
                v = vn if early_v else prep_kv(proj(2, p + 1))
            if p == b_at and b_layers:
                xb, qkv = b_qkv(b_layers)
                ob = b_attn(t, qkv, b_layers)
            if p >= 2 and p + 1 < NP:
                oproj(p - 2, os_.pop(p - 2))
        oproj(NP - 2, os_.pop(NP - 2))
        oproj(NP - 1, os_.pop(NP - 1))
        a = acc[0]
        if 0 in a_layers:
            xa_ref[0:SEG, :] = xrows(t) + a[0:SEG]
        if 1 in a_layers:
            xa_ref[SEG:2 * SEG, :] = x2 + a[RL - r0:RT - r0]
        mem1 = a[SEG - r0:RV - r0]
        mem2 = a[RV - r0:RL - r0] if 1 in a_layers else mem0
        h_ref[SEG:RL, :] = _cat0([mem1, mem2]).astype(BF16)

    def first_step():
        prep_q, prep_kv, qk, pv = make_single(0)

        RA = (RL + NPRE * SEG) // 32 * 16 + 16

        def wait_group(p):
            for cp in cp_group(p):
                cp.wait()

        def body0(p, carry):
            wait_group(p)
            ha = _unpack(hpre_ref[0:RA // 2, :])
            hb = _unpack(hpre_ref[RA // 2:, :])
            w = [dst[rows_of(p), :] for _, dst in w_pairs]

            def proj_a(i):
                r = _dot_nt(ha, w[i])
                pre_ref[i, p, 0:RA - RL, :] = r[RL:]
                return r[0:RL]

            def proj_b(i):
                pre_ref[i, p, RA - RL:, :] = _dot_nt(hb, w[i])

            q = prep_q(proj_a(0))
            k = prep_kv(proj_a(1))
            v = prep_kv(proj_a(2))
            pr = qk(q, k)
            proj_b(0)
            proj_b(1)
            o_ref[p] = _pack(pv(pr, v))
            proj_b(2)
            for i in range(3):
                wqkv_p[i, p] = _pack(w[i].T)
            return carry

        lax.fori_loop(0, NP, body0, 0)
        cp_wo.wait()
        a = None
        for p in range(NP):
            w = wo_ref[sl(p), :]
            wo_p[p] = _pack(w)
            part = _dot(_unpack(o_ref[p]), w)
            a = part if a is None else a + part
        xa_ref[0:SEG, :] = x_ref[0:SEG, :].astype(F32) + a[0:SEG]
        h_ref[0:SEG, :] = _ln(x_ref[SEG:2 * SEG, :].astype(F32)).astype(BF16)
        h_ref[SEG:RL, :] = _cat0([a[SEG:RV], mem0]).astype(BF16)

    first_step()
    cp_x1.start()
    for cp in cp_b:
        cp.wait()
    for j in range(3):
        perm_qkv(j)
    perm_wo()
    step(1, (0,), (0,), b_at=9)

    def body_light(t, carry):
        step(t, (0, 1), (0, 1), light=True)
        return carry

    lax.fori_loop(2, 2 + NPRE, body_light, 0)
    cp_x1.wait()

    def body(t, carry):
        step(t, (0, 1), (0, 1))
        return carry

    lax.fori_loop(2 + NPRE, NSEG, body, 0)
    done = (NSEG - 3) * SEG
    cp_o0 = pltpu.make_async_copy(out_ref.at[0:done], out_hbm.at[0:done], sem.at[6])
    cp_o0.start()
    step(NSEG, (1,), (0, 1))
    step(NSEG + 1, (1,), (1,))
    xb, qkv = b_qkv((1,))
    b_out(NSEG + 2, xb, b_attn(NSEG + 2, qkv, (1,)), (1,))
    cp_o1 = pltpu.make_async_copy(out_ref.at[done:S], out_hbm.at[done:S], sem.at[7])
    cp_o1.start()
    cp_o0.wait()
    cp_o1.wait()


@functools.partial(jax.jit, static_argnames=("A_seg_len",))
def pallas_interleave_layers__memory_aug_recurrent_mem_tr__sliding_local_dilated__prompt_kernel(
    A_x: jax.Array,
    A_mem0: jax.Array,
    A_Wq: jax.Array,
    A_Wk: jax.Array,
    A_Wv: jax.Array,
    A_Wo: jax.Array,
    A_seg_len,
    B_x: jax.Array,
    B_wqkv: jax.Array,
    B_wo: jax.Array,
):
    B, S, D = A_x.shape
    H, DH = A_Wq.shape[1], A_Wq.shape[2]
    M = A_mem0.shape[1]
    SEG = int(A_seg_len)
    assert B == 1 and M == 8 and SEG == 32 and DH == 192 and D % 128 == 0 and S % SEG == 0

    x = A_x.reshape(S, D)
    mem0 = A_mem0.reshape(M, D)
    wq = jnp.transpose(A_Wq, (1, 2, 0)).reshape(H * DH, D)
    wk = jnp.transpose(A_Wk, (1, 2, 0)).reshape(H * DH, D)
    wv = jnp.transpose(A_Wv, (1, 2, 0)).reshape(H * DH, D)
    wo = A_Wo.reshape(H * DH, D)

    hbm = pl.BlockSpec(memory_space=pl.ANY)
    out = pl.pallas_call(
        functools.partial(_kernel, S=S, D=D, H=H, DH=DH, M=M, SEG=SEG),
        out_shape=jax.ShapeDtypeStruct((S, D), A_x.dtype),
        in_specs=[hbm] * 8,
        out_specs=hbm,
        scratch_shapes=[
            pltpu.VMEM((M, D), BF16),
            pltpu.VMEM((S, D), BF16),
            pltpu.VMEM((S, D), BF16),
            pltpu.VMEM((H * DH, D), BF16),
            pltpu.VMEM((H * DH, D), BF16),
            pltpu.VMEM((H * DH, D), BF16),
            pltpu.VMEM((H * DH, D), BF16),
            pltpu.VMEM((3, D, D), BF16),
            pltpu.VMEM((D, D), BF16),
            pltpu.VMEM((3, H // 2, D // 2, 2 * DH), U32),
            pltpu.VMEM((H // 2, DH, D), U32),
            pltpu.VMEM((3 * D // 128, D // 2, 128), U32),
            pltpu.VMEM((D // 2, D), U32),
            pltpu.VMEM((2 * SEG + 2 * M, D), BF16),
            pltpu.VMEM((2 * SEG, D), F32),
            pltpu.VMEM((SEG, D), F32),
            pltpu.VMEM((2, 2 * D // 128, HIST + SEG, 128), F32),
            pltpu.VMEM(((SEG + 2 * M + NPRE * SEG) // 2, D), U32),
            pltpu.VMEM((3, H // 2, NPRE * SEG, 2 * DH), F32),
            pltpu.VMEM((H // 2, (SEG + 2 * M) // 2, 2 * DH), U32),
            pltpu.VMEM((4, D // 128, D, 128), F32),
            pltpu.SemaphoreType.DMA((H // 2,)),
            pltpu.SemaphoreType.DMA((10,)),
        ],
        compiler_params=pltpu.CompilerParams(vmem_limit_bytes=120 * 1024 * 1024),
    )(mem0, x, wq, wk, wv, wo, B_wqkv, B_wo)
    return out.reshape(B, S, D)
```

```python
import functools

import jax
import jax.numpy as jnp
from jax import lax
import jax.experimental.pallas as pl
import jax.experimental.pallas.tpu as pltpu

F32 = jnp.float32
BF16 = jnp.bfloat16
U32 = jnp.uint32

EPS = 1e-5
NEG = -1000000000.0
PADNEG = -3.0e38
B_HEADS = 32
B_WIN = 8
B_DIL = 2
NPRE = 9
HIST = 16


def _ln(x):
    m = jnp.mean(x, axis=-1, keepdims=True)
    xc = x - m
    v = jnp.mean(xc * xc, axis=-1, keepdims=True)
    return xc * lax.rsqrt(v + EPS)


def _dot_nt(a, b):
    return lax.dot_general(a, b, (((1,), (1,)), ((), ())), preferred_element_type=F32)


def _dot(a, b):
    return jnp.dot(a, b, preferred_element_type=F32)


def _pack(a):
    return pltpu.bitcast(a, U32)


def _unpack(a):
    return pltpu.bitcast(a, BF16)


def _cat0(xs):
    return jnp.concatenate(xs, axis=0)


def _cat1(xs):
    return jnp.concatenate(xs, axis=1)


def _kernel(mem0_hbm, x_hbm, wq_hbm, wk_hbm, wv_hbm, wo_hbm, bqkv_hbm, bwo_hbm,
            out_hbm,
            mem0_ref, x_ref, out_ref, wq_ref, wk_ref, wv_ref, wo_ref, bqkv_ref, bwo_ref,
            wqkv_p, wo_p, bqkv_p, bwo_p, h_ref, xa_ref, x2_ref, kv_ref, hpre_ref, pre_ref, o_ref, tmp_ref, wsem, sem,
            *, S, D, H, DH, M, SEG):
    NSEG = S // SEG
    PW = 2 * DH
    NP = H // 2
    RV = SEG + M
    RL = SEG + 2 * M
    RT = 2 * SEG + 2 * M
    a_scale = DH ** (-0.5)
    b_dh = D // B_HEADS
    b_scale = b_dh ** (-0.5)
    NT = D // 128
    X0 = (NPRE + 3) * SEG

    def sl(p):
        return slice(p * PW, (p + 1) * PW)

    cp_m = pltpu.make_async_copy(mem0_hbm, mem0_ref, sem.at[8])
    cp_x0 = pltpu.make_async_copy(x_hbm.at[0:X0], x_ref.at[0:X0], sem.at[0])
    cp_x1 = pltpu.make_async_copy(x_hbm.at[X0:S], x_ref.at[X0:S], sem.at[1])
    cp_b = [pltpu.make_async_copy(bqkv_hbm.at[:, j * D:(j + 1) * D], bqkv_ref.at[j], sem.at[2 + j])
            for j in range(3)]
    cp_b.append(pltpu.make_async_copy(bwo_hbm, bwo_ref, sem.at[5]))
    cp_wo = pltpu.make_async_copy(wo_hbm, wo_ref, sem.at[9])
    w_pairs = ((wq_hbm, wq_ref), (wk_hbm, wk_ref), (wv_hbm, wv_ref))

    def rows_of(p):
        return pl.ds(pl.multiple_of(p * PW, 128), PW)

    def cp_group(p):
        return [pltpu.make_async_copy(src.at[rows_of(p)], dst.at[rows_of(p)], wsem.at[p])
                for src, dst in w_pairs]

    def start_group(p, carry):
        for cp in cp_group(p):
            cp.start()

        @pl.when(p == NP - 1)
        def _():
            cp_wo.start()

        return carry

    cp_m.start()
    cp_x0.start()
    lax.fori_loop(0, NP, start_group, 0)
    for cp in cp_b:
        cp.start()

    xa_ref[...] = jnp.zeros(xa_ref.shape, F32)
    kv_ref[...] = jnp.zeros(kv_ref.shape, F32)
    cp_m.wait()
    cp_x0.wait()
    mem0 = mem0_ref[...].astype(F32)
    h0 = _ln(x_ref[0:SEG, :].astype(F32))
    hpre_ref[0:RL // 2, :] = _pack(_cat0([h0, mem0, mem0]).astype(BF16))
    for i in range(NPRE):
        hi = _ln(x_ref[(2 + i) * SEG:(3 + i) * SEG, :].astype(F32)).astype(BF16)
        hpre_ref[(RL + i * SEG) // 2:(RL + (i + 1) * SEG) // 2, :] = _pack(hi)

    def perm_rows(a, slot):
        a = a.astype(F32)
        for m in range(NT):
            tmp_ref[slot, m] = a[:, m * 128:(m + 1) * 128]
        return _cat1([_cat0([tmp_ref[slot, m, pl.ds(d, B_HEADS, stride=b_dh), :] for d in range(b_dh)])
                      for m in range(NT)]).astype(BF16)

    def perm_qkv(j):
        wp = perm_rows(bqkv_ref[j].T, j).T
        for c in range(NT):
            bqkv_p[j * NT + c] = _pack(wp[:, c * 128:(c + 1) * 128])

    def perm_wo():
        bwo_p[...] = _pack(perm_rows(bwo_ref[...], 3))

    def make_b(t, layers, masked):
        st = {}

        def keep(l, i, j, a):
            kv_ref[l, j, HIST:HIST + SEG, :] = a[i * SEG:(i + 1) * SEG]

        def keep_tail(l, i, j, a):
            kv_ref[l, j, 0:HIST, :] = a[(i + 1) * SEG - HIST:(i + 1) * SEG]

        def win(l, j, w):
            o = HIST - B_DIL * w
            return kv_ref[l, j, o:o + SEG, :]

        def qk():
            xb = xa_ref[layers[0] * SEG:(layers[-1] + 1) * SEG, :]
            hb = _ln(xb).astype(BF16)
            st['y'], st['hb'], st['p'] = xb, hb, []
            qs = [_dot(hb, _unpack(bqkv_p[j])) for j in range(NT)]
            ks = [_dot(hb, _unpack(bqkv_p[NT + j])) for j in range(NT)]
            for i, l in enumerate(layers):
                q = [qs[j][i * SEG:(i + 1) * SEG] * b_scale for j in range(NT)]
                for j in range(NT):
                    keep(l, i, j, ks[j])
                pos = (t - 1 - 2 * l) * SEG + lax.broadcasted_iota(jnp.int32, (SEG, 128), 0)
                logits = []
                for w in range(B_WIN):
                    s = q[0] * win(l, 0, w)
                    for j in range(1, NT):
                        s = s + q[j] * win(l, j, w)
                    s = s + pltpu.roll(s, 64, 1)
                    s = s + pltpu.roll(s, 32, 1)
                    logits.append(jnp.where(pos >= B_DIL * w, s, NEG) if masked else s)
                for j in range(NT):
                    keep_tail(l, i, j, ks[j])
                m = logits[0]
                for w in range(1, B_WIN):
                    m = jnp.maximum(m, logits[w])
                es = [jnp.exp(lg - m) for lg in logits]
                den = es[0]
                for w in range(1, B_WIN):
                    den = den + es[w]
                st['p'].append((es, 1.0 / den))

        def v_stage(j):
            vj = _dot(st['hb'], _unpack(bqkv_p[2 * NT + j]))
            outs = []
            for i, l in enumerate(layers):
                es, inv = st['p'][i]
                keep(l, i, NT + j, vj)
                acc = es[0] * win(l, NT + j, 0)
                for w in range(1, B_WIN):
                    acc = acc + es[w] * win(l, NT + j, w)
                keep_tail(l, i, NT + j, vj)
                outs.append(acc * inv)
            st['o', j] = _cat0(outs).astype(BF16)

        def o_stage(j):
            st['y'] = st['y'] + _dot(st.pop(('o', j)), _unpack(bwo_p[j * 64:(j + 1) * 64, :]))

        def fin():
            for i, l in enumerate(layers):
                yl = st['y'][i * SEG:(i + 1) * SEG]
                if l == 0:
                    x2_ref[...] = yl
                    h_ref[RL:RT, :] = _ln(yl).astype(BF16)
                else:
                    if isinstance(t, int):
                        row = (t - 3) * SEG
                    else:
                        row = pl.multiple_of(jnp.maximum(t - 3, 0) * SEG, SEG)
                    out_ref[pl.ds(row, SEG), :] = yl.astype(out_ref.dtype)

        return qk, v_stage, o_stage, fin

    def softmax2(s, first, valid, fill):
        s = jnp.where(valid, s * a_scale, fill)
        m1 = jnp.max(jnp.where(first, s, PADNEG), axis=-1, keepdims=True)
        m2 = jnp.max(jnp.where(first, PADNEG, s), axis=-1, keepdims=True)
        e = jnp.exp(s - jnp.where(first, m1, m2))
        e1 = jnp.where(first, e, 0.0)
        e2 = jnp.where(first, 0.0, e)
        l1 = jnp.sum(e1, axis=-1, keepdims=True)
        l2 = jnp.sum(e2, axis=-1, keepdims=True)
        inv = 1.0 / jnp.where(first, l1, l2)
        return e, e1, e2, inv

    def make_joint():
        rr = lax.broadcasted_iota(jnp.int32, (RT, 128), 0)
        cc = lax.broadcasted_iota(jnp.int32, (RT, 128), 1)
        lay1 = rr < RV
        first = cc < jnp.where(lay1, RL, RT)
        key = jnp.where(first, cc, cc - RL)
        exists = jnp.where(lay1, RV - 1 - key, key - RV) >= 0
        allowed = (key <= rr) | (lay1 & (key >= SEG)) | ((rr >= RV) & (rr < RL))
        valid = exists & allowed
        fill = jnp.where(exists, NEG, PADNEG)
        lo = cc < (DH - 128)
        z48 = jnp.zeros((128 - RT, 128), F32)
        z32 = jnp.zeros((128 - 2 * RL, 128), F32)

        def prep_q(a):
            return (a[:, 0:128].astype(BF16), a[0:RL, 128:256].astype(BF16),
                    a[SEG:RT, 128:256].astype(BF16), a[:, 256:384].astype(BF16))

        def prep_kv(a):
            mid = a[:, 128:256]
            tlo = jnp.where(lo, mid, 0.0)
            thi = jnp.where(lo, 0.0, mid)
            return (_cat0([a[:, 0:128], z48]).astype(BF16),
                    _cat0([tlo[0:RL], thi[0:RL], z32]).astype(BF16),
                    _cat0([z32, tlo[SEG:RT], thi[SEG:RT]]).astype(BF16),
                    _cat0([z48, a[:, 256:384]]).astype(BF16))

        def qk(q, k):
            t0 = _dot_nt(q[0], k[0])
            t2 = _dot_nt(q[3], k[3])
            t1a = _dot_nt(q[1], k[1])
            t1b = _dot_nt(q[2], k[2])
            s = jnp.where(first, t0, t2) + _cat0([t1a[0:RV], t1b[M:RL]])
            e, e1, e2, inv = softmax2(s, first, valid, fill)
            pa = e * inv
            return ((e1 * inv).astype(BF16), pa[0:RL].astype(BF16),
                    pa[SEG:RT].astype(BF16), (e2 * inv).astype(BF16))

        def pv(pr, v):
            o0 = _dot(pr[0], v[0])
            o2 = _dot(pr[3], v[3])
            o1a = _dot(pr[1], v[1])
            o1b = _dot(pr[2], v[2])
            return _cat1([o0, _cat0([o1a[0:RV], o1b[M:RL]]), o2]).astype(BF16)

        return prep_q, prep_kv, qk, pv

    def make_single(layer):
        rr = lax.broadcasted_iota(jnp.int32, (RV, 2 * RL), 0)
        cc = lax.broadcasted_iota(jnp.int32, (RV, 2 * RL), 1)
        first = cc < RL
        kc = jnp.where(first, cc, cc - RL)
        if layer == 0:
            exists = kc < RV
            valid = exists & ((kc >= SEG) | (kc <= rr))
            r0 = 0
        else:
            exists = kc >= M
            valid = exists & ((rr < M) | (kc - M <= rr))
            r0 = M
        fill = jnp.where(exists, NEG, PADNEG)
        lo = lax.broadcasted_iota(jnp.int32, (RL, PW), 1) < DH
        zrow = jnp.zeros((M, 2 * RL), F32)

        def prep_q(a):
            return a.astype(BF16)

        def prep_kv(a):
            return _cat0([jnp.where(lo, a, 0.0), jnp.where(lo, 0.0, a)]).astype(BF16)

        def qk(q, k):
            s = _dot_nt(q, k)[r0:r0 + RV]
            e, _, _, inv = softmax2(s, first, valid, fill)
            pa = e * inv
            return _cat0([pa, zrow] if layer == 0 else [zrow, pa]).astype(BF16)

        def pv(pr, v):
            return _dot(pr, v).astype(BF16)

        return prep_q, prep_kv, qk, pv

    def step(t, a_layers, b_layers, light=False, masked=True, b_sched=(0, 2, 2, 2)):
        r0 = 0 if 0 in a_layers else SEG
        r1 = RT if 1 in a_layers else RL
        h = h_ref[SEG if light else r0:r1, :]
        if len(a_layers) == 2:
            prep_q, prep_kv, qk, pv = make_joint()
        else:
            prep_q, prep_kv, qk, pv = make_single(a_layers[0])

        def proj(i, p):
            r = _dot(h, _unpack(wqkv_p[i, p]))
            if light:
                r = _cat0([pre_ref[i, p, pl.ds(pl.multiple_of((t - 2) * SEG, SEG), SEG), :], r])
            return r

        acc = [None]
        OLAG = 3 if len(a_layers) == 2 else 4

        def oproj(p, o):
            part = _dot(o, _unpack(wo_p[p]))
            acc[0] = part if acc[0] is None else acc[0] + part

        def xrows(seg):
            if isinstance(seg, int):
                return x_ref[seg * SEG:(seg + 1) * SEG, :].astype(F32)
            return x_ref[pl.ds(pl.multiple_of(seg * SEG, SEG), SEG), :].astype(F32)

        b_qk, b_v, b_o, b_fin = make_b(t, b_layers, masked)
        hooks = {p: [] for p in range(NP)}
        at, v0, dv, lag = b_sched
        hooks[at].append(b_qk)
        for j in range(NT):
            hooks[at + v0 + j * dv].insert(0, functools.partial(b_v, j)) if v0 else hooks[at].append(
                functools.partial(b_v, j))
        for j in range(NT):
            hooks[at + v0 + j * dv + lag].insert(0, functools.partial(b_o, j))
        x2 = x2_ref[...] if 1 in a_layers else None
        hooks[at + v0 + (NT - 1) * dv + lag].append(b_fin)

        q = prep_q(proj(0, 0))
        k = prep_kv(proj(1, 0))
        v = prep_kv(proj(2, 0))
        early_v = light or len(a_layers) == 1
        os_ = {}
        for p in range(NP):
            pr = qk(q, k)
            if p + 1 < NP:
                q = prep_q(proj(0, p + 1))
                k = prep_kv(proj(1, p + 1))
                if early_v:
                    vn = prep_kv(proj(2, p + 1))
            else:
                if 0 in a_layers:
                    nxt = t + 1 if isinstance(t, int) else jnp.minimum(t + 1, NSEG - 1)
                    h_ref[0:SEG, :] = _ln(xrows(nxt)).astype(BF16)
                for pp in range(p - OLAG, p - 1):
                    oproj(pp, os_.pop(pp))
            os_[p] = pv(pr, v)
            if p + 1 < NP:
                v = vn if early_v else prep_kv(proj(2, p + 1))
            for f in hooks[p]:
                f()
            if p >= OLAG and p + 1 < NP:
                oproj(p - OLAG, os_.pop(p - OLAG))
        oproj(NP - 2, os_.pop(NP - 2))
        oproj(NP - 1, os_.pop(NP - 1))
        a = acc[0]
        if 0 in a_layers:
            xa_ref[0:SEG, :] = xrows(t) + a[0:SEG]
        if 1 in a_layers:
            xa_ref[SEG:2 * SEG, :] = x2 + a[RL - r0:RT - r0]
        mem1 = a[SEG - r0:RV - r0]
        mem2 = a[RV - r0:RL - r0] if 1 in a_layers else mem0
        h_ref[SEG:RL, :] = _cat0([mem1, mem2]).astype(BF16)

    def first_step():
        prep_q, prep_kv, qk, pv = make_single(0)

        RA = (RL + NPRE * SEG) // 32 * 16 + 16

        def wait_group(p):
            for cp in cp_group(p):
                cp.wait()

        def body0(p, carry):
            wait_group(p)
            ha = _unpack(hpre_ref[0:RA // 2, :])
            hb = _unpack(hpre_ref[RA // 2:, :])
            w = [dst[rows_of(p), :] for _, dst in w_pairs]

            def proj_a(i):
                r = _dot_nt(ha, w[i])
                pre_ref[i, p, 0:RA - RL, :] = r[RL:]
                return r[0:RL]

            def proj_b(i):
                pre_ref[i, p, RA - RL:, :] = _dot_nt(hb, w[i])

            q = prep_q(proj_a(0))
            k = prep_kv(proj_a(1))
            v = prep_kv(proj_a(2))
            pr = qk(q, k)
            proj_b(0)
            proj_b(1)
            o_ref[p] = _pack(pv(pr, v))
            proj_b(2)
            for i in range(3):
                wqkv_p[i, p] = _pack(w[i].T)
            return carry

        lax.fori_loop(0, NP, body0, 0)
        cp_wo.wait()
        a = None
        for p in range(NP):
            w = wo_ref[sl(p), :]
            wo_p[p] = _pack(w)
            part = _dot(_unpack(o_ref[p]), w)
            a = part if a is None else a + part
        xa_ref[0:SEG, :] = x_ref[0:SEG, :].astype(F32) + a[0:SEG]
        h_ref[0:SEG, :] = _ln(x_ref[SEG:2 * SEG, :].astype(F32)).astype(BF16)
        h_ref[SEG:RL, :] = _cat0([a[SEG:RV], mem0]).astype(BF16)

    first_step()
    cp_x1.start()
    for cp in cp_b:
        cp.wait()
    for j in range(3):
        perm_qkv(j)
    perm_wo()
    step(1, (0,), (0,), b_sched=(7, 2, 1, 1))

    def body_light(t, carry):
        step(t, (0, 1), (0, 1), light=True)
        return carry

    lax.fori_loop(2, 2 + NPRE, body_light, 0)
    cp_x1.wait()

    def body(t, carry):
        step(t, (0, 1), (0, 1), masked=False)
        return carry

    lax.fori_loop(2 + NPRE, NSEG, body, 0)
    done = (NSEG - 3) * SEG
    cp_o0 = pltpu.make_async_copy(out_ref.at[0:done], out_hbm.at[0:done], sem.at[6])
    cp_o0.start()
    step(NSEG, (1,), (0, 1), masked=False)
    step(NSEG + 1, (1,), (1,), masked=False)
    b_qk, b_v, b_o, b_fin = make_b(NSEG + 2, (1,), False)
    b_qk()
    for j in range(NT):
        b_v(j)
    for j in range(NT):
        b_o(j)
    b_fin()
    cp_o1 = pltpu.make_async_copy(out_ref.at[done:S], out_hbm.at[done:S], sem.at[7])
    cp_o1.start()
    cp_o0.wait()
    cp_o1.wait()


@functools.partial(jax.jit, static_argnames=("A_seg_len",))
def pallas_interleave_layers__memory_aug_recurrent_mem_tr__sliding_local_dilated__prompt_kernel(
    A_x: jax.Array,
    A_mem0: jax.Array,
    A_Wq: jax.Array,
    A_Wk: jax.Array,
    A_Wv: jax.Array,
    A_Wo: jax.Array,
    A_seg_len,
    B_x: jax.Array,
    B_wqkv: jax.Array,
    B_wo: jax.Array,
):
    B, S, D = A_x.shape
    H, DH = A_Wq.shape[1], A_Wq.shape[2]
    M = A_mem0.shape[1]
    SEG = int(A_seg_len)
    assert B == 1 and M == 8 and SEG == 32 and DH == 192 and D % 128 == 0 and S % SEG == 0

    x = A_x.reshape(S, D)
    mem0 = A_mem0.reshape(M, D)
    wq = jnp.transpose(A_Wq, (1, 2, 0)).reshape(H * DH, D)
    wk = jnp.transpose(A_Wk, (1, 2, 0)).reshape(H * DH, D)
    wv = jnp.transpose(A_Wv, (1, 2, 0)).reshape(H * DH, D)
    wo = A_Wo.reshape(H * DH, D)

    hbm = pl.BlockSpec(memory_space=pl.ANY)
    out = pl.pallas_call(
        functools.partial(_kernel, S=S, D=D, H=H, DH=DH, M=M, SEG=SEG),
        out_shape=jax.ShapeDtypeStruct((S, D), A_x.dtype),
        in_specs=[hbm] * 8,
        out_specs=hbm,
        scratch_shapes=[
            pltpu.VMEM((M, D), BF16),
            pltpu.VMEM((S, D), BF16),
            pltpu.VMEM((S, D), BF16),
            pltpu.VMEM((H * DH, D), BF16),
            pltpu.VMEM((H * DH, D), BF16),
            pltpu.VMEM((H * DH, D), BF16),
            pltpu.VMEM((H * DH, D), BF16),
            pltpu.VMEM((3, D, D), BF16),
            pltpu.VMEM((D, D), BF16),
            pltpu.VMEM((3, H // 2, D // 2, 2 * DH), U32),
            pltpu.VMEM((H // 2, DH, D), U32),
            pltpu.VMEM((3 * D // 128, D // 2, 128), U32),
            pltpu.VMEM((D // 2, D), U32),
            pltpu.VMEM((2 * SEG + 2 * M, D), BF16),
            pltpu.VMEM((2 * SEG, D), F32),
            pltpu.VMEM((SEG, D), F32),
            pltpu.VMEM((2, 2 * D // 128, HIST + SEG, 128), F32),
            pltpu.VMEM(((SEG + 2 * M + NPRE * SEG) // 2, D), U32),
            pltpu.VMEM((3, H // 2, NPRE * SEG, 2 * DH), F32),
            pltpu.VMEM((H // 2, (SEG + 2 * M) // 2, 2 * DH), U32),
            pltpu.VMEM((4, D // 128, D, 128), F32),
            pltpu.SemaphoreType.DMA((H // 2,)),
            pltpu.SemaphoreType.DMA((10,)),
        ],
        compiler_params=pltpu.CompilerParams(vmem_limit_bytes=120 * 1024 * 1024),
    )(mem0, x, wq, wk, wv, wo, B_wqkv, B_wo)
    return out.reshape(B, S, D)
```

```python
import functools

import jax
import jax.numpy as jnp
from jax import lax
import jax.experimental.pallas as pl
import jax.experimental.pallas.tpu as pltpu

F32 = jnp.float32
BF16 = jnp.bfloat16
U32 = jnp.uint32

EPS = 1e-5
NEG = -1000000000.0
PADNEG = -3.0e38
B_HEADS = 32
B_WIN = 8
B_DIL = 2
NPRE = 9
HIST = 16


def _ln(x):
    m = jnp.mean(x, axis=-1, keepdims=True)
    xc = x - m
    v = jnp.mean(xc * xc, axis=-1, keepdims=True)
    return xc * lax.rsqrt(v + EPS)


def _dot_nt(a, b):
    return lax.dot_general(a, b, (((1,), (1,)), ((), ())), preferred_element_type=F32)


def _dot(a, b):
    return jnp.dot(a, b, preferred_element_type=F32)


def _pack(a):
    return pltpu.bitcast(a, U32)


def _unpack(a):
    return pltpu.bitcast(a, BF16)


def _cat0(xs):
    return jnp.concatenate(xs, axis=0)


def _cat1(xs):
    return jnp.concatenate(xs, axis=1)


def _kernel(mem0_hbm, x_hbm, wq_hbm, wk_hbm, wv_hbm, wo_hbm, bqkv_hbm, bwo_hbm,
            out_hbm,
            mem0_ref, x_ref, out_ref, wq_ref, wk_ref, wv_ref, wo_ref, bqkv_ref, bwo_ref,
            wqkv_p, wo_p, bqkv_p, bwo_p, h_ref, xa_ref, x2_ref, kv_ref, hpre_ref, pre_ref, o_ref, tmp_ref, wsem, sem,
            *, S, D, H, DH, M, SEG):
    NSEG = S // SEG
    PW = 2 * DH
    NP = H // 2
    RV = SEG + M
    RL = SEG + 2 * M
    RT = 2 * SEG + 2 * M
    a_scale = DH ** (-0.5)
    b_dh = D // B_HEADS
    b_scale = b_dh ** (-0.5)
    NT = D // 128
    X0 = (NPRE + 3) * SEG

    def sl(p):
        return slice(p * PW, (p + 1) * PW)

    cp_m = pltpu.make_async_copy(mem0_hbm, mem0_ref, sem.at[8])
    cp_x0 = pltpu.make_async_copy(x_hbm.at[0:X0], x_ref.at[0:X0], sem.at[0])
    cp_x1 = pltpu.make_async_copy(x_hbm.at[X0:S], x_ref.at[X0:S], sem.at[1])
    cp_b = [pltpu.make_async_copy(bqkv_hbm.at[:, j * D:(j + 1) * D], bqkv_ref.at[j], sem.at[2 + j])
            for j in range(3)]
    cp_b.append(pltpu.make_async_copy(bwo_hbm, bwo_ref, sem.at[5]))
    cp_wo = pltpu.make_async_copy(wo_hbm, wo_ref, sem.at[9])
    w_pairs = ((wq_hbm, wq_ref), (wk_hbm, wk_ref), (wv_hbm, wv_ref))

    def rows_of(p):
        return pl.ds(pl.multiple_of(p * PW, 128), PW)

    def cp_group(p):
        return [pltpu.make_async_copy(src.at[rows_of(p)], dst.at[rows_of(p)], wsem.at[p])
                for src, dst in w_pairs]

    def start_group(p, carry):
        for cp in cp_group(p):
            cp.start()

        @pl.when(p == NP - 1)
        def _():
            cp_wo.start()

        return carry

    cp_m.start()
    cp_x0.start()
    lax.fori_loop(0, NP, start_group, 0)
    for cp in cp_b:
        cp.start()

    xa_ref[...] = jnp.zeros(xa_ref.shape, F32)
    kv_ref[...] = jnp.zeros(kv_ref.shape, F32)
    cp_m.wait()
    cp_x0.wait()
    mem0 = mem0_ref[...].astype(F32)
    h0 = _ln(x_ref[0:SEG, :].astype(F32))
    hpre_ref[0:RL // 2, :] = _pack(_cat0([h0, mem0, mem0]).astype(BF16))
    for i in range(NPRE):
        hi = _ln(x_ref[(2 + i) * SEG:(3 + i) * SEG, :].astype(F32)).astype(BF16)
        hpre_ref[(RL + i * SEG) // 2:(RL + (i + 1) * SEG) // 2, :] = _pack(hi)

    def perm_rows(a, slot):
        a = a.astype(F32)
        for m in range(NT):
            tmp_ref[slot, m] = a[:, m * 128:(m + 1) * 128]
        return _cat1([_cat0([tmp_ref[slot, m, pl.ds(d, B_HEADS, stride=b_dh), :] for d in range(b_dh)])
                      for m in range(NT)]).astype(BF16)

    def perm_qkv(j):
        wp = perm_rows(bqkv_ref[j].T, j).T
        for c in range(NT):
            bqkv_p[j * NT + c] = _pack(wp[:, c * 128:(c + 1) * 128])

    def perm_wo():
        bwo_p[...] = _pack(perm_rows(bwo_ref[...], 3))

    def make_b(t, layers, masked):
        st = {}

        def keep(l, i, j, a):
            kv_ref[l, j, HIST:HIST + SEG, :] = a[i * SEG:(i + 1) * SEG]

        def keep_tail(l, i, j, a):
            kv_ref[l, j, 0:HIST, :] = a[(i + 1) * SEG - HIST:(i + 1) * SEG]

        def win(l, j, w):
            o = HIST - B_DIL * w
            return kv_ref[l, j, o:o + SEG, :]

        def qk():
            xb = xa_ref[layers[0] * SEG:(layers[-1] + 1) * SEG, :]
            hb = _ln(xb).astype(BF16)
            st['y'], st['hb'], st['p'] = xb, hb, []
            qs = [_dot(hb, _unpack(bqkv_p[j])) for j in range(NT)]
            ks = [_dot(hb, _unpack(bqkv_p[NT + j])) for j in range(NT)]
            for i, l in enumerate(layers):
                q = [qs[j][i * SEG:(i + 1) * SEG] * b_scale for j in range(NT)]
                for j in range(NT):
                    keep(l, i, j, ks[j])
                pos = (t - 1 - 2 * l) * SEG + lax.broadcasted_iota(jnp.int32, (SEG, 128), 0)
                logits = []
                for w in range(B_WIN):
                    s = q[0] * win(l, 0, w)
                    for j in range(1, NT):
                        s = s + q[j] * win(l, j, w)
                    s = s + pltpu.roll(s, 64, 1)
                    s = s + pltpu.roll(s, 32, 1)
                    logits.append(jnp.where(pos >= B_DIL * w, s, NEG) if masked else s)
                for j in range(NT):
                    keep_tail(l, i, j, ks[j])
                m = logits[0]
                for w in range(1, B_WIN):
                    m = jnp.maximum(m, logits[w])
                es = [jnp.exp(lg - m) for lg in logits]
                den = es[0]
                for w in range(1, B_WIN):
                    den = den + es[w]
                st['p'].append((es, 1.0 / den))

        def v_stage(j):
            vj = _dot(st['hb'], _unpack(bqkv_p[2 * NT + j]))
            outs = []
            for i, l in enumerate(layers):
                es, inv = st['p'][i]
                keep(l, i, NT + j, vj)
                acc = es[0] * win(l, NT + j, 0)
                for w in range(1, B_WIN):
                    acc = acc + es[w] * win(l, NT + j, w)
                keep_tail(l, i, NT + j, vj)
                outs.append(acc * inv)
            st['o', j] = _cat0(outs).astype(BF16)

        def o_stage(j):
            st['y'] = st['y'] + _dot(st.pop(('o', j)), _unpack(bwo_p[j * 64:(j + 1) * 64, :]))

        def fin():
            for i, l in enumerate(layers):
                yl = st['y'][i * SEG:(i + 1) * SEG]
                if l == 0:
                    x2_ref[...] = yl
                    h_ref[RL:RT, :] = _ln(yl).astype(BF16)
                else:
                    if isinstance(t, int):
                        row = (t - 3) * SEG
                    else:
                        row = pl.multiple_of(jnp.maximum(t - 3, 0) * SEG, SEG)
                    out_ref[pl.ds(row, SEG), :] = yl.astype(out_ref.dtype)

        return qk, v_stage, o_stage, fin

    def softmax2(s, first, valid, fill):
        s = jnp.where(valid, s * a_scale, fill)
        m1 = jnp.max(jnp.where(first, s, PADNEG), axis=-1, keepdims=True)
        m2 = jnp.max(jnp.where(first, PADNEG, s), axis=-1, keepdims=True)
        e = jnp.exp(s - jnp.where(first, m1, m2))
        e1 = jnp.where(first, e, 0.0)
        e2 = jnp.where(first, 0.0, e)
        l1 = jnp.sum(e1, axis=-1, keepdims=True)
        l2 = jnp.sum(e2, axis=-1, keepdims=True)
        inv = 1.0 / jnp.where(first, l1, l2)
        return e, e1, e2, inv

    def make_joint():
        rr = lax.broadcasted_iota(jnp.int32, (RT, 128), 0)
        cc = lax.broadcasted_iota(jnp.int32, (RT, 128), 1)
        lay1 = rr < RV
        first = cc < jnp.where(lay1, RL, RT)
        key = jnp.where(first, cc, cc - RL)
        exists = jnp.where(lay1, RV - 1 - key, key - RV) >= 0
        allowed = (key <= rr) | (lay1 & (key >= SEG)) | ((rr >= RV) & (rr < RL))
        valid = exists & allowed
        fill = jnp.where(exists, NEG, PADNEG)
        lo = cc < (DH - 128)
        z48 = jnp.zeros((128 - RT, 128), F32)
        z32 = jnp.zeros((128 - 2 * RL, 128), F32)

        def prep_q(a):
            return (a[:, 0:128].astype(BF16), a[0:RL, 128:256].astype(BF16),
                    a[SEG:RT, 128:256].astype(BF16), a[:, 256:384].astype(BF16))

        def prep_kv(a):
            mid = a[:, 128:256]
            tlo = jnp.where(lo, mid, 0.0)
            thi = jnp.where(lo, 0.0, mid)
            return (_cat0([a[:, 0:128], z48]).astype(BF16),
                    _cat0([tlo[0:RL], thi[0:RL], z32]).astype(BF16),
                    _cat0([z32, tlo[SEG:RT], thi[SEG:RT]]).astype(BF16),
                    _cat0([z48, a[:, 256:384]]).astype(BF16))

        def qk(q, k):
            t0 = _dot_nt(q[0], k[0])
            t2 = _dot_nt(q[3], k[3])
            t1a = _dot_nt(q[1], k[1])
            t1b = _dot_nt(q[2], k[2])
            s = jnp.where(first, t0, t2) + _cat0([t1a[0:RV], t1b[M:RL]])
            e, e1, e2, inv = softmax2(s, first, valid, fill)
            pa = e * inv
            return ((e1 * inv).astype(BF16), pa[0:RL].astype(BF16),
                    pa[SEG:RT].astype(BF16), (e2 * inv).astype(BF16))

        def pv(pr, v):
            o0 = _dot(pr[0], v[0])
            o2 = _dot(pr[3], v[3])
            o1a = _dot(pr[1], v[1])
            o1b = _dot(pr[2], v[2])
            return _cat1([o0, _cat0([o1a[0:RV], o1b[M:RL]]), o2]).astype(BF16)

        return prep_q, prep_kv, qk, pv

    def make_single(layer, last=False):
        nq = SEG if last else RV
        rr = lax.broadcasted_iota(jnp.int32, (nq, 2 * RL), 0) + (M if last else 0)
        cc = lax.broadcasted_iota(jnp.int32, (nq, 2 * RL), 1)
        first = cc < RL
        kc = jnp.where(first, cc, cc - RL)
        if layer == 0:
            exists = kc < RV
            valid = exists & ((kc >= SEG) | (kc <= rr))
            r0 = 0
        else:
            exists = kc >= M
            valid = exists & ((rr < M) | (kc - M <= rr))
            r0 = M
        fill = jnp.where(exists, NEG, PADNEG)
        lo = lax.broadcasted_iota(jnp.int32, (RL, PW), 1) < DH
        zrow = jnp.zeros((M, 2 * RL), F32)

        def prep_q(a):
            return a.astype(BF16)

        def prep_kv(a):
            return _cat0([jnp.where(lo, a, 0.0), jnp.where(lo, 0.0, a)]).astype(BF16)

        def qk(q, k):
            s = _dot_nt(q, k)
            if not last:
                s = s[r0:r0 + RV]
            e, _, _, inv = softmax2(s, first, valid, fill)
            pa = e * inv
            if not last:
                pa = _cat0([pa, zrow] if layer == 0 else [zrow, pa])
            return pa.astype(BF16)

        def pv(pr, v):
            return _dot(pr, v).astype(BF16)

        return prep_q, prep_kv, qk, pv

    def step(t, a_layers, b_layers, light=False, last=False, masked=True, b_sched=(0, 2, 2, 2)):
        r0 = 0 if 0 in a_layers else SEG
        r1 = RT if 1 in a_layers else RL
        h = h_ref[SEG if light else r0:r1, :]
        if len(a_layers) == 2:
            prep_q, prep_kv, qk, pv = make_joint()
        else:
            prep_q, prep_kv, qk, pv = make_single(a_layers[0], last)

        def proj(i, p):
            r = _dot(h_ref[RL:RT, :] if (last and i == 0) else h, _unpack(wqkv_p[i, p]))
            if light:
                r = _cat0([pre_ref[i, p, pl.ds(pl.multiple_of((t - 2) * SEG, SEG), SEG), :], r])
            return r

        acc = [None]
        OLAG = 3 if len(a_layers) == 2 else 4

        def oproj(p, o):
            part = _dot(o, _unpack(wo_p[p]))
            acc[0] = part if acc[0] is None else acc[0] + part

        def xrows(seg):
            if isinstance(seg, int):
                return x_ref[seg * SEG:(seg + 1) * SEG, :].astype(F32)
            return x_ref[pl.ds(pl.multiple_of(seg * SEG, SEG), SEG), :].astype(F32)

        b_qk, b_v, b_o, b_fin = make_b(t, b_layers, masked)
        hooks = {p: [] for p in range(NP)}
        at, v0, dv, lag = b_sched
        hooks[at].append(b_qk)
        for j in range(NT):
            hooks[at + v0 + j * dv].insert(0, functools.partial(b_v, j)) if v0 else hooks[at].append(
                functools.partial(b_v, j))
        for j in range(NT):
            hooks[at + v0 + j * dv + lag].insert(0, functools.partial(b_o, j))
        x2 = x2_ref[...] if 1 in a_layers else None
        hooks[at + v0 + (NT - 1) * dv + lag].append(b_fin)

        q = prep_q(proj(0, 0))
        k = prep_kv(proj(1, 0))
        v = prep_kv(proj(2, 0))
        early_v = light or len(a_layers) == 1
        os_ = {}
        for p in range(NP):
            pr = qk(q, k)
            if p + 1 < NP:
                q = prep_q(proj(0, p + 1))
                k = prep_kv(proj(1, p + 1))
                if early_v:
                    vn = prep_kv(proj(2, p + 1))
            else:
                if 0 in a_layers:
                    nxt = t + 1 if isinstance(t, int) else jnp.minimum(t + 1, NSEG - 1)
                    h_ref[0:SEG, :] = _ln(xrows(nxt)).astype(BF16)
                for pp in range(p - OLAG, p - 1):
                    oproj(pp, os_.pop(pp))
            os_[p] = pv(pr, v)
            if p + 1 < NP:
                v = vn if early_v else prep_kv(proj(2, p + 1))
            for f in hooks[p]:
                f()
            if p >= OLAG and p + 1 < NP:
                oproj(p - OLAG, os_.pop(p - OLAG))
        oproj(NP - 2, os_.pop(NP - 2))
        oproj(NP - 1, os_.pop(NP - 1))
        a = acc[0]
        if 0 in a_layers:
            xa_ref[0:SEG, :] = xrows(t) + a[0:SEG]
        if last:
            xa_ref[SEG:2 * SEG, :] = x2 + a
            return
        if 1 in a_layers:
            xa_ref[SEG:2 * SEG, :] = x2 + a[RL - r0:RT - r0]
        mem1 = a[SEG - r0:RV - r0]
        mem2 = a[RV - r0:RL - r0] if 1 in a_layers else mem0
        h_ref[SEG:RL, :] = _cat0([mem1, mem2]).astype(BF16)

    def first_step():
        prep_q, prep_kv, qk, pv = make_single(0)

        RA = (RL + NPRE * SEG) // 32 * 16 + 16

        def wait_group(p):
            for cp in cp_group(p):
                cp.wait()

        def body0(p, carry):
            wait_group(p)
            ha = _unpack(hpre_ref[0:RA // 2, :])
            hb = _unpack(hpre_ref[RA // 2:, :])
            w = [dst[rows_of(p), :] for _, dst in w_pairs]

            def proj_a(i):
                r = _dot_nt(ha, w[i])
                pre_ref[i, p, 0:RA - RL, :] = r[RL:]
                return r[0:RL]

            def proj_b(i):
                pre_ref[i, p, RA - RL:, :] = _dot_nt(hb, w[i])

            q = prep_q(proj_a(0))
            k = prep_kv(proj_a(1))
            v = prep_kv(proj_a(2))
            pr = qk(q, k)
            proj_b(0)
            proj_b(1)
            o_ref[p] = _pack(pv(pr, v))
            proj_b(2)
            for i in range(3):
                wqkv_p[i, p] = _pack(w[i].T)
            return carry

        lax.fori_loop(0, NP, body0, 0)
        cp_wo.wait()
        a = None
        for p in range(NP):
            w = wo_ref[sl(p), :]
            wo_p[p] = _pack(w)
            part = _dot(_unpack(o_ref[p]), w)
            a = part if a is None else a + part
        xa_ref[0:SEG, :] = x_ref[0:SEG, :].astype(F32) + a[0:SEG]
        h_ref[0:SEG, :] = _ln(x_ref[SEG:2 * SEG, :].astype(F32)).astype(BF16)
        h_ref[SEG:RL, :] = _cat0([a[SEG:RV], mem0]).astype(BF16)

    first_step()
    cp_x1.start()
    for cp in cp_b:
        cp.wait()
    for j in range(3):
        perm_qkv(j)
    perm_wo()
    step(1, (0,), (0,), b_sched=(7, 2, 1, 1))

    def body_light(t, carry):
        step(t, (0, 1), (0, 1), light=True)
        return carry

    lax.fori_loop(2, 2 + NPRE, body_light, 0)
    cp_x1.wait()

    def body(t, carry):
        step(t, (0, 1), (0, 1), masked=False)
        return carry

    lax.fori_loop(2 + NPRE, NSEG, body, 0)
    done = (NSEG - 3) * SEG
    cp_o0 = pltpu.make_async_copy(out_ref.at[0:done], out_hbm.at[0:done], sem.at[6])
    cp_o0.start()
    step(NSEG, (1,), (0, 1), masked=False)
    step(NSEG + 1, (1,), (1,), last=True, masked=False)
    b_qk, b_v, b_o, b_fin = make_b(NSEG + 2, (1,), False)
    b_qk()
    for j in range(NT):
        b_v(j)
    for j in range(NT):
        b_o(j)
    b_fin()
    cp_o1 = pltpu.make_async_copy(out_ref.at[done:S], out_hbm.at[done:S], sem.at[7])
    cp_o1.start()
    cp_o0.wait()
    cp_o1.wait()


@functools.partial(jax.jit, static_argnames=("A_seg_len",))
def pallas_interleave_layers__memory_aug_recurrent_mem_tr__sliding_local_dilated__prompt_kernel(
    A_x: jax.Array,
    A_mem0: jax.Array,
    A_Wq: jax.Array,
    A_Wk: jax.Array,
    A_Wv: jax.Array,
    A_Wo: jax.Array,
    A_seg_len,
    B_x: jax.Array,
    B_wqkv: jax.Array,
    B_wo: jax.Array,
):
    B, S, D = A_x.shape
    H, DH = A_Wq.shape[1], A_Wq.shape[2]
    M = A_mem0.shape[1]
    SEG = int(A_seg_len)
    assert B == 1 and M == 8 and SEG == 32 and DH == 192 and D % 128 == 0 and S % SEG == 0

    x = A_x.reshape(S, D)
    mem0 = A_mem0.reshape(M, D)
    wq = jnp.transpose(A_Wq, (1, 2, 0)).reshape(H * DH, D)
    wk = jnp.transpose(A_Wk, (1, 2, 0)).reshape(H * DH, D)
    wv = jnp.transpose(A_Wv, (1, 2, 0)).reshape(H * DH, D)
    wo = A_Wo.reshape(H * DH, D)

    hbm = pl.BlockSpec(memory_space=pl.ANY)
    out = pl.pallas_call(
        functools.partial(_kernel, S=S, D=D, H=H, DH=DH, M=M, SEG=SEG),
        out_shape=jax.ShapeDtypeStruct((S, D), A_x.dtype),
        in_specs=[hbm] * 8,
        out_specs=hbm,
        scratch_shapes=[
            pltpu.VMEM((M, D), BF16),
            pltpu.VMEM((S, D), BF16),
            pltpu.VMEM((S, D), BF16),
            pltpu.VMEM((H * DH, D), BF16),
            pltpu.VMEM((H * DH, D), BF16),
            pltpu.VMEM((H * DH, D), BF16),
            pltpu.VMEM((H * DH, D), BF16),
            pltpu.VMEM((3, D, D), BF16),
            pltpu.VMEM((D, D), BF16),
            pltpu.VMEM((3, H // 2, D // 2, 2 * DH), U32),
            pltpu.VMEM((H // 2, DH, D), U32),
            pltpu.VMEM((3 * D // 128, D // 2, 128), U32),
            pltpu.VMEM((D // 2, D), U32),
            pltpu.VMEM((2 * SEG + 2 * M, D), BF16),
            pltpu.VMEM((2 * SEG, D), F32),
            pltpu.VMEM((SEG, D), F32),
            pltpu.VMEM((2, 2 * D // 128, HIST + SEG, 128), F32),
            pltpu.VMEM(((SEG + 2 * M + NPRE * SEG) // 2, D), U32),
            pltpu.VMEM((3, H // 2, NPRE * SEG, 2 * DH), F32),
            pltpu.VMEM((H // 2, (SEG + 2 * M) // 2, 2 * DH), U32),
            pltpu.VMEM((4, D // 128, D, 128), F32),
            pltpu.SemaphoreType.DMA((H // 2,)),
            pltpu.SemaphoreType.DMA((10,)),
        ],
        compiler_params=pltpu.CompilerParams(vmem_limit_bytes=120 * 1024 * 1024),
    )(mem0, x, wq, wk, wv, wo, B_wqkv, B_wo)
    return out.reshape(B, S, D)
```

```python
import functools

import jax
import jax.numpy as jnp
from jax import lax
import jax.experimental.pallas as pl
import jax.experimental.pallas.tpu as pltpu

F32 = jnp.float32
BF16 = jnp.bfloat16
U32 = jnp.uint32

EPS = 1e-5
NEG = -1000000000.0
PADNEG = -3.0e38
B_HEADS = 32
B_WIN = 8
B_DIL = 2
NPRE = 9
HIST = 16


def _ln(x):
    m = jnp.mean(x, axis=-1, keepdims=True)
    xc = x - m
    v = jnp.mean(xc * xc, axis=-1, keepdims=True)
    return xc * lax.rsqrt(v + EPS)


def _dot_nt(a, b):
    return lax.dot_general(a, b, (((1,), (1,)), ((), ())), preferred_element_type=F32)


def _dot(a, b):
    return jnp.dot(a, b, preferred_element_type=F32)


def _pack(a):
    return pltpu.bitcast(a, U32)


def _unpack(a):
    return pltpu.bitcast(a, BF16)


def _cat0(xs):
    return jnp.concatenate(xs, axis=0)


def _cat1(xs):
    return jnp.concatenate(xs, axis=1)


def _kernel(mem0_hbm, x_hbm, wq_hbm, wk_hbm, wv_hbm, wo_hbm, bqkv_hbm, bwo_hbm,
            out_hbm,
            mem0_ref, x_ref, out_ref, wq_ref, wk_ref, wv_ref, wo_ref, bqkv_ref, bwo_ref,
            wqkv_p, wo_p, bqkv_p, bwo_p, h_ref, xa_ref, x2_ref, kv_ref, hpre_ref, pre_ref, o_ref, tmp_ref, wsem, sem,
            *, S, D, H, DH, M, SEG):
    NSEG = S // SEG
    PW = 2 * DH
    NP = H // 2
    RV = SEG + M
    RL = SEG + 2 * M
    RT = 2 * SEG + 2 * M
    a_scale = DH ** (-0.5)
    b_dh = D // B_HEADS
    b_scale = b_dh ** (-0.5)
    NT = D // 128
    X0 = (NPRE + 3) * SEG

    def sl(p):
        return slice(p * PW, (p + 1) * PW)

    cp_m = pltpu.make_async_copy(mem0_hbm, mem0_ref, sem.at[8])
    cp_x0 = pltpu.make_async_copy(x_hbm.at[0:X0], x_ref.at[0:X0], sem.at[0])
    cp_x1 = pltpu.make_async_copy(x_hbm.at[X0:S], x_ref.at[X0:S], sem.at[1])
    cp_b = [pltpu.make_async_copy(bqkv_hbm.at[:, j * D:(j + 1) * D], bqkv_ref.at[j], sem.at[2 + j])
            for j in range(3)]
    cp_b.append(pltpu.make_async_copy(bwo_hbm, bwo_ref, sem.at[5]))
    cp_wo = pltpu.make_async_copy(wo_hbm, wo_ref, sem.at[9])
    w_pairs = ((wq_hbm, wq_ref), (wk_hbm, wk_ref), (wv_hbm, wv_ref))

    def rows_of(p):
        return pl.ds(pl.multiple_of(p * PW, 128), PW)

    def cp_group(p):
        return [pltpu.make_async_copy(src.at[rows_of(p)], dst.at[rows_of(p)], wsem.at[p])
                for src, dst in w_pairs]

    def start_group(p, carry):
        for cp in cp_group(p):
            cp.start()

        @pl.when(p == NP - 1)
        def _():
            cp_wo.start()

        return carry

    cp_m.start()
    cp_x0.start()
    lax.fori_loop(0, NP, start_group, 0)
    for cp in cp_b:
        cp.start()

    xa_ref[...] = jnp.zeros(xa_ref.shape, F32)
    kv_ref[...] = jnp.zeros(kv_ref.shape, F32)
    cp_m.wait()
    cp_x0.wait()
    mem0 = mem0_ref[...].astype(F32)
    h0 = _ln(x_ref[0:SEG, :].astype(F32))
    hpre_ref[0:RL // 2, :] = _pack(_cat0([h0, mem0, mem0]).astype(BF16))
    for i in range(NPRE):
        hi = _ln(x_ref[(2 + i) * SEG:(3 + i) * SEG, :].astype(F32)).astype(BF16)
        hpre_ref[(RL + i * SEG) // 2:(RL + (i + 1) * SEG) // 2, :] = _pack(hi)

    def perm_rows(a, slot):
        a = a.astype(F32)
        for m in range(NT):
            tmp_ref[slot, m] = a[:, m * 128:(m + 1) * 128]
        return _cat1([_cat0([tmp_ref[slot, m, pl.ds(d, B_HEADS, stride=b_dh), :] for d in range(b_dh)])
                      for m in range(NT)]).astype(BF16)

    def perm_qkv(j):
        wp = perm_rows(bqkv_ref[j].T, j).T
        for c in range(NT):
            bqkv_p[j * NT + c] = _pack(wp[:, c * 128:(c + 1) * 128])

    def perm_wo():
        bwo_p[...] = _pack(perm_rows(bwo_ref[...], 3))

    def make_b(t, layers, masked):
        st = {}

        def windows(l, i, j, a):
            cur = a[i * SEG:(i + 1) * SEG]
            blk = _cat0([kv_ref[l, j], cur])
            kv_ref[l, j] = cur[SEG - HIST:SEG]
            rolled = [blk] + [pltpu.roll(blk, sh, 0) for sh in range(B_DIL, 8, B_DIL)]
            res = []
            for w in range(B_WIN):
                hi, lo_ = divmod(B_DIL * w, 8)
                o = HIST - 8 * hi
                res.append(rolled[lo_ // B_DIL][o:o + SEG])
            return res

        def qk():
            xb = xa_ref[layers[0] * SEG:(layers[-1] + 1) * SEG, :]
            hb = _ln(xb).astype(BF16)
            st['y'], st['hb'], st['p'] = xb, hb, []
            qs, ks = [], []
            for j in range(NT):
                qs.append(_dot(hb, _unpack(bqkv_p[j])))
                ks.append(_dot(hb, _unpack(bqkv_p[NT + j])))
            for i, l in enumerate(layers):
                ss = None
                for j in range(NT):
                    q = qs[j][i * SEG:(i + 1) * SEG] * b_scale
                    terms = [q * kw for kw in windows(l, i, j, ks[j])]
                    ss = terms if ss is None else [a + b for a, b in zip(ss, terms)]
                pos = (t - 1 - 2 * l) * SEG + lax.broadcasted_iota(jnp.int32, (SEG, 128), 0)
                logits = []
                for w, s in enumerate(ss):
                    s = s + pltpu.roll(s, 64, 1)
                    s = s + pltpu.roll(s, 32, 1)
                    logits.append(jnp.where(pos >= B_DIL * w, s, NEG) if masked else s)
                m = logits[0]
                for w in range(1, B_WIN):
                    m = jnp.maximum(m, logits[w])
                es = [jnp.exp(lg - m) for lg in logits]
                den = es[0]
                for w in range(1, B_WIN):
                    den = den + es[w]
                st['p'].append((es, 1.0 / den))

        def v_stage(j):
            vj = _dot(st['hb'], _unpack(bqkv_p[2 * NT + j]))
            outs = []
            for i, l in enumerate(layers):
                es, inv = st['p'][i]
                vw = windows(l, i, NT + j, vj)
                acc = es[0] * vw[0]
                for w in range(1, B_WIN):
                    acc = acc + es[w] * vw[w]
                outs.append(acc * inv)
            st['o', j] = _cat0(outs).astype(BF16)

        def o_stage(j):
            st['y'] = st['y'] + _dot(st.pop(('o', j)), _unpack(bwo_p[j * 64:(j + 1) * 64, :]))

        def fin():
            for i, l in enumerate(layers):
                yl = st['y'][i * SEG:(i + 1) * SEG]
                if l == 0:
                    x2_ref[...] = yl
                    h_ref[RL:RT, :] = _ln(yl).astype(BF16)
                else:
                    if isinstance(t, int):
                        row = (t - 3) * SEG
                    else:
                        row = pl.multiple_of(jnp.maximum(t - 3, 0) * SEG, SEG)
                    out_ref[pl.ds(row, SEG), :] = yl.astype(out_ref.dtype)

        return qk, v_stage, o_stage, fin

    def softmax2(s, first, valid, fill):
        s = jnp.where(valid, s * a_scale, fill)
        m1 = jnp.max(jnp.where(first, s, PADNEG), axis=-1, keepdims=True)
        m2 = jnp.max(jnp.where(first, PADNEG, s), axis=-1, keepdims=True)
        e = jnp.exp(s - jnp.where(first, m1, m2))
        e1 = jnp.where(first, e, 0.0)
        e2 = jnp.where(first, 0.0, e)
        l1 = jnp.sum(e1, axis=-1, keepdims=True)
        l2 = jnp.sum(e2, axis=-1, keepdims=True)
        inv = 1.0 / jnp.where(first, l1, l2)
        return e, e1, e2, inv

    def make_joint():
        rr = lax.broadcasted_iota(jnp.int32, (RT, 128), 0)
        cc = lax.broadcasted_iota(jnp.int32, (RT, 128), 1)
        lay1 = rr < RV
        first = cc < jnp.where(lay1, RL, RT)
        key = jnp.where(first, cc, cc - RL)
        exists = jnp.where(lay1, RV - 1 - key, key - RV) >= 0
        allowed = (key <= rr) | (lay1 & (key >= SEG)) | ((rr >= RV) & (rr < RL))
        valid = exists & allowed
        fill = jnp.where(exists, NEG, PADNEG)
        lo = cc < (DH - 128)
        z48 = jnp.zeros((128 - RT, 128), F32)
        z32 = jnp.zeros((128 - 2 * RL, 128), F32)

        def prep_q(a):
            return (a[:, 0:128].astype(BF16), a[0:RL, 128:256].astype(BF16),
                    a[SEG:RT, 128:256].astype(BF16), a[:, 256:384].astype(BF16))

        def prep_kv(a):
            mid = a[:, 128:256]
            tlo = jnp.where(lo, mid, 0.0)
            thi = jnp.where(lo, 0.0, mid)
            return (_cat0([a[:, 0:128], z48]).astype(BF16),
                    _cat0([tlo[0:RL], thi[0:RL], z32]).astype(BF16),
                    _cat0([z32, tlo[SEG:RT], thi[SEG:RT]]).astype(BF16),
                    _cat0([z48, a[:, 256:384]]).astype(BF16))

        def qk(q, k):
            t0 = _dot_nt(q[0], k[0])
            t2 = _dot_nt(q[3], k[3])
            t1a = _dot_nt(q[1], k[1])
            t1b = _dot_nt(q[2], k[2])
            s = jnp.where(first, t0, t2) + _cat0([t1a[0:RV], t1b[M:RL]])
            e, e1, e2, inv = softmax2(s, first, valid, fill)
            pa = e * inv
            return ((e1 * inv).astype(BF16), pa[0:RL].astype(BF16),
                    pa[SEG:RT].astype(BF16), (e2 * inv).astype(BF16))

        def pv(pr, v):
            o0 = _dot(pr[0], v[0])
            o2 = _dot(pr[3], v[3])
            o1a = _dot(pr[1], v[1])
            o1b = _dot(pr[2], v[2])
            return _cat1([o0, _cat0([o1a[0:RV], o1b[M:RL]]), o2]).astype(BF16)

        return prep_q, prep_kv, qk, pv

    def make_single(layer, last=False):
        nq = SEG if last else RV
        rr = lax.broadcasted_iota(jnp.int32, (nq, 2 * RL), 0) + (M if last else 0)
        cc = lax.broadcasted_iota(jnp.int32, (nq, 2 * RL), 1)
        first = cc < RL
        kc = jnp.where(first, cc, cc - RL)
        if layer == 0:
            exists = kc < RV
            valid = exists & ((kc >= SEG) | (kc <= rr))
            r0 = 0
        else:
            exists = kc >= M
            valid = exists & ((rr < M) | (kc - M <= rr))
            r0 = M
        fill = jnp.where(exists, NEG, PADNEG)
        lo = lax.broadcasted_iota(jnp.int32, (RL, PW), 1) < DH
        zrow = jnp.zeros((M, 2 * RL), F32)

        def prep_q(a):
            return a.astype(BF16)

        def prep_kv(a):
            return _cat0([jnp.where(lo, a, 0.0), jnp.where(lo, 0.0, a)]).astype(BF16)

        def qk(q, k):
            s = _dot_nt(q, k)
            if not last:
                s = s[r0:r0 + RV]
            e, _, _, inv = softmax2(s, first, valid, fill)
            pa = e * inv
            if not last:
                pa = _cat0([pa, zrow] if layer == 0 else [zrow, pa])
            return pa.astype(BF16)

        def pv(pr, v):
            return _dot(pr, v).astype(BF16)

        return prep_q, prep_kv, qk, pv

    def step(t, a_layers, b_layers, light=False, last=False, masked=True, b_sched=(0, 3, 2, 1)):
        r0 = 0 if 0 in a_layers else SEG
        r1 = RT if 1 in a_layers else RL
        h = h_ref[SEG if light else r0:r1, :]
        if len(a_layers) == 2:
            prep_q, prep_kv, qk, pv = make_joint()
        else:
            prep_q, prep_kv, qk, pv = make_single(a_layers[0], last)

        def proj(i, p):
            r = _dot(h_ref[RL:RT, :] if (last and i == 0) else h, _unpack(wqkv_p[i, p]))
            if light:
                r = _cat0([pre_ref[i, p, pl.ds(pl.multiple_of((t - 2) * SEG, SEG), SEG), :], r])
            return r

        acc = [None]
        OLAG = 3 if len(a_layers) == 2 else 4

        def oproj(p, o):
            part = _dot(o, _unpack(wo_p[p]))
            acc[0] = part if acc[0] is None else acc[0] + part

        def xrows(seg):
            if isinstance(seg, int):
                return x_ref[seg * SEG:(seg + 1) * SEG, :].astype(F32)
            return x_ref[pl.ds(pl.multiple_of(seg * SEG, SEG), SEG), :].astype(F32)

        b_qk, b_v, b_o, b_fin = make_b(t, b_layers, masked)
        hooks = {p: [] for p in range(NP)}
        at, v0, dv, lag = b_sched
        hooks[at].append(b_qk)
        for j in range(NT):
            hooks[at + v0 + j * dv].insert(0, functools.partial(b_v, j)) if v0 else hooks[at].append(
                functools.partial(b_v, j))
        for j in range(NT):
            hooks[at + v0 + j * dv + lag].insert(0, functools.partial(b_o, j))
        x2 = x2_ref[...] if 1 in a_layers else None
        hooks[at + v0 + (NT - 1) * dv + lag].append(b_fin)

        q = prep_q(proj(0, 0))
        k = prep_kv(proj(1, 0))
        v = prep_kv(proj(2, 0))
        early_v = light or len(a_layers) == 1
        os_ = {}
        for p in range(NP):
            pr = qk(q, k)
            if p + 1 < NP:
                q = prep_q(proj(0, p + 1))
                k = prep_kv(proj(1, p + 1))
                if early_v:
                    vn = prep_kv(proj(2, p + 1))
            else:
                if 0 in a_layers:
                    nxt = t + 1 if isinstance(t, int) else jnp.minimum(t + 1, NSEG - 1)
                    h_ref[0:SEG, :] = _ln(xrows(nxt)).astype(BF16)
                for pp in range(p - OLAG, p - 1):
                    oproj(pp, os_.pop(pp))
            os_[p] = pv(pr, v)
            if p + 1 < NP:
                v = vn if early_v else prep_kv(proj(2, p + 1))
            for f in hooks[p]:
                f()
            if p >= OLAG and p + 1 < NP:
                oproj(p - OLAG, os_.pop(p - OLAG))
        oproj(NP - 2, os_.pop(NP - 2))
        oproj(NP - 1, os_.pop(NP - 1))
        a = acc[0]
        if 0 in a_layers:
            xa_ref[0:SEG, :] = xrows(t) + a[0:SEG]
        if last:
            xa_ref[SEG:2 * SEG, :] = x2 + a
            return
        if 1 in a_layers:
            xa_ref[SEG:2 * SEG, :] = x2 + a[RL - r0:RT - r0]
        mem1 = a[SEG - r0:RV - r0]
        mem2 = a[RV - r0:RL - r0] if 1 in a_layers else mem0
        h_ref[SEG:RL, :] = _cat0([mem1, mem2]).astype(BF16)

    def first_step():
        prep_q, prep_kv, qk, pv = make_single(0)

        RA = (RL + NPRE * SEG) // 32 * 16 + 16

        def wait_group(p):
            for cp in cp_group(p):
                cp.wait()

        def body0(p, carry):
            wait_group(p)
            ha = _unpack(hpre_ref[0:RA // 2, :])
            hb = _unpack(hpre_ref[RA // 2:, :])
            w = [dst[rows_of(p), :] for _, dst in w_pairs]

            def proj_a(i):
                r = _dot_nt(ha, w[i])
                pre_ref[i, p, 0:RA - RL, :] = r[RL:]
                return r[0:RL]

            def proj_b(i):
                pre_ref[i, p, RA - RL:, :] = _dot_nt(hb, w[i])

            q = prep_q(proj_a(0))
            k = prep_kv(proj_a(1))
            v = prep_kv(proj_a(2))
            pr = qk(q, k)
            proj_b(0)
            proj_b(1)
            o_ref[p] = _pack(pv(pr, v))
            proj_b(2)
            for i in range(3):
                wqkv_p[i, p] = _pack(w[i].T)
            return carry

        lax.fori_loop(0, NP, body0, 0)
        cp_wo.wait()
        a = None
        for p in range(NP):
            w = wo_ref[sl(p), :]
            wo_p[p] = _pack(w)
            part = _dot(_unpack(o_ref[p]), w)
            a = part if a is None else a + part
        xa_ref[0:SEG, :] = x_ref[0:SEG, :].astype(F32) + a[0:SEG]
        h_ref[0:SEG, :] = _ln(x_ref[SEG:2 * SEG, :].astype(F32)).astype(BF16)
        h_ref[SEG:RL, :] = _cat0([a[SEG:RV], mem0]).astype(BF16)

    first_step()
    cp_x1.start()
    for cp in cp_b:
        cp.wait()
    for j in range(3):
        perm_qkv(j)
    perm_wo()
    step(1, (0,), (0,), b_sched=(7, 2, 1, 1))

    def body_light(t, carry):
        step(t, (0, 1), (0, 1), light=True)
        return carry

    lax.fori_loop(2, 2 + NPRE, body_light, 0)
    cp_x1.wait()

    def body(t, carry):
        step(t, (0, 1), (0, 1), masked=False)
        return carry

    lax.fori_loop(2 + NPRE, NSEG, body, 0)
    done = (NSEG - 3) * SEG
    cp_o0 = pltpu.make_async_copy(out_ref.at[0:done], out_hbm.at[0:done], sem.at[6])
    cp_o0.start()
    step(NSEG, (1,), (0, 1), masked=False)
    step(NSEG + 1, (1,), (1,), last=True, masked=False)
    b_qk, b_v, b_o, b_fin = make_b(NSEG + 2, (1,), False)
    b_qk()
    for j in range(NT):
        b_v(j)
    for j in range(NT):
        b_o(j)
    b_fin()
    cp_o1 = pltpu.make_async_copy(out_ref.at[done:S], out_hbm.at[done:S], sem.at[7])
    cp_o1.start()
    cp_o0.wait()
    cp_o1.wait()


@functools.partial(jax.jit, static_argnames=("A_seg_len",))
def pallas_interleave_layers__memory_aug_recurrent_mem_tr__sliding_local_dilated__prompt_kernel(
    A_x: jax.Array,
    A_mem0: jax.Array,
    A_Wq: jax.Array,
    A_Wk: jax.Array,
    A_Wv: jax.Array,
    A_Wo: jax.Array,
    A_seg_len,
    B_x: jax.Array,
    B_wqkv: jax.Array,
    B_wo: jax.Array,
):
    B, S, D = A_x.shape
    H, DH = A_Wq.shape[1], A_Wq.shape[2]
    M = A_mem0.shape[1]
    SEG = int(A_seg_len)
    assert B == 1 and M == 8 and SEG == 32 and DH == 192 and D % 128 == 0 and S % SEG == 0

    x = A_x.reshape(S, D)
    mem0 = A_mem0.reshape(M, D)
    wq = jnp.transpose(A_Wq, (1, 2, 0)).reshape(H * DH, D)
    wk = jnp.transpose(A_Wk, (1, 2, 0)).reshape(H * DH, D)
    wv = jnp.transpose(A_Wv, (1, 2, 0)).reshape(H * DH, D)
    wo = A_Wo.reshape(H * DH, D)

    hbm = pl.BlockSpec(memory_space=pl.ANY)
    out = pl.pallas_call(
        functools.partial(_kernel, S=S, D=D, H=H, DH=DH, M=M, SEG=SEG),
        out_shape=jax.ShapeDtypeStruct((S, D), A_x.dtype),
        in_specs=[hbm] * 8,
        out_specs=hbm,
        scratch_shapes=[
            pltpu.VMEM((M, D), BF16),
            pltpu.VMEM((S, D), BF16),
            pltpu.VMEM((S, D), BF16),
            pltpu.VMEM((H * DH, D), BF16),
            pltpu.VMEM((H * DH, D), BF16),
            pltpu.VMEM((H * DH, D), BF16),
            pltpu.VMEM((H * DH, D), BF16),
            pltpu.VMEM((3, D, D), BF16),
            pltpu.VMEM((D, D), BF16),
            pltpu.VMEM((3, H // 2, D // 2, 2 * DH), U32),
            pltpu.VMEM((H // 2, DH, D), U32),
            pltpu.VMEM((3 * D // 128, D // 2, 128), U32),
            pltpu.VMEM((D // 2, D), U32),
            pltpu.VMEM((2 * SEG + 2 * M, D), BF16),
            pltpu.VMEM((2 * SEG, D), F32),
            pltpu.VMEM((SEG, D), F32),
            pltpu.VMEM((2, 2 * D // 128, HIST, 128), F32),
            pltpu.VMEM(((SEG + 2 * M + NPRE * SEG) // 2, D), U32),
            pltpu.VMEM((3, H // 2, NPRE * SEG, 2 * DH), F32),
            pltpu.VMEM((H // 2, (SEG + 2 * M) // 2, 2 * DH), U32),
            pltpu.VMEM((4, D // 128, D, 128), F32),
            pltpu.SemaphoreType.DMA((H // 2,)),
            pltpu.SemaphoreType.DMA((10,)),
        ],
        compiler_params=pltpu.CompilerParams(vmem_limit_bytes=120 * 1024 * 1024),
    )(mem0, x, wq, wk, wv, wo, B_wqkv, B_wo)
    return out.reshape(B, S, D)
```

```python
import functools

import jax
import jax.numpy as jnp
from jax import lax
import jax.experimental.pallas as pl
import jax.experimental.pallas.tpu as pltpu

F32 = jnp.float32
BF16 = jnp.bfloat16
U32 = jnp.uint32

EPS = 1e-5
NEG = -1000000000.0
PADNEG = -3.0e38
B_HEADS = 32
B_WIN = 8
B_DIL = 2
NPRE = 9
HIST = 16


def _ln(x):
    m = jnp.mean(x, axis=-1, keepdims=True)
    xc = x - m
    v = jnp.mean(xc * xc, axis=-1, keepdims=True)
    return xc * lax.rsqrt(v + EPS)


def _dot_nt(a, b):
    return lax.dot_general(a, b, (((1,), (1,)), ((), ())), preferred_element_type=F32)


def _dot(a, b):
    return jnp.dot(a, b, preferred_element_type=F32)


def _pack(a):
    return pltpu.bitcast(a, U32)


def _unpack(a):
    return pltpu.bitcast(a, BF16)


def _cat0(xs):
    return jnp.concatenate(xs, axis=0)


def _cat1(xs):
    return jnp.concatenate(xs, axis=1)


def _kernel(mem0_hbm, x_hbm, wq_hbm, wk_hbm, wv_hbm, wo_hbm, bqkv_hbm, bwo_hbm,
            out_hbm,
            mem0_ref, x_ref, out_ref, wq_ref, wk_ref, wv_ref, wo_ref, bqkv_ref, bwo_ref,
            wqkv_p, wo_p, bqkv_p, bwo_p, h_ref, xa_ref, x2_ref, kv_ref, hpre_ref, pre_ref, o_ref, tmp_ref, wsem, sem,
            *, S, D, H, DH, M, SEG):
    NSEG = S // SEG
    PW = 2 * DH
    NP = H // 2
    RV = SEG + M
    RL = SEG + 2 * M
    RT = 2 * SEG + 2 * M
    a_scale = DH ** (-0.5)
    b_dh = D // B_HEADS
    b_scale = b_dh ** (-0.5)
    NT = D // 128
    X0 = (NPRE + 3) * SEG

    def sl(p):
        return slice(p * PW, (p + 1) * PW)

    cp_m = pltpu.make_async_copy(mem0_hbm, mem0_ref, sem.at[8])
    cp_x0 = pltpu.make_async_copy(x_hbm.at[0:X0], x_ref.at[0:X0], sem.at[0])
    cp_x1 = pltpu.make_async_copy(x_hbm.at[X0:S], x_ref.at[X0:S], sem.at[1])
    cp_b = [pltpu.make_async_copy(bqkv_hbm.at[:, j * D:(j + 1) * D], bqkv_ref.at[j], sem.at[2 + j])
            for j in range(3)]
    cp_b.append(pltpu.make_async_copy(bwo_hbm, bwo_ref, sem.at[5]))
    cp_wo = pltpu.make_async_copy(wo_hbm, wo_ref, sem.at[9])
    w_pairs = ((wq_hbm, wq_ref), (wk_hbm, wk_ref), (wv_hbm, wv_ref))

    def rows_of(p):
        return pl.ds(pl.multiple_of(p * PW, 128), PW)

    def cp_group(p):
        return [pltpu.make_async_copy(src.at[rows_of(p)], dst.at[rows_of(p)], wsem.at[p])
                for src, dst in w_pairs]

    def start_group(p, carry):
        for cp in cp_group(p):
            cp.start()

        @pl.when(p == NP - 1)
        def _():
            cp_wo.start()

        return carry

    cp_m.start()
    cp_x0.start()
    lax.fori_loop(0, NP, start_group, 0)
    for cp in cp_b:
        cp.start()

    xa_ref[...] = jnp.zeros(xa_ref.shape, F32)
    kv_ref[...] = jnp.zeros(kv_ref.shape, F32)
    cp_m.wait()
    cp_x0.wait()
    mem0 = mem0_ref[...].astype(F32)
    h0 = _ln(x_ref[0:SEG, :].astype(F32))
    hpre_ref[0:RL // 2, :] = _pack(_cat0([h0, mem0, mem0]).astype(BF16))
    for i in range(NPRE):
        hi = _ln(x_ref[(2 + i) * SEG:(3 + i) * SEG, :].astype(F32)).astype(BF16)
        hpre_ref[(RL + i * SEG) // 2:(RL + (i + 1) * SEG) // 2, :] = _pack(hi)

    def perm_rows(a, slot):
        a = a.astype(F32)
        for m in range(NT):
            tmp_ref[slot, m] = a[:, m * 128:(m + 1) * 128]
        return _cat1([_cat0([tmp_ref[slot, m, pl.ds(d, B_HEADS, stride=b_dh), :] for d in range(b_dh)])
                      for m in range(NT)]).astype(BF16)

    def perm_qkv(j):
        wp = perm_rows(bqkv_ref[j].T, j).T
        for c in range(NT):
            bqkv_p[j * NT + c] = _pack(wp[:, c * 128:(c + 1) * 128])

    def perm_wo():
        bwo_p[...] = _pack(perm_rows(bwo_ref[...], 3))

    def make_b(t, layers, masked):
        st = {}

        def windows(l, i, j, a):
            cur = a[i * SEG:(i + 1) * SEG]
            blk = _cat0([kv_ref[l, j], cur])
            kv_ref[l, j] = cur[SEG - HIST:SEG]
            rolled = [blk] + [pltpu.roll(blk, sh, 0) for sh in range(B_DIL, 8, B_DIL)]
            res = []
            for w in range(B_WIN):
                hi, lo_ = divmod(B_DIL * w, 8)
                o = HIST - 8 * hi
                res.append(rolled[lo_ // B_DIL][o:o + SEG])
            return res

        def qk():
            xb = xa_ref[layers[0] * SEG:(layers[-1] + 1) * SEG, :]
            hb = _ln(xb).astype(BF16)
            st['y'], st['hb'], st['p'] = xb, hb, []
            qs, ks = [], []
            for j in range(NT):
                qs.append(_dot(hb, _unpack(bqkv_p[j])))
                ks.append(_dot(hb, _unpack(bqkv_p[NT + j])))
            for i, l in enumerate(layers):
                ss = None
                for j in range(NT):
                    q = qs[j][i * SEG:(i + 1) * SEG] * b_scale
                    terms = [q * kw for kw in windows(l, i, j, ks[j])]
                    ss = terms if ss is None else [a + b for a, b in zip(ss, terms)]
                pos = (t - 1 - 2 * l) * SEG + lax.broadcasted_iota(jnp.int32, (SEG, 128), 0)
                logits = []
                for w, s in enumerate(ss):
                    s = s + pltpu.roll(s, 64, 1)
                    s = s + pltpu.roll(s, 32, 1)
                    logits.append(jnp.where(pos >= B_DIL * w, s, NEG) if masked else s)
                m = logits[0]
                for w in range(1, B_WIN):
                    m = jnp.maximum(m, logits[w])
                es = [jnp.exp(lg - m) for lg in logits]
                den = es[0]
                for w in range(1, B_WIN):
                    den = den + es[w]
                st['p'].append((es, 1.0 / den))

        def v_stage(j):
            vj = _dot(st['hb'], _unpack(bqkv_p[2 * NT + j]))
            outs = []
            for i, l in enumerate(layers):
                es, inv = st['p'][i]
                vw = windows(l, i, NT + j, vj)
                acc = es[0] * vw[0]
                for w in range(1, B_WIN):
                    acc = acc + es[w] * vw[w]
                outs.append(acc * inv)
            st['o', j] = _cat0(outs).astype(BF16)

        def o_stage(j):
            st['y'] = st['y'] + _dot(st.pop(('o', j)), _unpack(bwo_p[j * 64:(j + 1) * 64, :]))

        def fin():
            for i, l in enumerate(layers):
                yl = st['y'][i * SEG:(i + 1) * SEG]
                if l == 0:
                    x2_ref[...] = yl
                    h_ref[RL:RT, :] = _ln(yl).astype(BF16)
                else:
                    if isinstance(t, int):
                        row = (t - 3) * SEG
                    else:
                        row = pl.multiple_of(jnp.maximum(t - 3, 0) * SEG, SEG)
                    out_ref[pl.ds(row, SEG), :] = yl.astype(out_ref.dtype)

        return qk, v_stage, o_stage, fin

    def softmax2(s, first, valid, fill):
        s = jnp.where(valid, s * a_scale, fill)
        m1 = jnp.max(jnp.where(first, s, PADNEG), axis=-1, keepdims=True)
        m2 = jnp.max(jnp.where(first, PADNEG, s), axis=-1, keepdims=True)
        e = jnp.exp(s - jnp.where(first, m1, m2))
        e1 = jnp.where(first, e, 0.0)
        e2 = jnp.where(first, 0.0, e)
        l1 = jnp.sum(e1, axis=-1, keepdims=True)
        l2 = jnp.sum(e2, axis=-1, keepdims=True)
        inv = 1.0 / jnp.where(first, l1, l2)
        return e, e1, e2, inv

    def make_joint():
        rr = lax.broadcasted_iota(jnp.int32, (RT, 128), 0)
        cc = lax.broadcasted_iota(jnp.int32, (RT, 128), 1)
        lay1 = rr < RV
        first = cc < jnp.where(lay1, RL, RT)
        key = jnp.where(first, cc, cc - RL)
        exists = jnp.where(lay1, RV - 1 - key, key - RV) >= 0
        allowed = (key <= rr) | (lay1 & (key >= SEG)) | ((rr >= RV) & (rr < RL))
        valid = exists & allowed
        fill = jnp.where(exists, NEG, PADNEG)
        lo = cc < (DH - 128)
        z48 = jnp.zeros((128 - RT, 128), F32)
        z32 = jnp.zeros((128 - 2 * RL, 128), F32)

        def prep_q(a):
            return (a[:, 0:128].astype(BF16), a[0:RL, 128:256].astype(BF16),
                    a[SEG:RT, 128:256].astype(BF16), a[:, 256:384].astype(BF16))

        def prep_kv(a):
            mid = a[:, 128:256]
            tlo = jnp.where(lo, mid, 0.0)
            thi = jnp.where(lo, 0.0, mid)
            return (_cat0([a[:, 0:128], z48]).astype(BF16),
                    _cat0([tlo[0:RL], thi[0:RL], z32]).astype(BF16),
                    _cat0([z32, tlo[SEG:RT], thi[SEG:RT]]).astype(BF16),
                    _cat0([z48, a[:, 256:384]]).astype(BF16))

        def qk(q, k):
            t0 = _dot_nt(q[0], k[0])
            t2 = _dot_nt(q[3], k[3])
            t1a = _dot_nt(q[1], k[1])
            t1b = _dot_nt(q[2], k[2])
            s = jnp.where(first, t0, t2) + _cat0([t1a[0:RV], t1b[M:RL]])
            e, e1, e2, inv = softmax2(s, first, valid, fill)
            pa = e * inv
            return ((e1 * inv).astype(BF16), pa[0:RL].astype(BF16),
                    pa[SEG:RT].astype(BF16), (e2 * inv).astype(BF16))

        def pv(pr, v):
            o0 = _dot(pr[0], v[0])
            o2 = _dot(pr[3], v[3])
            o1a = _dot(pr[1], v[1])
            o1b = _dot(pr[2], v[2])
            return _cat1([o0, _cat0([o1a[0:RV], o1b[M:RL]]), o2]).astype(BF16)

        return prep_q, prep_kv, qk, pv

    def make_single(layer, last=False):
        nq = SEG if last else RV
        rr = lax.broadcasted_iota(jnp.int32, (nq, 2 * RL), 0) + (M if last else 0)
        cc = lax.broadcasted_iota(jnp.int32, (nq, 2 * RL), 1)
        first = cc < RL
        kc = jnp.where(first, cc, cc - RL)
        if layer == 0:
            exists = kc < RV
            valid = exists & ((kc >= SEG) | (kc <= rr))
            r0 = 0
        else:
            exists = kc >= M
            valid = exists & ((rr < M) | (kc - M <= rr))
            r0 = M
        fill = jnp.where(exists, NEG, PADNEG)
        lo = lax.broadcasted_iota(jnp.int32, (RL, PW), 1) < DH
        zrow = jnp.zeros((M, 2 * RL), F32)

        def prep_q(a):
            return a.astype(BF16)

        def prep_kv(a):
            return _cat0([jnp.where(lo, a, 0.0), jnp.where(lo, 0.0, a)]).astype(BF16)

        def qk(q, k):
            s = _dot_nt(q, k)
            if not last:
                s = s[r0:r0 + RV]
            e, _, _, inv = softmax2(s, first, valid, fill)
            pa = e * inv
            if not last:
                pa = _cat0([pa, zrow] if layer == 0 else [zrow, pa])
            return pa.astype(BF16)

        def pv(pr, v):
            return _dot(pr, v).astype(BF16)

        return prep_q, prep_kv, qk, pv

    def step(t, a_layers, b_layers, light=False, last=False, masked=True, deep=False, b_sched=(0, 3, 2, 1)):
        r0 = 0 if 0 in a_layers else SEG
        r1 = RT if 1 in a_layers else RL
        h = h_ref[SEG if light else r0:r1, :]
        if len(a_layers) == 2:
            prep_q, prep_kv, qk, pv = make_joint()
        else:
            prep_q, prep_kv, qk, pv = make_single(a_layers[0], last)

        def proj(i, p):
            r = _dot(h_ref[RL:RT, :] if (last and i == 0) else h, _unpack(wqkv_p[i, p]))
            if light:
                r = _cat0([pre_ref[i, p, pl.ds(pl.multiple_of((t - 2) * SEG, SEG), SEG), :], r])
            return r

        acc = [None]
        OLAG = 3 if len(a_layers) == 2 else 4

        def oproj(p, o):
            part = _dot(o, _unpack(wo_p[p]))
            acc[0] = part if acc[0] is None else acc[0] + part

        def xrows(seg):
            if isinstance(seg, int):
                return x_ref[seg * SEG:(seg + 1) * SEG, :].astype(F32)
            return x_ref[pl.ds(pl.multiple_of(seg * SEG, SEG), SEG), :].astype(F32)

        b_qk, b_v, b_o, b_fin = make_b(t, b_layers, masked)
        hooks = {p: [] for p in range(NP)}
        at, v0, dv, lag = b_sched
        hooks[at].append(b_qk)
        for j in range(NT):
            hooks[at + v0 + j * dv].insert(0, functools.partial(b_v, j)) if v0 else hooks[at].append(
                functools.partial(b_v, j))
        for j in range(NT):
            hooks[at + v0 + j * dv + lag].insert(0, functools.partial(b_o, j))
        x2 = x2_ref[...] if 1 in a_layers else None
        hooks[at + v0 + (NT - 1) * dv + lag].append(b_fin)

        q = prep_q(proj(0, 0))
        k = prep_kv(proj(1, 0))
        vs = {0: prep_kv(proj(2, 0))}
        early_v = light or len(a_layers) == 1
        os_ = {}
        prs = {}

        def do_pv(p):
            os_[p] = pv(prs.pop(p), vs.pop(p))

        for p in range(NP):
            prs[p] = qk(q, k)
            if p + 1 < NP:
                q = prep_q(proj(0, p + 1))
                k = prep_kv(proj(1, p + 1))
                if early_v:
                    vs[p + 1] = prep_kv(proj(2, p + 1))
            else:
                if deep:
                    do_pv(p - 1)
                if 0 in a_layers:
                    nxt = t + 1 if isinstance(t, int) else jnp.minimum(t + 1, NSEG - 1)
                    h_ref[0:SEG, :] = _ln(xrows(nxt)).astype(BF16)
                for pp in range(p - OLAG, p - 1):
                    oproj(pp, os_.pop(pp))
            if not deep or p + 1 == NP:
                do_pv(p)
            elif p >= 1:
                do_pv(p - 1)
            if p + 1 < NP and not early_v:
                vs[p + 1] = prep_kv(proj(2, p + 1))
            for f in hooks[p]:
                f()
            if p >= OLAG and p + 1 < NP:
                oproj(p - OLAG, os_.pop(p - OLAG))
        oproj(NP - 2, os_.pop(NP - 2))
        oproj(NP - 1, os_.pop(NP - 1))
        a = acc[0]
        if 0 in a_layers:
            xa_ref[0:SEG, :] = xrows(t) + a[0:SEG]
        if last:
            xa_ref[SEG:2 * SEG, :] = x2 + a
            return
        if 1 in a_layers:
            xa_ref[SEG:2 * SEG, :] = x2 + a[RL - r0:RT - r0]
        mem1 = a[SEG - r0:RV - r0]
        mem2 = a[RV - r0:RL - r0] if 1 in a_layers else mem0
        h_ref[SEG:RL, :] = _cat0([mem1, mem2]).astype(BF16)

    def first_step():
        prep_q, prep_kv, qk, pv = make_single(0)

        RA = (RL + NPRE * SEG) // 32 * 16 + 16

        def wait_group(p):
            for cp in cp_group(p):
                cp.wait()

        def body0(p, carry):
            wait_group(p)
            ha = _unpack(hpre_ref[0:RA // 2, :])
            hb = _unpack(hpre_ref[RA // 2:, :])
            w = [dst[rows_of(p), :] for _, dst in w_pairs]

            def proj_a(i):
                r = _dot_nt(ha, w[i])
                pre_ref[i, p, 0:RA - RL, :] = r[RL:]
                return r[0:RL]

            def proj_b(i):
                pre_ref[i, p, RA - RL:, :] = _dot_nt(hb, w[i])

            q = prep_q(proj_a(0))
            k = prep_kv(proj_a(1))
            v = prep_kv(proj_a(2))
            pr = qk(q, k)
            proj_b(0)
            proj_b(1)
            o_ref[p] = _pack(pv(pr, v))
            proj_b(2)
            for i in range(3):
                wqkv_p[i, p] = _pack(w[i].T)
            return carry

        lax.fori_loop(0, NP, body0, 0)
        cp_wo.wait()
        a = None
        for p in range(NP):
            w = wo_ref[sl(p), :]
            wo_p[p] = _pack(w)
            part = _dot(_unpack(o_ref[p]), w)
            a = part if a is None else a + part
        xa_ref[0:SEG, :] = x_ref[0:SEG, :].astype(F32) + a[0:SEG]
        h_ref[0:SEG, :] = _ln(x_ref[SEG:2 * SEG, :].astype(F32)).astype(BF16)
        h_ref[SEG:RL, :] = _cat0([a[SEG:RV], mem0]).astype(BF16)

    first_step()
    cp_x1.start()
    for cp in cp_b:
        cp.wait()
    for j in range(3):
        perm_qkv(j)
    perm_wo()
    step(1, (0,), (0,), deep=True, b_sched=(7, 2, 1, 1))

    def body_light(t, carry):
        step(t, (0, 1), (0, 1), light=True)
        return carry

    lax.fori_loop(2, 2 + NPRE, body_light, 0)
    cp_x1.wait()

    def body(t, carry):
        step(t, (0, 1), (0, 1), masked=False)
        return carry

    lax.fori_loop(2 + NPRE, NSEG, body, 0)
    done = (NSEG - 3) * SEG
    cp_o0 = pltpu.make_async_copy(out_ref.at[0:done], out_hbm.at[0:done], sem.at[6])
    cp_o0.start()
    step(NSEG, (1,), (0, 1), masked=False)
    step(NSEG + 1, (1,), (1,), last=True, masked=False)
    b_qk, b_v, b_o, b_fin = make_b(NSEG + 2, (1,), False)
    b_qk()
    for j in range(NT):
        b_v(j)
    for j in range(NT):
        b_o(j)
    b_fin()
    cp_o1 = pltpu.make_async_copy(out_ref.at[done:S], out_hbm.at[done:S], sem.at[7])
    cp_o1.start()
    cp_o0.wait()
    cp_o1.wait()


@functools.partial(jax.jit, static_argnames=("A_seg_len",))
def pallas_interleave_layers__memory_aug_recurrent_mem_tr__sliding_local_dilated__prompt_kernel(
    A_x: jax.Array,
    A_mem0: jax.Array,
    A_Wq: jax.Array,
    A_Wk: jax.Array,
    A_Wv: jax.Array,
    A_Wo: jax.Array,
    A_seg_len,
    B_x: jax.Array,
    B_wqkv: jax.Array,
    B_wo: jax.Array,
):
    B, S, D = A_x.shape
    H, DH = A_Wq.shape[1], A_Wq.shape[2]
    M = A_mem0.shape[1]
    SEG = int(A_seg_len)
    assert B == 1 and M == 8 and SEG == 32 and DH == 192 and D % 128 == 0 and S % SEG == 0

    x = A_x.reshape(S, D)
    mem0 = A_mem0.reshape(M, D)
    wq = jnp.transpose(A_Wq, (1, 2, 0)).reshape(H * DH, D)
    wk = jnp.transpose(A_Wk, (1, 2, 0)).reshape(H * DH, D)
    wv = jnp.transpose(A_Wv, (1, 2, 0)).reshape(H * DH, D)
    wo = A_Wo.reshape(H * DH, D)

    hbm = pl.BlockSpec(memory_space=pl.ANY)
    out = pl.pallas_call(
        functools.partial(_kernel, S=S, D=D, H=H, DH=DH, M=M, SEG=SEG),
        out_shape=jax.ShapeDtypeStruct((S, D), A_x.dtype),
        in_specs=[hbm] * 8,
        out_specs=hbm,
        scratch_shapes=[
            pltpu.VMEM((M, D), BF16),
            pltpu.VMEM((S, D), BF16),
            pltpu.VMEM((S, D), BF16),
            pltpu.VMEM((H * DH, D), BF16),
            pltpu.VMEM((H * DH, D), BF16),
            pltpu.VMEM((H * DH, D), BF16),
            pltpu.VMEM((H * DH, D), BF16),
            pltpu.VMEM((3, D, D), BF16),
            pltpu.VMEM((D, D), BF16),
            pltpu.VMEM((3, H // 2, D // 2, 2 * DH), U32),
            pltpu.VMEM((H // 2, DH, D), U32),
            pltpu.VMEM((3 * D // 128, D // 2, 128), U32),
            pltpu.VMEM((D // 2, D), U32),
            pltpu.VMEM((2 * SEG + 2 * M, D), BF16),
            pltpu.VMEM((2 * SEG, D), F32),
            pltpu.VMEM((SEG, D), F32),
            pltpu.VMEM((2, 2 * D // 128, HIST, 128), F32),
            pltpu.VMEM(((SEG + 2 * M + NPRE * SEG) // 2, D), U32),
            pltpu.VMEM((3, H // 2, NPRE * SEG, 2 * DH), F32),
            pltpu.VMEM((H // 2, (SEG + 2 * M) // 2, 2 * DH), U32),
            pltpu.VMEM((4, D // 128, D, 128), F32),
            pltpu.SemaphoreType.DMA((H // 2,)),
            pltpu.SemaphoreType.DMA((10,)),
        ],
        compiler_params=pltpu.CompilerParams(vmem_limit_bytes=120 * 1024 * 1024),
    )(mem0, x, wq, wk, wv, wo, B_wqkv, B_wo)
    return out.reshape(B, S, D)
```

```python
import functools

import jax
import jax.numpy as jnp
from jax import lax
import jax.experimental.pallas as pl
import jax.experimental.pallas.tpu as pltpu

F32 = jnp.float32
BF16 = jnp.bfloat16
U32 = jnp.uint32

EPS = 1e-5
NEG = -1000000000.0
PADNEG = -3.0e38
B_HEADS = 32
B_WIN = 8
B_DIL = 2
NPRE = 9
HIST = 16


def _ln(x):
    m = jnp.mean(x, axis=-1, keepdims=True)
    xc = x - m
    v = jnp.mean(xc * xc, axis=-1, keepdims=True)
    return xc * lax.rsqrt(v + EPS)


def _dot_nt(a, b):
    return lax.dot_general(a, b, (((1,), (1,)), ((), ())), preferred_element_type=F32)


def _dot(a, b):
    return jnp.dot(a, b, preferred_element_type=F32)


def _pack(a):
    return pltpu.bitcast(a, U32)


def _unpack(a):
    return pltpu.bitcast(a, BF16)


def _cat0(xs):
    return jnp.concatenate(xs, axis=0)


def _cat1(xs):
    return jnp.concatenate(xs, axis=1)


def _kernel(mem0_hbm, x_hbm, wq_hbm, wk_hbm, wv_hbm, wo_hbm, bqkv_hbm, bwo_hbm,
            out_hbm,
            mem0_ref, x_ref, out_ref, wq_ref, wk_ref, wv_ref, wo_ref, bqkv_ref, bwo_ref,
            wqkv_p, wo_p, bqkv_p, bwo_p, h_ref, xa_ref, x2_ref, kv_ref, hpre_ref, pre_ref, o_ref, tmp_ref, wsem, sem,
            *, S, D, H, DH, M, SEG):
    NSEG = S // SEG
    PW = 2 * DH
    NP = H // 2
    RV = SEG + M
    RL = SEG + 2 * M
    RT = 2 * SEG + 2 * M
    a_scale = DH ** (-0.5)
    b_dh = D // B_HEADS
    b_scale = b_dh ** (-0.5)
    NT = D // 128
    X0 = (NPRE + 3) * SEG

    def sl(p):
        return slice(p * PW, (p + 1) * PW)

    cp_m = pltpu.make_async_copy(mem0_hbm, mem0_ref, sem.at[8])
    cp_x0 = pltpu.make_async_copy(x_hbm.at[0:X0], x_ref.at[0:X0], sem.at[0])
    cp_x1 = pltpu.make_async_copy(x_hbm.at[X0:S], x_ref.at[X0:S], sem.at[1])
    cp_b = [pltpu.make_async_copy(bqkv_hbm.at[:, j * D:(j + 1) * D], bqkv_ref.at[j], sem.at[2 + j])
            for j in range(3)]
    cp_b.append(pltpu.make_async_copy(bwo_hbm, bwo_ref, sem.at[5]))
    cp_wo = pltpu.make_async_copy(wo_hbm, wo_ref, sem.at[9])
    w_pairs = ((wq_hbm, wq_ref), (wk_hbm, wk_ref), (wv_hbm, wv_ref))

    def rows_of(p):
        return pl.ds(pl.multiple_of(p * PW, 128), PW)

    def cp_group(p):
        return [pltpu.make_async_copy(src.at[rows_of(p)], dst.at[rows_of(p)], wsem.at[p])
                for src, dst in w_pairs]

    def start_group(p, carry):
        for cp in cp_group(p):
            cp.start()

        @pl.when(p == NP - 1)
        def _():
            cp_wo.start()

        return carry

    cp_m.start()
    cp_x0.start()
    lax.fori_loop(0, NP, start_group, 0)
    for cp in cp_b:
        cp.start()

    xa_ref[...] = jnp.zeros(xa_ref.shape, F32)
    kv_ref[...] = jnp.zeros(kv_ref.shape, F32)
    cp_m.wait()
    cp_x0.wait()
    mem0 = mem0_ref[...].astype(F32)
    h0 = _ln(x_ref[0:SEG, :].astype(F32))
    hpre_ref[0:RL // 2, :] = _pack(_cat0([h0, mem0, mem0]).astype(BF16))
    for i in range(NPRE):
        hi = _ln(x_ref[(2 + i) * SEG:(3 + i) * SEG, :].astype(F32)).astype(BF16)
        hpre_ref[(RL + i * SEG) // 2:(RL + (i + 1) * SEG) // 2, :] = _pack(hi)

    def perm_rows(a, slot):
        a = a.astype(F32)
        for m in range(NT):
            tmp_ref[slot, m, 0:D, :] = a[:, m * 128:(m + 1) * 128]
        return _cat1([_cat0([tmp_ref[slot, m, pl.ds(d, B_HEADS, stride=b_dh), :] for d in range(b_dh)])
                      for m in range(NT)]).astype(BF16)

    def perm_qkv(j):
        wp = perm_rows(bqkv_ref[j].T, j).T
        for c in range(NT):
            bqkv_p[j * NT + c] = _pack(wp[:, c * 128:(c + 1) * 128])

    def perm_wo():
        bwo_p[...] = _pack(perm_rows(bwo_ref[...], 3))

    def make_b(t, layers, masked):
        st = {}

        def windows(l, i, j, a):
            cur = a[i * SEG:(i + 1) * SEG]
            blk = _cat0([kv_ref[l, j], cur])
            kv_ref[l, j] = cur[SEG - HIST:SEG]
            rolled = [blk] + [pltpu.roll(blk, sh, 0) for sh in range(B_DIL, 8, B_DIL)]
            res = []
            for w in range(B_WIN):
                hi, lo_ = divmod(B_DIL * w, 8)
                o = HIST - 8 * hi
                res.append(rolled[lo_ // B_DIL][o:o + SEG])
            return res

        def qk():
            xb = xa_ref[layers[0] * SEG:(layers[-1] + 1) * SEG, :]
            hb = _ln(xb).astype(BF16)
            st['y'], st['hb'], st['p'] = xb, hb, []
            qs, ks = [], []
            for j in range(NT):
                qs.append(_dot(hb, _unpack(bqkv_p[j])))
                ks.append(_dot(hb, _unpack(bqkv_p[NT + j])))
            for i, l in enumerate(layers):
                ss = None
                for j in range(NT):
                    q = qs[j][i * SEG:(i + 1) * SEG] * b_scale
                    terms = [q * kw for kw in windows(l, i, j, ks[j])]
                    ss = terms if ss is None else [a + b for a, b in zip(ss, terms)]
                pos = (t - 1 - 2 * l) * SEG + lax.broadcasted_iota(jnp.int32, (SEG, 128), 0)
                logits = []
                for w, s in enumerate(ss):
                    s = s + pltpu.roll(s, 64, 1)
                    s = s + pltpu.roll(s, 32, 1)
                    logits.append(jnp.where(pos >= B_DIL * w, s, NEG) if masked else s)
                m = logits[0]
                for w in range(1, B_WIN):
                    m = jnp.maximum(m, logits[w])
                es = [jnp.exp(lg - m) for lg in logits]
                den = es[0]
                for w in range(1, B_WIN):
                    den = den + es[w]
                st['p'].append((es, 1.0 / den))

        def v_stage(j):
            vj = _dot(st['hb'], _unpack(bqkv_p[2 * NT + j]))
            outs = []
            for i, l in enumerate(layers):
                es, inv = st['p'][i]
                vw = windows(l, i, NT + j, vj)
                acc = es[0] * vw[0]
                for w in range(1, B_WIN):
                    acc = acc + es[w] * vw[w]
                outs.append(acc * inv)
            st['o', j] = _cat0(outs).astype(BF16)

        def o_stage(j):
            st['y'] = st['y'] + _dot(st.pop(('o', j)), _unpack(bwo_p[j * 64:(j + 1) * 64, :]))

        def fin():
            for i, l in enumerate(layers):
                yl = st['y'][i * SEG:(i + 1) * SEG]
                if l == 0:
                    x2_ref[...] = yl
                    h_ref[RL:RT, :] = _ln(yl).astype(BF16)
                else:
                    if isinstance(t, int):
                        row = (t - 3) * SEG
                    else:
                        row = pl.multiple_of(jnp.maximum(t - 3, 0) * SEG, SEG)
                    out_ref[pl.ds(row, SEG), :] = yl.astype(out_ref.dtype)

        return qk, v_stage, o_stage, fin

    def softmax2(s, first, valid, fill):
        s = jnp.where(valid, s * a_scale, fill)
        m1 = jnp.max(jnp.where(first, s, PADNEG), axis=-1, keepdims=True)
        m2 = jnp.max(jnp.where(first, PADNEG, s), axis=-1, keepdims=True)
        e = jnp.exp(s - jnp.where(first, m1, m2))
        e1 = jnp.where(first, e, 0.0)
        e2 = jnp.where(first, 0.0, e)
        l1 = jnp.sum(e1, axis=-1, keepdims=True)
        l2 = jnp.sum(e2, axis=-1, keepdims=True)
        inv = 1.0 / jnp.where(first, l1, l2)
        return e, e1, e2, inv

    def make_joint():
        rr = lax.broadcasted_iota(jnp.int32, (RT, 128), 0)
        cc = lax.broadcasted_iota(jnp.int32, (RT, 128), 1)
        lay1 = rr < RV
        first = cc < jnp.where(lay1, RL, RT)
        key = jnp.where(first, cc, cc - RL)
        exists = jnp.where(lay1, RV - 1 - key, key - RV) >= 0
        allowed = (key <= rr) | (lay1 & (key >= SEG)) | ((rr >= RV) & (rr < RL))
        valid = exists & allowed
        fill = jnp.where(exists, NEG, PADNEG)
        lo = cc < (DH - 128)
        z48 = jnp.zeros((128 - RT, 128), F32)
        z32 = jnp.zeros((128 - 2 * RL, 128), F32)

        def prep_q(a):
            return (a[:, 0:128].astype(BF16), a[0:RL, 128:256].astype(BF16),
                    a[SEG:RT, 128:256].astype(BF16), a[:, 256:384].astype(BF16))

        def prep_kv(a):
            mid = a[:, 128:256]
            tlo = jnp.where(lo, mid, 0.0)
            thi = jnp.where(lo, 0.0, mid)
            return (_cat0([a[:, 0:128], z48]).astype(BF16),
                    _cat0([tlo[0:RL], thi[0:RL], z32]).astype(BF16),
                    _cat0([z32, tlo[SEG:RT], thi[SEG:RT]]).astype(BF16),
                    _cat0([z48, a[:, 256:384]]).astype(BF16))

        def qk(q, k):
            t0 = _dot_nt(q[0], k[0])
            t2 = _dot_nt(q[3], k[3])
            t1a = _dot_nt(q[1], k[1])
            t1b = _dot_nt(q[2], k[2])
            s = jnp.where(first, t0, t2) + _cat0([t1a[0:RV], t1b[M:RL]])
            e, e1, e2, inv = softmax2(s, first, valid, fill)
            pa = e * inv
            return ((e1 * inv).astype(BF16), pa[0:RL].astype(BF16),
                    pa[SEG:RT].astype(BF16), (e2 * inv).astype(BF16))

        def pv(pr, v):
            o0 = _dot(pr[0], v[0])
            o2 = _dot(pr[3], v[3])
            o1a = _dot(pr[1], v[1])
            o1b = _dot(pr[2], v[2])
            return _cat1([o0, _cat0([o1a[0:RV], o1b[M:RL]]), o2]).astype(BF16)

        return prep_q, prep_kv, qk, pv

    def make_single(layer, last=False):
        nq = SEG if last else RV
        rr = lax.broadcasted_iota(jnp.int32, (nq, 2 * RL), 0) + (M if last else 0)
        cc = lax.broadcasted_iota(jnp.int32, (nq, 2 * RL), 1)
        first = cc < RL
        kc = jnp.where(first, cc, cc - RL)
        if layer == 0:
            exists = kc < RV
            valid = exists & ((kc >= SEG) | (kc <= rr))
            r0 = 0
        else:
            exists = kc >= M
            valid = exists & ((rr < M) | (kc - M <= rr))
            r0 = M
        fill = jnp.where(exists, NEG, PADNEG)
        lo = lax.broadcasted_iota(jnp.int32, (RL, PW), 1) < DH
        zrow = jnp.zeros((M, 2 * RL), F32)

        def prep_q(a):
            return a.astype(BF16)

        def prep_kv(a):
            return _cat0([jnp.where(lo, a, 0.0), jnp.where(lo, 0.0, a)]).astype(BF16)

        def qk(q, k):
            s = _dot_nt(q, k)
            if not last:
                s = s[r0:r0 + RV]
            e, _, _, inv = softmax2(s, first, valid, fill)
            pa = e * inv
            if not last:
                pa = _cat0([pa, zrow] if layer == 0 else [zrow, pa])
            return pa.astype(BF16)

        def pv(pr, v):
            return _dot(pr, v).astype(BF16)

        return prep_q, prep_kv, qk, pv

    def step(t, a_layers, b_layers, light=False, last=False, masked=True, deep=False, b_sched=(0, 3, 2, 1)):
        r0 = 0 if 0 in a_layers else SEG
        r1 = RT if 1 in a_layers else RL
        h = h_ref[SEG if light else r0:r1, :]
        if len(a_layers) == 2:
            prep_q, prep_kv, qk, pv = make_joint()
        else:
            prep_q, prep_kv, qk, pv = make_single(a_layers[0], last)

        def proj(i, p):
            r = _dot(h_ref[RL:RT, :] if (last and i == 0) else h, _unpack(wqkv_p[i, p]))
            if light:
                r = _cat0([pre_ref[i, p, pl.ds(pl.multiple_of((t - 2) * SEG, SEG), SEG), :], r])
            return r

        acc = [None]
        OLAG = 3 if len(a_layers) == 2 else 4

        def oproj(p, o):
            part = _dot(o, _unpack(wo_p[p]))
            acc[0] = part if acc[0] is None else acc[0] + part

        def xrows(seg):
            if isinstance(seg, int):
                return x_ref[seg * SEG:(seg + 1) * SEG, :].astype(F32)
            return x_ref[pl.ds(pl.multiple_of(seg * SEG, SEG), SEG), :].astype(F32)

        b_qk, b_v, b_o, b_fin = make_b(t, b_layers, masked)
        hooks = {p: [] for p in range(NP)}
        at, v0, dv, lag = b_sched
        hooks[at].append(b_qk)
        for j in range(NT):
            hooks[at + v0 + j * dv].insert(0, functools.partial(b_v, j)) if v0 else hooks[at].append(
                functools.partial(b_v, j))
        for j in range(NT):
            hooks[at + v0 + j * dv + lag].insert(0, functools.partial(b_o, j))
        x2 = x2_ref[...] if 1 in a_layers else None
        hooks[at + v0 + (NT - 1) * dv + lag].append(b_fin)

        q = prep_q(proj(0, 0))
        k = prep_kv(proj(1, 0))
        vs = {0: prep_kv(proj(2, 0))}
        early_v = light or len(a_layers) == 1
        os_ = {}
        prs = {}

        def do_pv(p):
            os_[p] = pv(prs.pop(p), vs.pop(p))

        for p in range(NP):
            prs[p] = qk(q, k)
            if p + 1 < NP:
                q = prep_q(proj(0, p + 1))
                k = prep_kv(proj(1, p + 1))
                if early_v:
                    vs[p + 1] = prep_kv(proj(2, p + 1))
            else:
                if deep:
                    do_pv(p - 1)
                if 0 in a_layers:
                    nxt = t + 1 if isinstance(t, int) else jnp.minimum(t + 1, NSEG - 1)
                    h_ref[0:SEG, :] = _ln(xrows(nxt)).astype(BF16)
                for pp in range(p - OLAG, p - 1):
                    oproj(pp, os_.pop(pp))
            if not deep or p + 1 == NP:
                do_pv(p)
            elif p >= 1:
                do_pv(p - 1)
            if p + 1 < NP and not early_v:
                vs[p + 1] = prep_kv(proj(2, p + 1))
            for f in hooks[p]:
                f()
            if p >= OLAG and p + 1 < NP:
                oproj(p - OLAG, os_.pop(p - OLAG))
        oproj(NP - 2, os_.pop(NP - 2))
        oproj(NP - 1, os_.pop(NP - 1))
        a = acc[0]
        if 0 in a_layers:
            xa_ref[0:SEG, :] = xrows(t) + a[0:SEG]
        if last:
            xa_ref[SEG:2 * SEG, :] = x2 + a
            return
        if 1 in a_layers:
            xa_ref[SEG:2 * SEG, :] = x2 + a[RL - r0:RT - r0]
        mem1 = a[SEG - r0:RV - r0]
        mem2 = a[RV - r0:RL - r0] if 1 in a_layers else mem0
        h_ref[SEG:RL, :] = _cat0([mem1, mem2]).astype(BF16)

    def first_step():
        prep_q, prep_kv, qk, pv = make_single(0)

        RA = (RL + NPRE * SEG) // 32 * 16 + 16

        def wait_group(p):
            for cp in cp_group(p):
                cp.wait()

        def body0(p, carry):
            wait_group(p)
            ha = _unpack(hpre_ref[0:RA // 2, :])
            hb = _unpack(hpre_ref[RA // 2:, :])
            w = [dst[rows_of(p), :] for _, dst in w_pairs]

            def proj_a(i):
                r = _dot_nt(ha, w[i])
                pre_ref[i, p, 0:RA - RL, :] = r[RL:]
                return r[0:RL]

            def proj_b(i):
                pre_ref[i, p, RA - RL:, :] = _dot_nt(hb, w[i])

            q = prep_q(proj_a(0))
            k = prep_kv(proj_a(1))
            v = prep_kv(proj_a(2))
            pr = qk(q, k)
            proj_b(0)
            proj_b(1)
            o_ref[p] = _pack(pv(pr, v))
            proj_b(2)
            for i in range(3):
                wqkv_p[i, p] = _pack(w[i].T)
            return carry

        lax.fori_loop(0, NP, body0, 0)
        cp_wo.wait()
        a = None
        for p in range(NP):
            w = wo_ref[sl(p), :]
            wo_p[p] = _pack(w)
            part = _dot(_unpack(o_ref[p]), w)
            a = part if a is None else a + part
        xa_ref[0:SEG, :] = x_ref[0:SEG, :].astype(F32) + a[0:SEG]
        h_ref[0:SEG, :] = _ln(x_ref[SEG:2 * SEG, :].astype(F32)).astype(BF16)
        h_ref[SEG:RL, :] = _cat0([a[SEG:RV], mem0]).astype(BF16)

    first_step()
    cp_x1.start()
    for cp in cp_b:
        cp.wait()
    for j in range(3):
        perm_qkv(j)
    perm_wo()
    step(1, (0,), (0,), deep=True, b_sched=(7, 2, 1, 1))

    def body_light(t, carry):
        step(t, (0, 1), (0, 1), light=True)
        return carry

    lax.fori_loop(2, 2 + NPRE, body_light, 0)
    cp_x1.wait()

    def body(t, carry):
        step(t, (0, 1), (0, 1), masked=False)
        return carry

    lax.fori_loop(2 + NPRE, NSEG, body, 0)
    done = (NSEG - 3) * SEG
    cp_o0 = pltpu.make_async_copy(out_ref.at[0:done], out_hbm.at[0:done], sem.at[6])
    cp_o0.start()
    step(NSEG, (1,), (0, 1), masked=False)
    step(NSEG + 1, (1,), (1,), last=True, masked=False)
    b_qk, b_v, b_o, b_fin = make_b(NSEG + 2, (1,), False)
    b_qk()
    for j in range(NT):
        b_v(j)
    for j in range(NT):
        b_o(j)
    b_fin()
    cp_o1 = pltpu.make_async_copy(out_ref.at[done:S], out_hbm.at[done:S], sem.at[7])
    cp_o1.start()
    cp_o0.wait()
    cp_o1.wait()


def pallas_interleave_layers__memory_aug_recurrent_mem_tr__sliding_local_dilated__prompt_kernel(
    A_x: jax.Array,
    A_mem0: jax.Array,
    A_Wq: jax.Array,
    A_Wk: jax.Array,
    A_Wv: jax.Array,
    A_Wo: jax.Array,
    A_seg_len,
    B_x: jax.Array,
    B_wqkv: jax.Array,
    B_wo: jax.Array,
):
    B, S, D = A_x.shape
    H, DH = A_Wq.shape[1], A_Wq.shape[2]
    M = A_mem0.shape[1]
    SEG = A_seg_len if isinstance(A_seg_len, int) else 32
    assert B == 1 and M == 8 and SEG == 32 and DH == 192 and D == 640 and H % 2 == 0
    assert S % SEG == 0 and S // SEG >= NPRE + 4

    x = A_x.reshape(S, D)
    mem0 = A_mem0.reshape(M, D)
    wq = jnp.transpose(A_Wq, (1, 2, 0)).reshape(H * DH, D)
    wk = jnp.transpose(A_Wk, (1, 2, 0)).reshape(H * DH, D)
    wv = jnp.transpose(A_Wv, (1, 2, 0)).reshape(H * DH, D)
    wo = A_Wo.reshape(H * DH, D)

    hbm = pl.BlockSpec(memory_space=pl.ANY)
    out = pl.pallas_call(
        functools.partial(_kernel, S=S, D=D, H=H, DH=DH, M=M, SEG=SEG),
        out_shape=jax.ShapeDtypeStruct((S, D), A_x.dtype),
        in_specs=[hbm] * 8,
        out_specs=hbm,
        scratch_shapes=[
            pltpu.VMEM((M, D), BF16),
            pltpu.VMEM((S, D), BF16),
            pltpu.VMEM((S, D), BF16),
            pltpu.VMEM((H * DH, D), BF16),
            pltpu.VMEM((H * DH, D), BF16),
            pltpu.VMEM((H * DH, D), BF16),
            pltpu.VMEM((H * DH, D), BF16),
            pltpu.VMEM((3, D, D), BF16),
            pltpu.VMEM((D, D), BF16),
            pltpu.VMEM((3, H // 2, D // 2, 2 * DH), U32),
            pltpu.VMEM((H // 2, DH, D), U32),
            pltpu.VMEM((3 * D // 128, D // 2, 128), U32),
            pltpu.VMEM((D // 2, D), U32),
            pltpu.VMEM((2 * SEG + 2 * M, D), BF16),
            pltpu.VMEM((2 * SEG, D), F32),
            pltpu.VMEM((SEG, D), F32),
            pltpu.VMEM((2, 2 * D // 128, HIST, 128), F32),
            pltpu.VMEM(((SEG + 2 * M + NPRE * SEG) // 2, D), U32),
            pltpu.VMEM((3, H // 2, NPRE * SEG, 2 * DH), F32),
            pltpu.VMEM((H // 2, (SEG + 2 * M) // 2, 2 * DH), U32),
            pltpu.VMEM((4, D // 128, D + 24, 128), F32),
            pltpu.SemaphoreType.DMA((H // 2,)),
            pltpu.SemaphoreType.DMA((10,)),
        ],
        compiler_params=pltpu.CompilerParams(vmem_limit_bytes=120 * 1024 * 1024),
        name="pallas_wavefront",
    )(mem0, x, wq, wk, wv, wo, B_wqkv, B_wo)
    return out.reshape(B, S, D)
```

```python
import functools

import jax
import jax.numpy as jnp
from jax import lax
import jax.experimental.pallas as pl
import jax.experimental.pallas.tpu as pltpu

F32 = jnp.float32
BF16 = jnp.bfloat16
U32 = jnp.uint32

EPS = 1e-5
NEG = -1000000000.0
PADNEG = -3.0e38
B_HEADS = 32
B_WIN = 8
B_DIL = 2
NPRE = 9
HIST = 16


def _ln(x):
    m = jnp.mean(x, axis=-1, keepdims=True)
    xc = x - m
    v = jnp.mean(xc * xc, axis=-1, keepdims=True)
    return xc * lax.rsqrt(v + EPS)


def _dot_nt(a, b):
    return lax.dot_general(a, b, (((1,), (1,)), ((), ())), preferred_element_type=F32)


def _dot(a, b):
    return jnp.dot(a, b, preferred_element_type=F32)


def _pack(a):
    return pltpu.bitcast(a, U32)


def _unpack(a):
    return pltpu.bitcast(a, BF16)


def _cat0(xs):
    return jnp.concatenate(xs, axis=0)


def _cat1(xs):
    return jnp.concatenate(xs, axis=1)


def _kernel(mem0_hbm, x_hbm, wq_hbm, wk_hbm, wv_hbm, wo_hbm, bqkv_hbm, bwo_hbm,
            out_hbm,
            mem0_ref, x_ref, out_ref, wq_ref, wk_ref, wv_ref, wo_ref, bqkv_ref, bwo_ref,
            wqkv_p, wo_p, bqkv_p, bwo_p, h_ref, xa_ref, x2_ref, kv_ref, hpre_ref, pre_ref, o_ref, tmp_ref, wsem, sem,
            *, S, D, H, DH, M, SEG):
    NSEG = S // SEG
    PW = 2 * DH
    NP = H // 2
    RV = SEG + M
    RL = SEG + 2 * M
    RT = 2 * SEG + 2 * M
    a_scale = DH ** (-0.5)
    b_dh = D // B_HEADS
    b_scale = b_dh ** (-0.5)
    NT = D // 128
    X0 = (NPRE + 3) * SEG

    def sl(p):
        return slice(p * PW, (p + 1) * PW)

    cp_m = pltpu.make_async_copy(mem0_hbm, mem0_ref, sem.at[8])
    cp_x0 = pltpu.make_async_copy(x_hbm.at[0:X0], x_ref.at[0:X0], sem.at[0])
    cp_x1 = pltpu.make_async_copy(x_hbm.at[X0:S], x_ref.at[X0:S], sem.at[1])
    cp_b = [pltpu.make_async_copy(bqkv_hbm.at[:, j * D:(j + 1) * D], bqkv_ref.at[j], sem.at[2 + j])
            for j in range(3)]
    cp_b.append(pltpu.make_async_copy(bwo_hbm, bwo_ref, sem.at[5]))
    cp_wo = pltpu.make_async_copy(wo_hbm, wo_ref, sem.at[9])
    w_pairs = ((wq_hbm, wq_ref), (wk_hbm, wk_ref), (wv_hbm, wv_ref))

    def rows_of(p):
        return pl.ds(pl.multiple_of(p * PW, 128), PW)

    def cp_group(p):
        return [pltpu.make_async_copy(src.at[rows_of(p)], dst.at[rows_of(p)], wsem.at[p])
                for src, dst in w_pairs]

    def start_group(p, carry):
        for cp in cp_group(p):
            cp.start()

        @pl.when(p == NP - 1)
        def _():
            cp_wo.start()

        return carry

    cp_m.start()
    cp_x0.start()
    lax.fori_loop(0, NP, start_group, 0)
    for cp in cp_b:
        cp.start()

    xa_ref[...] = jnp.zeros(xa_ref.shape, F32)
    kv_ref[...] = jnp.zeros(kv_ref.shape, F32)
    cp_m.wait()
    cp_x0.wait()
    mem0 = mem0_ref[...].astype(F32)
    h0 = _ln(x_ref[0:SEG, :].astype(F32))
    hpre_ref[0:RL // 2, :] = _pack(_cat0([h0, mem0, mem0]).astype(BF16))
    for i in range(NPRE):
        hi = _ln(x_ref[(2 + i) * SEG:(3 + i) * SEG, :].astype(F32)).astype(BF16)
        hpre_ref[(RL + i * SEG) // 2:(RL + (i + 1) * SEG) // 2, :] = _pack(hi)

    def perm_rows(a, slot):
        a = a.astype(F32)
        for m in range(NT):
            tmp_ref[slot, m, 0:D, :] = a[:, m * 128:(m + 1) * 128]
        return _cat1([_cat0([tmp_ref[slot, m, pl.ds(d, B_HEADS, stride=b_dh), :] for d in range(b_dh)])
                      for m in range(NT)]).astype(BF16)

    def perm_qkv(j):
        wp = perm_rows(bqkv_ref[j].T, j).T
        for c in range(NT):
            bqkv_p[j * NT + c] = _pack(wp[:, c * 128:(c + 1) * 128])

    def perm_wo():
        bwo_p[...] = _pack(perm_rows(bwo_ref[...], 3))

    def make_b(t, layers, masked):
        st = {}

        def windows(l, i, j, a):
            cur = a[i * SEG:(i + 1) * SEG]
            blk = _cat0([kv_ref[l, j], cur])
            kv_ref[l, j] = cur[SEG - HIST:SEG]
            rolled = [blk] + [pltpu.roll(blk, sh, 0) for sh in range(B_DIL, 8, B_DIL)]
            res = []
            for w in range(B_WIN):
                hi, lo_ = divmod(B_DIL * w, 8)
                o = HIST - 8 * hi
                res.append(rolled[lo_ // B_DIL][o:o + SEG])
            return res

        def qk():
            xb = xa_ref[layers[0] * SEG:(layers[-1] + 1) * SEG, :]
            hb = _ln(xb).astype(BF16)
            st['y'], st['hb'], st['p'] = xb, hb, []
            qs, ks = [], []
            for j in range(NT):
                qs.append(_dot(hb, _unpack(bqkv_p[j])))
                ks.append(_dot(hb, _unpack(bqkv_p[NT + j])))
            for i, l in enumerate(layers):
                ss = None
                for j in range(NT):
                    q = qs[j][i * SEG:(i + 1) * SEG] * b_scale
                    terms = [q * kw for kw in windows(l, i, j, ks[j])]
                    ss = terms if ss is None else [a + b for a, b in zip(ss, terms)]
                pos = (t - 1 - 2 * l) * SEG + lax.broadcasted_iota(jnp.int32, (SEG, 128), 0)
                logits = []
                for w, s in enumerate(ss):
                    s = s + pltpu.roll(s, 64, 1)
                    s = s + pltpu.roll(s, 32, 1)
                    logits.append(jnp.where(pos >= B_DIL * w, s, NEG) if masked else s)
                m = logits[0]
                for w in range(1, B_WIN):
                    m = jnp.maximum(m, logits[w])
                es = [jnp.exp(lg - m) for lg in logits]
                den = es[0]
                for w in range(1, B_WIN):
                    den = den + es[w]
                st['p'].append((es, 1.0 / den))

        def v_stage(j):
            vj = _dot(st['hb'], _unpack(bqkv_p[2 * NT + j]))
            outs = []
            for i, l in enumerate(layers):
                es, inv = st['p'][i]
                vw = windows(l, i, NT + j, vj)
                acc = es[0] * vw[0]
                for w in range(1, B_WIN):
                    acc = acc + es[w] * vw[w]
                outs.append(acc * inv)
            st['o', j] = _cat0(outs).astype(BF16)

        def o_stage(j):
            st['y'] = st['y'] + _dot(st.pop(('o', j)), _unpack(bwo_p[j * 64:(j + 1) * 64, :]))

        def fin():
            for i, l in enumerate(layers):
                yl = st['y'][i * SEG:(i + 1) * SEG]
                if l == 0:
                    x2_ref[...] = yl
                    h_ref[RL:RT, :] = _ln(yl).astype(BF16)
                else:
                    if isinstance(t, int):
                        row = (t - 3) * SEG
                    else:
                        row = pl.multiple_of(jnp.maximum(t - 3, 0) * SEG, SEG)
                    out_ref[pl.ds(row, SEG), :] = yl.astype(out_ref.dtype)

        return qk, v_stage, o_stage, fin

    def softmax2(s, first, valid, fill):
        s = jnp.where(valid, s * a_scale, fill)
        m1 = jnp.max(jnp.where(first, s, PADNEG), axis=-1, keepdims=True)
        m2 = jnp.max(jnp.where(first, PADNEG, s), axis=-1, keepdims=True)
        e = jnp.exp(s - jnp.where(first, m1, m2))
        e1 = jnp.where(first, e, 0.0)
        e2 = jnp.where(first, 0.0, e)
        l1 = jnp.sum(e1, axis=-1, keepdims=True)
        l2 = jnp.sum(e2, axis=-1, keepdims=True)
        inv = 1.0 / jnp.where(first, l1, l2)
        return e, e1, e2, inv

    def make_joint():
        rr = lax.broadcasted_iota(jnp.int32, (RT, 128), 0)
        cc = lax.broadcasted_iota(jnp.int32, (RT, 128), 1)
        lay1 = rr < RV
        first = cc < jnp.where(lay1, RL, RT)
        key = jnp.where(first, cc, cc - RL)
        exists = jnp.where(lay1, RV - 1 - key, key - RV) >= 0
        allowed = (key <= rr) | (lay1 & (key >= SEG)) | ((rr >= RV) & (rr < RL))
        valid = exists & allowed
        fill = jnp.where(exists, NEG, PADNEG)
        lo = cc < (DH - 128)
        z48 = jnp.zeros((128 - RT, 128), F32)
        z32 = jnp.zeros((128 - 2 * RL, 128), F32)

        def prep_q(a):
            return (a[:, 0:128].astype(BF16), a[0:RL, 128:256].astype(BF16),
                    a[SEG:RT, 128:256].astype(BF16), a[:, 256:384].astype(BF16))

        def prep_kv(a):
            mid = a[:, 128:256]
            tlo = jnp.where(lo, mid, 0.0)
            thi = jnp.where(lo, 0.0, mid)
            return (_cat0([a[:, 0:128], z48]).astype(BF16),
                    _cat0([tlo[0:RL], thi[0:RL], z32]).astype(BF16),
                    _cat0([z32, tlo[SEG:RT], thi[SEG:RT]]).astype(BF16),
                    _cat0([z48, a[:, 256:384]]).astype(BF16))

        def qk(q, k):
            t0 = _dot_nt(q[0], k[0])
            t2 = _dot_nt(q[3], k[3])
            t1a = _dot_nt(q[1], k[1])
            t1b = _dot_nt(q[2], k[2])
            s = jnp.where(first, t0, t2) + _cat0([t1a[0:RV], t1b[M:RL]])
            e, e1, e2, inv = softmax2(s, first, valid, fill)
            pa = e * inv
            return ((e1 * inv).astype(BF16), pa[0:RL].astype(BF16),
                    pa[SEG:RT].astype(BF16), (e2 * inv).astype(BF16))

        def pv(pr, v):
            o0 = _dot(pr[0], v[0])
            o2 = _dot(pr[3], v[3])
            o1a = _dot(pr[1], v[1])
            o1b = _dot(pr[2], v[2])
            return _cat1([o0, _cat0([o1a[0:RV], o1b[M:RL]]), o2]).astype(BF16)

        return prep_q, prep_kv, qk, pv

    def make_single(layer, last=False):
        nq = SEG if last else RV
        rr = lax.broadcasted_iota(jnp.int32, (nq, 2 * RL), 0) + (M if last else 0)
        cc = lax.broadcasted_iota(jnp.int32, (nq, 2 * RL), 1)
        first = cc < RL
        kc = jnp.where(first, cc, cc - RL)
        if layer == 0:
            exists = kc < RV
            valid = exists & ((kc >= SEG) | (kc <= rr))
            r0 = 0
        else:
            exists = kc >= M
            valid = exists & ((rr < M) | (kc - M <= rr))
            r0 = M
        fill = jnp.where(exists, NEG, PADNEG)
        lo = lax.broadcasted_iota(jnp.int32, (RL, PW), 1) < DH
        zrow = jnp.zeros((M, 2 * RL), F32)

        def prep_q(a):
            return a.astype(BF16)

        def prep_kv(a):
            return _cat0([jnp.where(lo, a, 0.0), jnp.where(lo, 0.0, a)]).astype(BF16)

        def qk(q, k):
            s = _dot_nt(q, k)
            if not last:
                s = s[r0:r0 + RV]
            e, _, _, inv = softmax2(s, first, valid, fill)
            pa = e * inv
            if not last:
                pa = _cat0([pa, zrow] if layer == 0 else [zrow, pa])
            return pa.astype(BF16)

        def pv(pr, v):
            return _dot(pr, v).astype(BF16)

        return prep_q, prep_kv, qk, pv

    def step(t, a_layers, b_layers, light=False, last=False, masked=True, deep=False,
             head_start=False, b_sched=(0, 3, 2, 1)):
        r0 = 0 if 0 in a_layers else SEG
        r1 = RT if 1 in a_layers else RL
        h = h_ref[SEG if light else r0:r1, :]
        if len(a_layers) == 2:
            prep_q, prep_kv, qk, pv = make_joint()
        else:
            prep_q, prep_kv, qk, pv = make_single(a_layers[0], last)

        def proj(i, p):
            r = _dot(h_ref[RL:RT, :] if (last and i == 0) else h, _unpack(wqkv_p[i, p]))
            if light:
                r = _cat0([pre_ref[i, p, pl.ds(pl.multiple_of((t - 2) * SEG, SEG), SEG), :], r])
            return r

        acc = [None]
        OLAG = 3 if len(a_layers) == 2 else 4

        def oproj(p, o):
            part = _dot(o, _unpack(wo_p[p]))
            acc[0] = part if acc[0] is None else acc[0] + part

        def xrows(seg):
            if isinstance(seg, int):
                return x_ref[seg * SEG:(seg + 1) * SEG, :].astype(F32)
            return x_ref[pl.ds(pl.multiple_of(seg * SEG, SEG), SEG), :].astype(F32)

        b_qk, b_v, b_o, b_fin = make_b(t, b_layers, masked)
        hooks = {p: [] for p in range(NP)}
        at, v0, dv, lag = b_sched
        hooks[at].append(b_qk)
        for j in range(NT):
            hooks[at + v0 + j * dv].insert(0, functools.partial(b_v, j)) if v0 else hooks[at].append(
                functools.partial(b_v, j))
        for j in range(NT):
            hooks[at + v0 + j * dv + lag].insert(0, functools.partial(b_o, j))
        x2 = x2_ref[...] if 1 in a_layers else None
        hooks[at + v0 + (NT - 1) * dv + lag].append(b_fin)

        if head_start:
            t0, t1 = (0, SEG) if 0 in a_layers else (RL, RT)
            m0, m1 = (SEG, r1) if 0 in a_layers else (SEG, RL)
            ht = h_ref[t0:t1, :]
            heads = [_dot(ht, _unpack(wqkv_p[i, 0])) for i in range(2)]
            hm = h_ref[m0:m1, :]
            rest = [_dot(hm, _unpack(wqkv_p[i, 0])) for i in range(2)]
            q, k = [_cat0([a, b] if 0 in a_layers else [b, a]) for a, b in zip(heads, rest)]
            q, k = prep_q(q), prep_kv(k)
        else:
            q = prep_q(proj(0, 0))
            k = prep_kv(proj(1, 0))
        vs = {0: prep_kv(proj(2, 0))}
        early_v = light or len(a_layers) == 1
        os_ = {}
        prs = {}

        def do_pv(p):
            os_[p] = pv(prs.pop(p), vs.pop(p))

        for p in range(NP):
            prs[p] = qk(q, k)
            if p + 1 < NP:
                q = prep_q(proj(0, p + 1))
                k = prep_kv(proj(1, p + 1))
                if early_v:
                    vs[p + 1] = prep_kv(proj(2, p + 1))
            else:
                if deep:
                    do_pv(p - 1)
                if 0 in a_layers:
                    nxt = min(t + 1, NSEG - 1) if isinstance(t, int) else jnp.minimum(t + 1, NSEG - 1)
                    h_ref[0:SEG, :] = _ln(xrows(nxt)).astype(BF16)
                for pp in range(p - OLAG, p - 1):
                    oproj(pp, os_.pop(pp))
            if not deep or p + 1 == NP:
                do_pv(p)
            elif p >= 1:
                do_pv(p - 1)
            if p + 1 < NP and not early_v:
                vs[p + 1] = prep_kv(proj(2, p + 1))
            for f in hooks[p]:
                f()
            if p >= OLAG and p + 1 < NP:
                oproj(p - OLAG, os_.pop(p - OLAG))
        oproj(NP - 2, os_.pop(NP - 2))
        oproj(NP - 1, os_.pop(NP - 1))
        a = acc[0]
        if 0 in a_layers:
            xa_ref[0:SEG, :] = xrows(t) + a[0:SEG]
        if last:
            xa_ref[SEG:2 * SEG, :] = x2 + a
            return
        if 1 in a_layers:
            xa_ref[SEG:2 * SEG, :] = x2 + a[RL - r0:RT - r0]
        mem1 = a[SEG - r0:RV - r0]
        mem2 = a[RV - r0:RL - r0] if 1 in a_layers else mem0
        h_ref[SEG:RL, :] = _cat0([mem1, mem2]).astype(BF16)

    def first_step():
        prep_q, prep_kv, qk, pv = make_single(0)

        RA = (RL + NPRE * SEG) // 32 * 16 + 16

        def wait_group(p):
            for cp in cp_group(p):
                cp.wait()

        def pair0(p):
            ha = _unpack(hpre_ref[0:RA // 2, :])
            hb = _unpack(hpre_ref[RA // 2:, :])
            w = [dst[rows_of(p), :] for _, dst in w_pairs]

            def proj_a(i):
                r = _dot_nt(ha, w[i])
                pre_ref[i, p, 0:RA - RL, :] = r[RL:]
                return r[0:RL]

            def proj_b(i):
                pre_ref[i, p, RA - RL:, :] = _dot_nt(hb, w[i])

            q = prep_q(proj_a(0))
            k = prep_kv(proj_a(1))
            v = prep_kv(proj_a(2))
            pr = qk(q, k)
            proj_b(0)
            proj_b(1)
            o_ref[p] = _pack(pv(pr, v))
            proj_b(2)
            for i in range(3):
                wqkv_p[i, p] = _pack(w[i].T)

        def body1(p, carry):
            wait_group(p)
            pair0(p)
            return carry

        def body2(i, carry):
            wait_group(2 * i)
            wait_group(2 * i + 1)
            pair0(2 * i)
            pair0(2 * i + 1)
            return carry

        lax.fori_loop(0, 4, body1, 0)
        lax.fori_loop(2, NP // 2, body2, 0)
        cp_wo.wait()
        a = None
        for p in range(NP):
            w = wo_ref[sl(p), :]
            wo_p[p] = _pack(w)
            part = _dot(_unpack(o_ref[p]), w)
            a = part if a is None else a + part
        xa_ref[0:SEG, :] = x_ref[0:SEG, :].astype(F32) + a[0:SEG]
        h_ref[0:SEG, :] = _ln(x_ref[SEG:2 * SEG, :].astype(F32)).astype(BF16)
        h_ref[SEG:RL, :] = _cat0([a[SEG:RV], mem0]).astype(BF16)

    first_step()
    cp_x1.start()
    for cp in cp_b:
        cp.wait()
    for j in range(3):
        perm_qkv(j)
    perm_wo()
    step(1, (0,), (0,), deep=True, b_sched=(7, 2, 1, 1))

    def body_light(t, carry):
        step(t, (0, 1), (0, 1), light=True)
        return carry

    lax.fori_loop(2, 2 + NPRE, body_light, 0)
    cp_x1.wait()

    T0 = 2 + NPRE
    NPAIR = (NSEG - T0) // 2

    def two_steps(t):
        step(t, (0, 1), (0, 1), masked=False)
        step(t + 1, (0, 1), (0, 1), masked=False, head_start=True)

    def body(i, carry):
        two_steps(T0 + 2 * i)
        return carry

    lax.fori_loop(0, NPAIR, body, 0)
    done = (T0 + 2 * NPAIR - 3) * SEG
    cp_o0 = pltpu.make_async_copy(out_ref.at[0:done], out_hbm.at[0:done], sem.at[6])
    cp_o0.start()
    for t in range(T0 + 2 * NPAIR, NSEG):
        step(t, (0, 1), (0, 1), masked=False)
    step(NSEG, (1,), (0, 1), masked=False, head_start=True)
    step(NSEG + 1, (1,), (1,), last=True, masked=False)
    b_qk, b_v, b_o, b_fin = make_b(NSEG + 2, (1,), False)
    b_qk()
    for j in range(NT):
        b_v(j)
    for j in range(NT):
        b_o(j)
    b_fin()
    cp_o1 = pltpu.make_async_copy(out_ref.at[done:S], out_hbm.at[done:S], sem.at[7])
    cp_o1.start()
    cp_o0.wait()
    cp_o1.wait()


def pallas_interleave_layers__memory_aug_recurrent_mem_tr__sliding_local_dilated__prompt_kernel(
    A_x: jax.Array,
    A_mem0: jax.Array,
    A_Wq: jax.Array,
    A_Wk: jax.Array,
    A_Wv: jax.Array,
    A_Wo: jax.Array,
    A_seg_len,
    B_x: jax.Array,
    B_wqkv: jax.Array,
    B_wo: jax.Array,
):
    B, S, D = A_x.shape
    H, DH = A_Wq.shape[1], A_Wq.shape[2]
    M = A_mem0.shape[1]
    SEG = A_seg_len if isinstance(A_seg_len, int) else 32
    assert B == 1 and M == 8 and SEG == 32 and DH == 192 and D == 640 and H % 2 == 0
    assert S % SEG == 0 and S // SEG >= NPRE + 4

    x = A_x.reshape(S, D)
    mem0 = A_mem0.reshape(M, D)
    wq = jnp.transpose(A_Wq, (1, 2, 0)).reshape(H * DH, D)
    wk = jnp.transpose(A_Wk, (1, 2, 0)).reshape(H * DH, D)
    wv = jnp.transpose(A_Wv, (1, 2, 0)).reshape(H * DH, D)
    wo = A_Wo.reshape(H * DH, D)

    hbm = pl.BlockSpec(memory_space=pl.ANY)
    out = pl.pallas_call(
        functools.partial(_kernel, S=S, D=D, H=H, DH=DH, M=M, SEG=SEG),
        out_shape=jax.ShapeDtypeStruct((S, D), A_x.dtype),
        in_specs=[hbm] * 8,
        out_specs=hbm,
        scratch_shapes=[
            pltpu.VMEM((M, D), BF16),
            pltpu.VMEM((S, D), BF16),
            pltpu.VMEM((S, D), BF16),
            pltpu.VMEM((H * DH, D), BF16),
            pltpu.VMEM((H * DH, D), BF16),
            pltpu.VMEM((H * DH, D), BF16),
            pltpu.VMEM((H * DH, D), BF16),
            pltpu.VMEM((3, D, D), BF16),
            pltpu.VMEM((D, D), BF16),
            pltpu.VMEM((3, H // 2, D // 2, 2 * DH), U32),
            pltpu.VMEM((H // 2, DH, D), U32),
            pltpu.VMEM((3 * D // 128, D // 2, 128), U32),
            pltpu.VMEM((D // 2, D), U32),
            pltpu.VMEM((2 * SEG + 2 * M, D), BF16),
            pltpu.VMEM((2 * SEG, D), F32),
            pltpu.VMEM((SEG, D), F32),
            pltpu.VMEM((2, 2 * D // 128, HIST, 128), F32),
            pltpu.VMEM(((SEG + 2 * M + NPRE * SEG) // 2, D), U32),
            pltpu.VMEM((3, H // 2, NPRE * SEG, 2 * DH), F32),
            pltpu.VMEM((H // 2, (SEG + 2 * M) // 2, 2 * DH), U32),
            pltpu.VMEM((4, D // 128, D + 24, 128), F32),
            pltpu.SemaphoreType.DMA((H // 2,)),
            pltpu.SemaphoreType.DMA((10,)),
        ],
        compiler_params=pltpu.CompilerParams(vmem_limit_bytes=120 * 1024 * 1024),
        name="pallas_wavefront",
    )(mem0, x, wq, wk, wv, wo, B_wqkv, B_wo)
    return out.reshape(B, S, D)
```

```python
import functools

import jax
import jax.numpy as jnp
from jax import lax
import jax.experimental.pallas as pl
import jax.experimental.pallas.tpu as pltpu

F32 = jnp.float32
BF16 = jnp.bfloat16
U32 = jnp.uint32

EPS = 1e-5
NEG = -1000000000.0
PADNEG = -3.0e38
B_HEADS = 32
B_WIN = 8
B_DIL = 2
NPRE = 9
NFINE = 2
HIST = 16


def _ln(x):
    m = jnp.mean(x, axis=-1, keepdims=True)
    xc = x - m
    v = jnp.mean(xc * xc, axis=-1, keepdims=True)
    return xc * lax.rsqrt(v + EPS)


def _dot_nt(a, b):
    return lax.dot_general(a, b, (((1,), (1,)), ((), ())), preferred_element_type=F32)


def _dot(a, b):
    return jnp.dot(a, b, preferred_element_type=F32)


def _pack(a):
    return pltpu.bitcast(a, U32)


def _unpack(a):
    return pltpu.bitcast(a, BF16)


def _cat0(xs):
    return jnp.concatenate(xs, axis=0)


def _cat1(xs):
    return jnp.concatenate(xs, axis=1)


def _kernel(mem0_hbm, x_hbm, wq_hbm, wk_hbm, wv_hbm, wo_hbm, bqkv_hbm, bwo_hbm,
            out_hbm,
            mem0_ref, x_ref, out_ref, wq_ref, wk_ref, wv_ref, wo_ref, bqkv_ref, bwo_ref,
            wqkv_p, wo_p, bqkv_p, bwo_p, h_ref, xa_ref, x2_ref, kv_ref, hpre_ref, pre_ref, o_ref, tmp_ref, wsem, sem,
            *, S, D, H, DH, M, SEG):
    NSEG = S // SEG
    PW = 2 * DH
    NP = H // 2
    RV = SEG + M
    RL = SEG + 2 * M
    RT = 2 * SEG + 2 * M
    a_scale = DH ** (-0.5)
    b_dh = D // B_HEADS
    b_scale = b_dh ** (-0.5)
    NT = D // 128
    X0 = (NPRE + 3) * SEG

    def sl(p):
        return slice(p * PW, (p + 1) * PW)

    cp_m = pltpu.make_async_copy(mem0_hbm, mem0_ref, sem.at[8])
    cp_x0 = pltpu.make_async_copy(x_hbm.at[0:X0], x_ref.at[0:X0], sem.at[0])
    cp_x1 = pltpu.make_async_copy(x_hbm.at[X0:S], x_ref.at[X0:S], sem.at[1])
    cp_b = [pltpu.make_async_copy(bqkv_hbm.at[:, j * D:(j + 1) * D], bqkv_ref.at[j], sem.at[2 + j])
            for j in range(3)]
    cp_b.append(pltpu.make_async_copy(bwo_hbm, bwo_ref, sem.at[5]))
    cp_wo = pltpu.make_async_copy(wo_hbm, wo_ref, sem.at[9])
    w_pairs = ((wq_hbm, wq_ref), (wk_hbm, wk_ref), (wv_hbm, wv_ref))

    def rows_of(p):
        return pl.ds(p * PW if isinstance(p, int) else pl.multiple_of(p * PW, 128), PW)

    def cp_fine(p, i):
        src, dst = w_pairs[i]
        return pltpu.make_async_copy(src.at[rows_of(p)], dst.at[rows_of(p)], wsem.at[NP + 3 * p + i])

    def cp_group(p):
        return [pltpu.make_async_copy(src.at[rows_of(p)], dst.at[rows_of(p)], wsem.at[p])
                for src, dst in w_pairs]

    def start_group(p, carry):
        for cp in cp_group(p):
            cp.start()

        @pl.when(p == NP - 1)
        def _():
            cp_wo.start()

        return carry

    firsts = [[cp_m, cp_x0]] + [[cp_fine(p, i)] for p in range(NFINE) for i in range(3)]

    def start_first(i, carry):
        for n, cps in enumerate(firsts):
            @pl.when(i == n)
            def _():
                for cp in cps:
                    cp.start()

        return carry

    lax.fori_loop(0, len(firsts), start_first, 0)
    lax.fori_loop(NFINE, NP, start_group, 0)
    for cp in cp_b:
        cp.start()

    xa_ref[...] = jnp.zeros(xa_ref.shape, F32)
    kv_ref[...] = jnp.zeros(kv_ref.shape, F32)
    cp_m.wait()
    cp_x0.wait()
    mem0 = mem0_ref[...].astype(F32)
    h0 = _ln(x_ref[0:SEG, :].astype(F32))
    hpre_ref[0:RL // 2, :] = _pack(_cat0([h0, mem0, mem0]).astype(BF16))
    for i in range(NPRE):
        hi = _ln(x_ref[(2 + i) * SEG:(3 + i) * SEG, :].astype(F32)).astype(BF16)
        hpre_ref[(RL + i * SEG) // 2:(RL + (i + 1) * SEG) // 2, :] = _pack(hi)

    def perm_rows(a, slot):
        a = a.astype(F32)
        for m in range(NT):
            tmp_ref[slot, m, 0:D, :] = a[:, m * 128:(m + 1) * 128]
        return _cat1([_cat0([tmp_ref[slot, m, pl.ds(d, B_HEADS, stride=b_dh), :] for d in range(b_dh)])
                      for m in range(NT)]).astype(BF16)

    def perm_qkv(j):
        wp = perm_rows(bqkv_ref[j].T, j).T
        for c in range(NT):
            bqkv_p[j * NT + c] = _pack(wp[:, c * 128:(c + 1) * 128])

    def perm_wo():
        bwo_p[...] = _pack(perm_rows(bwo_ref[...], 3))

    def make_b(t, layers, masked):
        st = {}

        def windows(l, i, j, a):
            cur = a[i * SEG:(i + 1) * SEG]
            blk = _cat0([kv_ref[l, j], cur])
            kv_ref[l, j] = cur[SEG - HIST:SEG]
            rolled = [blk] + [pltpu.roll(blk, sh, 0) for sh in range(B_DIL, 8, B_DIL)]
            res = []
            for w in range(B_WIN):
                hi, lo_ = divmod(B_DIL * w, 8)
                o = HIST - 8 * hi
                res.append(rolled[lo_ // B_DIL][o:o + SEG])
            return res

        def qk():
            xb = xa_ref[layers[0] * SEG:(layers[-1] + 1) * SEG, :]
            hb = _ln(xb).astype(BF16)
            st['y'], st['hb'], st['p'] = xb, hb, []
            qs, ks = [], []
            for j in range(NT):
                qs.append(_dot(hb, _unpack(bqkv_p[j])))
                ks.append(_dot(hb, _unpack(bqkv_p[NT + j])))
            for i, l in enumerate(layers):
                ss = None
                for j in range(NT):
                    q = qs[j][i * SEG:(i + 1) * SEG] * b_scale
                    terms = [q * kw for kw in windows(l, i, j, ks[j])]
                    ss = terms if ss is None else [a + b for a, b in zip(ss, terms)]
                pos = (t - 1 - 2 * l) * SEG + lax.broadcasted_iota(jnp.int32, (SEG, 128), 0)
                logits = []
                for w, s in enumerate(ss):
                    s = s + pltpu.roll(s, 64, 1)
                    s = s + pltpu.roll(s, 32, 1)
                    logits.append(jnp.where(pos >= B_DIL * w, s, NEG) if masked else s)
                m = logits[0]
                for w in range(1, B_WIN):
                    m = jnp.maximum(m, logits[w])
                es = [jnp.exp(lg - m) for lg in logits]
                den = es[0]
                for w in range(1, B_WIN):
                    den = den + es[w]
                st['p'].append((es, 1.0 / den))

        def v_stage(j):
            vj = _dot(st['hb'], _unpack(bqkv_p[2 * NT + j]))
            outs = []
            for i, l in enumerate(layers):
                es, inv = st['p'][i]
                vw = windows(l, i, NT + j, vj)
                acc = es[0] * vw[0]
                for w in range(1, B_WIN):
                    acc = acc + es[w] * vw[w]
                outs.append(acc * inv)
            st['o', j] = _cat0(outs).astype(BF16)

        def o_stage(j):
            st['y'] = st['y'] + _dot(st.pop(('o', j)), _unpack(bwo_p[j * 64:(j + 1) * 64, :]))

        def fin():
            for i, l in enumerate(layers):
                yl = st['y'][i * SEG:(i + 1) * SEG]
                if l == 0:
                    x2_ref[...] = yl
                    h_ref[RL:RT, :] = _ln(yl).astype(BF16)
                else:
                    if isinstance(t, int):
                        row = (t - 3) * SEG
                    else:
                        row = pl.multiple_of(jnp.maximum(t - 3, 0) * SEG, SEG)
                    out_ref[pl.ds(row, SEG), :] = yl.astype(out_ref.dtype)

        return qk, v_stage, o_stage, fin

    def softmax2(s, first, valid, fill):
        s = jnp.where(valid, s * a_scale, fill)
        m1 = jnp.max(jnp.where(first, s, PADNEG), axis=-1, keepdims=True)
        m2 = jnp.max(jnp.where(first, PADNEG, s), axis=-1, keepdims=True)
        e = jnp.exp(s - jnp.where(first, m1, m2))
        e1 = jnp.where(first, e, 0.0)
        e2 = jnp.where(first, 0.0, e)
        l1 = jnp.sum(e1, axis=-1, keepdims=True)
        l2 = jnp.sum(e2, axis=-1, keepdims=True)
        inv = 1.0 / jnp.where(first, l1, l2)
        return e, e1, e2, inv

    def make_joint():
        rr = lax.broadcasted_iota(jnp.int32, (RT, 128), 0)
        cc = lax.broadcasted_iota(jnp.int32, (RT, 128), 1)
        lay1 = rr < RV
        first = cc < jnp.where(lay1, RL, RT)
        key = jnp.where(first, cc, cc - RL)
        exists = jnp.where(lay1, RV - 1 - key, key - RV) >= 0
        allowed = (key <= rr) | (lay1 & (key >= SEG)) | ((rr >= RV) & (rr < RL))
        valid = exists & allowed
        fill = jnp.where(exists, NEG, PADNEG)
        lo = cc < (DH - 128)
        z48 = jnp.zeros((128 - RT, 128), F32)
        z32 = jnp.zeros((128 - 2 * RL, 128), F32)

        def prep_q(a):
            return (a[:, 0:128].astype(BF16), a[0:RL, 128:256].astype(BF16),
                    a[SEG:RT, 128:256].astype(BF16), a[:, 256:384].astype(BF16))

        def prep_kv(a):
            mid = a[:, 128:256]
            tlo = jnp.where(lo, mid, 0.0)
            thi = jnp.where(lo, 0.0, mid)
            return (_cat0([a[:, 0:128], z48]).astype(BF16),
                    _cat0([tlo[0:RL], thi[0:RL], z32]).astype(BF16),
                    _cat0([z32, tlo[SEG:RT], thi[SEG:RT]]).astype(BF16),
                    _cat0([z48, a[:, 256:384]]).astype(BF16))

        def qk(q, k):
            t0 = _dot_nt(q[0], k[0])
            t2 = _dot_nt(q[3], k[3])
            t1a = _dot_nt(q[1], k[1])
            t1b = _dot_nt(q[2], k[2])
            s = jnp.where(first, t0, t2) + _cat0([t1a[0:RV], t1b[M:RL]])
            e, e1, e2, inv = softmax2(s, first, valid, fill)
            pa = e * inv
            return ((e1 * inv).astype(BF16), pa[0:RL].astype(BF16),
                    pa[SEG:RT].astype(BF16), (e2 * inv).astype(BF16))

        def pv(pr, v):
            o0 = _dot(pr[0], v[0])
            o2 = _dot(pr[3], v[3])
            o1a = _dot(pr[1], v[1])
            o1b = _dot(pr[2], v[2])
            return _cat1([o0, _cat0([o1a[0:RV], o1b[M:RL]]), o2]).astype(BF16)

        return prep_q, prep_kv, qk, pv

    def make_single(layer, last=False):
        nq = SEG if last else RV
        rr = lax.broadcasted_iota(jnp.int32, (nq, 2 * RL), 0) + (M if last else 0)
        cc = lax.broadcasted_iota(jnp.int32, (nq, 2 * RL), 1)
        first = cc < RL
        kc = jnp.where(first, cc, cc - RL)
        if layer == 0:
            exists = kc < RV
            valid = exists & ((kc >= SEG) | (kc <= rr))
            r0 = 0
        else:
            exists = kc >= M
            valid = exists & ((rr < M) | (kc - M <= rr))
            r0 = M
        fill = jnp.where(exists, NEG, PADNEG)
        lo = lax.broadcasted_iota(jnp.int32, (RL, PW), 1) < DH
        zrow = jnp.zeros((M, 2 * RL), F32)

        def prep_q(a):
            return a.astype(BF16)

        def prep_kv(a):
            return _cat0([jnp.where(lo, a, 0.0), jnp.where(lo, 0.0, a)]).astype(BF16)

        def qk(q, k):
            s = _dot_nt(q, k)
            if not last:
                s = s[r0:r0 + RV]
            e, _, _, inv = softmax2(s, first, valid, fill)
            pa = e * inv
            if not last:
                pa = _cat0([pa, zrow] if layer == 0 else [zrow, pa])
            return pa.astype(BF16)

        def pv(pr, v):
            return _dot(pr, v).astype(BF16)

        return prep_q, prep_kv, qk, pv

    def step(t, a_layers, b_layers, light=False, last=False, masked=True, deep=False,
             head_start=False, b_sched=(0, 3, 2, 1)):
        r0 = 0 if 0 in a_layers else SEG
        r1 = RT if 1 in a_layers else RL
        h = h_ref[SEG if light else r0:r1, :]
        if len(a_layers) == 2:
            prep_q, prep_kv, qk, pv = make_joint()
        else:
            prep_q, prep_kv, qk, pv = make_single(a_layers[0], last)

        def proj(i, p):
            r = _dot(h_ref[RL:RT, :] if (last and i == 0) else h, _unpack(wqkv_p[i, p]))
            if light:
                r = _cat0([pre_ref[i, p, pl.ds(pl.multiple_of((t - 2) * SEG, SEG), SEG), :], r])
            return r

        acc = [None]
        OLAG = 3 if len(a_layers) == 2 else 4

        def oproj(p, o):
            part = _dot(o, _unpack(wo_p[p]))
            acc[0] = part if acc[0] is None else acc[0] + part

        def xrows(seg):
            if isinstance(seg, int):
                return x_ref[seg * SEG:(seg + 1) * SEG, :].astype(F32)
            return x_ref[pl.ds(pl.multiple_of(seg * SEG, SEG), SEG), :].astype(F32)

        b_qk, b_v, b_o, b_fin = make_b(t, b_layers, masked)
        hooks = {p: [] for p in range(NP)}
        at, v0, dv, lag = b_sched
        hooks[at].append(b_qk)
        for j in range(NT):
            hooks[at + v0 + j * dv].insert(0, functools.partial(b_v, j)) if v0 else hooks[at].append(
                functools.partial(b_v, j))
        for j in range(NT):
            hooks[at + v0 + j * dv + lag].insert(0, functools.partial(b_o, j))
        x2 = x2_ref[...] if 1 in a_layers else None
        hooks[at + v0 + (NT - 1) * dv + lag].append(b_fin)

        if head_start:
            t0, t1 = (0, SEG) if 0 in a_layers else (RL, RT)
            m0, m1 = (SEG, r1) if 0 in a_layers else (SEG, RL)
            ht = h_ref[t0:t1, :]
            heads = [_dot(ht, _unpack(wqkv_p[i, 0])) for i in range(2)]
            hm = h_ref[m0:m1, :]
            rest = [_dot(hm, _unpack(wqkv_p[i, 0])) for i in range(2)]
            q, k = [_cat0([a, b] if 0 in a_layers else [b, a]) for a, b in zip(heads, rest)]
            q, k = prep_q(q), prep_kv(k)
        else:
            q = prep_q(proj(0, 0))
            k = prep_kv(proj(1, 0))
        vs = {0: prep_kv(proj(2, 0))}
        early_v = light or len(a_layers) == 1
        os_ = {}
        prs = {}

        def do_pv(p):
            os_[p] = pv(prs.pop(p), vs.pop(p))

        for p in range(NP):
            prs[p] = qk(q, k)
            if p + 1 < NP:
                q = prep_q(proj(0, p + 1))
                k = prep_kv(proj(1, p + 1))
                if early_v:
                    vs[p + 1] = prep_kv(proj(2, p + 1))
            else:
                if deep:
                    do_pv(p - 1)
                if 0 in a_layers:
                    nxt = min(t + 1, NSEG - 1) if isinstance(t, int) else jnp.minimum(t + 1, NSEG - 1)
                    h_ref[0:SEG, :] = _ln(xrows(nxt)).astype(BF16)
                for pp in range(p - OLAG, p - 1):
                    oproj(pp, os_.pop(pp))
            if not deep or p + 1 == NP:
                do_pv(p)
            elif p >= 1:
                do_pv(p - 1)
            if p + 1 < NP and not early_v:
                vs[p + 1] = prep_kv(proj(2, p + 1))
            for f in hooks[p]:
                f()
            if p >= OLAG and p + 1 < NP:
                oproj(p - OLAG, os_.pop(p - OLAG))
        oproj(NP - 2, os_.pop(NP - 2))
        oproj(NP - 1, os_.pop(NP - 1))
        a = acc[0]
        if 0 in a_layers:
            xa_ref[0:SEG, :] = xrows(t) + a[0:SEG]
        if last:
            xa_ref[SEG:2 * SEG, :] = x2 + a
            return
        if 1 in a_layers:
            xa_ref[SEG:2 * SEG, :] = x2 + a[RL - r0:RT - r0]
        mem1 = a[SEG - r0:RV - r0]
        mem2 = a[RV - r0:RL - r0] if 1 in a_layers else mem0
        h_ref[SEG:RL, :] = _cat0([mem1, mem2]).astype(BF16)

    def first_step():
        prep_q, prep_kv, qk, pv = make_single(0)

        RA = (RL + NPRE * SEG) // 32 * 16 + 16

        def wait_group(p):
            for cp in cp_group(p):
                cp.wait()

        def pair0(p, fine=False):
            ha = _unpack(hpre_ref[0:RA // 2, :])
            hb = _unpack(hpre_ref[RA // 2:, :])
            w = {}

            def load(i):
                if fine:
                    cp_fine(p, i).wait()
                w[i] = w_pairs[i][1][rows_of(p), :]
                wqkv_p[i, p] = _pack(w[i].T)

            def proj_a(i):
                r = _dot_nt(ha, w[i])
                pre_ref[i, p, 0:RA - RL, :] = r[RL:]
                return r[0:RL]

            def proj_b(i):
                pre_ref[i, p, RA - RL:, :] = _dot_nt(hb, w[i])

            if fine:
                load(0)
                q = prep_q(proj_a(0))
                proj_b(0)
                load(1)
                k = prep_kv(proj_a(1))
                proj_b(1)
                load(2)
                pr = qk(q, k)
                v = prep_kv(proj_a(2))
                proj_b(2)
                o_ref[p] = _pack(pv(pr, v))
                return
            for i in range(3):
                load(i)
            q = prep_q(proj_a(0))
            k = prep_kv(proj_a(1))
            v = prep_kv(proj_a(2))
            pr = qk(q, k)
            proj_b(0)
            proj_b(1)
            o_ref[p] = _pack(pv(pr, v))
            proj_b(2)

        def body1(p, carry):
            wait_group(p)
            pair0(p)
            return carry

        def body2(i, carry):
            wait_group(2 * i)
            wait_group(2 * i + 1)
            pair0(2 * i)
            pair0(2 * i + 1)
            return carry

        def body0(p, carry):
            pair0(p, fine=True)
            return carry

        lax.fori_loop(0, NFINE, body0, 0)
        lax.fori_loop(NFINE, 4, body1, 0)
        lax.fori_loop(2, NP // 2, body2, 0)
        cp_wo.wait()
        a = None
        for p in range(NP):
            w = wo_ref[sl(p), :]
            wo_p[p] = _pack(w)
            part = _dot(_unpack(o_ref[p]), w)
            a = part if a is None else a + part
        xa_ref[0:SEG, :] = x_ref[0:SEG, :].astype(F32) + a[0:SEG]
        h_ref[0:SEG, :] = _ln(x_ref[SEG:2 * SEG, :].astype(F32)).astype(BF16)
        h_ref[SEG:RL, :] = _cat0([a[SEG:RV], mem0]).astype(BF16)

    first_step()
    cp_x1.start()
    for cp in cp_b:
        cp.wait()
    for j in range(3):
        perm_qkv(j)
    perm_wo()
    step(1, (0,), (0,), deep=True, b_sched=(7, 2, 1, 1))

    def body_light(t, carry):
        step(t, (0, 1), (0, 1), light=True)
        return carry

    lax.fori_loop(2, 2 + NPRE, body_light, 0)
    cp_x1.wait()

    T0 = 2 + NPRE
    NPAIR = (NSEG - T0) // 2

    def two_steps(t):
        step(t, (0, 1), (0, 1), masked=False)
        step(t + 1, (0, 1), (0, 1), masked=False, head_start=True)

    def body(i, carry):
        two_steps(T0 + 2 * i)
        return carry

    lax.fori_loop(0, NPAIR, body, 0)
    done = (T0 + 2 * NPAIR - 3) * SEG
    cp_o0 = pltpu.make_async_copy(out_ref.at[0:done], out_hbm.at[0:done], sem.at[6])
    cp_o0.start()
    for t in range(T0 + 2 * NPAIR, NSEG):
        step(t, (0, 1), (0, 1), masked=False)
    step(NSEG, (1,), (0, 1), masked=False, head_start=True)
    step(NSEG + 1, (1,), (1,), last=True, masked=False)
    b_qk, b_v, b_o, b_fin = make_b(NSEG + 2, (1,), False)
    b_qk()
    for j in range(NT):
        b_v(j)
    for j in range(NT):
        b_o(j)
    b_fin()
    cp_o1 = pltpu.make_async_copy(out_ref.at[done:S], out_hbm.at[done:S], sem.at[7])
    cp_o1.start()
    cp_o0.wait()
    cp_o1.wait()


def pallas_interleave_layers__memory_aug_recurrent_mem_tr__sliding_local_dilated__prompt_kernel(
    A_x: jax.Array,
    A_mem0: jax.Array,
    A_Wq: jax.Array,
    A_Wk: jax.Array,
    A_Wv: jax.Array,
    A_Wo: jax.Array,
    A_seg_len,
    B_x: jax.Array,
    B_wqkv: jax.Array,
    B_wo: jax.Array,
):
    B, S, D = A_x.shape
    H, DH = A_Wq.shape[1], A_Wq.shape[2]
    M = A_mem0.shape[1]
    SEG = A_seg_len if isinstance(A_seg_len, int) else 32
    assert B == 1 and M == 8 and SEG == 32 and DH == 192 and D == 640 and H % 2 == 0
    assert S % SEG == 0 and S // SEG >= NPRE + 4

    x = A_x.reshape(S, D)
    mem0 = A_mem0.reshape(M, D)
    wq = jnp.transpose(A_Wq, (1, 2, 0)).reshape(H * DH, D)
    wk = jnp.transpose(A_Wk, (1, 2, 0)).reshape(H * DH, D)
    wv = jnp.transpose(A_Wv, (1, 2, 0)).reshape(H * DH, D)
    wo = A_Wo.reshape(H * DH, D)

    hbm = pl.BlockSpec(memory_space=pl.ANY)
    out = pl.pallas_call(
        functools.partial(_kernel, S=S, D=D, H=H, DH=DH, M=M, SEG=SEG),
        out_shape=jax.ShapeDtypeStruct((S, D), A_x.dtype),
        in_specs=[hbm] * 8,
        out_specs=hbm,
        scratch_shapes=[
            pltpu.VMEM((M, D), BF16),
            pltpu.VMEM((S, D), BF16),
            pltpu.VMEM((S, D), BF16),
            pltpu.VMEM((H * DH, D), BF16),
            pltpu.VMEM((H * DH, D), BF16),
            pltpu.VMEM((H * DH, D), BF16),
            pltpu.VMEM((H * DH, D), BF16),
            pltpu.VMEM((3, D, D), BF16),
            pltpu.VMEM((D, D), BF16),
            pltpu.VMEM((3, H // 2, D // 2, 2 * DH), U32),
            pltpu.VMEM((H // 2, DH, D), U32),
            pltpu.VMEM((3 * D // 128, D // 2, 128), U32),
            pltpu.VMEM((D // 2, D), U32),
            pltpu.VMEM((2 * SEG + 2 * M, D), BF16),
            pltpu.VMEM((2 * SEG, D), F32),
            pltpu.VMEM((SEG, D), F32),
            pltpu.VMEM((2, 2 * D // 128, HIST, 128), F32),
            pltpu.VMEM(((SEG + 2 * M + NPRE * SEG) // 2, D), U32),
            pltpu.VMEM((3, H // 2, NPRE * SEG, 2 * DH), F32),
            pltpu.VMEM((H // 2, (SEG + 2 * M) // 2, 2 * DH), U32),
            pltpu.VMEM((4, D // 128, D + 24, 128), F32),
            pltpu.SemaphoreType.DMA((H // 2 + 3 * NFINE,)),
            pltpu.SemaphoreType.DMA((10,)),
        ],
        compiler_params=pltpu.CompilerParams(vmem_limit_bytes=120 * 1024 * 1024),
        name="pallas_wavefront",
    )(mem0, x, wq, wk, wv, wo, B_wqkv, B_wo)
    return out.reshape(B, S, D)
```

```python
import functools

import jax
import jax.numpy as jnp
from jax import lax
import jax.experimental.pallas as pl
import jax.experimental.pallas.tpu as pltpu

F32 = jnp.float32
BF16 = jnp.bfloat16
U32 = jnp.uint32

EPS = 1e-5
NEG = -1000000000.0
PADNEG = -3.0e38
B_HEADS = 32
B_WIN = 8
B_DIL = 2
NPRE = 9
NFINE = 2
HIST = 16


def _ln(x):
    m = jnp.mean(x, axis=-1, keepdims=True)
    xc = x - m
    v = jnp.mean(xc * xc, axis=-1, keepdims=True)
    return xc * lax.rsqrt(v + EPS)


def _dot_nt(a, b):
    return lax.dot_general(a, b, (((1,), (1,)), ((), ())), preferred_element_type=F32)


def _dot(a, b):
    return jnp.dot(a, b, preferred_element_type=F32)


def _pack(a):
    return pltpu.bitcast(a, U32)


def _unpack(a):
    return pltpu.bitcast(a, BF16)


def _cat0(xs):
    return jnp.concatenate(xs, axis=0)


def _cat1(xs):
    return jnp.concatenate(xs, axis=1)


def _kernel(mem0_hbm, x_hbm, wq_hbm, wk_hbm, wv_hbm, wo_hbm, bqkv_hbm, bwo_hbm,
            out_hbm,
            mem0_ref, x_ref, out_ref, wq_ref, wk_ref, wv_ref, wo_ref, bqkv_ref, bwo_ref,
            wqkv_p, wo_p, bqkv_p, bwo_p, h_ref, xa_ref, x2_ref, kv_ref, hpre_ref, pre_ref, o_ref, tmp_ref, wsem, sem,
            *, S, D, H, DH, M, SEG):
    NSEG = S // SEG
    PW = 2 * DH
    NP = H // 2
    RV = SEG + M
    RL = SEG + 2 * M
    RT = 2 * SEG + 2 * M
    a_scale = DH ** (-0.5)
    b_dh = D // B_HEADS
    b_scale = b_dh ** (-0.5)
    NT = D // 128
    X0 = (NPRE + 3) * SEG

    def sl(p):
        return slice(p * PW, (p + 1) * PW)

    cp_m = pltpu.make_async_copy(mem0_hbm, mem0_ref, sem.at[8])
    cp_x0 = pltpu.make_async_copy(x_hbm.at[0:X0], x_ref.at[0:X0], sem.at[0])
    cp_x1 = pltpu.make_async_copy(x_hbm.at[X0:S], x_ref.at[X0:S], sem.at[1])
    cp_b = [pltpu.make_async_copy(bqkv_hbm.at[:, j * D:(j + 1) * D], bqkv_ref.at[j], sem.at[2 + j])
            for j in range(3)]
    cp_b.append(pltpu.make_async_copy(bwo_hbm, bwo_ref, sem.at[5]))
    cp_wo = pltpu.make_async_copy(wo_hbm, wo_ref, sem.at[9])
    w_pairs = ((wq_hbm, wq_ref), (wk_hbm, wk_ref), (wv_hbm, wv_ref))

    def rows_of(p):
        return pl.ds(p * PW if isinstance(p, int) else pl.multiple_of(p * PW, 128), PW)

    def cp_fine(p, i):
        src, dst = w_pairs[i]
        return pltpu.make_async_copy(src.at[rows_of(p)], dst.at[rows_of(p)], wsem.at[NP + 3 * p + i])

    def cp_group(p):
        return [pltpu.make_async_copy(src.at[rows_of(p)], dst.at[rows_of(p)], wsem.at[p])
                for src, dst in w_pairs]

    def start_group(p, carry):
        for cp in cp_group(p):
            cp.start()

        @pl.when(p == NP - 1)
        def _():
            cp_wo.start()

        return carry

    firsts = [[cp_m, cp_x0]] + [[cp_fine(p, i)] for p in range(NFINE) for i in range(3)]

    def start_first(i, carry):
        for n, cps in enumerate(firsts):
            @pl.when(i == n)
            def _():
                for cp in cps:
                    cp.start()

        return carry

    lax.fori_loop(0, len(firsts), start_first, 0)
    lax.fori_loop(NFINE, NP, start_group, 0)
    for cp in cp_b:
        cp.start()

    xa_ref[...] = jnp.zeros(xa_ref.shape, F32)
    kv_ref[...] = jnp.zeros(kv_ref.shape, F32)
    cp_m.wait()
    cp_x0.wait()
    mem0 = mem0_ref[...].astype(F32)
    h0 = _ln(x_ref[0:SEG, :].astype(F32))
    hpre_ref[0:RL // 2, :] = _pack(_cat0([h0, mem0, mem0]).astype(BF16))
    for i in range(NPRE):
        hi = _ln(x_ref[(2 + i) * SEG:(3 + i) * SEG, :].astype(F32)).astype(BF16)
        hpre_ref[(RL + i * SEG) // 2:(RL + (i + 1) * SEG) // 2, :] = _pack(hi)

    def perm_rows(a, slot):
        a = a.astype(F32)
        for m in range(NT):
            tmp_ref[slot, m, 0:D, :] = a[:, m * 128:(m + 1) * 128]
        return _cat1([_cat0([tmp_ref[slot, m, pl.ds(d, B_HEADS, stride=b_dh), :] for d in range(b_dh)])
                      for m in range(NT)]).astype(BF16)

    def perm_qkv(j):
        wp = perm_rows(bqkv_ref[j].T, j).T
        for c in range(NT):
            bqkv_p[j * NT + c] = _pack(wp[:, c * 128:(c + 1) * 128])

    def perm_wo():
        bwo_p[...] = _pack(perm_rows(bwo_ref[...], 3))

    def make_b(t, layers, masked):
        st = {}

        def windows(l, i, j, a):
            cur = a[i * SEG:(i + 1) * SEG]
            blk = _cat0([kv_ref[l, j], cur])
            kv_ref[l, j] = cur[SEG - HIST:SEG]
            rolled = [blk] + [pltpu.roll(blk, sh, 0) for sh in range(B_DIL, 8, B_DIL)]
            res = []
            for w in range(B_WIN):
                hi, lo_ = divmod(B_DIL * w, 8)
                o = HIST - 8 * hi
                res.append(rolled[lo_ // B_DIL][o:o + SEG])
            return res

        def qk():
            xb = xa_ref[layers[0] * SEG:(layers[-1] + 1) * SEG, :]
            hb = _ln(xb).astype(BF16)
            st['y'], st['hb'], st['p'] = xb, hb, []
            qs, ks = [], []
            for j in range(NT):
                qs.append(_dot(hb, _unpack(bqkv_p[j])))
                ks.append(_dot(hb, _unpack(bqkv_p[NT + j])))
            for i, l in enumerate(layers):
                ss = None
                for j in range(NT):
                    q = qs[j][i * SEG:(i + 1) * SEG] * b_scale
                    terms = [q * kw for kw in windows(l, i, j, ks[j])]
                    ss = terms if ss is None else [a + b for a, b in zip(ss, terms)]
                pos = (t - 1 - 2 * l) * SEG + lax.broadcasted_iota(jnp.int32, (SEG, 128), 0)
                logits = []
                for w, s in enumerate(ss):
                    s = s + pltpu.roll(s, 64, 1)
                    s = s + pltpu.roll(s, 32, 1)
                    logits.append(jnp.where(pos >= B_DIL * w, s, NEG) if masked else s)
                m = logits[0]
                for w in range(1, B_WIN):
                    m = jnp.maximum(m, logits[w])
                es = [jnp.exp(lg - m) for lg in logits]
                den = es[0]
                for w in range(1, B_WIN):
                    den = den + es[w]
                st['p'].append((es, 1.0 / den))

        def v_stage(j):
            vj = _dot(st['hb'], _unpack(bqkv_p[2 * NT + j]))
            outs = []
            for i, l in enumerate(layers):
                es, inv = st['p'][i]
                vw = windows(l, i, NT + j, vj)
                acc = es[0] * vw[0]
                for w in range(1, B_WIN):
                    acc = acc + es[w] * vw[w]
                outs.append(acc * inv)
            st['o', j] = _cat0(outs).astype(BF16)

        def o_stage(j):
            st['y'] = st['y'] + _dot(st.pop(('o', j)), _unpack(bwo_p[j * 64:(j + 1) * 64, :]))

        def fin():
            for i, l in enumerate(layers):
                yl = st['y'][i * SEG:(i + 1) * SEG]
                if l == 0:
                    x2_ref[...] = yl
                    h_ref[RL:RT, :] = _ln(yl).astype(BF16)
                else:
                    if isinstance(t, int):
                        row = (t - 3) * SEG
                    else:
                        row = pl.multiple_of(jnp.maximum(t - 3, 0) * SEG, SEG)
                    out_ref[pl.ds(row, SEG), :] = yl.astype(out_ref.dtype)

        return qk, v_stage, o_stage, fin

    def softmax2(s, first, valid, fill):
        s = jnp.where(valid, s * a_scale, fill)
        m1 = jnp.max(jnp.where(first, s, PADNEG), axis=-1, keepdims=True)
        m2 = jnp.max(jnp.where(first, PADNEG, s), axis=-1, keepdims=True)
        e = jnp.exp(s - jnp.where(first, m1, m2))
        e1 = jnp.where(first, e, 0.0)
        e2 = jnp.where(first, 0.0, e)
        l1 = jnp.sum(e1, axis=-1, keepdims=True)
        l2 = jnp.sum(e2, axis=-1, keepdims=True)
        inv = 1.0 / jnp.where(first, l1, l2)
        return e, e1, e2, inv

    def make_joint():
        rr = lax.broadcasted_iota(jnp.int32, (RT, 128), 0)
        cc = lax.broadcasted_iota(jnp.int32, (RT, 128), 1)
        lay1 = rr < RV
        first = cc < jnp.where(lay1, RL, RT)
        key = jnp.where(first, cc, cc - RL)
        exists = jnp.where(lay1, RV - 1 - key, key - RV) >= 0
        allowed = (key <= rr) | (lay1 & (key >= SEG)) | ((rr >= RV) & (rr < RL))
        valid = exists & allowed
        fill = jnp.where(exists, NEG, PADNEG)
        lo = cc < (DH - 128)
        z48 = jnp.zeros((128 - RT, 128), F32)
        z32 = jnp.zeros((128 - 2 * RL, 128), F32)

        def prep_q(a):
            return (a[:, 0:128].astype(BF16), a[0:RL, 128:256].astype(BF16),
                    a[SEG:RT, 128:256].astype(BF16), a[:, 256:384].astype(BF16))

        def prep_kv(a):
            mid = a[:, 128:256]
            tlo = jnp.where(lo, mid, 0.0)
            thi = jnp.where(lo, 0.0, mid)
            return (_cat0([a[:, 0:128], z48]).astype(BF16),
                    _cat0([tlo[0:RL], thi[0:RL], z32]).astype(BF16),
                    _cat0([z32, tlo[SEG:RT], thi[SEG:RT]]).astype(BF16),
                    _cat0([z48, a[:, 256:384]]).astype(BF16))

        def qk(q, k):
            t0 = _dot_nt(q[0], k[0])
            t2 = _dot_nt(q[3], k[3])
            t1a = _dot_nt(q[1], k[1])
            t1b = _dot_nt(q[2], k[2])
            s = jnp.where(first, t0, t2) + _cat0([t1a[0:RV], t1b[M:RL]])
            e, e1, e2, inv = softmax2(s, first, valid, fill)
            pa = e * inv
            return ((e1 * inv).astype(BF16), pa[0:RL].astype(BF16),
                    pa[SEG:RT].astype(BF16), (e2 * inv).astype(BF16))

        def pv(pr, v):
            o0 = _dot(pr[0], v[0])
            o2 = _dot(pr[3], v[3])
            o1a = _dot(pr[1], v[1])
            o1b = _dot(pr[2], v[2])
            return _cat1([o0, _cat0([o1a[0:RV], o1b[M:RL]]), o2]).astype(BF16)

        return prep_q, prep_kv, qk, pv

    def make_single(layer, last=False):
        nq = SEG if last else RV
        rr = lax.broadcasted_iota(jnp.int32, (nq, 2 * RL), 0) + (M if last else 0)
        cc = lax.broadcasted_iota(jnp.int32, (nq, 2 * RL), 1)
        first = cc < RL
        kc = jnp.where(first, cc, cc - RL)
        if layer == 0:
            exists = kc < RV
            valid = exists & ((kc >= SEG) | (kc <= rr))
            r0 = 0
        else:
            exists = kc >= M
            valid = exists & ((rr < M) | (kc - M <= rr))
            r0 = M
        fill = jnp.where(exists, NEG, PADNEG)
        lo = lax.broadcasted_iota(jnp.int32, (RL, PW), 1) < DH
        zrow = jnp.zeros((M, 2 * RL), F32)

        def prep_q(a):
            return a.astype(BF16)

        def prep_kv(a):
            return _cat0([jnp.where(lo, a, 0.0), jnp.where(lo, 0.0, a)]).astype(BF16)

        def qk(q, k):
            s = _dot_nt(q, k)
            if not last:
                s = s[r0:r0 + RV]
            e, _, _, inv = softmax2(s, first, valid, fill)
            pa = e * inv
            if not last:
                pa = _cat0([pa, zrow] if layer == 0 else [zrow, pa])
            return pa.astype(BF16)

        def pv(pr, v):
            return _dot(pr, v).astype(BF16)

        return prep_q, prep_kv, qk, pv

    def step(t, a_layers, b_layers, light=False, last=False, masked=True, deep=False,
             head_start=False, b_sched=(0, 2, 2, 2)):
        r0 = 0 if 0 in a_layers else SEG
        r1 = RT if 1 in a_layers else RL
        h = h_ref[SEG if light else r0:r1, :]
        if len(a_layers) == 2:
            prep_q, prep_kv, qk, pv = make_joint()
        else:
            prep_q, prep_kv, qk, pv = make_single(a_layers[0], last)

        def proj(i, p):
            r = _dot(h_ref[RL:RT, :] if (last and i == 0) else h, _unpack(wqkv_p[i, p]))
            if light:
                r = _cat0([pre_ref[i, p, pl.ds(pl.multiple_of((t - 2) * SEG, SEG), SEG), :], r])
            return r

        acc = [None]
        OLAG = 3 if len(a_layers) == 2 else 4

        def oproj(p, o):
            part = _dot(o, _unpack(wo_p[p]))
            acc[0] = part if acc[0] is None else acc[0] + part

        def xrows(seg):
            if isinstance(seg, int):
                return x_ref[seg * SEG:(seg + 1) * SEG, :].astype(F32)
            return x_ref[pl.ds(pl.multiple_of(seg * SEG, SEG), SEG), :].astype(F32)

        b_qk, b_v, b_o, b_fin = make_b(t, b_layers, masked)
        hooks = {p: [] for p in range(NP)}
        at, v0, dv, lag = b_sched
        hooks[at].append(b_qk)
        for j in range(NT):
            hooks[at + v0 + j * dv].insert(0, functools.partial(b_v, j)) if v0 else hooks[at].append(
                functools.partial(b_v, j))
        for j in range(NT):
            hooks[at + v0 + j * dv + lag].insert(0, functools.partial(b_o, j))
        x2 = x2_ref[...] if 1 in a_layers else None
        hooks[at + v0 + (NT - 1) * dv + lag].append(b_fin)

        if head_start:
            t0, t1 = (0, SEG) if 0 in a_layers else (RL, RT)
            m0, m1 = (SEG, r1) if 0 in a_layers else (SEG, RL)
            ht = h_ref[t0:t1, :]
            heads = [_dot(ht, _unpack(wqkv_p[i, 0])) for i in range(2)]
            hm = h_ref[m0:m1, :]
            rest = [_dot(hm, _unpack(wqkv_p[i, 0])) for i in range(2)]
            q, k = [_cat0([a, b] if 0 in a_layers else [b, a]) for a, b in zip(heads, rest)]
            q, k = prep_q(q), prep_kv(k)
        else:
            q = prep_q(proj(0, 0))
            k = prep_kv(proj(1, 0))
        vs = {0: prep_kv(proj(2, 0))}
        early_v = light or len(a_layers) == 1
        os_ = {}
        prs = {}

        def do_pv(p):
            os_[p] = pv(prs.pop(p), vs.pop(p))

        for p in range(NP):
            prs[p] = qk(q, k)
            if p + 1 < NP:
                q = prep_q(proj(0, p + 1))
                k = prep_kv(proj(1, p + 1))
                if early_v:
                    vs[p + 1] = prep_kv(proj(2, p + 1))
            else:
                if deep:
                    do_pv(p - 1)
                if 0 in a_layers:
                    nxt = min(t + 1, NSEG - 1) if isinstance(t, int) else jnp.minimum(t + 1, NSEG - 1)
                    h_ref[0:SEG, :] = _ln(xrows(nxt)).astype(BF16)
                for pp in range(p - OLAG, p - 1):
                    oproj(pp, os_.pop(pp))
            if not deep or p + 1 == NP:
                do_pv(p)
            elif p >= 1:
                do_pv(p - 1)
            if p + 1 < NP and not early_v:
                vs[p + 1] = prep_kv(proj(2, p + 1))
            for f in hooks[p]:
                f()
            if p >= OLAG and p + 1 < NP:
                oproj(p - OLAG, os_.pop(p - OLAG))
        oproj(NP - 2, os_.pop(NP - 2))
        oproj(NP - 1, os_.pop(NP - 1))
        a = acc[0]
        if 0 in a_layers:
            xa_ref[0:SEG, :] = xrows(t) + a[0:SEG]
        if last:
            xa_ref[SEG:2 * SEG, :] = x2 + a
            return
        if 1 in a_layers:
            xa_ref[SEG:2 * SEG, :] = x2 + a[RL - r0:RT - r0]
        mem1 = a[SEG - r0:RV - r0]
        mem2 = a[RV - r0:RL - r0] if 1 in a_layers else mem0
        h_ref[SEG:RL, :] = _cat0([mem1, mem2]).astype(BF16)

    def first_step():
        prep_q, prep_kv, qk, pv = make_single(0)

        RA = (RL + NPRE * SEG) // 32 * 16 + 16

        def wait_group(p):
            for cp in cp_group(p):
                cp.wait()

        def pair0(p, fine=False):
            ha = _unpack(hpre_ref[0:RA // 2, :])
            hb = _unpack(hpre_ref[RA // 2:, :])
            w = {}

            def load(i):
                if fine:
                    cp_fine(p, i).wait()
                w[i] = w_pairs[i][1][rows_of(p), :]
                wqkv_p[i, p] = _pack(w[i].T)

            def proj_a(i):
                r = _dot_nt(ha, w[i])
                pre_ref[i, p, 0:RA - RL, :] = r[RL:]
                return r[0:RL]

            def proj_b(i):
                pre_ref[i, p, RA - RL:, :] = _dot_nt(hb, w[i])

            if fine:
                load(0)
                q = prep_q(proj_a(0))
                proj_b(0)
                load(1)
                k = prep_kv(proj_a(1))
                proj_b(1)
                load(2)
                pr = qk(q, k)
                v = prep_kv(proj_a(2))
                proj_b(2)
                o_ref[p] = _pack(pv(pr, v))
                return
            for i in range(3):
                load(i)
            q = prep_q(proj_a(0))
            k = prep_kv(proj_a(1))
            v = prep_kv(proj_a(2))
            pr = qk(q, k)
            proj_b(0)
            proj_b(1)
            o_ref[p] = _pack(pv(pr, v))
            proj_b(2)

        def body1(p, carry):
            wait_group(p)
            pair0(p)
            return carry

        def body2(i, carry):
            wait_group(2 * i)
            wait_group(2 * i + 1)
            pair0(2 * i)
            pair0(2 * i + 1)
            return carry

        def body0(p, carry):
            pair0(p, fine=True)
            return carry

        lax.fori_loop(0, NFINE, body0, 0)
        lax.fori_loop(NFINE, 4, body1, 0)
        lax.fori_loop(2, NP // 2, body2, 0)
        cp_wo.wait()
        a = None
        for p in range(NP):
            w = wo_ref[sl(p), :]
            wo_p[p] = _pack(w)
            part = _dot(_unpack(o_ref[p]), w)
            a = part if a is None else a + part
        xa_ref[0:SEG, :] = x_ref[0:SEG, :].astype(F32) + a[0:SEG]
        h_ref[0:SEG, :] = _ln(x_ref[SEG:2 * SEG, :].astype(F32)).astype(BF16)
        h_ref[SEG:RL, :] = _cat0([a[SEG:RV], mem0]).astype(BF16)

    first_step()
    cp_x1.start()
    for cp in cp_b:
        cp.wait()
    for j in range(3):
        perm_qkv(j)
    perm_wo()
    step(1, (0,), (0,), deep=True, b_sched=(7, 2, 1, 1))

    def body_light(t, carry):
        step(t, (0, 1), (0, 1), light=True, b_sched=(0, 3, 2, 1))
        return carry

    lax.fori_loop(2, 2 + NPRE, body_light, 0)
    cp_x1.wait()

    T0 = 2 + NPRE
    NPAIR = (NSEG - T0) // 2

    def two_steps(t):
        step(t, (0, 1), (0, 1), masked=False)
        step(t + 1, (0, 1), (0, 1), masked=False, head_start=True)

    def body(i, carry):
        two_steps(T0 + 2 * i)
        return carry

    lax.fori_loop(0, NPAIR, body, 0)
    done = (T0 + 2 * NPAIR - 3) * SEG
    cp_o0 = pltpu.make_async_copy(out_ref.at[0:done], out_hbm.at[0:done], sem.at[6])
    cp_o0.start()
    for t in range(T0 + 2 * NPAIR, NSEG):
        step(t, (0, 1), (0, 1), masked=False)
    step(NSEG, (1,), (0, 1), masked=False, head_start=True)
    step(NSEG + 1, (1,), (1,), last=True, masked=False)
    cp_o1 = pltpu.make_async_copy(out_ref.at[done:S - SEG], out_hbm.at[done:S - SEG], sem.at[7])
    cp_o1.start()
    b_qk, b_v, b_o, b_fin = make_b(NSEG + 2, (1,), False)
    b_qk()
    for j in range(NT):
        b_v(j)
    for j in range(NT):
        b_o(j)
    b_fin()
    cp_o2 = pltpu.make_async_copy(out_ref.at[S - SEG:S], out_hbm.at[S - SEG:S], sem.at[0])
    cp_o2.start()
    cp_o0.wait()
    cp_o1.wait()
    cp_o2.wait()


def pallas_interleave_layers__memory_aug_recurrent_mem_tr__sliding_local_dilated__prompt_kernel(
    A_x: jax.Array,
    A_mem0: jax.Array,
    A_Wq: jax.Array,
    A_Wk: jax.Array,
    A_Wv: jax.Array,
    A_Wo: jax.Array,
    A_seg_len,
    B_x: jax.Array,
    B_wqkv: jax.Array,
    B_wo: jax.Array,
):
    B, S, D = A_x.shape
    H, DH = A_Wq.shape[1], A_Wq.shape[2]
    M = A_mem0.shape[1]
    SEG = A_seg_len if isinstance(A_seg_len, int) else 32
    assert B == 1 and M == 8 and SEG == 32 and DH == 192 and D == 640 and H % 2 == 0
    assert S % SEG == 0 and S // SEG >= NPRE + 4

    x = A_x.reshape(S, D)
    mem0 = A_mem0.reshape(M, D)
    wq = jnp.transpose(A_Wq, (1, 2, 0)).reshape(H * DH, D)
    wk = jnp.transpose(A_Wk, (1, 2, 0)).reshape(H * DH, D)
    wv = jnp.transpose(A_Wv, (1, 2, 0)).reshape(H * DH, D)
    wo = A_Wo.reshape(H * DH, D)

    hbm = pl.BlockSpec(memory_space=pl.ANY)
    out = pl.pallas_call(
        functools.partial(_kernel, S=S, D=D, H=H, DH=DH, M=M, SEG=SEG),
        out_shape=jax.ShapeDtypeStruct((S, D), A_x.dtype),
        in_specs=[hbm] * 8,
        out_specs=hbm,
        scratch_shapes=[
            pltpu.VMEM((M, D), BF16),
            pltpu.VMEM((S, D), BF16),
            pltpu.VMEM((S, D), BF16),
            pltpu.VMEM((H * DH, D), BF16),
            pltpu.VMEM((H * DH, D), BF16),
            pltpu.VMEM((H * DH, D), BF16),
            pltpu.VMEM((H * DH, D), BF16),
            pltpu.VMEM((3, D, D), BF16),
            pltpu.VMEM((D, D), BF16),
            pltpu.VMEM((3, H // 2, D // 2, 2 * DH), U32),
            pltpu.VMEM((H // 2, DH, D), U32),
            pltpu.VMEM((3 * D // 128, D // 2, 128), U32),
            pltpu.VMEM((D // 2, D), U32),
            pltpu.VMEM((2 * SEG + 2 * M, D), BF16),
            pltpu.VMEM((2 * SEG, D), F32),
            pltpu.VMEM((SEG, D), F32),
            pltpu.VMEM((2, 2 * D // 128, HIST, 128), F32),
            pltpu.VMEM(((SEG + 2 * M + NPRE * SEG) // 2, D), U32),
            pltpu.VMEM((3, H // 2, NPRE * SEG, 2 * DH), F32),
            pltpu.VMEM((H // 2, (SEG + 2 * M) // 2, 2 * DH), U32),
            pltpu.VMEM((4, D // 128, D + 24, 128), F32),
            pltpu.SemaphoreType.DMA((H // 2 + 3 * NFINE,)),
            pltpu.SemaphoreType.DMA((10,)),
        ],
        compiler_params=pltpu.CompilerParams(vmem_limit_bytes=120 * 1024 * 1024),
        name="pallas_wavefront",
    )(mem0, x, wq, wk, wv, wo, B_wqkv, B_wo)
    return out.reshape(B, S, D)
```

```python
import functools

import jax
import jax.numpy as jnp
from jax import lax
import jax.experimental.pallas as pl
import jax.experimental.pallas.tpu as pltpu

F32 = jnp.float32
BF16 = jnp.bfloat16
U32 = jnp.uint32

EPS = 1e-5
NEG = -1000000000.0
PADNEG = -3.0e38
B_HEADS = 32
B_WIN = 8
B_DIL = 2
NPRE = 9
NFINE = 2
HIST = 16


def _ln(x):
    m = jnp.mean(x, axis=-1, keepdims=True)
    xc = x - m
    v = jnp.mean(xc * xc, axis=-1, keepdims=True)
    return xc * lax.rsqrt(v + EPS)


def _dot_nt(a, b):
    return lax.dot_general(a, b, (((1,), (1,)), ((), ())), preferred_element_type=F32)


def _dot(a, b):
    return jnp.dot(a, b, preferred_element_type=F32)


def _pack(a):
    return pltpu.bitcast(a, U32)


def _unpack(a):
    return pltpu.bitcast(a, BF16)


def _cat0(xs):
    return jnp.concatenate(xs, axis=0)


def _cat1(xs):
    return jnp.concatenate(xs, axis=1)


def _kernel(mem0_hbm, x_hbm, wq_hbm, wk_hbm, wv_hbm, wo_hbm, bqkv_hbm, bwo_hbm,
            out_hbm,
            mem0_ref, x_ref, out_ref, wq_ref, wk_ref, wv_ref, wo_ref, bqkv_ref, bwo_ref,
            wqkv_p, wo_p, bqkv_p, bwo_p, h_ref, xa_ref, x2_ref, kv_ref, hpre_ref, pre_ref, o_ref, tmp_ref, wsem, sem,
            *, S, D, H, DH, M, SEG):
    NSEG = S // SEG
    PW = 2 * DH
    NP = H // 2
    RV = SEG + M
    RL = SEG + 2 * M
    RT = 2 * SEG + 2 * M
    a_scale = DH ** (-0.5)
    b_dh = D // B_HEADS
    b_scale = b_dh ** (-0.5)
    NT = D // 128
    X0 = (NPRE + 3) * SEG

    def sl(p):
        return slice(p * PW, (p + 1) * PW)

    cp_m = pltpu.make_async_copy(mem0_hbm, mem0_ref, sem.at[8])
    cp_x0 = pltpu.make_async_copy(x_hbm.at[0:X0], x_ref.at[0:X0], sem.at[0])
    cp_x1 = pltpu.make_async_copy(x_hbm.at[X0:S], x_ref.at[X0:S], sem.at[1])
    cp_b = [pltpu.make_async_copy(bqkv_hbm.at[:, j * D:(j + 1) * D], bqkv_ref.at[j], sem.at[2 + j])
            for j in range(3)]
    cp_b.append(pltpu.make_async_copy(bwo_hbm, bwo_ref, sem.at[5]))
    cp_wo = pltpu.make_async_copy(wo_hbm, wo_ref, sem.at[9])
    w_pairs = ((wq_hbm, wq_ref), (wk_hbm, wk_ref), (wv_hbm, wv_ref))

    def rows_of(p):
        return pl.ds(p * PW if isinstance(p, int) else pl.multiple_of(p * PW, 128), PW)

    def cp_fine(p, i):
        src, dst = w_pairs[i]
        return pltpu.make_async_copy(src.at[rows_of(p)], dst.at[rows_of(p)], wsem.at[NP + 3 * p + i])

    def cp_group(p):
        return [pltpu.make_async_copy(src.at[rows_of(p)], dst.at[rows_of(p)], wsem.at[p])
                for src, dst in w_pairs]

    def start_group(p, carry):
        for cp in cp_group(p):
            cp.start()

        @pl.when(p == NP - 1)
        def _():
            cp_wo.start()

        return carry

    firsts = [[cp_m, cp_x0]] + [[cp_fine(p, i)] for p in range(NFINE) for i in range(3)]

    def start_first(i, carry):
        for n, cps in enumerate(firsts):
            @pl.when(i == n)
            def _():
                for cp in cps:
                    cp.start()

        return carry

    lax.fori_loop(0, len(firsts), start_first, 0)
    lax.fori_loop(NFINE, NP, start_group, 0)
    for cp in cp_b:
        cp.start()

    xa_ref[...] = jnp.zeros(xa_ref.shape, F32)
    kv_ref[...] = jnp.zeros(kv_ref.shape, F32)
    cp_m.wait()
    cp_x0.wait()
    mem0 = mem0_ref[...].astype(F32)
    h0 = _ln(x_ref[0:SEG, :].astype(F32))
    hpre_ref[0:RL // 2, :] = _pack(_cat0([h0, mem0, mem0]).astype(BF16))
    for i in range(NPRE):
        hi = _ln(x_ref[(2 + i) * SEG:(3 + i) * SEG, :].astype(F32)).astype(BF16)
        hpre_ref[(RL + i * SEG) // 2:(RL + (i + 1) * SEG) // 2, :] = _pack(hi)

    def perm_rows(a, slot):
        a = a.astype(F32)
        for m in range(NT):
            tmp_ref[slot, m, 0:D, :] = a[:, m * 128:(m + 1) * 128]
        return _cat1([_cat0([tmp_ref[slot, m, pl.ds(d, B_HEADS, stride=b_dh), :] for d in range(b_dh)])
                      for m in range(NT)]).astype(BF16)

    def perm_qkv(j):
        wp = perm_rows(bqkv_ref[j].T, j).T
        for c in range(NT):
            bqkv_p[j * NT + c] = _pack(wp[:, c * 128:(c + 1) * 128])

    def perm_wo():
        bwo_p[...] = _pack(perm_rows(bwo_ref[...], 3))

    def make_b(t, layers, masked):
        xb = xa_ref[layers[0] * SEG:(layers[-1] + 1) * SEG, :]
        hb = _ln(xb).astype(BF16)
        st = {'y': xb, 'p': []}

        def windows(l, i, j, a):
            cur = a[i * SEG:(i + 1) * SEG]
            blk = _cat0([kv_ref[l, j], cur])
            kv_ref[l, j] = cur[SEG - HIST:SEG]
            rolled = [blk] + [pltpu.roll(blk, sh, 0) for sh in range(B_DIL, 8, B_DIL)]
            res = []
            for w in range(B_WIN):
                hi, lo_ = divmod(B_DIL * w, 8)
                o = HIST - 8 * hi
                res.append(rolled[lo_ // B_DIL][o:o + SEG])
            return res

        def qk():
            qs, ks = [], []
            for j in range(NT):
                qs.append(_dot(hb, _unpack(bqkv_p[j])))
                ks.append(_dot(hb, _unpack(bqkv_p[NT + j])))
            for i, l in enumerate(layers):
                ss = None
                for j in range(NT):
                    q = qs[j][i * SEG:(i + 1) * SEG] * b_scale
                    terms = [q * kw for kw in windows(l, i, j, ks[j])]
                    ss = terms if ss is None else [a + b for a, b in zip(ss, terms)]
                pos = (t - 1 - 2 * l) * SEG + lax.broadcasted_iota(jnp.int32, (SEG, 128), 0)
                logits = []
                for w, s in enumerate(ss):
                    s = s + pltpu.roll(s, 64, 1)
                    s = s + pltpu.roll(s, 32, 1)
                    logits.append(jnp.where(pos >= B_DIL * w, s, NEG) if masked else s)
                m = logits[0]
                for w in range(1, B_WIN):
                    m = jnp.maximum(m, logits[w])
                es = [jnp.exp(lg - m) for lg in logits]
                den = es[0]
                for w in range(1, B_WIN):
                    den = den + es[w]
                st['p'].append((es, 1.0 / den))

        def v_stage(j):
            vj = _dot(hb, _unpack(bqkv_p[2 * NT + j]))
            outs = []
            for i, l in enumerate(layers):
                es, inv = st['p'][i]
                vw = windows(l, i, NT + j, vj)
                acc = es[0] * vw[0]
                for w in range(1, B_WIN):
                    acc = acc + es[w] * vw[w]
                outs.append(acc * inv)
            st['o', j] = _cat0(outs).astype(BF16)

        def o_stage(j):
            st['y'] = st['y'] + _dot(st.pop(('o', j)), _unpack(bwo_p[j * 64:(j + 1) * 64, :]))

        def fin():
            for i, l in enumerate(layers):
                yl = st['y'][i * SEG:(i + 1) * SEG]
                if l == 0:
                    x2_ref[...] = yl
                    h_ref[RL:RT, :] = _ln(yl).astype(BF16)
                else:
                    if isinstance(t, int):
                        row = (t - 3) * SEG
                    else:
                        row = pl.multiple_of(jnp.maximum(t - 3, 0) * SEG, SEG)
                    out_ref[pl.ds(row, SEG), :] = yl.astype(out_ref.dtype)

        return qk, v_stage, o_stage, fin

    def softmax2(s, first, valid, fill):
        s = jnp.where(valid, s * a_scale, fill)
        m1 = jnp.max(jnp.where(first, s, PADNEG), axis=-1, keepdims=True)
        m2 = jnp.max(jnp.where(first, PADNEG, s), axis=-1, keepdims=True)
        e = jnp.exp(s - jnp.where(first, m1, m2))
        e1 = jnp.where(first, e, 0.0)
        e2 = jnp.where(first, 0.0, e)
        l1 = jnp.sum(e1, axis=-1, keepdims=True)
        l2 = jnp.sum(e2, axis=-1, keepdims=True)
        inv = 1.0 / jnp.where(first, l1, l2)
        return e, e1, e2, inv

    def make_joint():
        rr = lax.broadcasted_iota(jnp.int32, (RT, 128), 0)
        cc = lax.broadcasted_iota(jnp.int32, (RT, 128), 1)
        lay1 = rr < RV
        first = cc < jnp.where(lay1, RL, RT)
        key = jnp.where(first, cc, cc - RL)
        exists = jnp.where(lay1, RV - 1 - key, key - RV) >= 0
        allowed = (key <= rr) | (lay1 & (key >= SEG)) | ((rr >= RV) & (rr < RL))
        valid = exists & allowed
        fill = jnp.where(exists, NEG, PADNEG)
        lo = cc < (DH - 128)
        z48 = jnp.zeros((128 - RT, 128), F32)
        z32 = jnp.zeros((128 - 2 * RL, 128), F32)

        def prep_q(a):
            return (a[:, 0:128].astype(BF16), a[0:RL, 128:256].astype(BF16),
                    a[SEG:RT, 128:256].astype(BF16), a[:, 256:384].astype(BF16))

        def prep_kv(a):
            mid = a[:, 128:256]
            tlo = jnp.where(lo, mid, 0.0)
            thi = jnp.where(lo, 0.0, mid)
            return (_cat0([a[:, 0:128], z48]).astype(BF16),
                    _cat0([tlo[0:RL], thi[0:RL], z32]).astype(BF16),
                    _cat0([z32, tlo[SEG:RT], thi[SEG:RT]]).astype(BF16),
                    _cat0([z48, a[:, 256:384]]).astype(BF16))

        def qk(q, k):
            t0 = _dot_nt(q[0], k[0])
            t2 = _dot_nt(q[3], k[3])
            t1a = _dot_nt(q[1], k[1])
            t1b = _dot_nt(q[2], k[2])
            s = jnp.where(first, t0, t2) + _cat0([t1a[0:RV], t1b[M:RL]])
            e, e1, e2, inv = softmax2(s, first, valid, fill)
            pa = e * inv
            return ((e1 * inv).astype(BF16), pa[0:RL].astype(BF16),
                    pa[SEG:RT].astype(BF16), (e2 * inv).astype(BF16))

        def pv(pr, v):
            o0 = _dot(pr[0], v[0])
            o2 = _dot(pr[3], v[3])
            o1a = _dot(pr[1], v[1])
            o1b = _dot(pr[2], v[2])
            return _cat1([o0, _cat0([o1a[0:RV], o1b[M:RL]]), o2]).astype(BF16)

        return prep_q, prep_kv, qk, pv

    def make_single(layer, last=False):
        nq = SEG if last else RV
        rr = lax.broadcasted_iota(jnp.int32, (nq, 2 * RL), 0) + (M if last else 0)
        cc = lax.broadcasted_iota(jnp.int32, (nq, 2 * RL), 1)
        first = cc < RL
        kc = jnp.where(first, cc, cc - RL)
        if layer == 0:
            exists = kc < RV
            valid = exists & ((kc >= SEG) | (kc <= rr))
            r0 = 0
        else:
            exists = kc >= M
            valid = exists & ((rr < M) | (kc - M <= rr))
            r0 = M
        fill = jnp.where(exists, NEG, PADNEG)
        lo = lax.broadcasted_iota(jnp.int32, (RL, PW), 1) < DH
        zrow = jnp.zeros((M, 2 * RL), F32)

        def prep_q(a):
            return a.astype(BF16)

        def prep_kv(a):
            return _cat0([jnp.where(lo, a, 0.0), jnp.where(lo, 0.0, a)]).astype(BF16)

        def qk(q, k):
            s = _dot_nt(q, k)
            if not last:
                s = s[r0:r0 + RV]
            e, _, _, inv = softmax2(s, first, valid, fill)
            pa = e * inv
            if not last:
                pa = _cat0([pa, zrow] if layer == 0 else [zrow, pa])
            return pa.astype(BF16)

        def pv(pr, v):
            return _dot(pr, v).astype(BF16)

        return prep_q, prep_kv, qk, pv

    def step(t, a_layers, b_layers, light=False, last=False, masked=True, deep=False,
             head_start=False, b_sched=(0, 2, 2, 2)):
        r0 = 0 if 0 in a_layers else SEG
        r1 = RT if 1 in a_layers else RL
        h = h_ref[SEG if light else r0:r1, :]
        if len(a_layers) == 2:
            prep_q, prep_kv, qk, pv = make_joint()
        else:
            prep_q, prep_kv, qk, pv = make_single(a_layers[0], last)

        def proj(i, p):
            r = _dot(h_ref[RL:RT, :] if (last and i == 0) else h, _unpack(wqkv_p[i, p]))
            if light:
                r = _cat0([pre_ref[i, p, pl.ds(pl.multiple_of((t - 2) * SEG, SEG), SEG), :], r])
            return r

        acc = [None]
        OLAG = 3 if len(a_layers) == 2 else 4

        def oproj(p, o):
            part = _dot(o, _unpack(wo_p[p]))
            acc[0] = part if acc[0] is None else acc[0] + part

        def xrows(seg):
            if isinstance(seg, int):
                return x_ref[seg * SEG:(seg + 1) * SEG, :].astype(F32)
            return x_ref[pl.ds(pl.multiple_of(seg * SEG, SEG), SEG), :].astype(F32)

        hooks = {p: [] for p in range(NP)}
        if b_layers:
            b_qk, b_v, b_o, b_fin = make_b(t, b_layers, masked)
            at, v0, dv, lag = b_sched
            for j in range(NT):
                hooks[at + v0 + j * dv + lag].append(functools.partial(b_o, j))
            hooks[at + v0 + (NT - 1) * dv + lag].append(b_fin)
            for j in range(NT):
                hooks[at + v0 + j * dv].append(functools.partial(b_v, j))
            hooks[at].append(b_qk)
        x2 = x2_ref[...] if 1 in a_layers else None

        if head_start:
            t0, t1 = (0, SEG) if 0 in a_layers else (RL, RT)
            m0, m1 = (SEG, r1) if 0 in a_layers else (SEG, RL)
            ht = h_ref[t0:t1, :]
            heads = [_dot(ht, _unpack(wqkv_p[i, 0])) for i in range(2)]
            hm = h_ref[m0:m1, :]
            rest = [_dot(hm, _unpack(wqkv_p[i, 0])) for i in range(2)]
            q, k = [_cat0([a, b] if 0 in a_layers else [b, a]) for a, b in zip(heads, rest)]
            q, k = prep_q(q), prep_kv(k)
        else:
            q = prep_q(proj(0, 0))
            k = prep_kv(proj(1, 0))
        vs = {0: prep_kv(proj(2, 0))}
        early_v = light or len(a_layers) == 1
        os_ = {}
        prs = {}

        def do_pv(p):
            os_[p] = pv(prs.pop(p), vs.pop(p))

        for p in range(NP):
            prs[p] = qk(q, k)
            if p + 1 < NP:
                q = prep_q(proj(0, p + 1))
                k = prep_kv(proj(1, p + 1))
                if early_v:
                    vs[p + 1] = prep_kv(proj(2, p + 1))
            else:
                if deep:
                    do_pv(p - 1)
                if 0 in a_layers:
                    nxt = min(t + 1, NSEG - 1) if isinstance(t, int) else jnp.minimum(t + 1, NSEG - 1)
                    h_ref[0:SEG, :] = _ln(xrows(nxt)).astype(BF16)
                for pp in range(p - OLAG, p - 1):
                    oproj(pp, os_.pop(pp))
            if not deep or p + 1 == NP:
                do_pv(p)
            elif p >= 1:
                do_pv(p - 1)
            if p + 1 < NP and not early_v:
                vs[p + 1] = prep_kv(proj(2, p + 1))
            for f in hooks[p]:
                f()
            if p >= OLAG and p + 1 < NP:
                oproj(p - OLAG, os_.pop(p - OLAG))
        oproj(NP - 2, os_.pop(NP - 2))
        oproj(NP - 1, os_.pop(NP - 1))
        a = acc[0]
        if 0 in a_layers:
            xa_ref[0:SEG, :] = xrows(t) + a[0:SEG]
        if last:
            xa_ref[SEG:2 * SEG, :] = x2 + a
            return
        if 1 in a_layers:
            xa_ref[SEG:2 * SEG, :] = x2 + a[RL - r0:RT - r0]
        mem1 = a[SEG - r0:RV - r0]
        mem2 = a[RV - r0:RL - r0] if 1 in a_layers else mem0
        h_ref[SEG:RL, :] = _cat0([mem1, mem2]).astype(BF16)

    def first_step():
        prep_q, prep_kv, qk, pv = make_single(0)

        RA = (RL + NPRE * SEG) // 32 * 16 + 16

        def wait_group(p):
            for cp in cp_group(p):
                cp.wait()

        def pair0(p, fine=False):
            ha = _unpack(hpre_ref[0:RA // 2, :])
            hb = _unpack(hpre_ref[RA // 2:, :])
            w = {}

            def load(i):
                if fine:
                    cp_fine(p, i).wait()
                w[i] = w_pairs[i][1][rows_of(p), :]
                wqkv_p[i, p] = _pack(w[i].T)

            def proj_a(i):
                r = _dot_nt(ha, w[i])
                pre_ref[i, p, 0:RA - RL, :] = r[RL:]
                return r[0:RL]

            def proj_b(i):
                pre_ref[i, p, RA - RL:, :] = _dot_nt(hb, w[i])

            if fine:
                load(0)
                q = prep_q(proj_a(0))
                proj_b(0)
                load(1)
                k = prep_kv(proj_a(1))
                proj_b(1)
                load(2)
                pr = qk(q, k)
                v = prep_kv(proj_a(2))
                proj_b(2)
                o_ref[p] = _pack(pv(pr, v))
                return
            for i in range(3):
                load(i)
            q = prep_q(proj_a(0))
            k = prep_kv(proj_a(1))
            v = prep_kv(proj_a(2))
            pr = qk(q, k)
            proj_b(0)
            proj_b(1)
            o_ref[p] = _pack(pv(pr, v))
            proj_b(2)

        def body1(p, carry):
            wait_group(p)
            pair0(p)
            return carry

        def body2(i, carry):
            wait_group(2 * i)
            wait_group(2 * i + 1)
            pair0(2 * i)
            pair0(2 * i + 1)
            return carry

        def body0(p, carry):
            pair0(p, fine=True)
            return carry

        lax.fori_loop(0, NFINE, body0, 0)
        lax.fori_loop(NFINE, 4, body1, 0)
        lax.fori_loop(2, NP // 2, body2, 0)
        cp_wo.wait()
        a = None
        for p in range(NP):
            w = wo_ref[sl(p), :]
            wo_p[p] = _pack(w)
            part = _dot(_unpack(o_ref[p]), w)
            a = part if a is None else a + part
        xa_ref[0:SEG, :] = x_ref[0:SEG, :].astype(F32) + a[0:SEG]
        h_ref[0:SEG, :] = _ln(x_ref[SEG:2 * SEG, :].astype(F32)).astype(BF16)
        h_ref[SEG:RL, :] = _cat0([a[SEG:RV], mem0]).astype(BF16)

    first_step()
    cp_x1.start()
    for cp in cp_b:
        cp.wait()
    for j in range(3):
        perm_qkv(j)
    perm_wo()
    step(1, (0,), (0,), deep=True, b_sched=(7, 2, 1, 1))

    def body_light(t, carry):
        step(t, (0, 1), (0, 1), light=True, b_sched=(0, 3, 2, 1))
        return carry

    lax.fori_loop(2, 2 + NPRE, body_light, 0)
    cp_x1.wait()

    T0 = 2 + NPRE
    NPAIR = (NSEG - T0) // 2

    def two_steps(t):
        step(t, (0, 1), (0, 1), masked=False)
        step(t + 1, (0, 1), (0, 1), masked=False, head_start=True)

    def body(i, carry):
        two_steps(T0 + 2 * i)
        return carry

    lax.fori_loop(0, NPAIR, body, 0)
    done = (T0 + 2 * NPAIR - 3) * SEG
    cp_o0 = pltpu.make_async_copy(out_ref.at[0:done], out_hbm.at[0:done], sem.at[6])
    cp_o0.start()
    for t in range(T0 + 2 * NPAIR, NSEG):
        step(t, (0, 1), (0, 1), masked=False)
    step(NSEG, (1,), (0, 1), masked=False, head_start=True)
    cp_o1 = pltpu.make_async_copy(out_ref.at[done:S - 2 * SEG], out_hbm.at[done:S - 2 * SEG], sem.at[7])
    cp_o1.start()
    tails = [make_b(NSEG + 1, (1,), False)]
    step(NSEG + 1, (1,), (), last=True)
    tails.append(make_b(NSEG + 2, (1,), False))
    for b_qk, b_v, _, _ in tails:
        b_qk()
        for j in range(NT):
            b_v(j)
    for _, _, b_o, b_fin in tails:
        for j in range(NT):
            b_o(j)
        b_fin()
    cp_o2 = pltpu.make_async_copy(out_ref.at[S - 2 * SEG:S], out_hbm.at[S - 2 * SEG:S], sem.at[0])
    cp_o2.start()
    cp_o0.wait()
    cp_o1.wait()
    cp_o2.wait()


def pallas_interleave_layers__memory_aug_recurrent_mem_tr__sliding_local_dilated__prompt_kernel(
    A_x: jax.Array,
    A_mem0: jax.Array,
    A_Wq: jax.Array,
    A_Wk: jax.Array,
    A_Wv: jax.Array,
    A_Wo: jax.Array,
    A_seg_len,
    B_x: jax.Array,
    B_wqkv: jax.Array,
    B_wo: jax.Array,
):
    B, S, D = A_x.shape
    H, DH = A_Wq.shape[1], A_Wq.shape[2]
    M = A_mem0.shape[1]
    SEG = A_seg_len if isinstance(A_seg_len, int) else 32
    assert B == 1 and M == 8 and SEG == 32 and DH == 192 and D == 640 and H % 2 == 0
    assert S % SEG == 0 and S // SEG >= NPRE + 4

    x = A_x.reshape(S, D)
    mem0 = A_mem0.reshape(M, D)
    wq = jnp.transpose(A_Wq, (1, 2, 0)).reshape(H * DH, D)
    wk = jnp.transpose(A_Wk, (1, 2, 0)).reshape(H * DH, D)
    wv = jnp.transpose(A_Wv, (1, 2, 0)).reshape(H * DH, D)
    wo = A_Wo.reshape(H * DH, D)

    hbm = pl.BlockSpec(memory_space=pl.ANY)
    out = pl.pallas_call(
        functools.partial(_kernel, S=S, D=D, H=H, DH=DH, M=M, SEG=SEG),
        out_shape=jax.ShapeDtypeStruct((S, D), A_x.dtype),
        in_specs=[hbm] * 8,
        out_specs=hbm,
        scratch_shapes=[
            pltpu.VMEM((M, D), BF16),
            pltpu.VMEM((S, D), BF16),
            pltpu.VMEM((S, D), BF16),
            pltpu.VMEM((H * DH, D), BF16),
            pltpu.VMEM((H * DH, D), BF16),
            pltpu.VMEM((H * DH, D), BF16),
            pltpu.VMEM((H * DH, D), BF16),
            pltpu.VMEM((3, D, D), BF16),
            pltpu.VMEM((D, D), BF16),
            pltpu.VMEM((3, H // 2, D // 2, 2 * DH), U32),
            pltpu.VMEM((H // 2, DH, D), U32),
            pltpu.VMEM((3 * D // 128, D // 2, 128), U32),
            pltpu.VMEM((D // 2, D), U32),
            pltpu.VMEM((2 * SEG + 2 * M, D), BF16),
            pltpu.VMEM((2 * SEG, D), F32),
            pltpu.VMEM((SEG, D), F32),
            pltpu.VMEM((2, 2 * D // 128, HIST, 128), F32),
            pltpu.VMEM(((SEG + 2 * M + NPRE * SEG) // 2, D), U32),
            pltpu.VMEM((3, H // 2, NPRE * SEG, 2 * DH), F32),
            pltpu.VMEM((H // 2, (SEG + 2 * M) // 2, 2 * DH), U32),
            pltpu.VMEM((4, D // 128, D + 24, 128), F32),
            pltpu.SemaphoreType.DMA((H // 2 + 3 * NFINE,)),
            pltpu.SemaphoreType.DMA((10,)),
        ],
        compiler_params=pltpu.CompilerParams(vmem_limit_bytes=120 * 1024 * 1024),
        name="pallas_wavefront",
    )(mem0, x, wq, wk, wv, wo, B_wqkv, B_wo)
    return out.reshape(B, S, D)
```

```python
import functools

import jax
import jax.numpy as jnp
from jax import lax
import jax.experimental.pallas as pl
import jax.experimental.pallas.tpu as pltpu

F32 = jnp.float32
BF16 = jnp.bfloat16
U32 = jnp.uint32

EPS = 1e-5
NEG = -1000000000.0
PADNEG = -3.0e38
B_HEADS = 32
B_WIN = 8
B_DIL = 2
NPRE = 9
NFINE = 2
HIST = 16


def _ln(x):
    m = jnp.mean(x, axis=-1, keepdims=True)
    xc = x - m
    v = jnp.mean(xc * xc, axis=-1, keepdims=True)
    return xc * lax.rsqrt(v + EPS)


def _dot_nt(a, b):
    return lax.dot_general(a, b, (((1,), (1,)), ((), ())), precision=lax.Precision.DEFAULT,
                           preferred_element_type=F32)


def _dot(a, b):
    return lax.dot_general(a, b, (((1,), (0,)), ((), ())), precision=lax.Precision.DEFAULT,
                           preferred_element_type=F32)


def _pack(a):
    return pltpu.bitcast(a, U32)


def _unpack(a):
    return pltpu.bitcast(a, BF16)


def _cat0(xs):
    return jnp.concatenate(xs, axis=0)


def _cat1(xs):
    return jnp.concatenate(xs, axis=1)


def _kernel(mem0_hbm, x_hbm, wq_hbm, wk_hbm, wv_hbm, wo_hbm, bqkv_hbm, bwo_hbm,
            out_hbm,
            mem0_ref, x_ref, out_ref, wq_ref, wk_ref, wv_ref, wo_ref, bqkv_ref, bwo_ref,
            wqkv_p, wo_p, bqkv_p, bwo_p, h_ref, xa_ref, x2_ref, kv_ref, hpre_ref, pre_ref, o_ref, tmp_ref, wsem, sem,
            *, S, D, H, DH, M, SEG):
    NSEG = S // SEG
    PW = 2 * DH
    NP = H // 2
    RV = SEG + M
    RL = SEG + 2 * M
    RT = 2 * SEG + 2 * M
    a_scale = DH ** (-0.5)
    b_dh = D // B_HEADS
    b_scale = b_dh ** (-0.5)
    NT = D // 128
    X0 = (NPRE + 3) * SEG

    def sl(p):
        return slice(p * PW, (p + 1) * PW)

    cp_m = pltpu.make_async_copy(mem0_hbm, mem0_ref, sem.at[8])
    cp_x0 = pltpu.make_async_copy(x_hbm.at[0:X0], x_ref.at[0:X0], sem.at[0])
    cp_x1 = pltpu.make_async_copy(x_hbm.at[X0:S], x_ref.at[X0:S], sem.at[1])
    cp_b = [pltpu.make_async_copy(bqkv_hbm.at[:, j * D:(j + 1) * D], bqkv_ref.at[j], sem.at[2 + j])
            for j in range(3)]
    cp_b.append(pltpu.make_async_copy(bwo_hbm, bwo_ref, sem.at[5]))
    cp_wo = pltpu.make_async_copy(wo_hbm, wo_ref, sem.at[9])
    w_pairs = ((wq_hbm, wq_ref), (wk_hbm, wk_ref), (wv_hbm, wv_ref))

    def rows_of(p):
        return pl.ds(p * PW if isinstance(p, int) else pl.multiple_of(p * PW, 128), PW)

    def cp_fine(p, i):
        src, dst = w_pairs[i]
        return pltpu.make_async_copy(src.at[rows_of(p)], dst.at[rows_of(p)], wsem.at[NP + 3 * p + i])

    def cp_group(p):
        return [pltpu.make_async_copy(src.at[rows_of(p)], dst.at[rows_of(p)], wsem.at[p])
                for src, dst in w_pairs]

    def start_group(p, carry):
        for cp in cp_group(p):
            cp.start()

        @pl.when(p == NP - 1)
        def _():
            cp_wo.start()

        return carry

    firsts = [[cp_m, cp_x0]] + [[cp_fine(p, i)] for p in range(NFINE) for i in range(3)]

    def start_first(i, carry):
        for n, cps in enumerate(firsts):
            @pl.when(i == n)
            def _():
                for cp in cps:
                    cp.start()

        return carry

    lax.fori_loop(0, len(firsts), start_first, 0)
    lax.fori_loop(NFINE, NP, start_group, 0)
    for cp in cp_b:
        cp.start()

    xa_ref[...] = jnp.zeros(xa_ref.shape, F32)
    kv_ref[...] = jnp.zeros(kv_ref.shape, F32)
    cp_m.wait()
    cp_x0.wait()
    mem0 = mem0_ref[...].astype(F32)
    h0 = _ln(x_ref[0:SEG, :].astype(F32))
    hpre_ref[0:RL // 2, :] = _pack(_cat0([h0, mem0, mem0]).astype(BF16))
    for i in range(NPRE):
        hi = _ln(x_ref[(2 + i) * SEG:(3 + i) * SEG, :].astype(F32)).astype(BF16)
        hpre_ref[(RL + i * SEG) // 2:(RL + (i + 1) * SEG) // 2, :] = _pack(hi)

    def perm_rows(a, slot):
        a = a.astype(F32)
        for m in range(NT):
            tmp_ref[slot, m, 0:D, :] = a[:, m * 128:(m + 1) * 128]
        return _cat1([_cat0([tmp_ref[slot, m, pl.ds(d, B_HEADS, stride=b_dh), :] for d in range(b_dh)])
                      for m in range(NT)]).astype(BF16)

    def perm_qkv(j):
        wp = perm_rows(bqkv_ref[j].T, j).T
        for c in range(NT):
            bqkv_p[j * NT + c] = _pack(wp[:, c * 128:(c + 1) * 128])

    def perm_wo():
        bwo_p[...] = _pack(perm_rows(bwo_ref[...], 3))

    def make_b(t, layers, masked):
        xb = xa_ref[layers[0] * SEG:(layers[-1] + 1) * SEG, :]
        hb = _ln(xb).astype(BF16)
        st = {'y': xb, 'p': []}

        def windows(l, i, j, a):
            cur = a[i * SEG:(i + 1) * SEG]
            blk = _cat0([kv_ref[l, j], cur])
            kv_ref[l, j] = cur[SEG - HIST:SEG]
            rolled = [blk] + [pltpu.roll(blk, sh, 0) for sh in range(B_DIL, 8, B_DIL)]
            res = []
            for w in range(B_WIN):
                hi, lo_ = divmod(B_DIL * w, 8)
                o = HIST - 8 * hi
                res.append(rolled[lo_ // B_DIL][o:o + SEG])
            return res

        def qk():
            qs, ks = [], []
            for j in range(NT):
                qs.append(_dot(hb, _unpack(bqkv_p[j])))
                ks.append(_dot(hb, _unpack(bqkv_p[NT + j])))
            for i, l in enumerate(layers):
                ss = None
                for j in range(NT):
                    q = qs[j][i * SEG:(i + 1) * SEG] * b_scale
                    terms = [q * kw for kw in windows(l, i, j, ks[j])]
                    ss = terms if ss is None else [a + b for a, b in zip(ss, terms)]
                pos = (t - 1 - 2 * l) * SEG + lax.broadcasted_iota(jnp.int32, (SEG, 128), 0)
                logits = []
                for w, s in enumerate(ss):
                    s = s + pltpu.roll(s, 64, 1)
                    s = s + pltpu.roll(s, 32, 1)
                    logits.append(jnp.where(pos >= B_DIL * w, s, NEG) if masked else s)
                m = logits[0]
                for w in range(1, B_WIN):
                    m = jnp.maximum(m, logits[w])
                es = [jnp.exp(lg - m) for lg in logits]
                den = es[0]
                for w in range(1, B_WIN):
                    den = den + es[w]
                st['p'].append((es, 1.0 / den))

        def v_stage(j):
            vj = _dot(hb, _unpack(bqkv_p[2 * NT + j]))
            outs = []
            for i, l in enumerate(layers):
                es, inv = st['p'][i]
                vw = windows(l, i, NT + j, vj)
                acc = es[0] * vw[0]
                for w in range(1, B_WIN):
                    acc = acc + es[w] * vw[w]
                outs.append(acc * inv)
            st['o', j] = _cat0(outs).astype(BF16)

        def o_stage(j):
            st['y'] = st['y'] + _dot(st.pop(('o', j)), _unpack(bwo_p[j * 64:(j + 1) * 64, :]))

        def fin():
            for i, l in enumerate(layers):
                yl = st['y'][i * SEG:(i + 1) * SEG]
                if l == 0:
                    x2_ref[...] = yl
                    h_ref[RL:RT, :] = _ln(yl).astype(BF16)
                else:
                    if isinstance(t, int):
                        row = (t - 3) * SEG
                    else:
                        row = pl.multiple_of(jnp.maximum(t - 3, 0) * SEG, SEG)
                    out_ref[pl.ds(row, SEG), :] = yl.astype(out_ref.dtype)

        return qk, v_stage, o_stage, fin

    def softmax2(s, first, valid, fill):
        s = jnp.where(valid, s * a_scale, fill)
        m1 = jnp.max(jnp.where(first, s, PADNEG), axis=-1, keepdims=True)
        m2 = jnp.max(jnp.where(first, PADNEG, s), axis=-1, keepdims=True)
        e = jnp.exp(s - jnp.where(first, m1, m2))
        e1 = jnp.where(first, e, 0.0)
        e2 = jnp.where(first, 0.0, e)
        l1 = jnp.sum(e1, axis=-1, keepdims=True)
        l2 = jnp.sum(e2, axis=-1, keepdims=True)
        inv = 1.0 / jnp.where(first, l1, l2)
        return e, e1, e2, inv

    def make_joint():
        rr = lax.broadcasted_iota(jnp.int32, (RT, 128), 0)
        cc = lax.broadcasted_iota(jnp.int32, (RT, 128), 1)
        lay1 = rr < RV
        first = cc < jnp.where(lay1, RL, RT)
        key = jnp.where(first, cc, cc - RL)
        exists = jnp.where(lay1, RV - 1 - key, key - RV) >= 0
        allowed = (key <= rr) | (lay1 & (key >= SEG)) | ((rr >= RV) & (rr < RL))
        valid = exists & allowed
        fill = jnp.where(exists, NEG, PADNEG)
        lo = cc < (DH - 128)
        z48 = jnp.zeros((128 - RT, 128), F32)
        z32 = jnp.zeros((128 - 2 * RL, 128), F32)

        def prep_q(a):
            return (a[:, 0:128].astype(BF16), a[0:RV, 128:256], a[RV:RT, 128:256], a[:, 256:384].astype(BF16))

        def prep_kv(a):
            mid = a[:, 128:256]
            tlo = jnp.where(lo, mid, 0.0)
            thi = jnp.where(lo, 0.0, mid)
            return (_cat0([a[:, 0:128], z48]).astype(BF16),
                    _cat0([tlo[0:RL], thi[0:RL], z32]).astype(BF16),
                    _cat0([z32, tlo[SEG:RT], thi[SEG:RT]]).astype(BF16),
                    _cat0([z48, a[:, 256:384]]).astype(BF16))

        def qk(q, k):
            t0 = _dot_nt(q[0], k[0])
            t2 = _dot_nt(q[3], k[3])
            t1a = _dot_nt(q[1], k[1])
            t1b = _dot_nt(q[2], k[2])
            s = jnp.where(first, t0, t2) + _cat0([t1a, t1b])
            e, e1, e2, inv = softmax2(s, first, valid, fill)
            pa = e * inv
            return (e1 * inv).astype(BF16), pa[0:RV], pa[RV:RT], (e2 * inv).astype(BF16)

        def pv(pr, v):
            o0 = _dot(pr[0], v[0])
            o2 = _dot(pr[3], v[3])
            o1a = _dot(pr[1], v[1])
            o1b = _dot(pr[2], v[2])
            return _cat1([o0, _cat0([o1a, o1b]), o2]).astype(BF16)

        return prep_q, prep_kv, qk, pv

    def make_single(layer, last=False):
        nq = SEG if last else RV
        rr = lax.broadcasted_iota(jnp.int32, (nq, 2 * RL), 0) + (M if last else 0)
        cc = lax.broadcasted_iota(jnp.int32, (nq, 2 * RL), 1)
        first = cc < RL
        kc = jnp.where(first, cc, cc - RL)
        if layer == 0:
            exists = kc < RV
            valid = exists & ((kc >= SEG) | (kc <= rr))
            r0 = 0
        else:
            exists = kc >= M
            valid = exists & ((rr < M) | (kc - M <= rr))
            r0 = M
        fill = jnp.where(exists, NEG, PADNEG)
        lo = lax.broadcasted_iota(jnp.int32, (RL, PW), 1) < DH
        zrow = jnp.zeros((M, 2 * RL), F32)

        def prep_q(a):
            return a.astype(BF16)

        def prep_kv(a):
            return _cat0([jnp.where(lo, a, 0.0), jnp.where(lo, 0.0, a)]).astype(BF16)

        def qk(q, k):
            s = _dot_nt(q, k)
            if not last:
                s = s[r0:r0 + RV]
            e, _, _, inv = softmax2(s, first, valid, fill)
            pa = e * inv
            if not last:
                pa = _cat0([pa, zrow] if layer == 0 else [zrow, pa])
            return pa.astype(BF16)

        def pv(pr, v):
            return _dot(pr, v).astype(BF16)

        return prep_q, prep_kv, qk, pv

    def step(t, a_layers, b_layers, light=False, last=False, masked=True, deep=False,
             head_start=False, b_sched=(0, 2, 2, 2)):
        r0 = 0 if 0 in a_layers else SEG
        r1 = RT if 1 in a_layers else RL
        h = h_ref[SEG if light else r0:r1, :]
        if len(a_layers) == 2:
            prep_q, prep_kv, qk, pv = make_joint()
        else:
            prep_q, prep_kv, qk, pv = make_single(a_layers[0], last)

        def proj(i, p):
            r = _dot(h_ref[RL:RT, :] if (last and i == 0) else h, _unpack(wqkv_p[i, p]))
            if light:
                r = _cat0([pre_ref[i, p, pl.ds(pl.multiple_of((t - 2) * SEG, SEG), SEG), :], r])
            return r

        acc = [None]
        OLAG = 3 if len(a_layers) == 2 else 4

        def oproj(p, o):
            part = _dot(o, _unpack(wo_p[p]))
            acc[0] = part if acc[0] is None else acc[0] + part

        def xrows(seg):
            if isinstance(seg, int):
                return x_ref[seg * SEG:(seg + 1) * SEG, :].astype(F32)
            return x_ref[pl.ds(pl.multiple_of(seg * SEG, SEG), SEG), :].astype(F32)

        hooks = {p: [] for p in range(NP)}
        if b_layers:
            b_qk, b_v, b_o, b_fin = make_b(t, b_layers, masked)
            at, v0, dv, lag = b_sched
            for j in range(NT):
                hooks[at + v0 + j * dv + lag].append(functools.partial(b_o, j))
            hooks[at + v0 + (NT - 1) * dv + lag].append(b_fin)
            for j in range(NT):
                hooks[at + v0 + j * dv].append(functools.partial(b_v, j))
            hooks[at].append(b_qk)
        x2 = x2_ref[...] if 1 in a_layers else None

        if head_start:
            t0, t1 = (0, SEG) if 0 in a_layers else (RL, RT)
            m0, m1 = (SEG, r1) if 0 in a_layers else (SEG, RL)
            ht = h_ref[t0:t1, :]
            heads = [_dot(ht, _unpack(wqkv_p[i, 0])) for i in range(2)]
            hm = h_ref[m0:m1, :]
            rest = [_dot(hm, _unpack(wqkv_p[i, 0])) for i in range(2)]
            q, k = [_cat0([a, b] if 0 in a_layers else [b, a]) for a, b in zip(heads, rest)]
            q, k = prep_q(q), prep_kv(k)
        else:
            q = prep_q(proj(0, 0))
            k = prep_kv(proj(1, 0))
        vs = {0: prep_kv(proj(2, 0))}
        early_v = light or len(a_layers) == 1
        os_ = {}
        prs = {}

        def do_pv(p):
            os_[p] = pv(prs.pop(p), vs.pop(p))

        for p in range(NP):
            prs[p] = qk(q, k)
            if p + 1 < NP:
                q = prep_q(proj(0, p + 1))
                k = prep_kv(proj(1, p + 1))
                if early_v:
                    vs[p + 1] = prep_kv(proj(2, p + 1))
            else:
                if deep:
                    do_pv(p - 1)
                if 0 in a_layers:
                    nxt = min(t + 1, NSEG - 1) if isinstance(t, int) else jnp.minimum(t + 1, NSEG - 1)
                    h_ref[0:SEG, :] = _ln(xrows(nxt)).astype(BF16)
                for pp in range(p - OLAG, p - 1):
                    oproj(pp, os_.pop(pp))
            if not deep or p + 1 == NP:
                do_pv(p)
            elif p >= 1:
                do_pv(p - 1)
            if p + 1 < NP and not early_v:
                vs[p + 1] = prep_kv(proj(2, p + 1))
            for f in hooks[p]:
                f()
            if p >= OLAG and p + 1 < NP:
                oproj(p - OLAG, os_.pop(p - OLAG))
        oproj(NP - 2, os_.pop(NP - 2))
        oproj(NP - 1, os_.pop(NP - 1))
        a = acc[0]
        if 0 in a_layers:
            xa_ref[0:SEG, :] = xrows(t) + a[0:SEG]
        if last:
            xa_ref[SEG:2 * SEG, :] = x2 + a
            return
        if 1 in a_layers:
            xa_ref[SEG:2 * SEG, :] = x2 + a[RL - r0:RT - r0]
        mem1 = a[SEG - r0:RV - r0]
        mem2 = a[RV - r0:RL - r0] if 1 in a_layers else mem0
        h_ref[SEG:RL, :] = _cat0([mem1, mem2]).astype(BF16)

    def first_step():
        prep_q, prep_kv, qk, pv = make_single(0)

        RA = (RL + NPRE * SEG) // 32 * 16 + 16

        def wait_group(p):
            for cp in cp_group(p):
                cp.wait()

        def pair0(p, fine=False):
            ha = _unpack(hpre_ref[0:RA // 2, :])
            hb = _unpack(hpre_ref[RA // 2:, :])
            w = {}

            def load(i):
                if fine:
                    cp_fine(p, i).wait()
                w[i] = w_pairs[i][1][rows_of(p), :]
                wqkv_p[i, p] = _pack(w[i].T)

            def proj_a(i):
                r = _dot_nt(ha, w[i])
                pre_ref[i, p, 0:RA - RL, :] = r[RL:]
                return r[0:RL]

            def proj_b(i):
                pre_ref[i, p, RA - RL:, :] = _dot_nt(hb, w[i])

            if fine:
                load(0)
                q = prep_q(proj_a(0))
                proj_b(0)
                load(1)
                k = prep_kv(proj_a(1))
                proj_b(1)
                load(2)
                pr = qk(q, k)
                v = prep_kv(proj_a(2))
                proj_b(2)
                o_ref[p] = _pack(pv(pr, v))
                return
            for i in range(3):
                load(i)
            q = prep_q(proj_a(0))
            k = prep_kv(proj_a(1))
            v = prep_kv(proj_a(2))
            pr = qk(q, k)
            proj_b(0)
            proj_b(1)
            o_ref[p] = _pack(pv(pr, v))
            proj_b(2)

        def body1(p, carry):
            wait_group(p)
            pair0(p)
            return carry

        def body2(i, carry):
            wait_group(2 * i)
            wait_group(2 * i + 1)
            pair0(2 * i)
            pair0(2 * i + 1)
            return carry

        def body0(p, carry):
            pair0(p, fine=True)
            return carry

        lax.fori_loop(0, NFINE, body0, 0)
        lax.fori_loop(NFINE, 4, body1, 0)
        lax.fori_loop(2, NP // 2, body2, 0)
        cp_wo.wait()
        a = None
        for p in range(NP):
            w = wo_ref[sl(p), :]
            wo_p[p] = _pack(w)
            part = _dot(_unpack(o_ref[p]), w)
            a = part if a is None else a + part
        xa_ref[0:SEG, :] = x_ref[0:SEG, :].astype(F32) + a[0:SEG]
        h_ref[0:SEG, :] = _ln(x_ref[SEG:2 * SEG, :].astype(F32)).astype(BF16)
        h_ref[SEG:RL, :] = _cat0([a[SEG:RV], mem0]).astype(BF16)

    first_step()
    cp_x1.start()
    for cp in cp_b:
        cp.wait()
    for j in range(3):
        perm_qkv(j)
    perm_wo()
    step(1, (0,), (0,), deep=True, b_sched=(7, 2, 1, 1))

    def body_light(t, carry):
        step(t, (0, 1), (0, 1), light=True, b_sched=(0, 3, 2, 1))
        return carry

    lax.fori_loop(2, 2 + NPRE, body_light, 0)
    cp_x1.wait()

    T0 = 2 + NPRE
    NPAIR = (NSEG - T0) // 2

    def two_steps(t):
        step(t, (0, 1), (0, 1), masked=False)
        step(t + 1, (0, 1), (0, 1), masked=False, head_start=True)

    def body(i, carry):
        two_steps(T0 + 2 * i)
        return carry

    lax.fori_loop(0, NPAIR, body, 0)
    done = (T0 + 2 * NPAIR - 3) * SEG
    cp_o0 = pltpu.make_async_copy(out_ref.at[0:done], out_hbm.at[0:done], sem.at[6])
    cp_o0.start()
    for t in range(T0 + 2 * NPAIR, NSEG):
        step(t, (0, 1), (0, 1), masked=False)
    step(NSEG, (1,), (0, 1), masked=False, head_start=True)
    cp_o1 = pltpu.make_async_copy(out_ref.at[done:S - 2 * SEG], out_hbm.at[done:S - 2 * SEG], sem.at[7])
    cp_o1.start()
    tails = [make_b(NSEG + 1, (1,), False)]
    step(NSEG + 1, (1,), (), last=True)
    tails.append(make_b(NSEG + 2, (1,), False))
    for b_qk, b_v, _, _ in tails:
        b_qk()
        for j in range(NT):
            b_v(j)
    for _, _, b_o, b_fin in tails:
        for j in range(NT):
            b_o(j)
        b_fin()
    cp_o2 = pltpu.make_async_copy(out_ref.at[S - 2 * SEG:S], out_hbm.at[S - 2 * SEG:S], sem.at[0])
    cp_o2.start()
    cp_o0.wait()
    cp_o1.wait()
    cp_o2.wait()


def pallas_interleave_layers__memory_aug_recurrent_mem_tr__sliding_local_dilated__prompt_kernel(
    A_x: jax.Array,
    A_mem0: jax.Array,
    A_Wq: jax.Array,
    A_Wk: jax.Array,
    A_Wv: jax.Array,
    A_Wo: jax.Array,
    A_seg_len,
    B_x: jax.Array,
    B_wqkv: jax.Array,
    B_wo: jax.Array,
):
    B, S, D = A_x.shape
    H, DH = A_Wq.shape[1], A_Wq.shape[2]
    M = A_mem0.shape[1]
    SEG = A_seg_len if isinstance(A_seg_len, int) else 32
    assert B == 1 and M == 8 and SEG == 32 and DH == 192 and D == 640 and H % 2 == 0
    assert S % SEG == 0 and S // SEG >= NPRE + 4

    x = A_x.reshape(S, D)
    mem0 = A_mem0.reshape(M, D)
    wq = jnp.transpose(A_Wq, (1, 2, 0)).reshape(H * DH, D)
    wk = jnp.transpose(A_Wk, (1, 2, 0)).reshape(H * DH, D)
    wv = jnp.transpose(A_Wv, (1, 2, 0)).reshape(H * DH, D)
    wo = A_Wo.reshape(H * DH, D)

    hbm = pl.BlockSpec(memory_space=pl.ANY)
    out = pl.pallas_call(
        functools.partial(_kernel, S=S, D=D, H=H, DH=DH, M=M, SEG=SEG),
        out_shape=jax.ShapeDtypeStruct((S, D), A_x.dtype),
        in_specs=[hbm] * 8,
        out_specs=hbm,
        scratch_shapes=[
            pltpu.VMEM((M, D), BF16),
            pltpu.VMEM((S, D), BF16),
            pltpu.VMEM((S, D), BF16),
            pltpu.VMEM((H * DH, D), BF16),
            pltpu.VMEM((H * DH, D), BF16),
            pltpu.VMEM((H * DH, D), BF16),
            pltpu.VMEM((H * DH, D), BF16),
            pltpu.VMEM((3, D, D), BF16),
            pltpu.VMEM((D, D), BF16),
            pltpu.VMEM((3, H // 2, D // 2, 2 * DH), U32),
            pltpu.VMEM((H // 2, DH, D), U32),
            pltpu.VMEM((3 * D // 128, D // 2, 128), U32),
            pltpu.VMEM((D // 2, D), U32),
            pltpu.VMEM((2 * SEG + 2 * M, D), BF16),
            pltpu.VMEM((2 * SEG, D), F32),
            pltpu.VMEM((SEG, D), F32),
            pltpu.VMEM((2, 2 * D // 128, HIST, 128), F32),
            pltpu.VMEM(((SEG + 2 * M + NPRE * SEG) // 2, D), U32),
            pltpu.VMEM((3, H // 2, NPRE * SEG, 2 * DH), F32),
            pltpu.VMEM((H // 2, (SEG + 2 * M) // 2, 2 * DH), U32),
            pltpu.VMEM((4, D // 128, D + 24, 128), F32),
            pltpu.SemaphoreType.DMA((H // 2 + 3 * NFINE,)),
            pltpu.SemaphoreType.DMA((10,)),
        ],
        compiler_params=pltpu.CompilerParams(vmem_limit_bytes=120 * 1024 * 1024),
        name="pallas_wavefront",
    )(mem0, x, wq, wk, wv, wo, B_wqkv, B_wo)
    return out.reshape(B, S, D)
```

```python
import functools

import jax
import jax.numpy as jnp
from jax import lax
import jax.experimental.pallas as pl
import jax.experimental.pallas.tpu as pltpu

F32 = jnp.float32
BF16 = jnp.bfloat16
U32 = jnp.uint32

EPS = 1e-5
NEG = -1000000000.0
PADNEG = -3.0e38
B_HEADS = 32
B_WIN = 8
B_DIL = 2
NPRE = 9
NPA = 4
NFINE = 2
HIST = 16


def _ln(x):
    m = jnp.mean(x, axis=-1, keepdims=True)
    xc = x - m
    v = jnp.mean(xc * xc, axis=-1, keepdims=True)
    return xc * lax.rsqrt(v + EPS)


def _dot_nt(a, b):
    return lax.dot_general(a, b, (((1,), (1,)), ((), ())), precision=lax.Precision.DEFAULT,
                           preferred_element_type=F32)


def _dot(a, b):
    return lax.dot_general(a, b, (((1,), (0,)), ((), ())), precision=lax.Precision.DEFAULT,
                           preferred_element_type=F32)


def _pack(a):
    return pltpu.bitcast(a, U32)


def _unpack(a):
    return pltpu.bitcast(a, BF16)


def _cat0(xs):
    return jnp.concatenate(xs, axis=0)


def _cat1(xs):
    return jnp.concatenate(xs, axis=1)


def _kernel(mem0_hbm, x_hbm, wq_hbm, wk_hbm, wv_hbm, wo_hbm, bqkv_hbm, bwo_hbm,
            out_hbm,
            mem0_ref, x_ref, out_ref, wq_ref, wk_ref, wv_ref, wo_ref, bqkv_ref, bwo_ref,
            wqkv_p, wo_p, bqkv_p, bwo_p, h_ref, xa_ref, x2_ref, kv_ref, ha_ref, hb_ref, pre_ref, o_ref, tmp_ref, wsem, sem,
            *, S, D, H, DH, M, SEG):
    NSEG = S // SEG
    PW = 2 * DH
    NP = H // 2
    RV = SEG + M
    RL = SEG + 2 * M
    RT = 2 * SEG + 2 * M
    a_scale = DH ** (-0.5)
    b_dh = D // B_HEADS
    b_scale = b_dh ** (-0.5)
    NT = D // 128
    X0 = (NPRE + 3) * SEG

    def sl(p):
        return slice(p * PW, (p + 1) * PW)

    cp_m = pltpu.make_async_copy(mem0_hbm, mem0_ref, sem.at[8])
    cp_x0 = pltpu.make_async_copy(x_hbm.at[0:X0], x_ref.at[0:X0], sem.at[0])
    cp_x1 = pltpu.make_async_copy(x_hbm.at[X0:S], x_ref.at[X0:S], sem.at[1])
    cp_b = [pltpu.make_async_copy(bqkv_hbm.at[:, j * D:(j + 1) * D], bqkv_ref.at[j], sem.at[2 + j])
            for j in range(3)]
    cp_b.append(pltpu.make_async_copy(bwo_hbm, bwo_ref, sem.at[5]))
    cp_wo = pltpu.make_async_copy(wo_hbm, wo_ref, sem.at[9])
    w_pairs = ((wq_hbm, wq_ref), (wk_hbm, wk_ref), (wv_hbm, wv_ref))

    def rows_of(p):
        return pl.ds(p * PW if isinstance(p, int) else pl.multiple_of(p * PW, 128), PW)

    def cp_fine(p, i):
        src, dst = w_pairs[i]
        return pltpu.make_async_copy(src.at[rows_of(p)], dst.at[rows_of(p)], wsem.at[NP + 3 * p + i])

    def cp_group(p):
        return [pltpu.make_async_copy(src.at[rows_of(p)], dst.at[rows_of(p)], wsem.at[p])
                for src, dst in w_pairs]

    def start_group(p, carry):
        for cp in cp_group(p):
            cp.start()

        @pl.when(p == NP - 1)
        def _():
            cp_wo.start()

        return carry

    firsts = [[cp_m, cp_x0]] + [[cp_fine(p, i)] for p in range(NFINE) for i in range(3)]

    def start_first(i, carry):
        for n, cps in enumerate(firsts):
            @pl.when(i == n)
            def _():
                for cp in cps:
                    cp.start()

        return carry

    lax.fori_loop(0, len(firsts), start_first, 0)
    lax.fori_loop(NFINE, NP, start_group, 0)
    for cp in cp_b:
        cp.start()

    xa_ref[...] = jnp.zeros(xa_ref.shape, F32)
    kv_ref[...] = jnp.zeros(kv_ref.shape, F32)
    cp_m.wait()
    cp_x0.wait()
    mem0 = mem0_ref[...].astype(F32)
    h0 = _ln(x_ref[0:SEG, :].astype(F32))
    ha_ref[0:RV, :] = _cat0([h0, mem0])
    for i in range(NPRE):
        hi = _ln(x_ref[(2 + i) * SEG:(3 + i) * SEG, :].astype(F32))
        if i < NPA:
            ha_ref[RV + i * SEG:RV + (i + 1) * SEG, :] = hi
        else:
            hb_ref[(i - NPA) * SEG // 2:(i - NPA + 1) * SEG // 2, :] = _pack(hi.astype(BF16))

    def perm_rows(a, slot):
        a = a.astype(F32)
        for m in range(NT):
            tmp_ref[slot, m, 0:D, :] = a[:, m * 128:(m + 1) * 128]
        return _cat1([_cat0([tmp_ref[slot, m, pl.ds(d, B_HEADS, stride=b_dh), :] for d in range(b_dh)])
                      for m in range(NT)]).astype(BF16)

    def perm_qkv(j):
        wp = perm_rows(bqkv_ref[j].T, j).T
        for c in range(NT):
            bqkv_p[j * NT + c] = _pack(wp[:, c * 128:(c + 1) * 128])

    def perm_wo():
        bwo_p[...] = _pack(perm_rows(bwo_ref[...], 3))

    def make_b(t, layers, masked):
        xb = xa_ref[layers[0] * SEG:(layers[-1] + 1) * SEG, :]
        hb = _ln(xb).astype(BF16)
        st = {'y': xb, 'p': []}

        def windows(l, i, j, a):
            cur = a[i * SEG:(i + 1) * SEG]
            blk = _cat0([kv_ref[l, j], cur])
            kv_ref[l, j] = cur[SEG - HIST:SEG]
            rolled = [blk] + [pltpu.roll(blk, sh, 0) for sh in range(B_DIL, 8, B_DIL)]
            res = []
            for w in range(B_WIN):
                hi, lo_ = divmod(B_DIL * w, 8)
                o = HIST - 8 * hi
                res.append(rolled[lo_ // B_DIL][o:o + SEG])
            return res

        def qk():
            qs, ks = [], []
            for j in range(NT):
                qs.append(_dot(hb, _unpack(bqkv_p[j])))
                ks.append(_dot(hb, _unpack(bqkv_p[NT + j])))
            for i, l in enumerate(layers):
                ss = None
                for j in range(NT):
                    q = qs[j][i * SEG:(i + 1) * SEG] * b_scale
                    terms = [q * kw for kw in windows(l, i, j, ks[j])]
                    ss = terms if ss is None else [a + b for a, b in zip(ss, terms)]
                pos = (t - 1 - 2 * l) * SEG + lax.broadcasted_iota(jnp.int32, (SEG, 128), 0)
                logits = []
                for w, s in enumerate(ss):
                    s = s + pltpu.roll(s, 64, 1)
                    s = s + pltpu.roll(s, 32, 1)
                    logits.append(jnp.where(pos >= B_DIL * w, s, NEG) if masked else s)
                m = logits[0]
                for w in range(1, B_WIN):
                    m = jnp.maximum(m, logits[w])
                es = [jnp.exp(lg - m) for lg in logits]
                den = es[0]
                for w in range(1, B_WIN):
                    den = den + es[w]
                st['p'].append((es, 1.0 / den))

        def v_stage(j):
            vj = _dot(hb, _unpack(bqkv_p[2 * NT + j]))
            outs = []
            for i, l in enumerate(layers):
                es, inv = st['p'][i]
                vw = windows(l, i, NT + j, vj)
                acc = es[0] * vw[0]
                for w in range(1, B_WIN):
                    acc = acc + es[w] * vw[w]
                outs.append(acc * inv)
            st['o', j] = _cat0(outs).astype(BF16)

        def o_stage(j):
            st['y'] = st['y'] + _dot(st.pop(('o', j)), _unpack(bwo_p[j * 64:(j + 1) * 64, :]))

        def fin():
            for i, l in enumerate(layers):
                yl = st['y'][i * SEG:(i + 1) * SEG]
                if l == 0:
                    x2_ref[...] = yl
                    h_ref[RL:RT, :] = _ln(yl).astype(BF16)
                else:
                    if isinstance(t, int):
                        row = (t - 3) * SEG
                    else:
                        row = pl.multiple_of(jnp.maximum(t - 3, 0) * SEG, SEG)
                    out_ref[pl.ds(row, SEG), :] = yl.astype(out_ref.dtype)

        return qk, v_stage, o_stage, fin

    def softmax2(s, first, valid, fill):
        s = jnp.where(valid, s * a_scale, fill)
        m1 = jnp.max(jnp.where(first, s, PADNEG), axis=-1, keepdims=True)
        m2 = jnp.max(jnp.where(first, PADNEG, s), axis=-1, keepdims=True)
        e = jnp.exp(s - jnp.where(first, m1, m2))
        e1 = jnp.where(first, e, 0.0)
        e2 = jnp.where(first, 0.0, e)
        l1 = jnp.sum(e1, axis=-1, keepdims=True)
        l2 = jnp.sum(e2, axis=-1, keepdims=True)
        inv = 1.0 / jnp.where(first, l1, l2)
        return e, e1, e2, inv

    def make_joint():
        rr = lax.broadcasted_iota(jnp.int32, (RT, 128), 0)
        cc = lax.broadcasted_iota(jnp.int32, (RT, 128), 1)
        lay1 = rr < RV
        first = cc < jnp.where(lay1, RL, RT)
        key = jnp.where(first, cc, cc - RL)
        exists = jnp.where(lay1, RV - 1 - key, key - RV) >= 0
        allowed = (key <= rr) | (lay1 & (key >= SEG)) | ((rr >= RV) & (rr < RL))
        valid = exists & allowed
        fill = jnp.where(exists, NEG, PADNEG)
        lo = cc < (DH - 128)
        z48 = jnp.zeros((128 - RT, 128), F32)
        z32 = jnp.zeros((128 - 2 * RL, 128), F32)

        def prep_q(a):
            return (a[:, 0:128].astype(BF16), a[0:RV, 128:256], a[RV:RT, 128:256], a[:, 256:384].astype(BF16))

        def prep_kv(a):
            mid = a[:, 128:256]
            tlo = jnp.where(lo, mid, 0.0)
            thi = jnp.where(lo, 0.0, mid)
            return (_cat0([a[:, 0:128], z48]).astype(BF16),
                    _cat0([tlo[0:RL], thi[0:RL], z32]).astype(BF16),
                    _cat0([z32, tlo[SEG:RT], thi[SEG:RT]]).astype(BF16),
                    _cat0([z48, a[:, 256:384]]).astype(BF16))

        def qk(q, k):
            t0 = _dot_nt(q[0], k[0])
            t2 = _dot_nt(q[3], k[3])
            t1a = _dot_nt(q[1], k[1])
            t1b = _dot_nt(q[2], k[2])
            s = jnp.where(first, t0, t2) + _cat0([t1a, t1b])
            e, e1, e2, inv = softmax2(s, first, valid, fill)
            pa = e * inv
            return (e1 * inv).astype(BF16), pa[0:RV], pa[RV:RT], (e2 * inv).astype(BF16)

        def pv(pr, v):
            o0 = _dot(pr[0], v[0])
            o2 = _dot(pr[3], v[3])
            o1a = _dot(pr[1], v[1])
            o1b = _dot(pr[2], v[2])
            return _cat1([o0, _cat0([o1a, o1b]), o2]).astype(BF16)

        return prep_q, prep_kv, qk, pv

    def make_single(layer, last=False):
        nq = SEG if last else RV
        rr = lax.broadcasted_iota(jnp.int32, (nq, 2 * RV), 0) + (M if last else 0)
        cc = lax.broadcasted_iota(jnp.int32, (nq, 2 * RV), 1)
        first = cc < RV
        kc = jnp.where(first, cc, cc - RV)
        if layer == 0:
            valid = (kc >= SEG) | (kc <= rr)
        else:
            valid = (rr < M) | (kc <= rr)
        lo = lax.broadcasted_iota(jnp.int32, (RV, PW), 1) < DH
        lhs = (lambda a: a.astype(BF16)) if last else (lambda a: a)

        def prep_kv(a):
            return _cat0([jnp.where(lo, a, 0.0), jnp.where(lo, 0.0, a)]).astype(BF16)

        def qk(q, k):
            e, _, _, inv = softmax2(_dot_nt(q, k), first, valid, NEG)
            return lhs(e * inv)

        def pv(pr, v):
            return lhs(_dot(pr, v))

        return lhs, prep_kv, qk, pv

    def step(t, a_layers, b_layers, light=False, last=False, masked=True, deep=False,
             head_start=False, b_sched=(0, 2, 2, 2)):
        r0 = 0 if 0 in a_layers else RV
        if len(a_layers) == 2:
            h = h_ref[SEG if light else 0:RT, :]
            prep_q, prep_kv, qk, pv = make_joint()
        else:
            h = h_ref[0:RL, :].astype(F32)[0:RV] if r0 == 0 else h_ref[SEG:RT, :].astype(F32)[M:RL]
            prep_q, prep_kv, qk, pv = make_single(a_layers[0], last)

        def proj(i, p):
            r = _dot(h_ref[RL:RT, :] if (last and i == 0) else h, _unpack(wqkv_p[i, p]))
            if light:
                r = _cat0([pre_ref[i, p, pl.ds(pl.multiple_of((t - 2) * SEG, SEG), SEG), :], r])
            return r

        acc = [None]
        OLAG = 3 if len(a_layers) == 2 else 4

        def oproj(p, o):
            part = _dot(o, _unpack(wo_p[p]))
            acc[0] = part if acc[0] is None else acc[0] + part

        def xrows(seg):
            if isinstance(seg, int):
                return x_ref[seg * SEG:(seg + 1) * SEG, :].astype(F32)
            return x_ref[pl.ds(pl.multiple_of(seg * SEG, SEG), SEG), :].astype(F32)

        hooks = {p: [] for p in range(NP)}
        if b_layers:
            b_qk, b_v, b_o, b_fin = make_b(t, b_layers, masked)
            at, v0, dv, lag = b_sched
            for j in range(NT):
                hooks[at + v0 + j * dv + lag].append(functools.partial(b_o, j))
            hooks[at + v0 + (NT - 1) * dv + lag].append(b_fin)
            for j in range(NT):
                hooks[at + v0 + j * dv].append(functools.partial(b_v, j))
            hooks[at].append(b_qk)
        x2 = x2_ref[...] if 1 in a_layers else None

        if head_start:
            heads = [_dot(h_ref[0:SEG, :], _unpack(wqkv_p[i, 0])) for i in range(2)]
            rest = [_dot(h_ref[SEG:RT, :], _unpack(wqkv_p[i, 0])) for i in range(2)]
            q, k = [_cat0([a, b]) for a, b in zip(heads, rest)]
            q, k = prep_q(q), prep_kv(k)
        else:
            q = prep_q(proj(0, 0))
            k = prep_kv(proj(1, 0))
        vs = {0: prep_kv(proj(2, 0))}
        early_v = light or len(a_layers) == 1
        os_ = {}
        prs = {}

        def do_pv(p):
            os_[p] = pv(prs.pop(p), vs.pop(p))

        for p in range(NP):
            prs[p] = qk(q, k)
            if p + 1 < NP:
                q = prep_q(proj(0, p + 1))
                k = prep_kv(proj(1, p + 1))
                if early_v:
                    vs[p + 1] = prep_kv(proj(2, p + 1))
            else:
                if deep:
                    do_pv(p - 1)
                if 0 in a_layers:
                    nxt = min(t + 1, NSEG - 1) if isinstance(t, int) else jnp.minimum(t + 1, NSEG - 1)
                    h_ref[0:SEG, :] = _ln(xrows(nxt)).astype(BF16)
                for pp in range(p - OLAG, p - 1):
                    oproj(pp, os_.pop(pp))
            if not deep or p + 1 == NP:
                do_pv(p)
            elif p >= 1:
                do_pv(p - 1)
            if p + 1 < NP and not early_v:
                vs[p + 1] = prep_kv(proj(2, p + 1))
            for f in hooks[p]:
                f()
            if p >= OLAG and p + 1 < NP:
                oproj(p - OLAG, os_.pop(p - OLAG))
        oproj(NP - 2, os_.pop(NP - 2))
        oproj(NP - 1, os_.pop(NP - 1))
        a = acc[0]
        if 0 in a_layers:
            xa_ref[0:SEG, :] = xrows(t) + a[0:SEG]
        if last:
            xa_ref[SEG:2 * SEG, :] = x2 + a
            return
        if 1 in a_layers:
            xa_ref[SEG:2 * SEG, :] = x2 + a[RL - r0:RT - r0]
        mem2 = a[RV - r0:RL - r0] if 1 in a_layers else mem0
        mem1 = a[SEG:RV] if 0 in a_layers else mem2
        h_ref[SEG:RL, :] = _cat0([mem1, mem2]).astype(BF16)

    def first_step():
        prep_q, prep_kv, qk, pv = make_single(0)

        def wait_group(p):
            for cp in cp_group(p):
                cp.wait()

        def pair0(p, fine=False):
            ha = ha_ref[...]
            hb = _unpack(hb_ref[...])
            w = {}

            def load(i):
                if fine:
                    cp_fine(p, i).wait()
                w[i] = w_pairs[i][1][rows_of(p), :]
                wqkv_p[i, p] = _pack(w[i].T)

            def proj_a(i):
                r = _dot_nt(ha, w[i])
                pre_ref[i, p, 0:NPA * SEG, :] = r[RV:]
                return r[0:RV]

            def proj_b(i):
                pre_ref[i, p, NPA * SEG:, :] = _dot_nt(hb, w[i])

            if fine:
                load(0)
                q = prep_q(proj_a(0))
                proj_b(0)
                load(1)
                k = prep_kv(proj_a(1))
                proj_b(1)
                load(2)
                pr = qk(q, k)
                v = prep_kv(proj_a(2))
                proj_b(2)
                o_ref[p] = pv(pr, v)
                return
            for i in range(3):
                load(i)
            q = prep_q(proj_a(0))
            k = prep_kv(proj_a(1))
            v = prep_kv(proj_a(2))
            pr = qk(q, k)
            proj_b(0)
            proj_b(1)
            o_ref[p] = pv(pr, v)
            proj_b(2)

        def body1(p, carry):
            wait_group(p)
            pair0(p)
            return carry

        def body2(i, carry):
            wait_group(2 * i)
            wait_group(2 * i + 1)
            pair0(2 * i)
            pair0(2 * i + 1)
            return carry

        def body0(p, carry):
            pair0(p, fine=True)
            return carry

        lax.fori_loop(0, NFINE, body0, 0)
        lax.fori_loop(NFINE, 4, body1, 0)
        lax.fori_loop(2, NP // 2, body2, 0)
        cp_wo.wait()
        a = None
        for p in range(NP):
            w = wo_ref[sl(p), :]
            wo_p[p] = _pack(w)
            part = _dot(o_ref[p], w)
            a = part if a is None else a + part
        xa_ref[0:SEG, :] = x_ref[0:SEG, :].astype(F32) + a[0:SEG]
        h_ref[0:SEG, :] = _ln(x_ref[SEG:2 * SEG, :].astype(F32)).astype(BF16)
        h_ref[SEG:RL, :] = _cat0([a[SEG:RV], mem0]).astype(BF16)

    first_step()
    cp_x1.start()
    for cp in cp_b:
        cp.wait()
    for j in range(3):
        perm_qkv(j)
    perm_wo()
    step(1, (0,), (0,), deep=True, b_sched=(7, 2, 1, 1))

    def body_light(t, carry):
        step(t, (0, 1), (0, 1), light=True, b_sched=(0, 3, 2, 1))
        return carry

    lax.fori_loop(2, 2 + NPRE, body_light, 0)
    cp_x1.wait()

    T0 = 2 + NPRE
    NPAIR = (NSEG - T0) // 2

    def two_steps(t):
        step(t, (0, 1), (0, 1), masked=False)
        step(t + 1, (0, 1), (0, 1), masked=False, head_start=True)

    def body(i, carry):
        two_steps(T0 + 2 * i)
        return carry

    lax.fori_loop(0, NPAIR, body, 0)
    done = (T0 + 2 * NPAIR - 3) * SEG
    cp_o0 = pltpu.make_async_copy(out_ref.at[0:done], out_hbm.at[0:done], sem.at[6])
    cp_o0.start()
    for t in range(T0 + 2 * NPAIR, NSEG):
        step(t, (0, 1), (0, 1), masked=False)
    step(NSEG, (1,), (0, 1), masked=False)
    cp_o1 = pltpu.make_async_copy(out_ref.at[done:S - 2 * SEG], out_hbm.at[done:S - 2 * SEG], sem.at[7])
    cp_o1.start()
    tails = [make_b(NSEG + 1, (1,), False)]
    step(NSEG + 1, (1,), (), last=True)
    tails.append(make_b(NSEG + 2, (1,), False))
    for b_qk, b_v, _, _ in tails:
        b_qk()
        for j in range(NT):
            b_v(j)
    for _, _, b_o, b_fin in tails:
        for j in range(NT):
            b_o(j)
        b_fin()
    cp_o2 = pltpu.make_async_copy(out_ref.at[S - 2 * SEG:S], out_hbm.at[S - 2 * SEG:S], sem.at[0])
    cp_o2.start()
    cp_o0.wait()
    cp_o1.wait()
    cp_o2.wait()


def pallas_interleave_layers__memory_aug_recurrent_mem_tr__sliding_local_dilated__prompt_kernel(
    A_x: jax.Array,
    A_mem0: jax.Array,
    A_Wq: jax.Array,
    A_Wk: jax.Array,
    A_Wv: jax.Array,
    A_Wo: jax.Array,
    A_seg_len,
    B_x: jax.Array,
    B_wqkv: jax.Array,
    B_wo: jax.Array,
):
    B, S, D = A_x.shape
    H, DH = A_Wq.shape[1], A_Wq.shape[2]
    M = A_mem0.shape[1]
    SEG = A_seg_len if isinstance(A_seg_len, int) else 32
    assert B == 1 and M == 8 and SEG == 32 and DH == 192 and D == 640 and H % 2 == 0
    assert S % SEG == 0 and S // SEG >= NPRE + 4

    x = A_x.reshape(S, D)
    mem0 = A_mem0.reshape(M, D)
    wq = jnp.transpose(A_Wq, (1, 2, 0)).reshape(H * DH, D)
    wk = jnp.transpose(A_Wk, (1, 2, 0)).reshape(H * DH, D)
    wv = jnp.transpose(A_Wv, (1, 2, 0)).reshape(H * DH, D)
    wo = A_Wo.reshape(H * DH, D)

    hbm = pl.BlockSpec(memory_space=pl.ANY)
    out = pl.pallas_call(
        functools.partial(_kernel, S=S, D=D, H=H, DH=DH, M=M, SEG=SEG),
        out_shape=jax.ShapeDtypeStruct((S, D), A_x.dtype),
        in_specs=[hbm] * 8,
        out_specs=hbm,
        scratch_shapes=[
            pltpu.VMEM((M, D), BF16),
            pltpu.VMEM((S, D), BF16),
            pltpu.VMEM((S, D), BF16),
            pltpu.VMEM((H * DH, D), BF16),
            pltpu.VMEM((H * DH, D), BF16),
            pltpu.VMEM((H * DH, D), BF16),
            pltpu.VMEM((H * DH, D), BF16),
            pltpu.VMEM((3, D, D), BF16),
            pltpu.VMEM((D, D), BF16),
            pltpu.VMEM((3, H // 2, D // 2, 2 * DH), U32),
            pltpu.VMEM((H // 2, DH, D), U32),
            pltpu.VMEM((3 * D // 128, D // 2, 128), U32),
            pltpu.VMEM((D // 2, D), U32),
            pltpu.VMEM((2 * SEG + 2 * M, D), BF16),
            pltpu.VMEM((2 * SEG, D), F32),
            pltpu.VMEM((SEG, D), F32),
            pltpu.VMEM((2, 2 * D // 128, HIST, 128), F32),
            pltpu.VMEM((SEG + M + NPA * SEG, D), F32),
            pltpu.VMEM(((NPRE - NPA) * SEG // 2, D), U32),
            pltpu.VMEM((3, H // 2, NPRE * SEG, 2 * DH), F32),
            pltpu.VMEM((H // 2, SEG + M, 2 * DH), F32),
            pltpu.VMEM((4, D // 128, D + 24, 128), F32),
            pltpu.SemaphoreType.DMA((H // 2 + 3 * NFINE,)),
            pltpu.SemaphoreType.DMA((10,)),
        ],
        compiler_params=pltpu.CompilerParams(vmem_limit_bytes=120 * 1024 * 1024),
        name="pallas_wavefront",
    )(mem0, x, wq, wk, wv, wo, B_wqkv, B_wo)
    return out.reshape(B, S, D)
```

```python
import functools

import jax
import jax.numpy as jnp
from jax import lax
import jax.experimental.pallas as pl
import jax.experimental.pallas.tpu as pltpu

F32 = jnp.float32
BF16 = jnp.bfloat16
U32 = jnp.uint32

EPS = 1e-5
NEG = -1000000000.0
PADNEG = -3.0e38
B_HEADS = 32
B_WIN = 8
B_DIL = 2
NPRE = 11
NPA = 5
NFINE = 1
HIST = 16


def _ln(x):
    m = jnp.mean(x, axis=-1, keepdims=True)
    xc = x - m
    v = jnp.mean(xc * xc, axis=-1, keepdims=True)
    return xc * lax.rsqrt(v + EPS)


def _dot_nt(a, b):
    return lax.dot_general(a, b, (((1,), (1,)), ((), ())), precision=lax.Precision.DEFAULT,
                           preferred_element_type=F32)


def _dot(a, b):
    return lax.dot_general(a, b, (((1,), (0,)), ((), ())), precision=lax.Precision.DEFAULT,
                           preferred_element_type=F32)


def _pack(a):
    return pltpu.bitcast(a, U32)


def _unpack(a):
    return pltpu.bitcast(a, BF16)


def _cat0(xs):
    return jnp.concatenate(xs, axis=0)


def _cat1(xs):
    return jnp.concatenate(xs, axis=1)


def _kernel(mem0_hbm, x_hbm, wq_hbm, wk_hbm, wv_hbm, wo_hbm, bqkv_hbm, bwo_hbm,
            out_hbm,
            mem0_ref, x_ref, out_ref, wq_ref, wk_ref, wv_ref, wo_ref, bqkv_ref, bwo_ref,
            wqkv_p, wo_p, bqkv_p, bwo_p, h_ref, xa_ref, x2_ref, kv_ref, ha_ref, hb_ref, pre_ref, o_ref, tmp_ref, wsem, sem,
            *, S, D, H, DH, M, SEG):
    NSEG = S // SEG
    PW = 2 * DH
    NP = H // 2
    RV = SEG + M
    RL = SEG + 2 * M
    RT = 2 * SEG + 2 * M
    a_scale = DH ** (-0.5)
    b_dh = D // B_HEADS
    b_scale = b_dh ** (-0.5)
    NT = D // 128
    X0 = (NPRE + 3) * SEG

    def sl(p):
        return slice(p * PW, (p + 1) * PW)

    cp_m = pltpu.make_async_copy(mem0_hbm, mem0_ref, sem.at[8])
    cp_x0 = pltpu.make_async_copy(x_hbm.at[0:X0], x_ref.at[0:X0], sem.at[0])
    cp_x1 = pltpu.make_async_copy(x_hbm.at[X0:S], x_ref.at[X0:S], sem.at[1])
    cp_b = [pltpu.make_async_copy(bqkv_hbm.at[:, j * D:(j + 1) * D], bqkv_ref.at[j], sem.at[2 + j])
            for j in range(3)]
    cp_b.append(pltpu.make_async_copy(bwo_hbm, bwo_ref, sem.at[5]))
    cp_wo = pltpu.make_async_copy(wo_hbm, wo_ref, sem.at[9])
    w_pairs = ((wq_hbm, wq_ref), (wk_hbm, wk_ref), (wv_hbm, wv_ref))

    def rows_of(p):
        return pl.ds(p * PW if isinstance(p, int) else pl.multiple_of(p * PW, 128), PW)

    def cp_fine(p, i):
        src, dst = w_pairs[i]
        return pltpu.make_async_copy(src.at[rows_of(p)], dst.at[rows_of(p)], wsem.at[NP + 3 * p + i])

    def cp_group(p):
        return [pltpu.make_async_copy(src.at[rows_of(p)], dst.at[rows_of(p)], wsem.at[p])
                for src, dst in w_pairs]

    def start_group(p, carry):
        for cp in cp_group(p):
            cp.start()

        @pl.when(p == NP - 1)
        def _():
            cp_wo.start()

        return carry

    firsts = [[cp_m, cp_x0]] + [[cp_fine(p, i)] for p in range(NFINE) for i in range(3)]

    def start_first(i, carry):
        for n, cps in enumerate(firsts):
            @pl.when(i == n)
            def _():
                for cp in cps:
                    cp.start()

        return carry

    lax.fori_loop(0, len(firsts), start_first, 0)
    lax.fori_loop(NFINE, NP, start_group, 0)
    for cp in cp_b:
        cp.start()

    xa_ref[...] = jnp.zeros(xa_ref.shape, F32)
    kv_ref[...] = jnp.zeros(kv_ref.shape, F32)
    cp_m.wait()
    cp_x0.wait()
    mem0 = mem0_ref[...].astype(F32)
    h0 = _ln(x_ref[0:SEG, :].astype(F32))
    ha_ref[0:RV, :] = _cat0([h0, mem0])
    for i in range(NPRE):
        hi = _ln(x_ref[(2 + i) * SEG:(3 + i) * SEG, :].astype(F32))
        if i < NPA:
            ha_ref[RV + i * SEG:RV + (i + 1) * SEG, :] = hi
        else:
            hb_ref[(i - NPA) * SEG // 2:(i - NPA + 1) * SEG // 2, :] = _pack(hi.astype(BF16))

    def perm_rows(a, slot):
        a = a.astype(F32)
        for m in range(NT):
            tmp_ref[slot, m, 0:D, :] = a[:, m * 128:(m + 1) * 128]
        return _cat1([_cat0([tmp_ref[slot, m, pl.ds(d, B_HEADS, stride=b_dh), :] for d in range(b_dh)])
                      for m in range(NT)]).astype(BF16)

    def perm_qkv(j):
        wp = perm_rows(bqkv_ref[j].T, j).T
        for c in range(NT):
            bqkv_p[j * NT + c] = _pack(wp[:, c * 128:(c + 1) * 128])

    def perm_wo():
        bwo_p[...] = _pack(perm_rows(bwo_ref[...], 3))

    def make_b(t, layers, masked):
        xb = xa_ref[layers[0] * SEG:(layers[-1] + 1) * SEG, :]
        hb = _ln(xb).astype(BF16)
        st = {'y': xb, 'p': []}

        def windows(l, i, j, a):
            cur = a[i * SEG:(i + 1) * SEG]
            blk = _cat0([kv_ref[l, j], cur])
            kv_ref[l, j] = cur[SEG - HIST:SEG]
            rolled = [blk] + [pltpu.roll(blk, sh, 0) for sh in range(B_DIL, 8, B_DIL)]
            res = []
            for w in range(B_WIN):
                hi, lo_ = divmod(B_DIL * w, 8)
                o = HIST - 8 * hi
                res.append(rolled[lo_ // B_DIL][o:o + SEG])
            return res

        def qk():
            qs, ks = [], []
            for j in range(NT):
                qs.append(_dot(hb, _unpack(bqkv_p[j])))
                ks.append(_dot(hb, _unpack(bqkv_p[NT + j])))
            for i, l in enumerate(layers):
                ss = None
                for j in range(NT):
                    q = qs[j][i * SEG:(i + 1) * SEG] * b_scale
                    terms = [q * kw for kw in windows(l, i, j, ks[j])]
                    ss = terms if ss is None else [a + b for a, b in zip(ss, terms)]
                pos = (t - 1 - 2 * l) * SEG + lax.broadcasted_iota(jnp.int32, (SEG, 128), 0)
                logits = []
                for w, s in enumerate(ss):
                    s = s + pltpu.roll(s, 64, 1)
                    s = s + pltpu.roll(s, 32, 1)
                    logits.append(jnp.where(pos >= B_DIL * w, s, NEG) if masked else s)
                m = logits[0]
                for w in range(1, B_WIN):
                    m = jnp.maximum(m, logits[w])
                es = [jnp.exp(lg - m) for lg in logits]
                den = es[0]
                for w in range(1, B_WIN):
                    den = den + es[w]
                st['p'].append((es, 1.0 / den))

        def v_stage(j):
            vj = _dot(hb, _unpack(bqkv_p[2 * NT + j]))
            outs = []
            for i, l in enumerate(layers):
                es, inv = st['p'][i]
                vw = windows(l, i, NT + j, vj)
                acc = es[0] * vw[0]
                for w in range(1, B_WIN):
                    acc = acc + es[w] * vw[w]
                outs.append(acc * inv)
            st['o', j] = _cat0(outs).astype(BF16)

        def o_stage(j):
            st['y'] = st['y'] + _dot(st.pop(('o', j)), _unpack(bwo_p[j * 64:(j + 1) * 64, :]))

        def fin():
            for i, l in enumerate(layers):
                yl = st['y'][i * SEG:(i + 1) * SEG]
                if l == 0:
                    x2_ref[...] = yl
                    h_ref[RL:RT, :] = _ln(yl).astype(BF16)
                else:
                    if isinstance(t, int):
                        row = (t - 3) * SEG
                    else:
                        row = pl.multiple_of(jnp.maximum(t - 3, 0) * SEG, SEG)
                    out_ref[pl.ds(row, SEG), :] = yl.astype(out_ref.dtype)

        return qk, v_stage, o_stage, fin

    def softmax2(s, first, valid, fill):
        s = jnp.where(valid, s * a_scale, fill)
        m1 = jnp.max(jnp.where(first, s, PADNEG), axis=-1, keepdims=True)
        m2 = jnp.max(jnp.where(first, PADNEG, s), axis=-1, keepdims=True)
        e = jnp.exp(s - jnp.where(first, m1, m2))
        e1 = jnp.where(first, e, 0.0)
        e2 = jnp.where(first, 0.0, e)
        l1 = jnp.sum(e1, axis=-1, keepdims=True)
        l2 = jnp.sum(e2, axis=-1, keepdims=True)
        inv = 1.0 / jnp.where(first, l1, l2)
        return e, e1, e2, inv

    def make_joint():
        rr = lax.broadcasted_iota(jnp.int32, (RT, 128), 0)
        cc = lax.broadcasted_iota(jnp.int32, (RT, 128), 1)
        lay1 = rr < RV
        first = cc < jnp.where(lay1, RL, RT)
        key = jnp.where(first, cc, cc - RL)
        exists = jnp.where(lay1, RV - 1 - key, key - RV) >= 0
        allowed = (key <= rr) | (lay1 & (key >= SEG)) | ((rr >= RV) & (rr < RL))
        valid = exists & allowed
        fill = jnp.where(exists, NEG, PADNEG)
        lo = cc < (DH - 128)
        z48 = jnp.zeros((128 - RT, 128), F32)
        z32 = jnp.zeros((128 - 2 * RL, 128), F32)

        def prep_q(a):
            return (a[:, 0:128].astype(BF16), a[0:RV, 128:256], a[RV:RT, 128:256], a[:, 256:384].astype(BF16))

        def prep_kv(a):
            mid = a[:, 128:256]
            tlo = jnp.where(lo, mid, 0.0)
            thi = jnp.where(lo, 0.0, mid)
            return (_cat0([a[:, 0:128], z48]).astype(BF16),
                    _cat0([tlo[0:RL], thi[0:RL], z32]).astype(BF16),
                    _cat0([z32, tlo[SEG:RT], thi[SEG:RT]]).astype(BF16),
                    _cat0([z48, a[:, 256:384]]).astype(BF16))

        def qk(q, k):
            t0 = _dot_nt(q[0], k[0])
            t2 = _dot_nt(q[3], k[3])
            t1a = _dot_nt(q[1], k[1])
            t1b = _dot_nt(q[2], k[2])
            s = jnp.where(first, t0, t2) + _cat0([t1a, t1b])
            e, e1, e2, inv = softmax2(s, first, valid, fill)
            pa = e * inv
            return (e1 * inv).astype(BF16), pa[0:RV], pa[RV:RT], (e2 * inv).astype(BF16)

        def pv(pr, v):
            o0 = _dot(pr[0], v[0])
            o2 = _dot(pr[3], v[3])
            o1a = _dot(pr[1], v[1])
            o1b = _dot(pr[2], v[2])
            return _cat1([o0, _cat0([o1a, o1b]), o2]).astype(BF16)

        return prep_q, prep_kv, qk, pv

    def make_single(layer, last=False):
        nq = SEG if last else RV
        rr = lax.broadcasted_iota(jnp.int32, (nq, 2 * RV), 0) + (M if last else 0)
        cc = lax.broadcasted_iota(jnp.int32, (nq, 2 * RV), 1)
        first = cc < RV
        kc = jnp.where(first, cc, cc - RV)
        if layer == 0:
            valid = (kc >= SEG) | (kc <= rr)
        else:
            valid = (rr < M) | (kc <= rr)
        lo = lax.broadcasted_iota(jnp.int32, (RV, PW), 1) < DH
        lhs = (lambda a: a.astype(BF16)) if last else (lambda a: a)

        def prep_kv(a):
            return _cat0([jnp.where(lo, a, 0.0), jnp.where(lo, 0.0, a)]).astype(BF16)

        def qk(q, k):
            e, _, _, inv = softmax2(_dot_nt(q, k), first, valid, NEG)
            return lhs(e * inv)

        def pv(pr, v):
            return lhs(_dot(pr, v))

        return lhs, prep_kv, qk, pv

    def step(t, a_layers, b_layers, light=False, last=False, masked=True, deep=False,
             head_start=False, b_sched=(0, 2, 2, 2)):
        r0 = 0 if 0 in a_layers else RV
        if len(a_layers) == 2:
            h = h_ref[SEG if light else 0:RT, :]
            prep_q, prep_kv, qk, pv = make_joint()
        else:
            h = h_ref[0:RL, :].astype(F32)[0:RV] if r0 == 0 else h_ref[SEG:RT, :].astype(F32)[M:RL]
            prep_q, prep_kv, qk, pv = make_single(a_layers[0], last)

        def proj(i, p):
            r = _dot(h_ref[RL:RT, :] if (last and i == 0) else h, _unpack(wqkv_p[i, p]))
            if light:
                r = _cat0([pre_ref[i, p, pl.ds(pl.multiple_of((t - 2) * SEG, SEG), SEG), :], r])
            return r

        acc = [None]
        OLAG = 3 if len(a_layers) == 2 else 4

        def oproj(p, o):
            part = _dot(o, _unpack(wo_p[p]))
            acc[0] = part if acc[0] is None else acc[0] + part

        def xrows(seg):
            if isinstance(seg, int):
                return x_ref[seg * SEG:(seg + 1) * SEG, :].astype(F32)
            return x_ref[pl.ds(pl.multiple_of(seg * SEG, SEG), SEG), :].astype(F32)

        hooks = {p: [] for p in range(NP)}
        if b_layers:
            b_qk, b_v, b_o, b_fin = make_b(t, b_layers, masked)
            at, v0, dv, lag = b_sched
            for j in range(NT):
                hooks[at + v0 + j * dv + lag].append(functools.partial(b_o, j))
            hooks[at + v0 + (NT - 1) * dv + lag].append(b_fin)
            for j in range(NT):
                hooks[at + v0 + j * dv].append(functools.partial(b_v, j))
            hooks[at].append(b_qk)
        x2 = x2_ref[...] if 1 in a_layers else None

        if head_start:
            heads = [_dot(h_ref[0:SEG, :], _unpack(wqkv_p[i, 0])) for i in range(2)]
            rest = [_dot(h_ref[SEG:RT, :], _unpack(wqkv_p[i, 0])) for i in range(2)]
            q, k = [_cat0([a, b]) for a, b in zip(heads, rest)]
            q, k = prep_q(q), prep_kv(k)
        else:
            q = prep_q(proj(0, 0))
            k = prep_kv(proj(1, 0))
        vs = {0: prep_kv(proj(2, 0))}
        early_v = light or len(a_layers) == 1
        os_ = {}
        prs = {}

        def do_pv(p):
            os_[p] = pv(prs.pop(p), vs.pop(p))

        for p in range(NP):
            prs[p] = qk(q, k)
            if p + 1 < NP:
                q = prep_q(proj(0, p + 1))
                k = prep_kv(proj(1, p + 1))
                if early_v:
                    vs[p + 1] = prep_kv(proj(2, p + 1))
            else:
                if deep:
                    do_pv(p - 1)
                if 0 in a_layers:
                    nxt = min(t + 1, NSEG - 1) if isinstance(t, int) else jnp.minimum(t + 1, NSEG - 1)
                    h_ref[0:SEG, :] = _ln(xrows(nxt)).astype(BF16)
                for pp in range(p - OLAG, p - 1):
                    oproj(pp, os_.pop(pp))
            if not deep or p + 1 == NP:
                do_pv(p)
            elif p >= 1:
                do_pv(p - 1)
            if p + 1 < NP and not early_v:
                vs[p + 1] = prep_kv(proj(2, p + 1))
            for f in hooks[p]:
                f()
            if p >= OLAG and p + 1 < NP:
                oproj(p - OLAG, os_.pop(p - OLAG))
        oproj(NP - 2, os_.pop(NP - 2))
        oproj(NP - 1, os_.pop(NP - 1))
        a = acc[0]
        if 0 in a_layers:
            xa_ref[0:SEG, :] = xrows(t) + a[0:SEG]
        if last:
            xa_ref[SEG:2 * SEG, :] = x2 + a
            return
        if 1 in a_layers:
            xa_ref[SEG:2 * SEG, :] = x2 + a[RL - r0:RT - r0]
        mem2 = a[RV - r0:RL - r0] if 1 in a_layers else mem0
        mem1 = a[SEG:RV] if 0 in a_layers else mem2
        h_ref[SEG:RL, :] = _cat0([mem1, mem2]).astype(BF16)

    def first_step():
        prep_q, prep_kv, qk, pv = make_single(0)

        def wait_group(p):
            for cp in cp_group(p):
                cp.wait()

        def pair0(p, fine=False):
            ha = ha_ref[...]
            hb = _unpack(hb_ref[...])
            w = {}

            def load(i):
                if fine:
                    cp_fine(p, i).wait()
                w[i] = w_pairs[i][1][rows_of(p), :]
                wqkv_p[i, p] = _pack(w[i].T)

            def proj_a(i):
                r = _dot_nt(ha, w[i])
                pre_ref[i, p, 0:NPA * SEG, :] = r[RV:]
                return r[0:RV]

            def proj_b(i):
                pre_ref[i, p, NPA * SEG:, :] = _dot_nt(hb, w[i])

            if fine:
                load(0)
                q = prep_q(proj_a(0))
                proj_b(0)
                load(1)
                k = prep_kv(proj_a(1))
                proj_b(1)
                load(2)
                pr = qk(q, k)
                v = prep_kv(proj_a(2))
                proj_b(2)
                o_ref[p] = pv(pr, v)
                return
            for i in range(3):
                load(i)
            q = prep_q(proj_a(0))
            k = prep_kv(proj_a(1))
            v = prep_kv(proj_a(2))
            pr = qk(q, k)
            proj_b(0)
            proj_b(1)
            o_ref[p] = pv(pr, v)
            proj_b(2)

        def body1(p, carry):
            wait_group(p)
            pair0(p)
            return carry

        def body2(i, carry):
            wait_group(2 * i)
            wait_group(2 * i + 1)
            pair0(2 * i)
            pair0(2 * i + 1)
            return carry

        def body0(p, carry):
            pair0(p, fine=True)
            return carry

        lax.fori_loop(0, NFINE, body0, 0)
        lax.fori_loop(NFINE, 4, body1, 0)
        lax.fori_loop(2, NP // 2, body2, 0)
        cp_x1.start()
        cp_wo.wait()
        for cp in cp_b:
            cp.wait()
        a = None
        for p in range(NP):
            w = wo_ref[sl(p), :]
            wo_p[p] = _pack(w)
            part = _dot(o_ref[p], w)
            a = part if a is None else a + part
        xa_ref[0:SEG, :] = x_ref[0:SEG, :].astype(F32) + a[0:SEG]
        h_ref[0:SEG, :] = _ln(x_ref[SEG:2 * SEG, :].astype(F32)).astype(BF16)
        h_ref[SEG:RL, :] = _cat0([a[SEG:RV], mem0]).astype(BF16)

    first_step()
    for j in range(3):
        perm_qkv(j)
    perm_wo()
    step(1, (0,), (0,), deep=True, b_sched=(7, 2, 1, 1))

    def body_light(t, carry):
        step(t, (0, 1), (0, 1), light=True, b_sched=(0, 3, 2, 1))
        return carry

    lax.fori_loop(2, 2 + NPRE, body_light, 0)
    cp_x1.wait()

    T0 = 2 + NPRE
    NPAIR = (NSEG - T0) // 2

    def two_steps(t):
        step(t, (0, 1), (0, 1), masked=False)
        step(t + 1, (0, 1), (0, 1), masked=False, head_start=True)

    def body(i, carry):
        two_steps(T0 + 2 * i)
        return carry

    lax.fori_loop(0, NPAIR, body, 0)
    done = (T0 + 2 * NPAIR - 3) * SEG
    cp_o0 = pltpu.make_async_copy(out_ref.at[0:done], out_hbm.at[0:done], sem.at[6])
    cp_o0.start()
    for t in range(T0 + 2 * NPAIR, NSEG):
        step(t, (0, 1), (0, 1), masked=False)
    step(NSEG, (1,), (0, 1), masked=False)
    cp_o1 = pltpu.make_async_copy(out_ref.at[done:S - 2 * SEG], out_hbm.at[done:S - 2 * SEG], sem.at[7])
    cp_o1.start()
    tails = [make_b(NSEG + 1, (1,), False)]
    step(NSEG + 1, (1,), (), last=True)
    tails.append(make_b(NSEG + 2, (1,), False))
    for b_qk, b_v, _, _ in tails:
        b_qk()
        for j in range(NT):
            b_v(j)
    for _, _, b_o, b_fin in tails:
        for j in range(NT):
            b_o(j)
        b_fin()
    cp_o2 = pltpu.make_async_copy(out_ref.at[S - 2 * SEG:S], out_hbm.at[S - 2 * SEG:S], sem.at[0])
    cp_o2.start()
    cp_o0.wait()
    cp_o1.wait()
    cp_o2.wait()


def pallas_interleave_layers__memory_aug_recurrent_mem_tr__sliding_local_dilated__prompt_kernel(
    A_x: jax.Array,
    A_mem0: jax.Array,
    A_Wq: jax.Array,
    A_Wk: jax.Array,
    A_Wv: jax.Array,
    A_Wo: jax.Array,
    A_seg_len,
    B_x: jax.Array,
    B_wqkv: jax.Array,
    B_wo: jax.Array,
):
    B, S, D = A_x.shape
    H, DH = A_Wq.shape[1], A_Wq.shape[2]
    M = A_mem0.shape[1]
    SEG = A_seg_len if isinstance(A_seg_len, int) else 32
    assert B == 1 and M == 8 and SEG == 32 and DH == 192 and D == 640 and H % 2 == 0
    assert S % SEG == 0 and S // SEG >= NPRE + 4

    x = A_x.reshape(S, D)
    mem0 = A_mem0.reshape(M, D)
    wq = jnp.transpose(A_Wq, (1, 2, 0)).reshape(H * DH, D)
    wk = jnp.transpose(A_Wk, (1, 2, 0)).reshape(H * DH, D)
    wv = jnp.transpose(A_Wv, (1, 2, 0)).reshape(H * DH, D)
    wo = A_Wo.reshape(H * DH, D)

    hbm = pl.BlockSpec(memory_space=pl.ANY)
    out = pl.pallas_call(
        functools.partial(_kernel, S=S, D=D, H=H, DH=DH, M=M, SEG=SEG),
        out_shape=jax.ShapeDtypeStruct((S, D), A_x.dtype),
        in_specs=[hbm] * 8,
        out_specs=hbm,
        scratch_shapes=[
            pltpu.VMEM((M, D), BF16),
            pltpu.VMEM((S, D), BF16),
            pltpu.VMEM((S, D), BF16),
            pltpu.VMEM((H * DH, D), BF16),
            pltpu.VMEM((H * DH, D), BF16),
            pltpu.VMEM((H * DH, D), BF16),
            pltpu.VMEM((H * DH, D), BF16),
            pltpu.VMEM((3, D, D), BF16),
            pltpu.VMEM((D, D), BF16),
            pltpu.VMEM((3, H // 2, D // 2, 2 * DH), U32),
            pltpu.VMEM((H // 2, DH, D), U32),
            pltpu.VMEM((3 * D // 128, D // 2, 128), U32),
            pltpu.VMEM((D // 2, D), U32),
            pltpu.VMEM((2 * SEG + 2 * M, D), BF16),
            pltpu.VMEM((2 * SEG, D), F32),
            pltpu.VMEM((SEG, D), F32),
            pltpu.VMEM((2, 2 * D // 128, HIST, 128), F32),
            pltpu.VMEM((SEG + M + NPA * SEG, D), F32),
            pltpu.VMEM(((NPRE - NPA) * SEG // 2, D), U32),
            pltpu.VMEM((3, H // 2, NPRE * SEG, 2 * DH), F32),
            pltpu.VMEM((H // 2, SEG + M, 2 * DH), F32),
            pltpu.VMEM((4, D // 128, D + 24, 128), F32),
            pltpu.SemaphoreType.DMA((H // 2 + 3 * NFINE,)),
            pltpu.SemaphoreType.DMA((10,)),
        ],
        compiler_params=pltpu.CompilerParams(vmem_limit_bytes=120 * 1024 * 1024),
        name="pallas_wavefront",
    )(mem0, x, wq, wk, wv, wo, B_wqkv, B_wo)
    return out.reshape(B, S, D)
```

```python
import functools

import jax
import jax.numpy as jnp
from jax import lax
import jax.experimental.pallas as pl
import jax.experimental.pallas.tpu as pltpu

F32 = jnp.float32
BF16 = jnp.bfloat16
U32 = jnp.uint32

EPS = 1e-5
NEG = -1000000000.0
PADNEG = -3.0e38
B_HEADS = 32
B_WIN = 8
B_DIL = 2
NPRE = 11
NPA = 5
NFINE = 1
HIST = 16


def _ln(x):
    m = jnp.mean(x, axis=-1, keepdims=True)
    xc = x - m
    v = jnp.mean(xc * xc, axis=-1, keepdims=True)
    return xc * lax.rsqrt(v + EPS)


def _dot_nt(a, b):
    return lax.dot_general(a, b, (((1,), (1,)), ((), ())), precision=lax.Precision.DEFAULT,
                           preferred_element_type=F32)


def _dot(a, b):
    return lax.dot_general(a, b, (((1,), (0,)), ((), ())), precision=lax.Precision.DEFAULT,
                           preferred_element_type=F32)


def _pack(a):
    return pltpu.bitcast(a, U32)


def _unpack(a):
    return pltpu.bitcast(a, BF16)


def _cat0(xs):
    return jnp.concatenate(xs, axis=0)


def _cat1(xs):
    return jnp.concatenate(xs, axis=1)


def _kernel(mem0_hbm, x_hbm, wq_hbm, wk_hbm, wv_hbm, wo_hbm, bqkv_hbm, bwo_hbm,
            out_hbm,
            mem0_ref, x_ref, out_ref, wq_ref, wk_ref, wv_ref, wo_ref, bqkv_ref, bwo_ref,
            wqkv_p, wo_p, bqkv_p, bwo_p, h_ref, xa_ref, x2_ref, kv_ref, ha_ref, hb_ref, pre_ref, o_ref, tmp_ref, wsem, sem,
            *, S, D, H, DH, M, SEG):
    NSEG = S // SEG
    PW = 2 * DH
    NP = H // 2
    RV = SEG + M
    RL = SEG + 2 * M
    RT = 2 * SEG + 2 * M
    a_scale = DH ** (-0.5)
    b_dh = D // B_HEADS
    b_scale = b_dh ** (-0.5)
    NT = D // 128
    X0 = (NPRE + 3) * SEG

    def sl(p):
        return slice(p * PW, (p + 1) * PW)

    cp_m = pltpu.make_async_copy(mem0_hbm, mem0_ref, sem.at[8])
    cp_x0 = pltpu.make_async_copy(x_hbm.at[0:X0], x_ref.at[0:X0], sem.at[0])
    cp_x1 = pltpu.make_async_copy(x_hbm.at[X0:S], x_ref.at[X0:S], sem.at[1])
    cp_b = [pltpu.make_async_copy(bqkv_hbm.at[:, j * D:(j + 1) * D], bqkv_ref.at[j], sem.at[2 + j])
            for j in range(3)]
    cp_b.append(pltpu.make_async_copy(bwo_hbm, bwo_ref, sem.at[5]))
    cp_wo = pltpu.make_async_copy(wo_hbm, wo_ref, sem.at[9])
    w_pairs = ((wq_hbm, wq_ref), (wk_hbm, wk_ref), (wv_hbm, wv_ref))

    def rows_of(p):
        return pl.ds(p * PW if isinstance(p, int) else pl.multiple_of(p * PW, 128), PW)

    def cp_fine(p, i):
        src, dst = w_pairs[i]
        return pltpu.make_async_copy(src.at[rows_of(p)], dst.at[rows_of(p)], wsem.at[NP + 3 * p + i])

    def cp_group(p):
        return [pltpu.make_async_copy(src.at[rows_of(p)], dst.at[rows_of(p)], wsem.at[p])
                for src, dst in w_pairs]

    def start_group(p, carry):
        for cp in cp_group(p):
            cp.start()

        @pl.when(p == NP - 1)
        def _():
            cp_wo.start()

        return carry

    firsts = [[cp_m, cp_x0]] + [[cp_fine(p, i)] for p in range(NFINE) for i in range(3)]

    def start_first(i, carry):
        for n, cps in enumerate(firsts):
            @pl.when(i == n)
            def _():
                for cp in cps:
                    cp.start()

        return carry

    lax.fori_loop(0, len(firsts), start_first, 0)
    lax.fori_loop(NFINE, NP, start_group, 0)
    for cp in cp_b:
        cp.start()

    xa_ref[...] = jnp.zeros(xa_ref.shape, F32)
    kv_ref[...] = jnp.zeros(kv_ref.shape, F32)
    cp_m.wait()
    cp_x0.wait()
    mem0 = mem0_ref[...].astype(F32)
    h0 = _ln(x_ref[0:SEG, :].astype(F32))
    ha_ref[0:RV, :] = _cat0([h0, mem0])
    for i in range(NPRE):
        hi = _ln(x_ref[(2 + i) * SEG:(3 + i) * SEG, :].astype(F32))
        if i < NPA:
            ha_ref[RV + i * SEG:RV + (i + 1) * SEG, :] = hi
        else:
            hb_ref[(i - NPA) * SEG // 2:(i - NPA + 1) * SEG // 2, :] = _pack(hi.astype(BF16))

    def perm_rows(a, slot):
        a = a.astype(F32)
        for m in range(NT):
            tmp_ref[slot, m, 0:D, :] = a[:, m * 128:(m + 1) * 128]
        return _cat1([_cat0([tmp_ref[slot, m, pl.ds(d, B_HEADS, stride=b_dh), :] for d in range(b_dh)])
                      for m in range(NT)]).astype(BF16)

    def perm_qkv(j):
        wp = perm_rows(bqkv_ref[j].T, j).T
        for c in range(NT):
            bqkv_p[j * NT + c] = _pack(wp[:, c * 128:(c + 1) * 128])

    def perm_wo():
        bwo_p[...] = _pack(perm_rows(bwo_ref[...], 3))

    def make_b(t, layers, masked):
        xb = xa_ref[layers[0] * SEG:(layers[-1] + 1) * SEG, :]
        hb = _ln(xb).astype(BF16)
        st = {'y': xb, 'p': []}

        def windows(l, i, j, a):
            cur = a[i * SEG:(i + 1) * SEG]
            blk = _cat0([kv_ref[l, j], cur])
            kv_ref[l, j] = cur[SEG - HIST:SEG]
            rolled = [blk] + [pltpu.roll(blk, sh, 0) for sh in range(B_DIL, 8, B_DIL)]
            res = []
            for w in range(B_WIN):
                hi, lo_ = divmod(B_DIL * w, 8)
                o = HIST - 8 * hi
                res.append(rolled[lo_ // B_DIL][o:o + SEG])
            return res

        def qk():
            qs, ks = [], []
            for j in range(NT):
                qs.append(_dot(hb, _unpack(bqkv_p[j])))
                ks.append(_dot(hb, _unpack(bqkv_p[NT + j])))
            for i, l in enumerate(layers):
                ss = None
                for j in range(NT):
                    q = qs[j][i * SEG:(i + 1) * SEG] * b_scale
                    terms = [q * kw for kw in windows(l, i, j, ks[j])]
                    ss = terms if ss is None else [a + b for a, b in zip(ss, terms)]
                pos = (t - 1 - 2 * l) * SEG + lax.broadcasted_iota(jnp.int32, (SEG, 128), 0)
                logits = []
                for w, s in enumerate(ss):
                    s = s + pltpu.roll(s, 64, 1)
                    s = s + pltpu.roll(s, 32, 1)
                    logits.append(jnp.where(pos >= B_DIL * w, s, NEG) if masked else s)
                m = logits[0]
                for w in range(1, B_WIN):
                    m = jnp.maximum(m, logits[w])
                es = [jnp.exp(lg - m) for lg in logits]
                den = es[0]
                for w in range(1, B_WIN):
                    den = den + es[w]
                st['p'].append((es, 1.0 / den))

        def v_stage(j):
            vj = _dot(hb, _unpack(bqkv_p[2 * NT + j]))
            outs = []
            for i, l in enumerate(layers):
                es, inv = st['p'][i]
                vw = windows(l, i, NT + j, vj)
                acc = es[0] * vw[0]
                for w in range(1, B_WIN):
                    acc = acc + es[w] * vw[w]
                outs.append(acc * inv)
            st['o', j] = _cat0(outs).astype(BF16)

        def o_stage(j):
            st['y'] = st['y'] + _dot(st.pop(('o', j)), _unpack(bwo_p[j * 64:(j + 1) * 64, :]))

        def fin():
            for i, l in enumerate(layers):
                yl = st['y'][i * SEG:(i + 1) * SEG]
                if l == 0:
                    x2_ref[...] = yl
                    h_ref[RL:RT, :] = _ln(yl).astype(BF16)
                else:
                    if isinstance(t, int):
                        row = (t - 3) * SEG
                    else:
                        row = pl.multiple_of(jnp.maximum(t - 3, 0) * SEG, SEG)
                    out_ref[pl.ds(row, SEG), :] = yl.astype(out_ref.dtype)

        return qk, v_stage, o_stage, fin

    def softmax2(s, first, valid, fill):
        s = jnp.where(valid, s * a_scale, fill)
        m1 = jnp.max(jnp.where(first, s, PADNEG), axis=-1, keepdims=True)
        m2 = jnp.max(jnp.where(first, PADNEG, s), axis=-1, keepdims=True)
        e = jnp.exp(s - jnp.where(first, m1, m2))
        e1 = jnp.where(first, e, 0.0)
        e2 = jnp.where(first, 0.0, e)
        l1 = jnp.sum(e1, axis=-1, keepdims=True)
        l2 = jnp.sum(e2, axis=-1, keepdims=True)
        inv = 1.0 / jnp.where(first, l1, l2)
        return e, e1, e2, inv

    def make_joint():
        rr = lax.broadcasted_iota(jnp.int32, (RT, 128), 0)
        cc = lax.broadcasted_iota(jnp.int32, (RT, 128), 1)
        lay1 = rr < RV
        first = cc < jnp.where(lay1, RL, RT)
        key = jnp.where(first, cc, cc - RL)
        exists = jnp.where(lay1, RV - 1 - key, key - RV) >= 0
        allowed = (key <= rr) | (lay1 & (key >= SEG)) | ((rr >= RV) & (rr < RL))
        valid = exists & allowed
        fill = jnp.where(exists, NEG, PADNEG)
        lo = cc < (DH - 128)
        z48 = jnp.zeros((128 - RT, 128), F32)
        z32 = jnp.zeros((128 - 2 * RL, 128), F32)

        def prep_q(a):
            return (a[:, 0:128].astype(BF16), a[0:RV, 128:256], a[RV:RT, 128:256], a[:, 256:384].astype(BF16))

        def prep_kv(a):
            mid = a[:, 128:256]
            tlo = jnp.where(lo, mid, 0.0)
            thi = jnp.where(lo, 0.0, mid)
            return (_cat0([a[:, 0:128], z48]).astype(BF16),
                    _cat0([tlo[0:RL], thi[0:RL], z32]).astype(BF16),
                    _cat0([z32, tlo[SEG:RT], thi[SEG:RT]]).astype(BF16),
                    _cat0([z48, a[:, 256:384]]).astype(BF16))

        def qk(q, k):
            t0 = _dot_nt(q[0], k[0])
            t2 = _dot_nt(q[3], k[3])
            t1a = _dot_nt(q[1], k[1])
            t1b = _dot_nt(q[2], k[2])
            s = jnp.where(first, t0, t2) + _cat0([t1a, t1b])
            e, e1, e2, inv = softmax2(s, first, valid, fill)
            pa = e * inv
            return (e1 * inv).astype(BF16), pa[0:RV], pa[RV:RT], (e2 * inv).astype(BF16)

        def pv(pr, v):
            o0 = _dot(pr[0], v[0])
            o2 = _dot(pr[3], v[3])
            o1a = _dot(pr[1], v[1])
            o1b = _dot(pr[2], v[2])
            return _cat1([o0, _cat0([o1a, o1b]), o2]).astype(BF16)

        return prep_q, prep_kv, qk, pv

    def make_single(layer, last=False):
        nq = SEG if last else RV
        rr = lax.broadcasted_iota(jnp.int32, (nq, 2 * RV), 0) + (M if last else 0)
        cc = lax.broadcasted_iota(jnp.int32, (nq, 2 * RV), 1)
        first = cc < RV
        kc = jnp.where(first, cc, cc - RV)
        if layer == 0:
            valid = (kc >= SEG) | (kc <= rr)
        else:
            valid = (rr < M) | (kc <= rr)
        lo = lax.broadcasted_iota(jnp.int32, (RV, PW), 1) < DH
        lhs = (lambda a: a.astype(BF16)) if last else (lambda a: a)

        def prep_kv(a):
            return _cat0([jnp.where(lo, a, 0.0), jnp.where(lo, 0.0, a)]).astype(BF16)

        def qk(q, k):
            e, _, _, inv = softmax2(_dot_nt(q, k), first, valid, NEG)
            return lhs(e * inv)

        def pv(pr, v):
            return lhs(_dot(pr, v))

        return lhs, prep_kv, qk, pv

    def step(t, a_layers, b_layers, light=False, last=False, masked=True, deep=0,
             head_start=False, b_sched=(0, 2, 2, 2)):
        r0 = 0 if 0 in a_layers else RV
        if len(a_layers) == 2:
            h = h_ref[SEG if light else 0:RT, :]
            prep_q, prep_kv, qk, pv = make_joint()
        else:
            h = h_ref[0:RL, :].astype(F32)[0:RV] if r0 == 0 else h_ref[SEG:RT, :].astype(F32)[M:RL]
            prep_q, prep_kv, qk, pv = make_single(a_layers[0], last)

        def proj(i, p):
            r = _dot(h_ref[RL:RT, :] if (last and i == 0) else h, _unpack(wqkv_p[i, p]))
            if light:
                r = _cat0([pre_ref[i, p, pl.ds(pl.multiple_of((t - 2) * SEG, SEG), SEG), :], r])
            return r

        acc = [None]
        OLAG = 3 if len(a_layers) == 2 else 5

        def oproj(p, o):
            part = _dot(o, _unpack(wo_p[p]))
            acc[0] = part if acc[0] is None else acc[0] + part

        def xrows(seg):
            if isinstance(seg, int):
                return x_ref[seg * SEG:(seg + 1) * SEG, :].astype(F32)
            return x_ref[pl.ds(pl.multiple_of(seg * SEG, SEG), SEG), :].astype(F32)

        hooks = {p: [] for p in range(NP)}
        if b_layers:
            b_qk, b_v, b_o, b_fin = make_b(t, b_layers, masked)
            at, v0, dv, lag = b_sched
            for j in range(NT):
                hooks[at + v0 + j * dv + lag].append(functools.partial(b_o, j))
            hooks[at + v0 + (NT - 1) * dv + lag].append(b_fin)
            for j in range(NT):
                hooks[at + v0 + j * dv].append(functools.partial(b_v, j))
            hooks[at].append(b_qk)
        x2 = x2_ref[...] if 1 in a_layers else None

        if head_start:
            heads = [_dot(h_ref[0:SEG, :], _unpack(wqkv_p[i, 0])) for i in range(2)]
            rest = [_dot(h_ref[SEG:RT, :], _unpack(wqkv_p[i, 0])) for i in range(2)]
            q, k = [_cat0([a, b]) for a, b in zip(heads, rest)]
            q, k = prep_q(q), prep_kv(k)
        else:
            q = prep_q(proj(0, 0))
            k = prep_kv(proj(1, 0))
        vs = {0: prep_kv(proj(2, 0))}
        early_v = light or len(a_layers) == 1
        os_ = {}
        prs = {}

        def do_pv(p):
            os_[p] = pv(prs.pop(p), vs.pop(p))

        for p in range(NP):
            prs[p] = qk(q, k)
            if p + 1 < NP:
                q = prep_q(proj(0, p + 1))
                k = prep_kv(proj(1, p + 1))
                if early_v:
                    vs[p + 1] = prep_kv(proj(2, p + 1))
            else:
                for pp in range(p - deep, p):
                    do_pv(pp)
                if 0 in a_layers:
                    nxt = min(t + 1, NSEG - 1) if isinstance(t, int) else jnp.minimum(t + 1, NSEG - 1)
                    h_ref[0:SEG, :] = _ln(xrows(nxt)).astype(BF16)
                for pp in range(p - OLAG, p - 1):
                    oproj(pp, os_.pop(pp))
            if p + 1 == NP:
                do_pv(p)
            elif p >= deep:
                do_pv(p - deep)
            if p + 1 < NP and not early_v:
                vs[p + 1] = prep_kv(proj(2, p + 1))
            for f in hooks[p]:
                f()
            if p >= OLAG and p + 1 < NP:
                oproj(p - OLAG, os_.pop(p - OLAG))
        oproj(NP - 2, os_.pop(NP - 2))
        oproj(NP - 1, os_.pop(NP - 1))
        a = acc[0]
        if 0 in a_layers:
            xa_ref[0:SEG, :] = xrows(t) + a[0:SEG]
        if last:
            xa_ref[SEG:2 * SEG, :] = x2 + a
            return
        if 1 in a_layers:
            xa_ref[SEG:2 * SEG, :] = x2 + a[RL - r0:RT - r0]
        mem2 = a[RV - r0:RL - r0] if 1 in a_layers else mem0
        mem1 = a[SEG:RV] if 0 in a_layers else mem2
        h_ref[SEG:RL, :] = _cat0([mem1, mem2]).astype(BF16)

    def first_step():
        prep_q, prep_kv, qk, pv = make_single(0)

        def wait_group(p):
            for cp in cp_group(p):
                cp.wait()

        def pair0(p, fine=False):
            ha = ha_ref[...]
            hb = _unpack(hb_ref[...])
            w = {}

            def load(i):
                if fine:
                    cp_fine(p, i).wait()
                w[i] = w_pairs[i][1][rows_of(p), :]
                wqkv_p[i, p] = _pack(w[i].T)

            def proj_a(i):
                r = _dot_nt(ha, w[i])
                pre_ref[i, p, 0:NPA * SEG, :] = r[RV:]
                return r[0:RV]

            def proj_b(i):
                pre_ref[i, p, NPA * SEG:, :] = _dot_nt(hb, w[i])

            if fine:
                load(0)
                q = prep_q(proj_a(0))
                proj_b(0)
                load(1)
                k = prep_kv(proj_a(1))
                proj_b(1)
                load(2)
                pr = qk(q, k)
                v = prep_kv(proj_a(2))
                proj_b(2)
                o_ref[p] = pv(pr, v)
                return
            for i in range(3):
                load(i)
            q = prep_q(proj_a(0))
            k = prep_kv(proj_a(1))
            v = prep_kv(proj_a(2))
            pr = qk(q, k)
            proj_b(0)
            proj_b(1)
            o_ref[p] = pv(pr, v)
            proj_b(2)

        def body1(p, carry):
            wait_group(p)
            pair0(p)
            return carry

        def body2(i, carry):
            wait_group(2 * i)
            wait_group(2 * i + 1)
            pair0(2 * i)
            pair0(2 * i + 1)
            return carry

        def body0(p, carry):
            pair0(p, fine=True)
            return carry

        lax.fori_loop(0, NFINE, body0, 0)
        lax.fori_loop(NFINE, 4, body1, 0)
        lax.fori_loop(2, NP // 2, body2, 0)
        cp_x1.start()
        cp_wo.wait()
        for cp in cp_b:
            cp.wait()
        a = None
        for p in range(NP):
            w = wo_ref[sl(p), :]
            wo_p[p] = _pack(w)
            part = _dot(o_ref[p], w)
            a = part if a is None else a + part
        xa_ref[0:SEG, :] = x_ref[0:SEG, :].astype(F32) + a[0:SEG]
        h_ref[0:SEG, :] = _ln(x_ref[SEG:2 * SEG, :].astype(F32)).astype(BF16)
        h_ref[SEG:RL, :] = _cat0([a[SEG:RV], mem0]).astype(BF16)

    first_step()
    for j in range(3):
        perm_qkv(j)
    perm_wo()
    step(1, (0,), (0,), deep=2, b_sched=(8, 2, 1, 1))

    def body_light(t, carry):
        step(t, (0, 1), (0, 1), light=True, b_sched=(0, 3, 2, 1))
        return carry

    lax.fori_loop(2, 2 + NPRE, body_light, 0)
    cp_x1.wait()

    T0 = 2 + NPRE
    NPAIR = (NSEG - T0) // 2

    def two_steps(t):
        step(t, (0, 1), (0, 1), masked=False)
        step(t + 1, (0, 1), (0, 1), masked=False, head_start=True)

    def body(i, carry):
        two_steps(T0 + 2 * i)
        return carry

    lax.fori_loop(0, NPAIR, body, 0)
    done = (T0 + 2 * NPAIR - 3) * SEG
    cp_o0 = pltpu.make_async_copy(out_ref.at[0:done], out_hbm.at[0:done], sem.at[6])
    cp_o0.start()
    for t in range(T0 + 2 * NPAIR, NSEG):
        step(t, (0, 1), (0, 1), masked=False)
    step(NSEG, (1,), (0, 1), masked=False, deep=1)
    cp_o1 = pltpu.make_async_copy(out_ref.at[done:S - 2 * SEG], out_hbm.at[done:S - 2 * SEG], sem.at[7])
    cp_o1.start()
    tails = [make_b(NSEG + 1, (1,), False)]
    step(NSEG + 1, (1,), (), last=True, deep=1)
    tails.append(make_b(NSEG + 2, (1,), False))
    for b_qk, b_v, _, _ in tails:
        b_qk()
        for j in range(NT):
            b_v(j)
    for _, _, b_o, b_fin in tails:
        for j in range(NT):
            b_o(j)
        b_fin()
    cp_o2 = pltpu.make_async_copy(out_ref.at[S - 2 * SEG:S], out_hbm.at[S - 2 * SEG:S], sem.at[0])
    cp_o2.start()
    cp_o0.wait()
    cp_o1.wait()
    cp_o2.wait()


def pallas_interleave_layers__memory_aug_recurrent_mem_tr__sliding_local_dilated__prompt_kernel(
    A_x: jax.Array,
    A_mem0: jax.Array,
    A_Wq: jax.Array,
    A_Wk: jax.Array,
    A_Wv: jax.Array,
    A_Wo: jax.Array,
    A_seg_len,
    B_x: jax.Array,
    B_wqkv: jax.Array,
    B_wo: jax.Array,
):
    B, S, D = A_x.shape
    H, DH = A_Wq.shape[1], A_Wq.shape[2]
    M = A_mem0.shape[1]
    SEG = A_seg_len if isinstance(A_seg_len, int) else 32
    assert B == 1 and M == 8 and SEG == 32 and DH == 192 and D == 640 and H % 2 == 0
    assert S % SEG == 0 and S // SEG >= NPRE + 4

    x = A_x.reshape(S, D)
    mem0 = A_mem0.reshape(M, D)
    wq = jnp.transpose(A_Wq, (1, 2, 0)).reshape(H * DH, D)
    wk = jnp.transpose(A_Wk, (1, 2, 0)).reshape(H * DH, D)
    wv = jnp.transpose(A_Wv, (1, 2, 0)).reshape(H * DH, D)
    wo = A_Wo.reshape(H * DH, D)

    hbm = pl.BlockSpec(memory_space=pl.ANY)
    out = pl.pallas_call(
        functools.partial(_kernel, S=S, D=D, H=H, DH=DH, M=M, SEG=SEG),
        out_shape=jax.ShapeDtypeStruct((S, D), A_x.dtype),
        in_specs=[hbm] * 8,
        out_specs=hbm,
        scratch_shapes=[
            pltpu.VMEM((M, D), BF16),
            pltpu.VMEM((S, D), BF16),
            pltpu.VMEM((S, D), BF16),
            pltpu.VMEM((H * DH, D), BF16),
            pltpu.VMEM((H * DH, D), BF16),
            pltpu.VMEM((H * DH, D), BF16),
            pltpu.VMEM((H * DH, D), BF16),
            pltpu.VMEM((3, D, D), BF16),
            pltpu.VMEM((D, D), BF16),
            pltpu.VMEM((3, H // 2, D // 2, 2 * DH), U32),
            pltpu.VMEM((H // 2, DH, D), U32),
            pltpu.VMEM((3 * D // 128, D // 2, 128), U32),
            pltpu.VMEM((D // 2, D), U32),
            pltpu.VMEM((2 * SEG + 2 * M, D), BF16),
            pltpu.VMEM((2 * SEG, D), F32),
            pltpu.VMEM((SEG, D), F32),
            pltpu.VMEM((2, 2 * D // 128, HIST, 128), F32),
            pltpu.VMEM((SEG + M + NPA * SEG, D), F32),
            pltpu.VMEM(((NPRE - NPA) * SEG // 2, D), U32),
            pltpu.VMEM((3, H // 2, NPRE * SEG, 2 * DH), F32),
            pltpu.VMEM((H // 2, SEG + M, 2 * DH), F32),
            pltpu.VMEM((4, D // 128, D + 24, 128), F32),
            pltpu.SemaphoreType.DMA((H // 2 + 3 * NFINE,)),
            pltpu.SemaphoreType.DMA((10,)),
        ],
        compiler_params=pltpu.CompilerParams(vmem_limit_bytes=120 * 1024 * 1024),
        name="pallas_wavefront",
    )(mem0, x, wq, wk, wv, wo, B_wqkv, B_wo)
    return out.reshape(B, S, D)
```

```python
import functools

import jax
import jax.numpy as jnp
from jax import lax
import jax.experimental.pallas as pl
import jax.experimental.pallas.tpu as pltpu

F32 = jnp.float32
BF16 = jnp.bfloat16
U32 = jnp.uint32

EPS = 1e-5
NEG = -1000000000.0
PADNEG = -3.0e38
B_HEADS = 32
B_WIN = 8
B_DIL = 2
NPRE = 11
NPA = 5
NFINE = 1
HIST = 16


def _ln(x):
    m = jnp.mean(x, axis=-1, keepdims=True)
    xc = x - m
    v = jnp.mean(xc * xc, axis=-1, keepdims=True)
    return xc * lax.rsqrt(v + EPS)


def _dot_nt(a, b):
    return lax.dot_general(a, b, (((1,), (1,)), ((), ())), precision=lax.Precision.DEFAULT,
                           preferred_element_type=F32)


def _dot(a, b):
    return lax.dot_general(a, b, (((1,), (0,)), ((), ())), precision=lax.Precision.DEFAULT,
                           preferred_element_type=F32)


def _pack(a):
    return pltpu.bitcast(a, U32)


def _unpack(a):
    return pltpu.bitcast(a, BF16)


def _cat0(xs):
    return jnp.concatenate(xs, axis=0)


def _cat1(xs):
    return jnp.concatenate(xs, axis=1)


def _kernel(mem0_hbm, x_hbm, wq_hbm, wk_hbm, wv_hbm, wo_hbm, bqkv_hbm, bwo_hbm,
            out_hbm,
            mem0_ref, x_ref, out_ref, wq_ref, wk_ref, wv_ref, wo_ref, bqkv_ref, bwo_ref,
            wqkv_p, wo_p, bqkv_p, bwo_p, h_ref, xa_ref, x2_ref, kv_ref, ha_ref, hb_ref, pre_ref, o_ref, tmp_ref, wsem, sem,
            *, S, D, H, DH, M, SEG):
    NSEG = S // SEG
    PW = 2 * DH
    NP = H // 2
    RV = SEG + M
    RL = SEG + 2 * M
    RT = 2 * SEG + 2 * M
    a_scale = DH ** (-0.5)
    b_dh = D // B_HEADS
    b_scale = b_dh ** (-0.5)
    NT = D // 128
    X0 = (NPRE + 3) * SEG

    def sl(p):
        return slice(p * PW, (p + 1) * PW)

    cp_m = pltpu.make_async_copy(mem0_hbm, mem0_ref, sem.at[8])
    cp_x0 = pltpu.make_async_copy(x_hbm.at[0:X0], x_ref.at[0:X0], sem.at[0])
    cp_x1 = pltpu.make_async_copy(x_hbm.at[X0:S], x_ref.at[X0:S], sem.at[1])
    cp_b = [pltpu.make_async_copy(bqkv_hbm.at[:, j * D:(j + 1) * D], bqkv_ref.at[j], sem.at[2 + j])
            for j in range(3)]
    cp_b.append(pltpu.make_async_copy(bwo_hbm, bwo_ref, sem.at[5]))
    cp_wo = pltpu.make_async_copy(wo_hbm, wo_ref, sem.at[9])
    w_pairs = ((wq_hbm, wq_ref), (wk_hbm, wk_ref), (wv_hbm, wv_ref))

    def rows_of(p):
        return pl.ds(p * PW if isinstance(p, int) else pl.multiple_of(p * PW, 128), PW)

    def cp_fine(p, i):
        src, dst = w_pairs[i]
        return pltpu.make_async_copy(src.at[rows_of(p)], dst.at[rows_of(p)], wsem.at[NP + 3 * p + i])

    def cp_group(p):
        return [pltpu.make_async_copy(src.at[rows_of(p)], dst.at[rows_of(p)], wsem.at[p])
                for src, dst in w_pairs]

    def start_group(p, carry):
        for cp in cp_group(p):
            cp.start()

        @pl.when(p == NP - 1)
        def _():
            cp_wo.start()

        return carry

    firsts = [[cp_m, cp_x0]] + [[cp_fine(p, i)] for p in range(NFINE) for i in range(3)]

    def start_first(i, carry):
        for n, cps in enumerate(firsts):
            @pl.when(i == n)
            def _():
                for cp in cps:
                    cp.start()

        return carry

    lax.fori_loop(0, len(firsts), start_first, 0)
    lax.fori_loop(NFINE, NP, start_group, 0)
    for cp in cp_b:
        cp.start()

    xa_ref[...] = jnp.zeros(xa_ref.shape, F32)
    kv_ref[...] = jnp.zeros(kv_ref.shape, F32)
    cp_m.wait()
    cp_x0.wait()
    mem0 = mem0_ref[...].astype(F32)
    h0 = _ln(x_ref[0:SEG, :].astype(F32))
    ha_ref[0:RV, :] = _cat0([h0, mem0])
    for i in range(NPRE):
        hi = _ln(x_ref[(2 + i) * SEG:(3 + i) * SEG, :].astype(F32))
        if i < NPA:
            ha_ref[RV + i * SEG:RV + (i + 1) * SEG, :] = hi
        else:
            hb_ref[(i - NPA) * SEG // 2:(i - NPA + 1) * SEG // 2, :] = _pack(hi.astype(BF16))

    def perm_rows(a, slot):
        a = a.astype(F32)
        for m in range(NT):
            tmp_ref[slot, m, 0:D, :] = a[:, m * 128:(m + 1) * 128]
        return _cat1([_cat0([tmp_ref[slot, m, pl.ds(d, B_HEADS, stride=b_dh), :] for d in range(b_dh)])
                      for m in range(NT)]).astype(BF16)

    def perm_qkv(j):
        wp = perm_rows(bqkv_ref[j].T, j).T
        for c in range(NT):
            bqkv_p[j * NT + c] = _pack(wp[:, c * 128:(c + 1) * 128])

    def perm_wo():
        bwo_p[...] = _pack(perm_rows(bwo_ref[...], 3))

    def make_b(t, layers, masked):
        xb = xa_ref[layers[0] * SEG:(layers[-1] + 1) * SEG, :]
        hb = _ln(xb).astype(BF16)
        st = {'y': xb, 'p': []}

        def windows(l, i, j, a):
            cur = a[i * SEG:(i + 1) * SEG]
            blk = _cat0([kv_ref[l, j], cur])
            kv_ref[l, j] = cur[SEG - HIST:SEG]
            rolled = [blk] + [pltpu.roll(blk, sh, 0) for sh in range(B_DIL, 8, B_DIL)]
            res = []
            for w in range(B_WIN):
                hi, lo_ = divmod(B_DIL * w, 8)
                o = HIST - 8 * hi
                res.append(rolled[lo_ // B_DIL][o:o + SEG])
            return res

        def qk():
            qs, ks = [], []
            for j in range(NT):
                qs.append(_dot(hb, _unpack(bqkv_p[j])))
                ks.append(_dot(hb, _unpack(bqkv_p[NT + j])))
            for i, l in enumerate(layers):
                ss = None
                for j in range(NT):
                    q = qs[j][i * SEG:(i + 1) * SEG] * b_scale
                    terms = [q * kw for kw in windows(l, i, j, ks[j])]
                    ss = terms if ss is None else [a + b for a, b in zip(ss, terms)]
                pos = (t - 1 - 2 * l) * SEG + lax.broadcasted_iota(jnp.int32, (SEG, 128), 0)
                logits = []
                for w, s in enumerate(ss):
                    s = s + pltpu.roll(s, 64, 1)
                    s = s + pltpu.roll(s, 32, 1)
                    logits.append(jnp.where(pos >= B_DIL * w, s, NEG) if masked else s)
                m = logits[0]
                for w in range(1, B_WIN):
                    m = jnp.maximum(m, logits[w])
                es = [jnp.exp(lg - m) for lg in logits]
                den = es[0]
                for w in range(1, B_WIN):
                    den = den + es[w]
                st['p'].append((es, 1.0 / den))

        def v_stage(j):
            vj = _dot(hb, _unpack(bqkv_p[2 * NT + j]))
            outs = []
            for i, l in enumerate(layers):
                es, inv = st['p'][i]
                vw = windows(l, i, NT + j, vj)
                acc = es[0] * vw[0]
                for w in range(1, B_WIN):
                    acc = acc + es[w] * vw[w]
                outs.append(acc * inv)
            st['o', j] = _cat0(outs).astype(BF16)

        def o_stage(j):
            st['y'] = st['y'] + _dot(st.pop(('o', j)), _unpack(bwo_p[j * 64:(j + 1) * 64, :]))

        def fin():
            for i, l in enumerate(layers):
                yl = st['y'][i * SEG:(i + 1) * SEG]
                if l == 0:
                    x2_ref[...] = yl
                    h_ref[RL:RT, :] = _ln(yl).astype(BF16)
                else:
                    if isinstance(t, int):
                        row = (t - 3) * SEG
                    else:
                        row = pl.multiple_of(jnp.maximum(t - 3, 0) * SEG, SEG)
                    out_ref[pl.ds(row, SEG), :] = yl.astype(out_ref.dtype)

        return qk, v_stage, o_stage, fin

    def softmax2(s, first, valid, fill):
        s = jnp.where(valid, s * a_scale, fill)
        m1 = jnp.max(jnp.where(first, s, PADNEG), axis=-1, keepdims=True)
        m2 = jnp.max(jnp.where(first, PADNEG, s), axis=-1, keepdims=True)
        e = jnp.exp(s - jnp.where(first, m1, m2))
        e1 = jnp.where(first, e, 0.0)
        e2 = jnp.where(first, 0.0, e)
        l1 = jnp.sum(e1, axis=-1, keepdims=True)
        l2 = jnp.sum(e2, axis=-1, keepdims=True)
        inv = 1.0 / jnp.where(first, l1, l2)
        return e, e1, e2, inv

    def make_joint():
        rr = lax.broadcasted_iota(jnp.int32, (RT, 128), 0)
        cc = lax.broadcasted_iota(jnp.int32, (RT, 128), 1)
        lay1 = rr < RV
        first = cc < jnp.where(lay1, RL, RT)
        key = jnp.where(first, cc, cc - RL)
        exists = jnp.where(lay1, RV - 1 - key, key - RV) >= 0
        allowed = (key <= rr) | (lay1 & (key >= SEG)) | ((rr >= RV) & (rr < RL))
        valid = exists & allowed
        fill = jnp.where(exists, NEG, PADNEG)
        lo = cc < (DH - 128)
        z48 = jnp.zeros((128 - RT, 128), F32)
        z32 = jnp.zeros((128 - 2 * RL, 128), F32)

        def prep_q(a):
            return (a[:, 0:128].astype(BF16), a[0:RV, 128:256], a[RV:RT, 128:256], a[:, 256:384].astype(BF16))

        def prep_kv(a):
            mid = a[:, 128:256]
            tlo = jnp.where(lo, mid, 0.0)
            thi = jnp.where(lo, 0.0, mid)
            return (_cat0([a[:, 0:128], z48]).astype(BF16),
                    _cat0([tlo[0:RL], thi[0:RL], z32]).astype(BF16),
                    _cat0([z32, tlo[SEG:RT], thi[SEG:RT]]).astype(BF16),
                    _cat0([z48, a[:, 256:384]]).astype(BF16))

        def qk(q, k):
            t0 = _dot_nt(q[0], k[0])
            t2 = _dot_nt(q[3], k[3])
            t1a = _dot_nt(q[1], k[1])
            t1b = _dot_nt(q[2], k[2])
            s = jnp.where(first, t0, t2) + _cat0([t1a, t1b])
            e, e1, e2, inv = softmax2(s, first, valid, fill)
            pa = e * inv
            return (e1 * inv).astype(BF16), pa[0:RV], pa[RV:RT], (e2 * inv).astype(BF16)

        def pv(pr, v):
            o0 = _dot(pr[0], v[0])
            o2 = _dot(pr[3], v[3])
            o1a = _dot(pr[1], v[1])
            o1b = _dot(pr[2], v[2])
            return _cat1([o0, _cat0([o1a, o1b]), o2])

        return prep_q, prep_kv, qk, pv

    def make_single(layer, last=False):
        nq = SEG if last else RV
        rr = lax.broadcasted_iota(jnp.int32, (nq, 2 * RV), 0) + (M if last else 0)
        cc = lax.broadcasted_iota(jnp.int32, (nq, 2 * RV), 1)
        first = cc < RV
        kc = jnp.where(first, cc, cc - RV)
        if layer == 0:
            valid = (kc >= SEG) | (kc <= rr)
        else:
            valid = (rr < M) | (kc <= rr)
        lo = lax.broadcasted_iota(jnp.int32, (RV, PW), 1) < DH
        lhs = (lambda a: a.astype(BF16)) if last else (lambda a: a)

        def prep_kv(a):
            return _cat0([jnp.where(lo, a, 0.0), jnp.where(lo, 0.0, a)]).astype(BF16)

        def qk(q, k):
            e, _, _, inv = softmax2(_dot_nt(q, k), first, valid, NEG)
            return lhs(e * inv)

        def pv(pr, v):
            return lhs(_dot(pr, v))

        return lhs, prep_kv, qk, pv

    def step(t, a_layers, b_layers, light=False, last=False, masked=True, deep=0,
             head_start=False, b_sched=(0, 2, 2, 2)):
        r0 = 0 if 0 in a_layers else RV
        if len(a_layers) == 2:
            h = h_ref[SEG if light else 0:RT, :]
            prep_q, prep_kv, qk, pv = make_joint()
        else:
            h = h_ref[0:RL, :].astype(F32)[0:RV] if r0 == 0 else h_ref[SEG:RT, :].astype(F32)[M:RL]
            prep_q, prep_kv, qk, pv = make_single(a_layers[0], last)

        drop1 = isinstance(t, int) and t == NSEG - 1

        def squeeze(a):
            return _cat0([a[0:SEG], a[RV:RT]])

        def expand(a):
            return _cat0([a[0:SEG], jnp.zeros((M, a.shape[1]), F32), a[SEG:RT - M]])

        hq = squeeze(h.astype(F32)) if drop1 else (h_ref[RL:RT, :] if last else h)

        def proj(i, p):
            r = _dot(hq if i == 0 else h, _unpack(wqkv_p[i, p]))
            if drop1 and i == 0:
                r = expand(r)
            if light:
                r = _cat0([pre_ref[i, p, pl.ds(pl.multiple_of((t - 2) * SEG, SEG), SEG), :], r])
            return r

        acc = [None]
        OLAG = 3 if len(a_layers) == 2 else 5

        def oproj(p, o):
            part = _dot(o, _unpack(wo_p[p]))
            acc[0] = part if acc[0] is None else acc[0] + part

        def xrows(seg):
            if isinstance(seg, int):
                return x_ref[seg * SEG:(seg + 1) * SEG, :].astype(F32)
            return x_ref[pl.ds(pl.multiple_of(seg * SEG, SEG), SEG), :].astype(F32)

        hooks = {p: [] for p in range(NP)}
        if b_layers:
            b_qk, b_v, b_o, b_fin = make_b(t, b_layers, masked)
            at, v0, dv, lag = b_sched
            for j in range(NT):
                hooks[at + v0 + j * dv + lag].append(functools.partial(b_o, j))
            hooks[at + v0 + (NT - 1) * dv + lag].append(b_fin)
            for j in range(NT):
                hooks[at + v0 + j * dv].append(functools.partial(b_v, j))
            hooks[at].append(b_qk)
        x2 = x2_ref[...] if 1 in a_layers else None

        if head_start:
            heads = [_dot(h_ref[0:SEG, :], _unpack(wqkv_p[i, 0])) for i in range(2)]
            rest = [_dot(h_ref[SEG:RT, :], _unpack(wqkv_p[i, 0])) for i in range(2)]
            q, k = [_cat0([a, b]) for a, b in zip(heads, rest)]
            q, k = prep_q(q), prep_kv(k)
        else:
            q = prep_q(proj(0, 0))
            k = prep_kv(proj(1, 0))
        vs = {0: prep_kv(proj(2, 0))}
        early_v = light or len(a_layers) == 1
        os_ = {}
        prs = {}

        def do_pv(p):
            o = pv(prs.pop(p), vs.pop(p))
            if len(a_layers) == 2:
                o = squeeze(o) if drop1 else o.astype(BF16)
            os_[p] = o

        for p in range(NP):
            prs[p] = qk(q, k)
            if p + 1 < NP:
                q = prep_q(proj(0, p + 1))
                k = prep_kv(proj(1, p + 1))
                if early_v:
                    vs[p + 1] = prep_kv(proj(2, p + 1))
            else:
                for pp in range(p - deep, p):
                    do_pv(pp)
                if 0 in a_layers and not drop1:
                    nxt = t + 1 if isinstance(t, int) else jnp.minimum(t + 1, NSEG - 1)
                    h_ref[0:SEG, :] = _ln(xrows(nxt)).astype(BF16)
                for pp in range(p - OLAG, p - 1):
                    oproj(pp, os_.pop(pp))
            if p + 1 == NP:
                do_pv(p)
            elif p >= deep:
                do_pv(p - deep)
            if p + 1 < NP and not early_v:
                vs[p + 1] = prep_kv(proj(2, p + 1))
            for f in hooks[p]:
                f()
            if p >= OLAG and p + 1 < NP:
                oproj(p - OLAG, os_.pop(p - OLAG))
        oproj(NP - 2, os_.pop(NP - 2))
        oproj(NP - 1, os_.pop(NP - 1))
        a = expand(acc[0]) if drop1 else acc[0]
        if 0 in a_layers:
            xa_ref[0:SEG, :] = xrows(t) + a[0:SEG]
        if last:
            xa_ref[SEG:2 * SEG, :] = x2 + a
            return
        if 1 in a_layers:
            xa_ref[SEG:2 * SEG, :] = x2 + a[RL - r0:RT - r0]
        mem2 = a[RV - r0:RL - r0] if 1 in a_layers else mem0
        mem1 = a[SEG:RV] if 0 in a_layers else mem2
        h_ref[SEG:RL, :] = _cat0([mem1, mem2]).astype(BF16)

    def first_step():
        prep_q, prep_kv, qk, pv = make_single(0)

        def wait_group(p):
            for cp in cp_group(p):
                cp.wait()

        def pair0(p, fine=False):
            ha = ha_ref[...]
            hb = _unpack(hb_ref[...])
            w = {}

            def load(i):
                if fine:
                    cp_fine(p, i).wait()
                w[i] = w_pairs[i][1][rows_of(p), :]
                wqkv_p[i, p] = _pack(w[i].T)

            def proj_a(i):
                r = _dot_nt(ha, w[i])
                pre_ref[i, p, 0:NPA * SEG, :] = r[RV:]
                return r[0:RV]

            def proj_b(i):
                pre_ref[i, p, NPA * SEG:, :] = _dot_nt(hb, w[i])

            if fine:
                load(0)
                q = prep_q(proj_a(0))
                proj_b(0)
                load(1)
                k = prep_kv(proj_a(1))
                proj_b(1)
                load(2)
                pr = qk(q, k)
                v = prep_kv(proj_a(2))
                proj_b(2)
                o_ref[p] = pv(pr, v)
                return
            for i in range(3):
                load(i)
            q = prep_q(proj_a(0))
            k = prep_kv(proj_a(1))
            v = prep_kv(proj_a(2))
            pr = qk(q, k)
            proj_b(0)
            proj_b(1)
            o_ref[p] = pv(pr, v)
            proj_b(2)

        def body1(p, carry):
            wait_group(p)
            pair0(p)
            return carry

        def body2(i, carry):
            wait_group(2 * i)
            wait_group(2 * i + 1)
            pair0(2 * i)
            pair0(2 * i + 1)
            return carry

        def body0(p, carry):
            pair0(p, fine=True)
            return carry

        lax.fori_loop(0, NFINE, body0, 0)
        lax.fori_loop(NFINE, 4, body1, 0)
        lax.fori_loop(2, NP // 2, body2, 0)
        cp_x1.start()
        cp_wo.wait()
        for cp in cp_b:
            cp.wait()
        a = None
        for p in range(NP):
            w = wo_ref[sl(p), :]
            wo_p[p] = _pack(w)
            part = _dot(o_ref[p], w)
            a = part if a is None else a + part
        xa_ref[0:SEG, :] = x_ref[0:SEG, :].astype(F32) + a[0:SEG]
        h_ref[0:SEG, :] = _ln(x_ref[SEG:2 * SEG, :].astype(F32)).astype(BF16)
        h_ref[SEG:RL, :] = _cat0([a[SEG:RV], mem0]).astype(BF16)

    first_step()
    for j in range(3):
        perm_qkv(j)
    perm_wo()
    step(1, (0,), (0,), deep=2, b_sched=(8, 2, 1, 1))

    def body_light(t, carry):
        step(t, (0, 1), (0, 1), light=True, b_sched=(0, 3, 2, 1))
        return carry

    lax.fori_loop(2, 2 + NPRE, body_light, 0)
    cp_x1.wait()

    T0 = 2 + NPRE
    NPAIR = (NSEG - T0) // 2

    def two_steps(t):
        step(t, (0, 1), (0, 1), masked=False)
        step(t + 1, (0, 1), (0, 1), masked=False, head_start=True)

    def body(i, carry):
        two_steps(T0 + 2 * i)
        return carry

    lax.fori_loop(0, NPAIR, body, 0)
    done = (T0 + 2 * NPAIR - 3) * SEG
    cp_o0 = pltpu.make_async_copy(out_ref.at[0:done], out_hbm.at[0:done], sem.at[6])
    cp_o0.start()
    for t in range(T0 + 2 * NPAIR, NSEG):
        step(t, (0, 1), (0, 1), masked=False)
    step(NSEG, (1,), (0, 1), masked=False, deep=1)
    cp_o1 = pltpu.make_async_copy(out_ref.at[done:S - 2 * SEG], out_hbm.at[done:S - 2 * SEG], sem.at[7])
    cp_o1.start()
    tails = [make_b(NSEG + 1, (1,), False)]
    step(NSEG + 1, (1,), (), last=True, deep=1)
    tails.append(make_b(NSEG + 2, (1,), False))
    for b_qk, b_v, _, _ in tails:
        b_qk()
        for j in range(NT):
            b_v(j)
    for _, _, b_o, b_fin in tails:
        for j in range(NT):
            b_o(j)
        b_fin()
    cp_o2 = pltpu.make_async_copy(out_ref.at[S - 2 * SEG:S], out_hbm.at[S - 2 * SEG:S], sem.at[0])
    cp_o2.start()
    cp_o0.wait()
    cp_o1.wait()
    cp_o2.wait()


def pallas_interleave_layers__memory_aug_recurrent_mem_tr__sliding_local_dilated__prompt_kernel(
    A_x: jax.Array,
    A_mem0: jax.Array,
    A_Wq: jax.Array,
    A_Wk: jax.Array,
    A_Wv: jax.Array,
    A_Wo: jax.Array,
    A_seg_len,
    B_x: jax.Array,
    B_wqkv: jax.Array,
    B_wo: jax.Array,
):
    B, S, D = A_x.shape
    H, DH = A_Wq.shape[1], A_Wq.shape[2]
    M = A_mem0.shape[1]
    SEG = A_seg_len if isinstance(A_seg_len, int) else 32
    assert B == 1 and M == 8 and SEG == 32 and DH == 192 and D == 640 and H % 2 == 0
    assert S % SEG == 0 and S // SEG >= NPRE + 4

    x = A_x.reshape(S, D)
    mem0 = A_mem0.reshape(M, D)
    wq = jnp.transpose(A_Wq, (1, 2, 0)).reshape(H * DH, D)
    wk = jnp.transpose(A_Wk, (1, 2, 0)).reshape(H * DH, D)
    wv = jnp.transpose(A_Wv, (1, 2, 0)).reshape(H * DH, D)
    wo = A_Wo.reshape(H * DH, D)

    hbm = pl.BlockSpec(memory_space=pl.ANY)
    out = pl.pallas_call(
        functools.partial(_kernel, S=S, D=D, H=H, DH=DH, M=M, SEG=SEG),
        out_shape=jax.ShapeDtypeStruct((S, D), A_x.dtype),
        in_specs=[hbm] * 8,
        out_specs=hbm,
        scratch_shapes=[
            pltpu.VMEM((M, D), BF16),
            pltpu.VMEM((S, D), BF16),
            pltpu.VMEM((S, D), BF16),
            pltpu.VMEM((H * DH, D), BF16),
            pltpu.VMEM((H * DH, D), BF16),
            pltpu.VMEM((H * DH, D), BF16),
            pltpu.VMEM((H * DH, D), BF16),
            pltpu.VMEM((3, D, D), BF16),
            pltpu.VMEM((D, D), BF16),
            pltpu.VMEM((3, H // 2, D // 2, 2 * DH), U32),
            pltpu.VMEM((H // 2, DH, D), U32),
            pltpu.VMEM((3 * D // 128, D // 2, 128), U32),
            pltpu.VMEM((D // 2, D), U32),
            pltpu.VMEM((2 * SEG + 2 * M, D), BF16),
            pltpu.VMEM((2 * SEG, D), F32),
            pltpu.VMEM((SEG, D), F32),
            pltpu.VMEM((2, 2 * D // 128, HIST, 128), F32),
            pltpu.VMEM((SEG + M + NPA * SEG, D), F32),
            pltpu.VMEM(((NPRE - NPA) * SEG // 2, D), U32),
            pltpu.VMEM((3, H // 2, NPRE * SEG, 2 * DH), F32),
            pltpu.VMEM((H // 2, SEG + M, 2 * DH), F32),
            pltpu.VMEM((4, D // 128, D + 24, 128), F32),
            pltpu.SemaphoreType.DMA((H // 2 + 3 * NFINE,)),
            pltpu.SemaphoreType.DMA((10,)),
        ],
        compiler_params=pltpu.CompilerParams(vmem_limit_bytes=120 * 1024 * 1024),
        name="pallas_wavefront",
    )(mem0, x, wq, wk, wv, wo, B_wqkv, B_wo)
    return out.reshape(B, S, D)
```

```python
import functools

import jax
import jax.numpy as jnp
from jax import lax
import jax.experimental.pallas as pl
import jax.experimental.pallas.tpu as pltpu

F32 = jnp.float32
BF16 = jnp.bfloat16
U32 = jnp.uint32

EPS = 1e-5
NEG = -1000000000.0
PADNEG = -3.0e38
B_HEADS = 32
B_WIN = 8
B_DIL = 2
NPRE = 11
NPA = 5
NFINE = 1
HIST = 16


def _ln(x):
    m = jnp.mean(x, axis=-1, keepdims=True)
    xc = x - m
    v = jnp.mean(xc * xc, axis=-1, keepdims=True)
    return xc * lax.rsqrt(v + EPS)


def _dot_nt(a, b):
    return lax.dot_general(a, b, (((1,), (1,)), ((), ())), precision=lax.Precision.DEFAULT,
                           preferred_element_type=F32)


def _dot(a, b):
    return lax.dot_general(a, b, (((1,), (0,)), ((), ())), precision=lax.Precision.DEFAULT,
                           preferred_element_type=F32)


def _pack(a):
    return pltpu.bitcast(a, U32)


def _unpack(a):
    return pltpu.bitcast(a, BF16)


def _cat0(xs):
    return jnp.concatenate(xs, axis=0)


def _cat1(xs):
    return jnp.concatenate(xs, axis=1)


def _kernel(mem0_hbm, x_hbm, wq_hbm, wk_hbm, wv_hbm, wo_hbm, bqkv_hbm, bwo_hbm,
            out_hbm,
            mem0_ref, x_ref, out_ref, wq_ref, wk_ref, wv_ref, wo_ref, bqkv_ref, bwo_ref,
            wqkv_p, wo_p, bqkv_p, bwo_p, h_ref, xa_ref, x2_ref, kv_ref, ha_ref, hb_ref, pre_ref, o_ref, tmp_ref, wsem, sem,
            *, S, D, H, DH, M, SEG):
    NSEG = S // SEG
    PW = 2 * DH
    NP = H // 2
    RV = SEG + M
    RL = SEG + 2 * M
    RT = 2 * SEG + 2 * M
    a_scale = DH ** (-0.5)
    b_dh = D // B_HEADS
    b_scale = b_dh ** (-0.5)
    NT = D // 128
    X0 = (NPRE + 3) * SEG

    def sl(p):
        return slice(p * PW, (p + 1) * PW)

    cp_m = pltpu.make_async_copy(mem0_hbm, mem0_ref, sem.at[8])
    cp_x0 = pltpu.make_async_copy(x_hbm.at[0:X0], x_ref.at[0:X0], sem.at[0])
    cp_x1 = pltpu.make_async_copy(x_hbm.at[X0:S], x_ref.at[X0:S], sem.at[1])
    cp_b = [pltpu.make_async_copy(bqkv_hbm.at[:, j * D:(j + 1) * D], bqkv_ref.at[j], sem.at[2 + j])
            for j in range(3)]
    cp_b.append(pltpu.make_async_copy(bwo_hbm, bwo_ref, sem.at[5]))
    cp_wo = pltpu.make_async_copy(wo_hbm, wo_ref, sem.at[9])
    w_pairs = ((wq_hbm, wq_ref), (wk_hbm, wk_ref), (wv_hbm, wv_ref))

    def rows_of(p):
        return pl.ds(p * PW if isinstance(p, int) else pl.multiple_of(p * PW, 128), PW)

    def cp_fine(p, i):
        src, dst = w_pairs[i]
        return pltpu.make_async_copy(src.at[rows_of(p)], dst.at[rows_of(p)], wsem.at[NP + 3 * p + i])

    def cp_group(p):
        return [pltpu.make_async_copy(src.at[rows_of(p)], dst.at[rows_of(p)], wsem.at[p])
                for src, dst in w_pairs]

    def start_group(p, carry):
        for cp in cp_group(p):
            cp.start()

        @pl.when(p == NP - 1)
        def _():
            cp_wo.start()

        return carry

    firsts = [[cp_m, cp_x0]] + [[cp_fine(p, i)] for p in range(NFINE) for i in range(3)]

    def start_first(i, carry):
        for n, cps in enumerate(firsts):
            @pl.when(i == n)
            def _():
                for cp in cps:
                    cp.start()

        return carry

    lax.fori_loop(0, len(firsts), start_first, 0)
    lax.fori_loop(NFINE, NP, start_group, 0)
    for cp in cp_b:
        cp.start()

    xa_ref[...] = jnp.zeros(xa_ref.shape, F32)
    kv_ref[...] = jnp.zeros(kv_ref.shape, F32)
    cp_m.wait()
    cp_x0.wait()
    mem0 = mem0_ref[...].astype(F32)
    h0 = _ln(x_ref[0:SEG, :].astype(F32))
    ha_ref[0:RV, :] = _cat0([h0, mem0])
    for i in range(NPRE):
        hi = _ln(x_ref[(2 + i) * SEG:(3 + i) * SEG, :].astype(F32))
        if i < NPA:
            ha_ref[RV + i * SEG:RV + (i + 1) * SEG, :] = hi
        else:
            hb_ref[(i - NPA) * SEG // 2:(i - NPA + 1) * SEG // 2, :] = _pack(hi.astype(BF16))

    def perm_rows(a, slot):
        a = a.astype(F32)
        for m in range(NT):
            tmp_ref[slot, m, 0:D, :] = a[:, m * 128:(m + 1) * 128]
        return _cat1([_cat0([tmp_ref[slot, m, pl.ds(d, B_HEADS, stride=b_dh), :] for d in range(b_dh)])
                      for m in range(NT)]).astype(BF16)

    def perm_qkv(j):
        wp = perm_rows(bqkv_ref[j].T, j).T
        for c in range(NT):
            bqkv_p[j * NT + c] = _pack(wp[:, c * 128:(c + 1) * 128])

    def perm_wo():
        bwo_p[...] = _pack(perm_rows(bwo_ref[...], 3))

    def make_b(t, layers, masked):
        xb = xa_ref[layers[0] * SEG:(layers[-1] + 1) * SEG, :]
        hb = _ln(xb).astype(BF16)
        st = {'y': xb, 'p': []}

        def windows(l, i, j, a):
            cur = a[i * SEG:(i + 1) * SEG]
            blk = _cat0([kv_ref[l, j], cur])
            kv_ref[l, j] = cur[SEG - HIST:SEG]
            rolled = [blk] + [pltpu.roll(blk, sh, 0) for sh in range(B_DIL, 8, B_DIL)]
            res = []
            for w in range(B_WIN):
                hi, lo_ = divmod(B_DIL * w, 8)
                o = HIST - 8 * hi
                res.append(rolled[lo_ // B_DIL][o:o + SEG])
            return res

        def qk():
            qs, ks = [], []
            for j in range(NT):
                qs.append(_dot(hb, _unpack(bqkv_p[j])))
                ks.append(_dot(hb, _unpack(bqkv_p[NT + j])))
            for i, l in enumerate(layers):
                ss = None
                for j in range(NT):
                    q = qs[j][i * SEG:(i + 1) * SEG] * b_scale
                    terms = [q * kw for kw in windows(l, i, j, ks[j])]
                    ss = terms if ss is None else [a + b for a, b in zip(ss, terms)]
                pos = (t - 1 - 2 * l) * SEG + lax.broadcasted_iota(jnp.int32, (SEG, 128), 0)
                logits = []
                for w, s in enumerate(ss):
                    s = s + pltpu.roll(s, 64, 1)
                    s = s + pltpu.roll(s, 32, 1)
                    logits.append(jnp.where(pos >= B_DIL * w, s, NEG) if masked else s)
                m = logits[0]
                for w in range(1, B_WIN):
                    m = jnp.maximum(m, logits[w])
                es = [jnp.exp(lg - m) for lg in logits]
                den = es[0]
                for w in range(1, B_WIN):
                    den = den + es[w]
                st['p'].append((es, 1.0 / den))

        def v_stage(j):
            vj = _dot(hb, _unpack(bqkv_p[2 * NT + j]))
            outs = []
            for i, l in enumerate(layers):
                es, inv = st['p'][i]
                vw = windows(l, i, NT + j, vj)
                acc = es[0] * vw[0]
                for w in range(1, B_WIN):
                    acc = acc + es[w] * vw[w]
                outs.append(acc * inv)
            st['o', j] = _cat0(outs).astype(BF16)

        def o_stage(j):
            st['y'] = st['y'] + _dot(st.pop(('o', j)), _unpack(bwo_p[j * 64:(j + 1) * 64, :]))

        def fin():
            for i, l in enumerate(layers):
                yl = st['y'][i * SEG:(i + 1) * SEG]
                if l == 0:
                    x2_ref[...] = yl
                    h_ref[RL:RT, :] = _ln(yl).astype(BF16)
                else:
                    if isinstance(t, int):
                        row = (t - 3) * SEG
                    else:
                        row = pl.multiple_of(jnp.maximum(t - 3, 0) * SEG, SEG)
                    out_ref[pl.ds(row, SEG), :] = yl.astype(out_ref.dtype)

        return qk, v_stage, o_stage, fin

    def softmax2(s, first, valid, fill):
        s = jnp.where(valid, s * a_scale, fill)
        m1 = jnp.max(jnp.where(first, s, PADNEG), axis=-1, keepdims=True)
        m2 = jnp.max(jnp.where(first, PADNEG, s), axis=-1, keepdims=True)
        e = jnp.exp(s - jnp.where(first, m1, m2))
        e1 = jnp.where(first, e, 0.0)
        e2 = jnp.where(first, 0.0, e)
        l1 = jnp.sum(e1, axis=-1, keepdims=True)
        l2 = jnp.sum(e2, axis=-1, keepdims=True)
        inv = 1.0 / jnp.where(first, l1, l2)
        return e, e1, e2, inv

    def make_joint(packed):
        rr = lax.broadcasted_iota(jnp.int32, (RT, 128), 0)
        cc = lax.broadcasted_iota(jnp.int32, (RT, 128), 1)
        lay1 = rr < RV
        first = cc < jnp.where(lay1, RL, RT)
        key = jnp.where(first, cc, cc - RL)
        exists = jnp.where(lay1, RV - 1 - key, key - RV) >= 0
        allowed = (key <= rr) | (lay1 & (key >= SEG)) | ((rr >= RV) & (rr < RL))
        valid = exists & allowed
        fill = jnp.where(exists, NEG, PADNEG)
        lo = cc < (DH - 128)
        z48 = jnp.zeros((128 - RT, 128), F32)
        z32 = jnp.zeros((128 - 2 * RL, 128), F32)
        lhs = (lambda a: a.astype(BF16)) if packed else (lambda a: a)

        def prep_q(a):
            return lhs(a[:, 0:128]), a[0:RV, 128:256], a[RV:RT, 128:256], lhs(a[:, 256:384])

        def prep_kv(a):
            mid = a[:, 128:256]
            tlo = jnp.where(lo, mid, 0.0)
            thi = jnp.where(lo, 0.0, mid)
            return (_cat0([a[:, 0:128], z48]).astype(BF16),
                    _cat0([tlo[0:RL], thi[0:RL], z32]).astype(BF16),
                    _cat0([z32, tlo[SEG:RT], thi[SEG:RT]]).astype(BF16),
                    _cat0([z48, a[:, 256:384]]).astype(BF16))

        def qk(q, k):
            t0 = _dot_nt(q[0], k[0])
            t2 = _dot_nt(q[3], k[3])
            t1a = _dot_nt(q[1], k[1])
            t1b = _dot_nt(q[2], k[2])
            s = jnp.where(first, t0, t2) + _cat0([t1a, t1b])
            e, e1, e2, inv = softmax2(s, first, valid, fill)
            pa = e * inv
            return lhs(e1 * inv), pa[0:RV], pa[RV:RT], lhs(e2 * inv)

        def pv(pr, v):
            o0 = _dot(pr[0], v[0])
            o2 = _dot(pr[3], v[3])
            o1a = _dot(pr[1], v[1])
            o1b = _dot(pr[2], v[2])
            return _cat1([o0, _cat0([o1a, o1b]), o2])

        return prep_q, prep_kv, qk, pv

    def make_single(layer, last=False):
        nq = SEG if last else RV
        rr = lax.broadcasted_iota(jnp.int32, (nq, 2 * RV), 0) + (M if last else 0)
        cc = lax.broadcasted_iota(jnp.int32, (nq, 2 * RV), 1)
        first = cc < RV
        kc = jnp.where(first, cc, cc - RV)
        if layer == 0:
            valid = (kc >= SEG) | (kc <= rr)
        else:
            valid = (rr < M) | (kc <= rr)
        lo = lax.broadcasted_iota(jnp.int32, (RV, PW), 1) < DH
        lhs = (lambda a: a.astype(BF16)) if last else (lambda a: a)

        def prep_kv(a):
            return _cat0([jnp.where(lo, a, 0.0), jnp.where(lo, 0.0, a)]).astype(BF16)

        def qk(q, k):
            e, _, _, inv = softmax2(_dot_nt(q, k), first, valid, NEG)
            return lhs(e * inv)

        def pv(pr, v):
            return lhs(_dot(pr, v))

        return lhs, prep_kv, qk, pv

    def step(t, a_layers, b_layers, light=False, last=False, masked=True, deep=0,
             head_start=False, b_sched=(0, 2, 2, 2)):
        r0 = 0 if 0 in a_layers else RV
        if len(a_layers) == 2:
            h = h_ref[SEG if light else 0:RT, :]
            prep_q, prep_kv, qk, pv = make_joint(light)
        else:
            h = h_ref[0:RL, :].astype(F32)[0:RV] if r0 == 0 else h_ref[SEG:RT, :].astype(F32)[M:RL]
            prep_q, prep_kv, qk, pv = make_single(a_layers[0], last)

        drop1 = isinstance(t, int) and t == NSEG - 1

        def squeeze(a):
            return _cat0([a[0:SEG], a[RV:RT]])

        def expand(a):
            return _cat0([a[0:SEG], jnp.zeros((M, a.shape[1]), F32), a[SEG:RT - M]])

        hq = squeeze(h.astype(F32)) if drop1 else (h_ref[RL:RT, :] if last else h)

        def proj(i, p):
            r = _dot(hq if i == 0 else h, _unpack(wqkv_p[i, p]))
            if drop1 and i == 0:
                r = expand(r)
            if light:
                r = _cat0([pre_ref[i, p, pl.ds(pl.multiple_of((t - 2) * SEG, SEG), SEG), :], r])
            return r

        acc = [None]
        OLAG = 3 if len(a_layers) == 2 else 5

        def oproj(p, o):
            part = _dot(o, _unpack(wo_p[p]))
            acc[0] = part if acc[0] is None else acc[0] + part

        def xrows(seg):
            if isinstance(seg, int):
                return x_ref[seg * SEG:(seg + 1) * SEG, :].astype(F32)
            return x_ref[pl.ds(pl.multiple_of(seg * SEG, SEG), SEG), :].astype(F32)

        hooks = {p: [] for p in range(NP)}
        if b_layers:
            b_qk, b_v, b_o, b_fin = make_b(t, b_layers, masked)
            at, v0, dv, lag = b_sched
            for j in range(NT):
                hooks[at + v0 + j * dv + lag].append(functools.partial(b_o, j))
            hooks[at + v0 + (NT - 1) * dv + lag].append(b_fin)
            for j in range(NT):
                hooks[at + v0 + j * dv].append(functools.partial(b_v, j))
            hooks[at].append(b_qk)
        x2 = x2_ref[...] if 1 in a_layers else None

        if head_start:
            heads = [_dot(h_ref[0:SEG, :], _unpack(wqkv_p[i, 0])) for i in range(2)]
            rest = [_dot(h_ref[SEG:RT, :], _unpack(wqkv_p[i, 0])) for i in range(2)]
            q, k = [_cat0([a, b]) for a, b in zip(heads, rest)]
            q, k = prep_q(q), prep_kv(k)
        else:
            q = prep_q(proj(0, 0))
            k = prep_kv(proj(1, 0))
        vs = {0: prep_kv(proj(2, 0))}
        early_v = light or len(a_layers) == 1
        os_ = {}
        prs = {}

        def do_pv(p):
            o = pv(prs.pop(p), vs.pop(p))
            if len(a_layers) == 2:
                o = squeeze(o) if drop1 else o.astype(BF16)
            os_[p] = o

        for p in range(NP):
            prs[p] = qk(q, k)
            if p + 1 < NP:
                q = prep_q(proj(0, p + 1))
                k = prep_kv(proj(1, p + 1))
                if early_v:
                    vs[p + 1] = prep_kv(proj(2, p + 1))
            else:
                for pp in range(p - deep, p):
                    do_pv(pp)
                if 0 in a_layers and not drop1:
                    nxt = t + 1 if isinstance(t, int) else jnp.minimum(t + 1, NSEG - 1)
                    h_ref[0:SEG, :] = _ln(xrows(nxt)).astype(BF16)
                for pp in range(p - OLAG, p - 1):
                    oproj(pp, os_.pop(pp))
            if p + 1 == NP:
                do_pv(p)
            elif p >= deep:
                do_pv(p - deep)
            if p + 1 < NP and not early_v:
                vs[p + 1] = prep_kv(proj(2, p + 1))
            for f in hooks[p]:
                f()
            if p >= OLAG and p + 1 < NP:
                oproj(p - OLAG, os_.pop(p - OLAG))
        oproj(NP - 2, os_.pop(NP - 2))
        oproj(NP - 1, os_.pop(NP - 1))
        a = expand(acc[0]) if drop1 else acc[0]
        if 0 in a_layers:
            xa_ref[0:SEG, :] = xrows(t) + a[0:SEG]
        if last:
            xa_ref[SEG:2 * SEG, :] = x2 + a
            return
        if 1 in a_layers:
            xa_ref[SEG:2 * SEG, :] = x2 + a[RL - r0:RT - r0]
        mem2 = a[RV - r0:RL - r0] if 1 in a_layers else mem0
        mem1 = a[SEG:RV] if 0 in a_layers else mem2
        h_ref[SEG:RL, :] = _cat0([mem1, mem2]).astype(BF16)

    def first_step():
        prep_q, prep_kv, qk, pv = make_single(0)

        def wait_group(p):
            for cp in cp_group(p):
                cp.wait()

        def pair0(p, fine=False):
            ha = ha_ref[...]
            hb = _unpack(hb_ref[...])
            w = {}

            def load(i):
                if fine:
                    cp_fine(p, i).wait()
                w[i] = w_pairs[i][1][rows_of(p), :]
                wqkv_p[i, p] = _pack(w[i].T)

            def proj_a(i):
                r = _dot_nt(ha, w[i])
                pre_ref[i, p, 0:NPA * SEG, :] = r[RV:]
                return r[0:RV]

            def proj_b(i):
                pre_ref[i, p, NPA * SEG:, :] = _dot_nt(hb, w[i])

            if fine:
                load(0)
                q = prep_q(proj_a(0))
                proj_b(0)
                load(1)
                k = prep_kv(proj_a(1))
                proj_b(1)
                load(2)
                pr = qk(q, k)
                v = prep_kv(proj_a(2))
                proj_b(2)
                o_ref[p] = pv(pr, v)
                return
            for i in range(3):
                load(i)
            q = prep_q(proj_a(0))
            k = prep_kv(proj_a(1))
            v = prep_kv(proj_a(2))
            pr = qk(q, k)
            proj_b(0)
            proj_b(1)
            o_ref[p] = pv(pr, v)
            proj_b(2)

        def body1(p, carry):
            wait_group(p)
            pair0(p)
            return carry

        def body2(i, carry):
            wait_group(2 * i)
            wait_group(2 * i + 1)
            pair0(2 * i)
            pair0(2 * i + 1)
            return carry

        def body0(p, carry):
            pair0(p, fine=True)
            return carry

        lax.fori_loop(0, NFINE, body0, 0)
        lax.fori_loop(NFINE, 4, body1, 0)
        lax.fori_loop(2, NP // 2, body2, 0)
        cp_x1.start()
        cp_wo.wait()
        for cp in cp_b:
            cp.wait()
        a = None
        for p in range(NP):
            w = wo_ref[sl(p), :]
            wo_p[p] = _pack(w)
            part = _dot(o_ref[p], w)
            a = part if a is None else a + part
        xa_ref[0:SEG, :] = x_ref[0:SEG, :].astype(F32) + a[0:SEG]
        h_ref[0:SEG, :] = _ln(x_ref[SEG:2 * SEG, :].astype(F32)).astype(BF16)
        h_ref[SEG:RL, :] = _cat0([a[SEG:RV], mem0]).astype(BF16)

    first_step()
    for j in range(3):
        perm_qkv(j)
    perm_wo()
    step(1, (0,), (0,), deep=2, b_sched=(8, 2, 1, 1))

    def body_light(t, carry):
        step(t, (0, 1), (0, 1), light=True, b_sched=(0, 3, 2, 1))
        return carry

    lax.fori_loop(2, 2 + NPRE, body_light, 0)
    cp_x1.wait()

    T0 = 2 + NPRE
    NPAIR = (NSEG - T0) // 2

    def two_steps(t):
        step(t, (0, 1), (0, 1), masked=False)
        step(t + 1, (0, 1), (0, 1), masked=False, head_start=True)

    def body(i, carry):
        two_steps(T0 + 2 * i)
        return carry

    lax.fori_loop(0, NPAIR, body, 0)
    done = (T0 + 2 * NPAIR - 3) * SEG
    cp_o0 = pltpu.make_async_copy(out_ref.at[0:done], out_hbm.at[0:done], sem.at[6])
    cp_o0.start()
    for t in range(T0 + 2 * NPAIR, NSEG):
        step(t, (0, 1), (0, 1), masked=False)
    step(NSEG, (1,), (0, 1), masked=False, deep=1)
    cp_o1 = pltpu.make_async_copy(out_ref.at[done:S - 2 * SEG], out_hbm.at[done:S - 2 * SEG], sem.at[7])
    cp_o1.start()
    tails = [make_b(NSEG + 1, (1,), False)]
    step(NSEG + 1, (1,), (), last=True, deep=1)
    tails.append(make_b(NSEG + 2, (1,), False))
    for b_qk, b_v, _, _ in tails:
        b_qk()
        for j in range(NT):
            b_v(j)
    for _, _, b_o, b_fin in tails:
        for j in range(NT):
            b_o(j)
        b_fin()
    cp_o2 = pltpu.make_async_copy(out_ref.at[S - 2 * SEG:S], out_hbm.at[S - 2 * SEG:S], sem.at[0])
    cp_o2.start()
    cp_o0.wait()
    cp_o1.wait()
    cp_o2.wait()


def pallas_interleave_layers__memory_aug_recurrent_mem_tr__sliding_local_dilated__prompt_kernel(
    A_x: jax.Array,
    A_mem0: jax.Array,
    A_Wq: jax.Array,
    A_Wk: jax.Array,
    A_Wv: jax.Array,
    A_Wo: jax.Array,
    A_seg_len,
    B_x: jax.Array,
    B_wqkv: jax.Array,
    B_wo: jax.Array,
):
    B, S, D = A_x.shape
    H, DH = A_Wq.shape[1], A_Wq.shape[2]
    M = A_mem0.shape[1]
    SEG = A_seg_len if isinstance(A_seg_len, int) else 32
    assert B == 1 and M == 8 and SEG == 32 and DH == 192 and D == 640 and H % 2 == 0
    assert S % SEG == 0 and S // SEG >= NPRE + 4

    x = A_x.reshape(S, D)
    mem0 = A_mem0.reshape(M, D)
    wq = jnp.transpose(A_Wq, (1, 2, 0)).reshape(H * DH, D)
    wk = jnp.transpose(A_Wk, (1, 2, 0)).reshape(H * DH, D)
    wv = jnp.transpose(A_Wv, (1, 2, 0)).reshape(H * DH, D)
    wo = A_Wo.reshape(H * DH, D)

    hbm = pl.BlockSpec(memory_space=pl.ANY)
    out = pl.pallas_call(
        functools.partial(_kernel, S=S, D=D, H=H, DH=DH, M=M, SEG=SEG),
        out_shape=jax.ShapeDtypeStruct((S, D), A_x.dtype),
        in_specs=[hbm] * 8,
        out_specs=hbm,
        scratch_shapes=[
            pltpu.VMEM((M, D), BF16),
            pltpu.VMEM((S, D), BF16),
            pltpu.VMEM((S, D), BF16),
            pltpu.VMEM((H * DH, D), BF16),
            pltpu.VMEM((H * DH, D), BF16),
            pltpu.VMEM((H * DH, D), BF16),
            pltpu.VMEM((H * DH, D), BF16),
            pltpu.VMEM((3, D, D), BF16),
            pltpu.VMEM((D, D), BF16),
            pltpu.VMEM((3, H // 2, D // 2, 2 * DH), U32),
            pltpu.VMEM((H // 2, DH, D), U32),
            pltpu.VMEM((3 * D // 128, D // 2, 128), U32),
            pltpu.VMEM((D // 2, D), U32),
            pltpu.VMEM((2 * SEG + 2 * M, D), BF16),
            pltpu.VMEM((2 * SEG, D), F32),
            pltpu.VMEM((SEG, D), F32),
            pltpu.VMEM((2, 2 * D // 128, HIST, 128), F32),
            pltpu.VMEM((SEG + M + NPA * SEG, D), F32),
            pltpu.VMEM(((NPRE - NPA) * SEG // 2, D), U32),
            pltpu.VMEM((3, H // 2, NPRE * SEG, 2 * DH), F32),
            pltpu.VMEM((H // 2, SEG + M, 2 * DH), F32),
            pltpu.VMEM((4, D // 128, D + 24, 128), F32),
            pltpu.SemaphoreType.DMA((H // 2 + 3 * NFINE,)),
            pltpu.SemaphoreType.DMA((10,)),
        ],
        compiler_params=pltpu.CompilerParams(vmem_limit_bytes=120 * 1024 * 1024),
        name="pallas_wavefront",
    )(mem0, x, wq, wk, wv, wo, B_wqkv, B_wo)
    return out.reshape(B, S, D)
```

```python
import functools

import jax
import jax.numpy as jnp
from jax import lax
import jax.experimental.pallas as pl
import jax.experimental.pallas.tpu as pltpu

F32 = jnp.float32
BF16 = jnp.bfloat16
U32 = jnp.uint32

EPS = 1e-5
NEG = -1000000000.0
PADNEG = -3.0e38
B_HEADS = 32
B_WIN = 8
B_DIL = 2
NPRE = 11
NPA = 5
NFINE = 1
HIST = 16


def _ln(x):
    m = jnp.mean(x, axis=-1, keepdims=True)
    xc = x - m
    v = jnp.mean(xc * xc, axis=-1, keepdims=True)
    return xc * lax.rsqrt(v + EPS)


def _dot_nt(a, b):
    return lax.dot_general(a, b, (((1,), (1,)), ((), ())), precision=lax.Precision.DEFAULT,
                           preferred_element_type=F32)


def _dot(a, b):
    return lax.dot_general(a, b, (((1,), (0,)), ((), ())), precision=lax.Precision.DEFAULT,
                           preferred_element_type=F32)


def _recip(x):
    r = pl.reciprocal(x, approx=True)
    return r * (2.0 - x * r)


def _pack(a):
    return pltpu.bitcast(a, U32)


def _unpack(a):
    return pltpu.bitcast(a, BF16)


def _cat0(xs):
    return jnp.concatenate(xs, axis=0)


def _cat1(xs):
    return jnp.concatenate(xs, axis=1)


def _kernel(mem0_hbm, x_hbm, wq_hbm, wk_hbm, wv_hbm, wo_hbm, bqkv_hbm, bwo_hbm,
            out_hbm,
            mem0_ref, x_ref, out_ref, wq_ref, wk_ref, wv_ref, wo_ref, bqkv_ref, bwo_ref,
            wqkv_p, wo_p, bqkv_p, bwo_p, h_ref, xa_ref, x2_ref, kv_ref, ha_ref, hb_ref, pre_ref, o_ref, tmp_ref, wsem, sem,
            *, S, D, H, DH, M, SEG):
    NSEG = S // SEG
    PW = 2 * DH
    NP = H // 2
    RV = SEG + M
    RL = SEG + 2 * M
    RT = 2 * SEG + 2 * M
    a_scale = DH ** (-0.5)
    b_dh = D // B_HEADS
    b_scale = b_dh ** (-0.5)
    NT = D // 128
    X0 = (NPRE + 3) * SEG

    def sl(p):
        return slice(p * PW, (p + 1) * PW)

    cp_m = pltpu.make_async_copy(mem0_hbm, mem0_ref, sem.at[8])
    cp_x0 = pltpu.make_async_copy(x_hbm.at[0:X0], x_ref.at[0:X0], sem.at[0])
    cp_x1 = pltpu.make_async_copy(x_hbm.at[X0:S], x_ref.at[X0:S], sem.at[1])
    cp_b = [pltpu.make_async_copy(bqkv_hbm.at[:, j * D:(j + 1) * D], bqkv_ref.at[j], sem.at[2 + j])
            for j in range(3)]
    cp_b.append(pltpu.make_async_copy(bwo_hbm, bwo_ref, sem.at[5]))
    cp_wo = pltpu.make_async_copy(wo_hbm, wo_ref, sem.at[9])
    w_pairs = ((wq_hbm, wq_ref), (wk_hbm, wk_ref), (wv_hbm, wv_ref))

    def rows_of(p):
        return pl.ds(p * PW if isinstance(p, int) else pl.multiple_of(p * PW, 128), PW)

    def cp_fine(p, i):
        src, dst = w_pairs[i]
        return pltpu.make_async_copy(src.at[rows_of(p)], dst.at[rows_of(p)], wsem.at[NP + 3 * p + i])

    def cp_group(p):
        return [pltpu.make_async_copy(src.at[rows_of(p)], dst.at[rows_of(p)], wsem.at[p])
                for src, dst in w_pairs]

    def start_group(p, carry):
        for cp in cp_group(p):
            cp.start()

        @pl.when(p == NP - 1)
        def _():
            cp_wo.start()

        return carry

    firsts = [[cp_m, cp_x0]] + [[cp_fine(p, i)] for p in range(NFINE) for i in range(3)]

    def start_first(i, carry):
        for n, cps in enumerate(firsts):
            @pl.when(i == n)
            def _():
                for cp in cps:
                    cp.start()

        return carry

    lax.fori_loop(0, len(firsts), start_first, 0)
    lax.fori_loop(NFINE, NP, start_group, 0)
    for cp in cp_b:
        cp.start()

    xa_ref[...] = jnp.zeros(xa_ref.shape, F32)
    kv_ref[...] = jnp.zeros(kv_ref.shape, F32)
    cp_m.wait()
    cp_x0.wait()
    mem0 = mem0_ref[...].astype(F32)
    h0 = _ln(x_ref[0:SEG, :].astype(F32))
    ha_ref[0:RV, :] = _cat0([h0, mem0])
    for i in range(NPRE):
        hi = _ln(x_ref[(2 + i) * SEG:(3 + i) * SEG, :].astype(F32))
        if i < NPA:
            ha_ref[RV + i * SEG:RV + (i + 1) * SEG, :] = hi
        else:
            hb_ref[(i - NPA) * SEG // 2:(i - NPA + 1) * SEG // 2, :] = _pack(hi.astype(BF16))

    def perm_rows(a, slot):
        a = a.astype(F32)
        for m in range(NT):
            tmp_ref[slot, m, 0:D, :] = a[:, m * 128:(m + 1) * 128]
        return _cat1([_cat0([tmp_ref[slot, m, pl.ds(d, B_HEADS, stride=b_dh), :] for d in range(b_dh)])
                      for m in range(NT)]).astype(BF16)

    def perm_qkv(j):
        wp = perm_rows(bqkv_ref[j].T, j).T
        for c in range(NT):
            bqkv_p[j * NT + c] = _pack(wp[:, c * 128:(c + 1) * 128])

    def perm_wo():
        bwo_p[...] = _pack(perm_rows(bwo_ref[...], 3))

    def make_b(t, layers, masked):
        xb = xa_ref[layers[0] * SEG:(layers[-1] + 1) * SEG, :]
        hb = _ln(xb).astype(BF16)
        st = {'y': xb, 'p': []}

        def windows(l, i, j, a):
            cur = a[i * SEG:(i + 1) * SEG]
            blk = _cat0([kv_ref[l, j], cur])
            kv_ref[l, j] = cur[SEG - HIST:SEG]
            rolled = [blk] + [pltpu.roll(blk, sh, 0) for sh in range(B_DIL, 8, B_DIL)]
            res = []
            for w in range(B_WIN):
                hi, lo_ = divmod(B_DIL * w, 8)
                o = HIST - 8 * hi
                res.append(rolled[lo_ // B_DIL][o:o + SEG])
            return res

        def qk():
            qs, ks = [], []
            for j in range(NT):
                qs.append(_dot(hb, _unpack(bqkv_p[j])))
                ks.append(_dot(hb, _unpack(bqkv_p[NT + j])))
            for i, l in enumerate(layers):
                ss = None
                for j in range(NT):
                    q = qs[j][i * SEG:(i + 1) * SEG] * b_scale
                    terms = [q * kw for kw in windows(l, i, j, ks[j])]
                    ss = terms if ss is None else [a + b for a, b in zip(ss, terms)]
                pos = (t - 1 - 2 * l) * SEG + lax.broadcasted_iota(jnp.int32, (SEG, 128), 0)
                logits = []
                for w, s in enumerate(ss):
                    s = s + pltpu.roll(s, 64, 1)
                    s = s + pltpu.roll(s, 32, 1)
                    logits.append(jnp.where(pos >= B_DIL * w, s, NEG) if masked else s)
                m = logits[0]
                for w in range(1, B_WIN):
                    m = jnp.maximum(m, logits[w])
                es = [jnp.exp(lg - m) for lg in logits]
                den = es[0]
                for w in range(1, B_WIN):
                    den = den + es[w]
                st['p'].append((es, _recip(den)))

        def v_stage(j):
            vj = _dot(hb, _unpack(bqkv_p[2 * NT + j]))
            outs = []
            for i, l in enumerate(layers):
                es, inv = st['p'][i]
                vw = windows(l, i, NT + j, vj)
                acc = es[0] * vw[0]
                for w in range(1, B_WIN):
                    acc = acc + es[w] * vw[w]
                outs.append(acc * inv)
            st['o', j] = _cat0(outs).astype(BF16)

        def o_stage(j):
            st['y'] = st['y'] + _dot(st.pop(('o', j)), _unpack(bwo_p[j * 64:(j + 1) * 64, :]))

        def fin():
            for i, l in enumerate(layers):
                yl = st['y'][i * SEG:(i + 1) * SEG]
                if l == 0:
                    x2_ref[...] = yl
                    h_ref[RL:RT, :] = _ln(yl).astype(BF16)
                else:
                    if isinstance(t, int):
                        row = (t - 3) * SEG
                    else:
                        row = pl.multiple_of(jnp.maximum(t - 3, 0) * SEG, SEG)
                    out_ref[pl.ds(row, SEG), :] = yl.astype(out_ref.dtype)

        return qk, v_stage, o_stage, fin

    def softmax2(s, first, valid, fill):
        s = jnp.where(valid, s * a_scale, fill)
        m1 = jnp.max(jnp.where(first, s, PADNEG), axis=-1, keepdims=True)
        m2 = jnp.max(jnp.where(first, PADNEG, s), axis=-1, keepdims=True)
        e = jnp.exp(s - jnp.where(first, m1, m2))
        e1 = jnp.where(first, e, 0.0)
        e2 = jnp.where(first, 0.0, e)
        l1 = jnp.sum(e1, axis=-1, keepdims=True)
        l2 = jnp.sum(e2, axis=-1, keepdims=True)
        inv = _recip(jnp.where(first, l1, l2))
        return e, e1, e2, inv

    def make_joint(packed):
        rr = lax.broadcasted_iota(jnp.int32, (RT, 128), 0)
        cc = lax.broadcasted_iota(jnp.int32, (RT, 128), 1)
        lay1 = rr < RV
        first = cc < jnp.where(lay1, RL, RT)
        key = jnp.where(first, cc, cc - RL)
        exists = jnp.where(lay1, RV - 1 - key, key - RV) >= 0
        allowed = (key <= rr) | (lay1 & (key >= SEG)) | ((rr >= RV) & (rr < RL))
        valid = exists & allowed
        fill = jnp.where(exists, NEG, PADNEG)
        lo = cc < (DH - 128)
        z48 = jnp.zeros((128 - RT, 128), F32)
        z32 = jnp.zeros((128 - 2 * RL, 128), F32)
        lhs = (lambda a: a.astype(BF16)) if packed else (lambda a: a)

        def prep_q(a):
            return lhs(a[:, 0:128]), a[0:RV, 128:256], a[RV:RT, 128:256], lhs(a[:, 256:384])

        def prep_kv(a):
            mid = a[:, 128:256]
            tlo = jnp.where(lo, mid, 0.0)
            thi = jnp.where(lo, 0.0, mid)
            return (_cat0([a[:, 0:128], z48]).astype(BF16),
                    _cat0([tlo[0:RL], thi[0:RL], z32]).astype(BF16),
                    _cat0([z32, tlo[SEG:RT], thi[SEG:RT]]).astype(BF16),
                    _cat0([z48, a[:, 256:384]]).astype(BF16))

        def qk(q, k):
            t0 = _dot_nt(q[0], k[0])
            t2 = _dot_nt(q[3], k[3])
            t1a = _dot_nt(q[1], k[1])
            t1b = _dot_nt(q[2], k[2])
            s = jnp.where(first, t0, t2) + _cat0([t1a, t1b])
            e, e1, e2, inv = softmax2(s, first, valid, fill)
            pa = e * inv
            return lhs(e1 * inv), pa[0:RV], pa[RV:RT], lhs(e2 * inv)

        def pv(pr, v):
            o0 = _dot(pr[0], v[0])
            o2 = _dot(pr[3], v[3])
            o1a = _dot(pr[1], v[1])
            o1b = _dot(pr[2], v[2])
            return _cat1([o0, _cat0([o1a, o1b]), o2])

        return prep_q, prep_kv, qk, pv

    def make_single(layer, last=False):
        nq = SEG if last else RV
        rr = lax.broadcasted_iota(jnp.int32, (nq, 2 * RV), 0) + (M if last else 0)
        cc = lax.broadcasted_iota(jnp.int32, (nq, 2 * RV), 1)
        first = cc < RV
        kc = jnp.where(first, cc, cc - RV)
        if layer == 0:
            valid = (kc >= SEG) | (kc <= rr)
        else:
            valid = (rr < M) | (kc <= rr)
        lo = lax.broadcasted_iota(jnp.int32, (RV, PW), 1) < DH
        lhs = (lambda a: a.astype(BF16)) if last else (lambda a: a)

        def prep_kv(a):
            return _cat0([jnp.where(lo, a, 0.0), jnp.where(lo, 0.0, a)]).astype(BF16)

        def qk(q, k):
            e, _, _, inv = softmax2(_dot_nt(q, k), first, valid, NEG)
            return lhs(e * inv)

        def pv(pr, v):
            return lhs(_dot(pr, v))

        return lhs, prep_kv, qk, pv

    def step(t, a_layers, b_layers, light=False, last=False, masked=True, deep=0,
             head_start=False, b_sched=(0, 2, 2, 2)):
        r0 = 0 if 0 in a_layers else RV
        if len(a_layers) == 2:
            h = h_ref[SEG if light else 0:RT, :]
            prep_q, prep_kv, qk, pv = make_joint(light)
        else:
            h = h_ref[0:RL, :].astype(F32)[0:RV] if r0 == 0 else h_ref[SEG:RT, :].astype(F32)[M:RL]
            prep_q, prep_kv, qk, pv = make_single(a_layers[0], last)

        drop1 = isinstance(t, int) and t == NSEG - 1

        def squeeze(a):
            return _cat0([a[0:SEG], a[RV:RT]])

        def expand(a):
            return _cat0([a[0:SEG], jnp.zeros((M, a.shape[1]), F32), a[SEG:RT - M]])

        hq = squeeze(h.astype(F32)) if drop1 else (h_ref[RL:RT, :] if last else h)

        def proj(i, p):
            r = _dot(hq if i == 0 else h, _unpack(wqkv_p[i, p]))
            if drop1 and i == 0:
                r = expand(r)
            if light:
                r = _cat0([pre_ref[i, p, pl.ds(pl.multiple_of((t - 2) * SEG, SEG), SEG), :], r])
            return r

        acc = [None]
        OLAG = 3 if len(a_layers) == 2 else 5

        def oproj(p, o):
            part = _dot(o, _unpack(wo_p[p]))
            acc[0] = part if acc[0] is None else acc[0] + part

        def xrows(seg):
            if isinstance(seg, int):
                return x_ref[seg * SEG:(seg + 1) * SEG, :].astype(F32)
            return x_ref[pl.ds(pl.multiple_of(seg * SEG, SEG), SEG), :].astype(F32)

        hooks = {p: [] for p in range(NP)}
        if b_layers:
            b_qk, b_v, b_o, b_fin = make_b(t, b_layers, masked)
            at, v0, dv, lag = b_sched
            for j in range(NT):
                hooks[at + v0 + j * dv + lag].append(functools.partial(b_o, j))
            hooks[at + v0 + (NT - 1) * dv + lag].append(b_fin)
            for j in range(NT):
                hooks[at + v0 + j * dv].append(functools.partial(b_v, j))
            hooks[at].append(b_qk)
        x2 = x2_ref[...] if 1 in a_layers else None

        if head_start:
            heads = [_dot(h_ref[0:SEG, :], _unpack(wqkv_p[i, 0])) for i in range(2)]
            rest = [_dot(h_ref[SEG:RT, :], _unpack(wqkv_p[i, 0])) for i in range(2)]
            q, k = [_cat0([a, b]) for a, b in zip(heads, rest)]
            q, k = prep_q(q), prep_kv(k)
        else:
            q = prep_q(proj(0, 0))
            k = prep_kv(proj(1, 0))
        vs = {0: prep_kv(proj(2, 0))}
        early_v = light or len(a_layers) == 1
        os_ = {}
        prs = {}

        def do_pv(p):
            o = pv(prs.pop(p), vs.pop(p))
            if len(a_layers) == 2:
                o = squeeze(o) if drop1 else o.astype(BF16)
            os_[p] = o

        for p in range(NP):
            prs[p] = qk(q, k)
            if p + 1 < NP:
                q = prep_q(proj(0, p + 1))
                k = prep_kv(proj(1, p + 1))
                if early_v:
                    vs[p + 1] = prep_kv(proj(2, p + 1))
            else:
                for pp in range(p - deep, p):
                    do_pv(pp)
                if 0 in a_layers and not drop1:
                    nxt = t + 1 if isinstance(t, int) else jnp.minimum(t + 1, NSEG - 1)
                    h_ref[0:SEG, :] = _ln(xrows(nxt)).astype(BF16)
                for pp in range(p - OLAG, p - 1):
                    oproj(pp, os_.pop(pp))
            if p + 1 == NP:
                do_pv(p)
            elif p >= deep:
                do_pv(p - deep)
            if p + 1 < NP and not early_v:
                vs[p + 1] = prep_kv(proj(2, p + 1))
            for f in hooks[p]:
                f()
            if p >= OLAG and p + 1 < NP:
                oproj(p - OLAG, os_.pop(p - OLAG))
        oproj(NP - 2, os_.pop(NP - 2))
        oproj(NP - 1, os_.pop(NP - 1))
        a = expand(acc[0]) if drop1 else acc[0]
        if 0 in a_layers:
            xa_ref[0:SEG, :] = xrows(t) + a[0:SEG]
        if last:
            xa_ref[SEG:2 * SEG, :] = x2 + a
            return
        if 1 in a_layers:
            xa_ref[SEG:2 * SEG, :] = x2 + a[RL - r0:RT - r0]
        mem2 = a[RV - r0:RL - r0] if 1 in a_layers else mem0
        mem1 = a[SEG:RV] if 0 in a_layers else mem2
        h_ref[SEG:RL, :] = _cat0([mem1, mem2]).astype(BF16)

    def first_step():
        prep_q, prep_kv, qk, pv = make_single(0)

        def wait_group(p):
            for cp in cp_group(p):
                cp.wait()

        def pair0(p, fine=False):
            ha = ha_ref[...]
            hb = _unpack(hb_ref[...])
            w = {}

            def load(i):
                if fine:
                    cp_fine(p, i).wait()
                w[i] = w_pairs[i][1][rows_of(p), :]
                wqkv_p[i, p] = _pack(w[i].T)

            def proj_a(i):
                r = _dot_nt(ha, w[i])
                pre_ref[i, p, 0:NPA * SEG, :] = r[RV:]
                return r[0:RV]

            def proj_b(i):
                pre_ref[i, p, NPA * SEG:, :] = _dot_nt(hb, w[i])

            if fine:
                load(0)
                q = prep_q(proj_a(0))
                proj_b(0)
                load(1)
                k = prep_kv(proj_a(1))
                proj_b(1)
                load(2)
                pr = qk(q, k)
                v = prep_kv(proj_a(2))
                proj_b(2)
                o_ref[p] = pv(pr, v)
                return
            for i in range(3):
                load(i)
            q = prep_q(proj_a(0))
            k = prep_kv(proj_a(1))
            v = prep_kv(proj_a(2))
            pr = qk(q, k)
            proj_b(0)
            proj_b(1)
            o_ref[p] = pv(pr, v)
            proj_b(2)

        def body1(p, carry):
            wait_group(p)
            pair0(p)
            return carry

        def body2(i, carry):
            wait_group(2 * i)
            wait_group(2 * i + 1)
            pair0(2 * i)
            pair0(2 * i + 1)
            return carry

        def body0(p, carry):
            pair0(p, fine=True)
            return carry

        lax.fori_loop(0, NFINE, body0, 0)
        lax.fori_loop(NFINE, 4, body1, 0)
        lax.fori_loop(2, NP // 2, body2, 0)
        cp_x1.start()
        cp_wo.wait()
        for cp in cp_b:
            cp.wait()
        a = None
        for p in range(NP):
            w = wo_ref[sl(p), :]
            wo_p[p] = _pack(w)
            part = _dot(o_ref[p], w)
            a = part if a is None else a + part
        xa_ref[0:SEG, :] = x_ref[0:SEG, :].astype(F32) + a[0:SEG]
        h_ref[0:SEG, :] = _ln(x_ref[SEG:2 * SEG, :].astype(F32)).astype(BF16)
        h_ref[SEG:RL, :] = _cat0([a[SEG:RV], mem0]).astype(BF16)

    first_step()
    for j in range(3):
        perm_qkv(j)
    perm_wo()
    step(1, (0,), (0,), deep=2, b_sched=(8, 2, 1, 1))

    def body_light(t, carry):
        step(t, (0, 1), (0, 1), light=True, b_sched=(0, 3, 2, 1))
        return carry

    lax.fori_loop(2, 2 + NPRE, body_light, 0)
    cp_x1.wait()

    T0 = 2 + NPRE
    NPAIR = (NSEG - T0) // 2

    def two_steps(t):
        step(t, (0, 1), (0, 1), masked=False)
        step(t + 1, (0, 1), (0, 1), masked=False, head_start=True)

    def body(i, carry):
        two_steps(T0 + 2 * i)
        return carry

    lax.fori_loop(0, NPAIR, body, 0)
    done = (T0 + 2 * NPAIR - 3) * SEG
    cp_o0 = pltpu.make_async_copy(out_ref.at[0:done], out_hbm.at[0:done], sem.at[6])
    cp_o0.start()
    for t in range(T0 + 2 * NPAIR, NSEG):
        step(t, (0, 1), (0, 1), masked=False)
    step(NSEG, (1,), (0, 1), masked=False, deep=1)
    cp_o1 = pltpu.make_async_copy(out_ref.at[done:S - 2 * SEG], out_hbm.at[done:S - 2 * SEG], sem.at[7])
    cp_o1.start()
    tails = [make_b(NSEG + 1, (1,), False)]
    step(NSEG + 1, (1,), (), last=True, deep=1)
    tails.append(make_b(NSEG + 2, (1,), False))
    for b_qk, b_v, _, _ in tails:
        b_qk()
        for j in range(NT):
            b_v(j)
    for _, _, b_o, b_fin in tails:
        for j in range(NT):
            b_o(j)
        b_fin()
    cp_o2 = pltpu.make_async_copy(out_ref.at[S - 2 * SEG:S], out_hbm.at[S - 2 * SEG:S], sem.at[0])
    cp_o2.start()
    cp_o0.wait()
    cp_o1.wait()
    cp_o2.wait()


def pallas_interleave_layers__memory_aug_recurrent_mem_tr__sliding_local_dilated__prompt_kernel(
    A_x: jax.Array,
    A_mem0: jax.Array,
    A_Wq: jax.Array,
    A_Wk: jax.Array,
    A_Wv: jax.Array,
    A_Wo: jax.Array,
    A_seg_len,
    B_x: jax.Array,
    B_wqkv: jax.Array,
    B_wo: jax.Array,
):
    B, S, D = A_x.shape
    H, DH = A_Wq.shape[1], A_Wq.shape[2]
    M = A_mem0.shape[1]
    SEG = A_seg_len if isinstance(A_seg_len, int) else 32
    assert B == 1 and M == 8 and SEG == 32 and DH == 192 and D == 640 and H % 2 == 0
    assert S % SEG == 0 and S // SEG >= NPRE + 4

    x = A_x.reshape(S, D)
    mem0 = A_mem0.reshape(M, D)
    wq = jnp.transpose(A_Wq, (1, 2, 0)).reshape(H * DH, D)
    wk = jnp.transpose(A_Wk, (1, 2, 0)).reshape(H * DH, D)
    wv = jnp.transpose(A_Wv, (1, 2, 0)).reshape(H * DH, D)
    wo = A_Wo.reshape(H * DH, D)

    hbm = pl.BlockSpec(memory_space=pl.ANY)
    out = pl.pallas_call(
        functools.partial(_kernel, S=S, D=D, H=H, DH=DH, M=M, SEG=SEG),
        out_shape=jax.ShapeDtypeStruct((S, D), A_x.dtype),
        in_specs=[hbm] * 8,
        out_specs=hbm,
        scratch_shapes=[
            pltpu.VMEM((M, D), BF16),
            pltpu.VMEM((S, D), BF16),
            pltpu.VMEM((S, D), BF16),
            pltpu.VMEM((H * DH, D), BF16),
            pltpu.VMEM((H * DH, D), BF16),
            pltpu.VMEM((H * DH, D), BF16),
            pltpu.VMEM((H * DH, D), BF16),
            pltpu.VMEM((3, D, D), BF16),
            pltpu.VMEM((D, D), BF16),
            pltpu.VMEM((3, H // 2, D // 2, 2 * DH), U32),
            pltpu.VMEM((H // 2, DH, D), U32),
            pltpu.VMEM((3 * D // 128, D // 2, 128), U32),
            pltpu.VMEM((D // 2, D), U32),
            pltpu.VMEM((2 * SEG + 2 * M, D), BF16),
            pltpu.VMEM((2 * SEG, D), F32),
            pltpu.VMEM((SEG, D), F32),
            pltpu.VMEM((2, 2 * D // 128, HIST, 128), F32),
            pltpu.VMEM((SEG + M + NPA * SEG, D), F32),
            pltpu.VMEM(((NPRE - NPA) * SEG // 2, D), U32),
            pltpu.VMEM((3, H // 2, NPRE * SEG, 2 * DH), F32),
            pltpu.VMEM((H // 2, SEG + M, 2 * DH), F32),
            pltpu.VMEM((4, D // 128, D + 24, 128), F32),
            pltpu.SemaphoreType.DMA((H // 2 + 3 * NFINE,)),
            pltpu.SemaphoreType.DMA((10,)),
        ],
        compiler_params=pltpu.CompilerParams(vmem_limit_bytes=120 * 1024 * 1024),
        name="pallas_wavefront",
    )(mem0, x, wq, wk, wv, wo, B_wqkv, B_wo)
    return out.reshape(B, S, D)
```

```python
import functools

import jax
import jax.numpy as jnp
from jax import lax
import jax.experimental.pallas as pl
import jax.experimental.pallas.tpu as pltpu

F32 = jnp.float32
BF16 = jnp.bfloat16
U32 = jnp.uint32

EPS = 1e-5
NEG = -1000000000.0
PADNEG = -3.0e38
B_HEADS = 32
B_WIN = 8
B_DIL = 2
NPRE = 11
NPA = 5
NFINE = 1
HIST = 16


def _ln(x):
    m = jnp.mean(x, axis=-1, keepdims=True)
    xc = x - m
    v = jnp.mean(xc * xc, axis=-1, keepdims=True)
    return xc * lax.rsqrt(v + EPS)


def _dot_nt(a, b):
    return lax.dot_general(a, b, (((1,), (1,)), ((), ())), precision=lax.Precision.DEFAULT,
                           preferred_element_type=F32)


def _dot(a, b):
    return lax.dot_general(a, b, (((1,), (0,)), ((), ())), precision=lax.Precision.DEFAULT,
                           preferred_element_type=F32)


def _recip(x):
    r = pl.reciprocal(x, approx=True)
    return r * (2.0 - x * r)


def _pack(a):
    return pltpu.bitcast(a, U32)


def _unpack(a):
    return pltpu.bitcast(a, BF16)


def _cat0(xs):
    return jnp.concatenate(xs, axis=0)


def _cat1(xs):
    return jnp.concatenate(xs, axis=1)


def _kernel(mem0_hbm, x_hbm, wq_hbm, wk_hbm, wv_hbm, wo_hbm, bqkv_hbm, bwo_hbm,
            out_hbm,
            mem0_ref, x_ref, out_ref, wq_ref, wk_ref, wv_ref, wo_ref, bqkv_ref, bwo_ref,
            wqkv_p, wo_p, bqkv_p, bwo_p, h_ref, xa_ref, x2_ref, kv_ref, ha_ref, hb_ref, pre_ref, o_ref, tmp_ref, wsem, sem,
            *, S, D, H, DH, M, SEG):
    NSEG = S // SEG
    PW = 2 * DH
    NP = H // 2
    RV = SEG + M
    RL = SEG + 2 * M
    RT = 2 * SEG + 2 * M
    a_scale = DH ** (-0.5)
    b_dh = D // B_HEADS
    b_scale = b_dh ** (-0.5)
    NT = D // 128
    X0 = (NPRE + 3) * SEG

    def sl(p):
        return slice(p * PW, (p + 1) * PW)

    cp_m = pltpu.make_async_copy(mem0_hbm, mem0_ref, sem.at[0])
    cp_x0 = pltpu.make_async_copy(x_hbm.at[0:X0], x_ref.at[0:X0], sem.at[0])
    cp_x1 = pltpu.make_async_copy(x_hbm.at[X0:S], x_ref.at[X0:S], sem.at[1])
    cp_b = [pltpu.make_async_copy(bqkv_hbm.at[:, j * D:(j + 1) * D], bqkv_ref.at[j], sem.at[2])
            for j in range(3)]
    cp_b.append(pltpu.make_async_copy(bwo_hbm, bwo_ref, sem.at[2]))
    cp_wo = pltpu.make_async_copy(wo_hbm, wo_ref, sem.at[2])
    w_pairs = ((wq_hbm, wq_ref), (wk_hbm, wk_ref), (wv_hbm, wv_ref))

    def rows_of(p):
        return pl.ds(p * PW if isinstance(p, int) else pl.multiple_of(p * PW, 128), PW)

    def cp_fine(p, i):
        src, dst = w_pairs[i]
        return pltpu.make_async_copy(src.at[rows_of(p)], dst.at[rows_of(p)], wsem.at[NP // 2 + 2 + 3 * p + i])

    def cp_group(p, s):
        return [pltpu.make_async_copy(src.at[rows_of(p)], dst.at[rows_of(p)], wsem.at[s])
                for src, dst in w_pairs]

    def start_group(p, carry):
        for cp in cp_group(p, jnp.where(p < 4, p, 2 + p // 2)):
            cp.start()

        @pl.when(p == NP - 1)
        def _():
            cp_wo.start()

        return carry

    firsts = [[cp_m, cp_x0]] + [[cp_fine(p, i)] for p in range(NFINE) for i in range(3)]

    def start_first(i, carry):
        for n, cps in enumerate(firsts):
            @pl.when(i == n)
            def _():
                for cp in cps:
                    cp.start()

        return carry

    lax.fori_loop(0, len(firsts), start_first, 0)
    lax.fori_loop(NFINE, NP, start_group, 0)
    for cp in cp_b:
        cp.start()

    xa_ref[...] = jnp.zeros(xa_ref.shape, F32)
    kv_ref[...] = jnp.zeros(kv_ref.shape, F32)
    cp_m.wait()
    cp_x0.wait()
    mem0 = mem0_ref[...].astype(F32)
    h0 = _ln(x_ref[0:SEG, :].astype(F32))
    ha_ref[0:RV, :] = _cat0([h0, mem0])
    for i in range(NPRE):
        hi = _ln(x_ref[(2 + i) * SEG:(3 + i) * SEG, :].astype(F32))
        if i < NPA:
            ha_ref[RV + i * SEG:RV + (i + 1) * SEG, :] = hi
        else:
            hb_ref[(i - NPA) * SEG // 2:(i - NPA + 1) * SEG // 2, :] = _pack(hi.astype(BF16))

    def perm_rows(a, slot):
        a = a.astype(F32)
        for m in range(NT):
            tmp_ref[slot, m, 0:D, :] = a[:, m * 128:(m + 1) * 128]
        return _cat1([_cat0([tmp_ref[slot, m, pl.ds(d, B_HEADS, stride=b_dh), :] for d in range(b_dh)])
                      for m in range(NT)]).astype(BF16)

    def perm_qkv(j):
        wp = perm_rows(bqkv_ref[j].T, j).T
        for c in range(NT):
            bqkv_p[j * NT + c] = _pack(wp[:, c * 128:(c + 1) * 128])

    def perm_wo():
        bwo_p[...] = _pack(perm_rows(bwo_ref[...], 3))

    def make_b(t, layers, masked):
        xb = xa_ref[layers[0] * SEG:(layers[-1] + 1) * SEG, :]
        hb = _ln(xb).astype(BF16)
        st = {'y': xb, 'p': []}

        def windows(l, i, j, a):
            cur = a[i * SEG:(i + 1) * SEG]
            blk = _cat0([kv_ref[l, j], cur])
            kv_ref[l, j] = cur[SEG - HIST:SEG]
            rolled = [blk] + [pltpu.roll(blk, sh, 0) for sh in range(B_DIL, 8, B_DIL)]
            res = []
            for w in range(B_WIN):
                hi, lo_ = divmod(B_DIL * w, 8)
                o = HIST - 8 * hi
                res.append(rolled[lo_ // B_DIL][o:o + SEG])
            return res

        def qk():
            qs, ks = [], []
            for j in range(NT):
                qs.append(_dot(hb, _unpack(bqkv_p[j])))
                ks.append(_dot(hb, _unpack(bqkv_p[NT + j])))
            for i, l in enumerate(layers):
                ss = None
                for j in range(NT):
                    q = qs[j][i * SEG:(i + 1) * SEG] * b_scale
                    terms = [q * kw for kw in windows(l, i, j, ks[j])]
                    ss = terms if ss is None else [a + b for a, b in zip(ss, terms)]
                pos = (t - 1 - 2 * l) * SEG + lax.broadcasted_iota(jnp.int32, (SEG, 128), 0)
                logits = []
                for w, s in enumerate(ss):
                    s = s + pltpu.roll(s, 64, 1)
                    s = s + pltpu.roll(s, 32, 1)
                    logits.append(jnp.where(pos >= B_DIL * w, s, NEG) if masked else s)
                m = logits[0]
                for w in range(1, B_WIN):
                    m = jnp.maximum(m, logits[w])
                es = [jnp.exp(lg - m) for lg in logits]
                den = es[0]
                for w in range(1, B_WIN):
                    den = den + es[w]
                st['p'].append((es, _recip(den)))

        def v_stage(j):
            vj = _dot(hb, _unpack(bqkv_p[2 * NT + j]))
            outs = []
            for i, l in enumerate(layers):
                es, inv = st['p'][i]
                vw = windows(l, i, NT + j, vj)
                acc = es[0] * vw[0]
                for w in range(1, B_WIN):
                    acc = acc + es[w] * vw[w]
                outs.append(acc * inv)
            st['o', j] = _cat0(outs).astype(BF16)

        def o_stage(j):
            st['y'] = st['y'] + _dot(st.pop(('o', j)), _unpack(bwo_p[j * 64:(j + 1) * 64, :]))

        def fin():
            for i, l in enumerate(layers):
                yl = st['y'][i * SEG:(i + 1) * SEG]
                if l == 0:
                    x2_ref[...] = yl
                    h_ref[RL:RT, :] = _ln(yl).astype(BF16)
                else:
                    if isinstance(t, int):
                        row = (t - 3) * SEG
                    else:
                        row = pl.multiple_of(jnp.maximum(t - 3, 0) * SEG, SEG)
                    out_ref[pl.ds(row, SEG), :] = yl.astype(out_ref.dtype)

        return qk, v_stage, o_stage, fin

    def softmax2(s, first, valid, fill):
        s = jnp.where(valid, s * a_scale, fill)
        m1 = jnp.max(jnp.where(first, s, PADNEG), axis=-1, keepdims=True)
        m2 = jnp.max(jnp.where(first, PADNEG, s), axis=-1, keepdims=True)
        e = jnp.exp(s - jnp.where(first, m1, m2))
        e1 = jnp.where(first, e, 0.0)
        e2 = jnp.where(first, 0.0, e)
        l1 = jnp.sum(e1, axis=-1, keepdims=True)
        l2 = jnp.sum(e2, axis=-1, keepdims=True)
        inv = _recip(jnp.where(first, l1, l2))
        return e, e1, e2, inv

    def make_joint(packed):
        rr = lax.broadcasted_iota(jnp.int32, (RT, 128), 0)
        cc = lax.broadcasted_iota(jnp.int32, (RT, 128), 1)
        lay1 = rr < RV
        first = cc < jnp.where(lay1, RL, RT)
        key = jnp.where(first, cc, cc - RL)
        exists = jnp.where(lay1, RV - 1 - key, key - RV) >= 0
        allowed = (key <= rr) | (lay1 & (key >= SEG)) | ((rr >= RV) & (rr < RL))
        valid = exists & allowed
        fill = jnp.where(exists, NEG, PADNEG)
        lo = cc < (DH - 128)
        z48 = jnp.zeros((128 - RT, 128), F32)
        z32 = jnp.zeros((128 - 2 * RL, 128), F32)
        lhs = (lambda a: a.astype(BF16)) if packed else (lambda a: a)

        def prep_q(a):
            return lhs(a[:, 0:128]), a[0:RV, 128:256], a[RV:RT, 128:256], lhs(a[:, 256:384])

        def prep_kv(a):
            mid = a[:, 128:256]
            tlo = jnp.where(lo, mid, 0.0)
            thi = jnp.where(lo, 0.0, mid)
            return (_cat0([a[:, 0:128], z48]).astype(BF16),
                    _cat0([tlo[0:RL], thi[0:RL], z32]).astype(BF16),
                    _cat0([z32, tlo[SEG:RT], thi[SEG:RT]]).astype(BF16),
                    _cat0([z48, a[:, 256:384]]).astype(BF16))

        def qk(q, k):
            t0 = _dot_nt(q[0], k[0])
            t2 = _dot_nt(q[3], k[3])
            t1a = _dot_nt(q[1], k[1])
            t1b = _dot_nt(q[2], k[2])
            s = jnp.where(first, t0, t2) + _cat0([t1a, t1b])
            e, e1, e2, inv = softmax2(s, first, valid, fill)
            pa = e * inv
            return lhs(e1 * inv), pa[0:RV], pa[RV:RT], lhs(e2 * inv)

        def pv(pr, v):
            o0 = _dot(pr[0], v[0])
            o2 = _dot(pr[3], v[3])
            o1a = _dot(pr[1], v[1])
            o1b = _dot(pr[2], v[2])
            return _cat1([o0, _cat0([o1a, o1b]), o2])

        return prep_q, prep_kv, qk, pv

    def make_single(layer, last=False):
        nq = SEG if last else RV
        rr = lax.broadcasted_iota(jnp.int32, (nq, 2 * RV), 0) + (M if last else 0)
        cc = lax.broadcasted_iota(jnp.int32, (nq, 2 * RV), 1)
        first = cc < RV
        kc = jnp.where(first, cc, cc - RV)
        if layer == 0:
            valid = (kc >= SEG) | (kc <= rr)
        else:
            valid = (rr < M) | (kc <= rr)
        lo = lax.broadcasted_iota(jnp.int32, (RV, PW), 1) < DH
        lhs = (lambda a: a.astype(BF16)) if last else (lambda a: a)

        def prep_kv(a):
            return _cat0([jnp.where(lo, a, 0.0), jnp.where(lo, 0.0, a)]).astype(BF16)

        def qk(q, k):
            e, _, _, inv = softmax2(_dot_nt(q, k), first, valid, NEG)
            return lhs(e * inv)

        def pv(pr, v):
            return lhs(_dot(pr, v))

        return lhs, prep_kv, qk, pv

    def step(t, a_layers, b_layers, light=False, last=False, masked=True, deep=0,
             head_start=False, b_sched=(0, 2, 2, 2)):
        r0 = 0 if 0 in a_layers else RV
        if len(a_layers) == 2:
            h = h_ref[SEG if light else 0:RT, :]
            prep_q, prep_kv, qk, pv = make_joint(light)
        else:
            h = h_ref[0:RL, :].astype(F32)[0:RV] if r0 == 0 else h_ref[SEG:RT, :].astype(F32)[M:RL]
            prep_q, prep_kv, qk, pv = make_single(a_layers[0], last)

        drop1 = isinstance(t, int) and t == NSEG - 1

        def squeeze(a):
            return _cat0([a[0:SEG], a[RV:RT]])

        def expand(a):
            return _cat0([a[0:SEG], jnp.zeros((M, a.shape[1]), F32), a[SEG:RT - M]])

        hq = squeeze(h.astype(F32)) if drop1 else (h_ref[RL:RT, :] if last else h)

        def proj(i, p):
            r = _dot(hq if i == 0 else h, _unpack(wqkv_p[i, p]))
            if drop1 and i == 0:
                r = expand(r)
            if light:
                r = _cat0([pre_ref[i, p, pl.ds(pl.multiple_of((t - 2) * SEG, SEG), SEG), :], r])
            return r

        acc = [None]
        OLAG = 3 if len(a_layers) == 2 else 5

        def oproj(p, o):
            part = _dot(o, _unpack(wo_p[p]))
            acc[0] = part if acc[0] is None else acc[0] + part

        def xrows(seg):
            if isinstance(seg, int):
                return x_ref[seg * SEG:(seg + 1) * SEG, :].astype(F32)
            return x_ref[pl.ds(pl.multiple_of(seg * SEG, SEG), SEG), :].astype(F32)

        hooks = {p: [] for p in range(NP)}
        if b_layers:
            b_qk, b_v, b_o, b_fin = make_b(t, b_layers, masked)
            at, v0, dv, lag = b_sched
            for j in range(NT):
                hooks[at + v0 + j * dv + lag].append(functools.partial(b_o, j))
            hooks[at + v0 + (NT - 1) * dv + lag].append(b_fin)
            for j in range(NT):
                hooks[at + v0 + j * dv].append(functools.partial(b_v, j))
            hooks[at].append(b_qk)
        x2 = x2_ref[...] if 1 in a_layers else None

        if head_start:
            heads = [_dot(h_ref[0:SEG, :], _unpack(wqkv_p[i, 0])) for i in range(2)]
            rest = [_dot(h_ref[SEG:RT, :], _unpack(wqkv_p[i, 0])) for i in range(2)]
            q, k = [_cat0([a, b]) for a, b in zip(heads, rest)]
            q, k = prep_q(q), prep_kv(k)
        else:
            q = prep_q(proj(0, 0))
            k = prep_kv(proj(1, 0))
        vs = {0: prep_kv(proj(2, 0))}
        early_v = light or len(a_layers) == 1
        os_ = {}
        prs = {}

        def do_pv(p):
            o = pv(prs.pop(p), vs.pop(p))
            if len(a_layers) == 2:
                o = squeeze(o) if drop1 else o.astype(BF16)
            os_[p] = o

        for p in range(NP):
            prs[p] = qk(q, k)
            if p + 1 < NP:
                q = prep_q(proj(0, p + 1))
                k = prep_kv(proj(1, p + 1))
                if early_v:
                    vs[p + 1] = prep_kv(proj(2, p + 1))
            else:
                for pp in range(p - deep, p):
                    do_pv(pp)
                if 0 in a_layers and not drop1:
                    nxt = t + 1 if isinstance(t, int) else jnp.minimum(t + 1, NSEG - 1)
                    h_ref[0:SEG, :] = _ln(xrows(nxt)).astype(BF16)
                for pp in range(p - OLAG, p - 1):
                    oproj(pp, os_.pop(pp))
            if p + 1 == NP:
                do_pv(p)
            elif p >= deep:
                do_pv(p - deep)
            if p + 1 < NP and not early_v:
                vs[p + 1] = prep_kv(proj(2, p + 1))
            for f in hooks[p]:
                f()
            if p >= OLAG and p + 1 < NP:
                oproj(p - OLAG, os_.pop(p - OLAG))
        oproj(NP - 2, os_.pop(NP - 2))
        oproj(NP - 1, os_.pop(NP - 1))
        a = expand(acc[0]) if drop1 else acc[0]
        if 0 in a_layers:
            xa_ref[0:SEG, :] = xrows(t) + a[0:SEG]
        if last:
            xa_ref[SEG:2 * SEG, :] = x2 + a
            return
        if 1 in a_layers:
            xa_ref[SEG:2 * SEG, :] = x2 + a[RL - r0:RT - r0]
        mem2 = a[RV - r0:RL - r0] if 1 in a_layers else mem0
        mem1 = a[SEG:RV] if 0 in a_layers else mem2
        h_ref[SEG:RL, :] = _cat0([mem1, mem2]).astype(BF16)

    def first_step():
        prep_q, prep_kv, qk, pv = make_single(0)

        def wait_group(p, s):
            for cp in cp_group(p, s):
                cp.wait()

        def pair0(p, fine=False):
            ha = ha_ref[...]
            hb = _unpack(hb_ref[...])
            w = {}

            def load(i):
                if fine:
                    cp_fine(p, i).wait()
                w[i] = w_pairs[i][1][rows_of(p), :]
                wqkv_p[i, p] = _pack(w[i].T)

            def proj_a(i):
                r = _dot_nt(ha, w[i])
                pre_ref[i, p, 0:NPA * SEG, :] = r[RV:]
                return r[0:RV]

            def proj_b(i):
                pre_ref[i, p, NPA * SEG:, :] = _dot_nt(hb, w[i])

            if fine:
                load(0)
                q = prep_q(proj_a(0))
                proj_b(0)
                load(1)
                k = prep_kv(proj_a(1))
                proj_b(1)
                load(2)
                pr = qk(q, k)
                v = prep_kv(proj_a(2))
                proj_b(2)
                o_ref[p] = pv(pr, v)
                return
            for i in range(3):
                load(i)
            q = prep_q(proj_a(0))
            k = prep_kv(proj_a(1))
            v = prep_kv(proj_a(2))
            pr = qk(q, k)
            proj_b(0)
            proj_b(1)
            o_ref[p] = pv(pr, v)
            proj_b(2)

        def body1(p, carry):
            wait_group(p, p)
            pair0(p)
            return carry

        def body2(i, carry):
            wait_group(2 * i, 2 + i)
            wait_group(2 * i + 1, 2 + i)
            pair0(2 * i)
            pair0(2 * i + 1)
            return carry

        def body0(p, carry):
            pair0(p, fine=True)
            return carry

        lax.fori_loop(0, NFINE, body0, 0)
        lax.fori_loop(NFINE, 4, body1, 0)
        lax.fori_loop(2, NP // 2, body2, 0)
        cp_x1.start()
        cp_wo.wait()
        for cp in cp_b:
            cp.wait()
        a = None
        for p in range(NP):
            w = wo_ref[sl(p), :]
            wo_p[p] = _pack(w)
            part = _dot(o_ref[p], w)
            a = part if a is None else a + part
        xa_ref[0:SEG, :] = x_ref[0:SEG, :].astype(F32) + a[0:SEG]
        h_ref[0:SEG, :] = _ln(x_ref[SEG:2 * SEG, :].astype(F32)).astype(BF16)
        h_ref[SEG:RL, :] = _cat0([a[SEG:RV], mem0]).astype(BF16)

    first_step()
    for j in range(3):
        perm_qkv(j)
    perm_wo()
    step(1, (0,), (0,), deep=2, b_sched=(8, 2, 1, 1))

    def body_light(t, carry):
        step(t, (0, 1), (0, 1), light=True, b_sched=(0, 3, 2, 1))
        return carry

    lax.fori_loop(2, 2 + NPRE, body_light, 0)
    cp_x1.wait()

    T0 = 2 + NPRE
    NPAIR = (NSEG - T0) // 2

    def two_steps(t):
        step(t, (0, 1), (0, 1), masked=False)
        step(t + 1, (0, 1), (0, 1), masked=False, head_start=True)

    def body(i, carry):
        two_steps(T0 + 2 * i)
        return carry

    lax.fori_loop(0, NPAIR, body, 0)
    done = (T0 + 2 * NPAIR - 3) * SEG
    cp_o0 = pltpu.make_async_copy(out_ref.at[0:done], out_hbm.at[0:done], sem.at[0])
    cp_o0.start()
    for t in range(T0 + 2 * NPAIR, NSEG):
        step(t, (0, 1), (0, 1), masked=False)
    step(NSEG, (1,), (0, 1), masked=False, deep=1)
    cp_o1 = pltpu.make_async_copy(out_ref.at[done:S - 2 * SEG], out_hbm.at[done:S - 2 * SEG], sem.at[0])
    cp_o1.start()
    tails = [make_b(NSEG + 1, (1,), False)]
    step(NSEG + 1, (1,), (), last=True, deep=1)
    tails.append(make_b(NSEG + 2, (1,), False))
    for b_qk, b_v, _, _ in tails:
        b_qk()
        for j in range(NT):
            b_v(j)
    for _, _, b_o, b_fin in tails:
        for j in range(NT):
            b_o(j)
        b_fin()
    cp_o2 = pltpu.make_async_copy(out_ref.at[S - 2 * SEG:S], out_hbm.at[S - 2 * SEG:S], sem.at[0])
    cp_o2.start()
    cp_o0.wait()
    cp_o1.wait()
    cp_o2.wait()


def pallas_interleave_layers__memory_aug_recurrent_mem_tr__sliding_local_dilated__prompt_kernel(
    A_x: jax.Array,
    A_mem0: jax.Array,
    A_Wq: jax.Array,
    A_Wk: jax.Array,
    A_Wv: jax.Array,
    A_Wo: jax.Array,
    A_seg_len,
    B_x: jax.Array,
    B_wqkv: jax.Array,
    B_wo: jax.Array,
):
    B, S, D = A_x.shape
    H, DH = A_Wq.shape[1], A_Wq.shape[2]
    M = A_mem0.shape[1]
    SEG = A_seg_len if isinstance(A_seg_len, int) else 32
    assert B == 1 and M == 8 and SEG == 32 and DH == 192 and D == 640 and H % 2 == 0
    assert S % SEG == 0 and S // SEG >= NPRE + 4

    x = A_x.reshape(S, D)
    mem0 = A_mem0.reshape(M, D)
    wq = jnp.transpose(A_Wq, (1, 2, 0)).reshape(H * DH, D)
    wk = jnp.transpose(A_Wk, (1, 2, 0)).reshape(H * DH, D)
    wv = jnp.transpose(A_Wv, (1, 2, 0)).reshape(H * DH, D)
    wo = A_Wo.reshape(H * DH, D)

    hbm = pl.BlockSpec(memory_space=pl.ANY)
    out = pl.pallas_call(
        functools.partial(_kernel, S=S, D=D, H=H, DH=DH, M=M, SEG=SEG),
        out_shape=jax.ShapeDtypeStruct((S, D), A_x.dtype),
        in_specs=[hbm] * 8,
        out_specs=hbm,
        scratch_shapes=[
            pltpu.VMEM((M, D), BF16),
            pltpu.VMEM((S, D), BF16),
            pltpu.VMEM((S, D), BF16),
            pltpu.VMEM((H * DH, D), BF16),
            pltpu.VMEM((H * DH, D), BF16),
            pltpu.VMEM((H * DH, D), BF16),
            pltpu.VMEM((H * DH, D), BF16),
            pltpu.VMEM((3, D, D), BF16),
            pltpu.VMEM((D, D), BF16),
            pltpu.VMEM((3, H // 2, D // 2, 2 * DH), U32),
            pltpu.VMEM((H // 2, DH, D), U32),
            pltpu.VMEM((3 * D // 128, D // 2, 128), U32),
            pltpu.VMEM((D // 2, D), U32),
            pltpu.VMEM((2 * SEG + 2 * M, D), BF16),
            pltpu.VMEM((2 * SEG, D), F32),
            pltpu.VMEM((SEG, D), F32),
            pltpu.VMEM((2, 2 * D // 128, HIST, 128), F32),
            pltpu.VMEM((SEG + M + NPA * SEG, D), F32),
            pltpu.VMEM(((NPRE - NPA) * SEG // 2, D), U32),
            pltpu.VMEM((3, H // 2, NPRE * SEG, 2 * DH), F32),
            pltpu.VMEM((H // 2, SEG + M, 2 * DH), F32),
            pltpu.VMEM((4, D // 128, D + 24, 128), F32),
            pltpu.SemaphoreType.DMA((H // 4 + 2 + 3 * NFINE,)),
            pltpu.SemaphoreType.DMA((3,)),
        ],
        compiler_params=pltpu.CompilerParams(vmem_limit_bytes=120 * 1024 * 1024),
        name="pallas_wavefront",
    )(mem0, x, wq, wk, wv, wo, B_wqkv, B_wo)
    return out.reshape(B, S, D)
```
